```python
import jax
import jax.numpy as jnp

def _softmax(x, axis=-1):
    return jax.nn.softmax(x, axis=axis)
def _gelu(x):
    return jax.nn.gelu(x, approximate=True)
def _silu(x):
    return jax.nn.silu(x)
def _sigmoid(x):
    return jax.nn.sigmoid(x)
def _layernorm(x, axis=-1, eps=1e-5):
    m = jnp.mean(x, axis=axis, keepdims=True)
    v = jnp.var(x, axis=axis, keepdims=True)
    return (x - m) / jnp.sqrt(v + eps)
def _scatter_add(tgt, idx, src, axis=0):
    return tgt.at[idx].add(src)
def _segment_sum(src, seg, n):
    return jax.ops.segment_sum(src, seg, n)
class _Rng:
    def __init__(self, key):
        self._k = key
    def _next(self):
        self._k, sub = jax.random.split(self._k)
        return sub
    def normal(self, shape):
        return jax.random.normal(self._next(), shape, dtype=jnp.bfloat16)
    def randint(self, lo, hi, shape):
        return jax.random.randint(self._next(), shape, lo, hi, dtype=jnp.int32)
    def uniform(self, shape, lo=0.0, hi=1.0):
        return jax.random.uniform(self._next(), shape, jnp.bfloat16, lo, hi)
    def permutation(self, n):
        return jax.random.permutation(self._next(), n)


kernel_name = 'interleave_layers__ssm_conv_s4__sliding_local_dilated__prompt'

def setup_inputs():
    _rng = _Rng(jax.random.key(int.from_bytes(__import__("os").urandom(4), "little")))
    _w = (lambda a: (lambda t: t.astype(jnp.bfloat16) if jnp.issubdtype(t.dtype, jnp.floating) else t)(jnp.asarray(a)))
    def _A_setup():
        B, L, D, N = 1, 2048, 512, 128
        A_re = -jnp.exp((lambda *s: _rng.normal(s) * 0.05)(D, N))
        A_im = jnp.pi * (lambda *s: _rng.normal(s) * 0.05)(D, N)
        B_re = (lambda *s: _rng.normal(s) * 0.05)(D, N)
        B_im = (lambda *s: _rng.normal(s) * 0.05)(D, N)
        C_re = (lambda *s: _rng.normal(s) * 0.05)(D, N)
        C_im = (lambda *s: _rng.normal(s) * 0.05)(D, N)
        log_dt = (lambda *s: _rng.normal(s) * 0.05)(D) * 0.5 - 4.0
        Dskip = (lambda *s: _rng.normal(s) * 0.05)(D)
        return {
            "u": _w((lambda *s: _rng.normal(s) * 0.05)(B, L, D)),
            "A_re": _w(A_re),
            "A_im": _w(A_im),
            "B_re": _w(B_re),
            "B_im": _w(B_im),
            "C_re": _w(C_re),
            "C_im": _w(C_im),
            "log_dt": _w(log_dt),
            "Dskip": _w(Dskip),
        }
    _A_in = _A_setup()

    def _B_setup():
        B, S, D = 1, 2048, 512
        return {
            "x": _w((lambda *s: _rng.normal(s) * 0.05)(B, S, D)),
            "wqkv": _w((lambda *s: _rng.normal(s) * 0.05)(D, 3 * D)),
            "wo": _w((lambda *s: _rng.normal(s) * 0.05)(D, D)),
        }
    _B_in = _B_setup()

    return {
        "A_u": _A_in["u"],
        "A_A_re": _A_in["A_re"],
        "A_A_im": _A_in["A_im"],
        "A_B_re": _A_in["B_re"],
        "A_B_im": _A_in["B_im"],
        "A_C_re": _A_in["C_re"],
        "A_C_im": _A_in["C_im"],
        "A_log_dt": _A_in["log_dt"],
        "A_Dskip": _A_in["Dskip"],
        "B_x": _B_in["x"],
        "B_wqkv": _B_in["wqkv"],
        "B_wo": _B_in["wo"],
    }

def reference(A_u, A_A_re, A_A_im, A_B_re, A_B_im, A_C_re, A_C_im, A_log_dt, A_Dskip, B_x, B_wqkv, B_wo):
    def _A_ref(u, A_re, A_im, B_re, B_im, C_re, C_im, log_dt, Dskip):
        Bsz, L, D = u.shape
        dt = jnp.exp(log_dt)[:, None]
        A = A_re + 1j * A_im
        Bc = B_re + 1j * B_im
        Cc = C_re + 1j * C_im
        logdA = dt * A
        dB = dt * Bc
        l = (lambda x, dt: x.astype(dt))(jnp.arange(L), A_re.dtype)
        P = jnp.exp(logdA[:, :, None] * l[None, None, :])
        K = jnp.einsum("dn,dnl,dn->dl", Cc, P, dB).real
        L2 = 2 * L
        Kp = jnp.pad(K, ((0, 0), (0, L)))
        up = (lambda x, *d: x.transpose(*d))(u, 0, 2, 1)
        up = jnp.pad(up, ((0, 0), (0, 0), (0, L)))
        Kf = (lambda x, axes=(-2,-1): jnp.fft.rfft2(x.astype(jnp.float32), axes=axes))(Kp[:, None, :], axes=(-2, -1))
        Uf = (lambda x, axes=(-2,-1): jnp.fft.rfft2(x.astype(jnp.float32), axes=axes))(up[:, :, None, :], axes=(-2, -1))
        Yf = Uf * Kf[None, :, :, :]
        y = (lambda x, s, axes=(-2,-1): jnp.fft.irfft2(x, s=s, axes=axes).astype(jnp.bfloat16))(Yf, (1, L2), axes=(-2, -1))[:, :, 0, :L]
        y = (lambda x, *d: x.transpose(*d))(y, 0, 2, 1) + u * Dskip[None, None, :]
        return y

    def _B_ref(x, wqkv, wo):
        B, S, D = x.shape
        H = 32; Dh = D // H
        W, dil = 8, 2
        qkv = (lambda x, *d: x.transpose(*d))((x @ wqkv).reshape(B, S, 3, H, Dh), 2, 0, 3, 1, 4)
        q, k, v = qkv[0], qkv[1], qkv[2]
        scale = Dh ** -0.5
        pos = jnp.arange(S)
        off = jnp.arange(W) * dil
        idx = pos[:, None] - off[None, :]
        mask = idx >= 0
        idx_c = jnp.where(mask, idx, 0).reshape(-1)
        kg = k[:, :, idx_c, :].reshape(B, H, S, W, Dh)
        vg = v[:, :, idx_c, :].reshape(B, H, S, W, Dh)
        logits = jnp.einsum("bhsd,bhswd->bhsw", q, kg) * scale
        logits = jnp.where(mask[None, None, :, :], logits, -1e9)
        attn = _softmax(logits, axis=-1)
        o = jnp.einsum("bhsw,bhswd->bhsd", attn, vg)
        return (lambda x, *d: x.transpose(*d))(o, 0, 2, 1, 3).reshape(B, S, D) @ wo

    x = A_u
    x = x + _A_ref(_layernorm(x, axis=-1), A_A_re, A_A_im, A_B_re, A_B_im, A_C_re, A_C_im, A_log_dt, A_Dskip)
    x = x + _B_ref(_layernorm(x, axis=-1), B_wqkv, B_wo)
    x = x + _A_ref(_layernorm(x, axis=-1), A_A_re, A_A_im, A_B_re, A_B_im, A_C_re, A_C_im, A_log_dt, A_Dskip)
    x = x + _B_ref(_layernorm(x, axis=-1), B_wqkv, B_wo)
    return x
```

```python
import numpy as np

import jax
import jax.numpy as jnp
import jax.experimental.pallas as pl
import jax.experimental.pallas.tpu as pltpu

F32, BF16, U32, I32 = jnp.float32, jnp.bfloat16, jnp.uint32, jnp.int32
L, D, NS = 2048, 512, 128
PH, T1 = 16, 128
WIN = 8
NT = (((1,), (1,)), ((), ()))
QS = 116
ZS = 28
CB = 64


def _dft_matrices():
    t = 16 * np.arange(T1)[None, :, None] + np.arange(PH)[:, None, None]
    k = np.arange(T1)[None, None, :] + 0.5
    phi = 2.0 * np.pi * k * t / (2 * L)
    f = np.concatenate([np.cos(phi), -np.sin(phi)], axis=-1).astype(np.float32)
    bits = f.astype(BF16).view(np.uint16).astype(np.uint32)
    return bits[:, 0::2] | (bits[:, 1::2] << 16)


def _cmul(a, b):
    return a[0] * b[0] - a[1] * b[1], a[0] * b[1] + a[1] * b[0]


def _csq(a):
    t = a[0] * a[1]
    return a[0] * a[0] - a[1] * a[1], t + t


def _cadd(a, b):
    return a[0] + b[0], a[1] + b[1]


def _csub(a, b):
    return a[0] - b[0], a[1] - b[1]


def _radix4(x0, x1, x2, x3, sign, rot2=False):
    if rot2:
        m, p = (x0[0] - x2[1], x0[1] + x2[0]), (x0[0] + x2[1], x0[1] - x2[0])
        a, b = (m, p) if sign > 0 else (p, m)
    else:
        a, b = _cadd(x0, x2), _csub(x0, x2)
    c, d = _cadd(x1, x3), _csub(x1, x3)
    m, p = (b[0] - d[1], b[1] + d[0]), (b[0] + d[1], b[1] - d[0])
    y1, y3 = (m, p) if sign > 0 else (p, m)
    return _cadd(a, c), y1, _csub(a, c), y3


def _twiddle(x, e, sign):
    h = float(np.sqrt(0.5))
    if e == 2:
        s, d = x[0] + x[1], x[0] - x[1]
        return (d * h, s * h) if sign > 0 else (s * h, d * -h)
    if e == 6:
        s, d = x[0] + x[1], x[0] - x[1]
        return (s * -h, d * h) if sign > 0 else (d * -h, s * -h)
    ang = sign * 2.0 * np.pi * e / 16
    return _cmul(x, (float(np.cos(ang)), float(np.sin(ang))))


def _fft16(x, sign):
    g = [_radix4(x[c], x[4 + c], x[8 + c], x[12 + c], sign) for c in range(4)]
    y = [None] * 16
    for m in range(4):
        t = [g[c][m] if c * m in (0, 4) else _twiddle(g[c][m], c * m, sign) for c in range(4)]
        y[m], y[m + 4], y[m + 8], y[m + 12] = _radix4(*t, sign, rot2=(m == 2))
    return y


def _sincos(x):
    n = jnp.floor(x * float(2.0 / np.pi) + 0.5)
    r = ((x - n * 1.5703125) - n * 4.837512969970703125e-4) - n * 7.54978995489188216e-8
    z = r * r
    s = r + r * z * ((-1.9515295891e-4 * z + 8.3321608736e-3) * z - 1.6666654611e-1)
    c = 1.0 + z * (((2.443315711809948e-5 * z - 1.388731625493765e-3) * z
                    + 4.166664568298827e-2) * z - 0.5)
    q = n.astype(I32)
    odd = (q & 1) == 1
    s, c = jnp.where(odd, c, s), jnp.where(odd, s, c)
    return jnp.where((q & 2) == 2, -s, s), jnp.where(((q + 1) & 2) == 2, -c, c)


def _pk(x):
    return pltpu.bitcast(x.astype(BF16), U32)


def _bf(words):
    return pltpu.bitcast(words, BF16)


def _layernorm(x):
    d = x - jnp.sum(x, axis=0, keepdims=True) * (1.0 / D)
    v = jnp.sum(d * d, axis=0, keepdims=True) * (1.0 / D)
    return _pk(d * jax.lax.rsqrt(v + 1e-5))


def _kernel(u_hbm, are, aim, bre, bim, cre, cim, ldt, dsk, wqkv_hbm, wo_hbm, f_hbm, out_hbm,
            io, wq_in, wo_in, fm, wt, wot, lam, dtc, tab, ztab, kb, kf,
            xs, xn, ua, va, kx, vx, qs, ob, sems):
    cp_u = [pltpu.make_async_copy(u_hbm.bitcast(U32).at[:, pl.ds(128 * j, 128)],
                                  io.at[j, pl.ds(0, L // 2)], sems.at[j]) for j in range(4)]
    cp_f = pltpu.make_async_copy(f_hbm, fm, sems.at[4])
    cp_wq = pltpu.make_async_copy(wqkv_hbm, wq_in, sems.at[5])
    cp_wo = pltpu.make_async_copy(wo_hbm, wo_in, sems.at[6])
    for cp in [cp_f] + cp_u + [cp_wq, cp_wo]:
        cp.start()

    lane = jax.lax.broadcasted_iota(I32, (8, T1), 1)

    dt_row = jnp.exp(ldt[...].astype(F32)).astype(BF16).astype(F32)
    ds_row = dsk[...].astype(F32)
    for j in range(4):
        rows = slice(128 * j, 128 * j + 128)
        dtc[0, rows, :] = jnp.broadcast_to(dt_row[:, rows], (128, 128)).T
        dtc[1, rows, :] = jnp.broadcast_to(ds_row[:, rows], (128, 128)).T
    theta = dtc[0] * aim[...].astype(F32)
    mag = jnp.exp(dtc[0] * are[...].astype(F32))
    sn, cs = _sincos(theta)
    lam[0] = mag * cs
    lam[1] = mag * sn

    @pl.when(jnp.logical_not(jnp.max(jnp.abs(theta)) <= 8192.0))
    def _():
        def body(i, _):
            rows = pl.ds(pl.multiple_of(i * 16, 16), 16)
            th = dtc[0, rows, :] * aim[rows, :].astype(F32)
            mg = jnp.exp(dtc[0, rows, :] * are[rows, :].astype(F32))
            lam[0, rows, :] = mg * jnp.cos(th)
            lam[1, rows, :] = mg * jnp.sin(th)
        jax.lax.fori_loop(0, D // 16, body, None)

    def taps(blk, _):
        rows32 = pl.ds(pl.multiple_of(blk * 32, 32), 32)
        sc = dtc[0, rows32, :] * (1.0 / L)
        w32 = _cmul((cre[rows32, :].astype(F32), cim[rows32, :].astype(F32)),
                    (bre[rows32, :].astype(F32) * sc, bim[rows32, :].astype(F32) * sc))
        k0 = jnp.sum(w32[0], axis=1, keepdims=True) + dtc[1, rows32, :] * (1.0 / L)
        for e in range(4):
            rows = pl.ds(pl.multiple_of(blk * 32 + 8 * e, 8), 8)

            def put(row, a, b):
                for z in range(2):
                    tab[z, pl.ds(row, 8, stride=QS), :] = pltpu.pack_elementwise(
                        [a[z], b[z]], packed_dtype=BF16)

            l1 = (lam[0, rows, :], lam[1, rows, :])
            l2 = _csq(l1)
            w = (w32[0][8 * e:8 * e + 8], w32[1][8 * e:8 * e + 8])
            a, b = _cmul(w, l1), _cmul(w, l2)
            keep = {}
            for j in range(8):
                put(64 + 12 * e + j, a, b)
                keep[2 * j + 2] = b
                if j < 7:
                    a, b = _cmul(a, l2), _cmul(b, l2)
            l16 = _csq(_csq(_csq(l2)))
            m1 = (l16[0], -l16[1])
            m2 = _csq(m1)
            put(16 * e, (jnp.ones_like(m1[0]), jnp.zeros_like(m1[0])), m1)
            a, b = m2, _cmul(m1, m2)
            for j in range(1, 16):
                put(16 * e + j, a, b)
                if j == 8:
                    l512 = _csq((a[0], -a[1]))
                if j < 15:
                    a, b = _cmul(a, m2), _cmul(b, m2)
            put(64 + 12 * e + 8, _cmul(keep[4], l512), _cmul(keep[12], l512))
            a, b = keep[8], keep[16]
            for j in range(3):
                a, b = _cmul(a, l512), _cmul(b, l512)
                put(64 + 12 * e + 9 + j, a, b)
        for i in range(8):
            acc = None
            for z in range(2):
                rhs = pltpu.bitcast(tab[z, pl.ds(QS * i, 64), :], BF16)
                lhs = pltpu.bitcast(tab[z, pl.ds(QS * i + 64, 48), :], BF16)
                d = jax.lax.dot_general(lhs, rhs, NT, preferred_element_type=F32)
                acc = d if acc is None else acc + d
            for r in range(3):
                pc = [acc[24 * e + 8 * r:24 * e + 8 * r + 8] for e in range(4)]
                ztab[pl.ds(ZS * i + 8 * r, 8), :] = jnp.where(
                    lane < 64, jnp.where(lane < 32, pc[0], pc[1]),
                    jnp.where(lane < 96, pc[2], pc[3]))
        zr = [ztab[pl.ds(r, 8, stride=ZS), :] for r in range(24)]
        taps_e = []
        for e in range(4):
            def at(r, g):
                return zr[r] if g == e else pltpu.roll(zr[r], (32 * (g - e)) % 128, 1)

            def full(r, r1):
                return jnp.where(lane < 64, jnp.where(lane < 32, at(r, 0), at(r1, 1)),
                                 jnp.where(lane < 96, at(r1 + 2, 2), at(r1 + 4, 3)))

            e8, e16 = full(7, 18), full(15, 19)
            e0 = jnp.where(lane == 0, k0[8 * e:8 * e + 8], pltpu.roll(e16, 1, 1))
            e4 = jnp.where(lane < 32, at(3, 0), at(16, 1))
            e12 = jnp.where(lane < 32, at(11, 0), at(17, 1))
            k4, k12 = jnp.where(lane < 64, e4, e0), jnp.where(lane < 64, e12, e16)
            far = {1: e0, 2: e0, 3: k4, 5: jnp.where(lane < 64, e4, e8), 6: e8, 7: e8, 9: e8,
                   10: e8, 11: jnp.where(lane < 64, e12, e8), 13: k12, 14: e16, 15: e16}
            kt = {0: e0, 4: k4, 8: e8, 12: k12}
            for p, v in far.items():
                kt[p] = jnp.where(lane < (16 if p % 2 else 32), at(p - 1, 0), v)
            taps_e.append(kt)
        for p in range(PH):
            kb[p, pl.ds(pl.multiple_of(blk * 16, 16), 16), :] = _pk(
                jnp.concatenate([t[p] for t in taps_e], axis=0))

    jax.lax.fori_loop(0, D // 32, taps, None)

    cp_f.wait()

    def tap_spectrum(blk, _):
        half = pl.ds(pl.multiple_of(blk * (CB // 2), CB // 2), CB // 2)
        for p in range(PH):
            ua[p] = jnp.dot(_bf(kb[p, half, :]), _bf(fm[p]), preferred_element_type=F32)
        for g in range(CB // 8):
            r = slice(8 * g, 8 * g + 8)
            y = _fft16([(ua[p, r, :T1], ua[p, r, T1:]) for p in range(PH)], -1)
            ro = pl.ds(pl.multiple_of(blk * CB + 8 * g, 8), 8)
            for k in range(PH):
                kf[k, ro, :T1] = y[k][0]
                kf[k, ro, T1:] = y[k][1]

    jax.lax.fori_loop(0, D // CB, tap_spectrum, None)

    for cp in cp_u:
        cp.wait()

    def load_pair(h, _):
        wds = jnp.concatenate([io[j, pl.ds(h, T1, stride=8), :].T for j in range(4)], axis=0)
        for z, bits in enumerate((wds << 16, wds & jnp.uint32(0xFFFF0000))):
            x = pltpu.bitcast(bits, F32)
            xs[2 * h + z] = x
            xn[2 * h + z] = _layernorm(x)

    jax.lax.fori_loop(0, PH // 2, load_pair, None)

    ri = jax.lax.broadcasted_iota(I32, (128, 128), 0)
    ci = jax.lax.broadcasted_iota(I32, (128, 128), 1)
    hit = ci == (ri & 7) * 16 + (ri >> 3)
    perm = jnp.where(hit, 1.0, 0.0).astype(BF16)
    perm_q = jnp.where(hit, 0.25, 0.0).astype(BF16)
    eye = jnp.where(ri == ci, 1.0, 0.0).astype(BF16)
    cp_wq.wait()
    cp_wo.wait()
    for j in range(12):
        cols = slice(128 * j, 128 * j + 128)
        wt[64 * j:64 * j + 64, :] = _pk(jax.lax.dot_general(
            perm_q if j < 4 else perm, wq_in[:, cols], NT, preferred_element_type=F32))
    wp = jnp.concatenate(
        [jnp.dot(perm, wo_in[128 * j:128 * j + 128, :], preferred_element_type=F32).astype(BF16)
         for j in range(4)], axis=0)
    for j in range(4):
        cols = slice(128 * j, 128 * j + 128)
        wot[64 * j:64 * j + 64, :] = _pk(jax.lax.dot_general(
            eye, wp[:, cols], NT, preferred_element_type=F32))

    def long_conv(blk, _):
        rows = pl.ds(pl.multiple_of(blk * CB, CB), CB)
        half = pl.ds(pl.multiple_of(blk * (CB // 2), CB // 2), CB // 2)
        for p in range(PH):
            ua[p] = jnp.dot(_bf(xn[p, half, :]), _bf(fm[p]), preferred_element_type=F32)
        for g in range(CB // 16):
            halves = []
            for s in range(2):
                r = slice(16 * g + 8 * s, 16 * g + 8 * s + 8)
                ro = pl.ds(pl.multiple_of(blk * CB + 16 * g + 8 * s, 8), 8)
                y = _fft16([(ua[p, r, :T1], ua[p, r, T1:]) for p in range(PH)], -1)
                y = [_cmul(y[k], (kf[k, ro, :T1], kf[k, ro, T1:])) for k in range(PH)]
                halves.append(_fft16(y, 1))
            r = slice(8 * g, 8 * g + 8)
            for p in range(PH):
                for z in range(2):
                    va[p, r, T1 * z:T1 * z + T1] = _pk(jnp.concatenate(
                        [halves[0][p][z], halves[1][p][z]], axis=0))
        for p in range(PH):
            xs[p, rows, :] += jax.lax.dot_general(_bf(va[p]), _bf(fm[p]), NT,
                                                  preferred_element_type=F32)

    def keys_values(par, m):
        p = 2 * m + par
        xb = _layernorm(xs[p])
        xn[p] = xb
        for dst, lo in ((kx, D), (vx, 2 * D)):
            y = jnp.dot(_bf(wt[lo // 2:(lo + D) // 2, :]), _bf(xb), preferred_element_type=F32)
            dst[par, WIN + m] = y
            dst[par, m] = pltpu.roll(y, 1, 1)

    def attend(par, m):
        p = 2 * m + par
        qs[...] = jnp.dot(_bf(wt[:D // 2, :]), _bf(xn[p]), preferred_element_type=F32)
        for hg in range(4):
            lg = [None] * WIN
            for dh in range(16):
                r = slice(128 * hg + 8 * dh, 128 * hg + 8 * dh + 8)
                q = qs[r, :]
                for j in range(WIN):
                    t = q * kx[par, WIN + m - j, r, :]
                    lg[j] = t if dh == 0 else lg[j] + t
            for j in range(1, WIN):
                lg[j] = jnp.where(lane < jnp.where(j > m, 1, 0), -1e9, lg[j])
            mx = lg[0]
            for j in range(1, WIN):
                mx = jnp.maximum(mx, lg[j])
            ex = [jnp.exp(t - mx) for t in lg]
            den = ex[0]
            for j in range(1, WIN):
                den = den + ex[j]
            inv = 1.0 / den
            pr = [t * inv for t in ex]
            for d2 in range(8):
                o = []
                for s in range(2):
                    r = slice(128 * hg + 16 * d2 + 8 * s, 128 * hg + 16 * d2 + 8 * s + 8)
                    acc = pr[0] * vx[par, WIN + m, r, :]
                    for j in range(1, WIN):
                        acc = acc + pr[j] * vx[par, WIN + m - j, r, :]
                    o.append(acc)
                ob[64 * hg + 8 * d2:64 * hg + 8 * d2 + 8, :] = _pk(jnp.concatenate(o, axis=0))
        x = xs[p] + jnp.dot(_bf(wot[...]), _bf(ob[...]), preferred_element_type=F32)
        xs[p] = x
        xn[p] = _layernorm(x)

    def layer(_, c):
        jax.lax.fori_loop(0, D // CB, long_conv, None)
        jax.lax.fori_loop(0, WIN, lambda m, _: keys_values(0, m), None)

        def even(m, _):
            keys_values(1, m)
            attend(0, m)

        jax.lax.fori_loop(0, WIN, even, None)
        jax.lax.fori_loop(0, WIN, lambda m, _: attend(1, m), None)

    jax.lax.fori_loop(0, 2, layer, None)

    cp_o = [pltpu.make_async_copy(io.at[j, pl.ds(0, L // 2)],
                                  out_hbm.bitcast(U32).at[:, pl.ds(128 * j, 128)], sems.at[j])
            for j in range(4)]
    for j in range(4):
        rows = slice(128 * j, 128 * j + 128)
        for h in range(PH // 2):
            wds = pltpu.pack_elementwise([xs[2 * h, rows, :], xs[2 * h + 1, rows, :]],
                                         packed_dtype=BF16)
            io[j, pl.ds(h, T1, stride=8), :] = wds.T
        cp_o[j].start()
    for cp in cp_o:
        cp.wait()


@jax.jit
def pallas_interleave_layers__ssm_conv_s4__sliding_local_dilated__prompt_kernel(
    A_u: jax.Array,
    A_A_re: jax.Array,
    A_A_im: jax.Array,
    A_B_re: jax.Array,
    A_B_im: jax.Array,
    A_C_re: jax.Array,
    A_C_im: jax.Array,
    A_log_dt: jax.Array,
    A_Dskip: jax.Array,
    B_x: jax.Array,
    B_wqkv: jax.Array,
    B_wo: jax.Array,
):
    del B_x
    hbm = pl.BlockSpec(memory_space=pl.ANY)
    vmem = pl.BlockSpec(memory_space=pltpu.VMEM)
    out = pl.pallas_call(
        _kernel,
        in_specs=[hbm] + [vmem] * 8 + [hbm] * 3,
        out_specs=hbm,
        out_shape=jax.ShapeDtypeStruct((L, D), BF16),
        scratch_shapes=[
            pltpu.VMEM((4, L // 2 + 8, 128), U32),
            pltpu.VMEM((D, 3 * D), BF16),
            pltpu.VMEM((D, D), BF16),
            pltpu.VMEM((PH, T1 // 2, 2 * T1), U32),
            pltpu.VMEM((3 * D // 2, D), U32),
            pltpu.VMEM((D // 2, D), U32),
            pltpu.VMEM((2, D, NS), F32),
            pltpu.VMEM((2, D, NS), F32),
            pltpu.VMEM((2, 9 * QS + 4, NS), U32),
            pltpu.VMEM((9 * ZS + 4, T1), F32),
            pltpu.VMEM((PH, D // 2, T1), U32),
            pltpu.VMEM((PH, D, 2 * T1), F32),
            pltpu.VMEM((PH, D, T1), F32),
            pltpu.VMEM((PH, D // 2, T1), U32),
            pltpu.VMEM((PH, CB, 2 * T1), F32),
            pltpu.VMEM((PH, CB // 2, 2 * T1), U32),
            pltpu.VMEM((2, 2 * WIN, D, T1), F32),
            pltpu.VMEM((2, 2 * WIN, D, T1), F32),
            pltpu.VMEM((D, T1), F32),
            pltpu.VMEM((D // 2, T1), U32),
            pltpu.SemaphoreType.DMA((7,)),
        ],
        compiler_params=pltpu.CompilerParams(vmem_limit_bytes=100 * 1024 * 1024),
    )(A_u.reshape(L, D), A_A_re, A_A_im, A_B_re, A_B_im, A_C_re, A_C_im,
      A_log_dt.reshape(1, D), A_Dskip.reshape(1, D), B_wqkv, B_wo,
      _dft_matrices())
    return out.reshape(1, L, D)
```

```python
import numpy as np

import jax
import jax.numpy as jnp
import jax.experimental.pallas as pl
import jax.experimental.pallas.tpu as pltpu

F32, BF16, U32, I32 = jnp.float32, jnp.bfloat16, jnp.uint32, jnp.int32
L, D, NS = 2048, 512, 128
PH, T1 = 16, 128
WIN = 8
NN = (((1,), (0,)), ((), ()))
NT = (((1,), (1,)), ((), ()))
QS = 116
TZ = 8 * QS
ZS = 28
_H = float(np.sqrt(0.5))
NCOEF = 22
CB = 64


def _dft_matrices():
    t = 16 * np.arange(T1)[None, :, None] + np.arange(PH)[:, None, None]
    k = np.arange(T1)[None, None, :] + 0.5
    phi = 2.0 * np.pi * k * t / (2 * L)
    f = np.concatenate([np.cos(phi), -np.sin(phi)], axis=-1).astype(np.float32)
    bits = f.astype(BF16).view(np.uint16).astype(np.uint32)
    return bits[:, 0::2] | (bits[:, 1::2] << 16)


def _cmul(a, b):
    return a[0] * b[0] - a[1] * b[1], a[0] * b[1] + a[1] * b[0]


def _csq(a):
    t = a[0] * a[1]
    return a[0] * a[0] - a[1] * a[1], t + t


def _cadd(a, b):
    return a[0] + b[0], a[1] + b[1]


def _csub(a, b):
    return a[0] - b[0], a[1] - b[1]


def _rot8(x, e):
    s, d = x[0] + x[1], x[0] - x[1]
    return {1: (d * _H, s * _H), 3: (s * -_H, d * _H), 5: (d * -_H, s * -_H), 7: (s * _H, d * -_H)}[e]


def _split(x, e):
    n = len(x) // 2
    lo, hi = x[:n], x[n:]
    if e == 4:
        return ([(a[0] - b[1], a[1] + b[0]) for a, b in zip(lo, hi)],
                [(a[0] + b[1], a[1] - b[0]) for a, b in zip(lo, hi)])
    if e:
        hi = [_rot8(b, e // 2) for b in hi]
    return [_cadd(a, b) for a, b in zip(lo, hi)], [_csub(a, b) for a, b in zip(lo, hi)]


def _merge(p, m, e):
    lo = [_cadd(a, b) for a, b in zip(p, m)]
    if e == 4:
        return lo + [(a[1] - b[1], b[0] - a[0]) for a, b in zip(p, m)]
    hi = [_csub(a, b) for a, b in zip(p, m)]
    return lo + ([_rot8(b, 8 - e // 2) for b in hi] if e else hi)


def _conv_coefs(k, e):
    if len(k) == 1:
        return [(k[0][0] * 0.5, k[0][1] * 0.5)]
    if len(k) == 2 and e % 4:
        if e % 2:
            top = _csub(_rot8(k[1], e), k[0])
        elif e == 2:
            top = (-k[1][1] - k[0][0], k[1][0] - k[0][1])
        else:
            top = (k[1][1] - k[0][0], -k[1][0] - k[0][1])
        return [k[0], top, _csub(k[1], k[0])]
    p, m = _split(k, e)
    return _conv_coefs(p, e // 2) + _conv_coefs(m, e // 2 + 4)


def _conv(x, e, coef):
    if len(x) == 1:
        return [_cmul(x[0], coef())]
    if len(x) == 2 and e % 4:
        both = _cmul(_cadd(x[0], x[1]), coef())
        return [_cadd(both, _cmul(x[1], coef())), _cadd(both, _cmul(x[0], coef()))]
    p, m = _split(x, e)
    return _merge(_conv(p, e // 2, coef), _conv(m, e // 2 + 4, coef), e)


def _sincos(x):
    n = jnp.floor(x * float(2.0 / np.pi) + 0.5)
    r = ((x - n * 1.5703125) - n * 4.837512969970703125e-4) - n * 7.54978995489188216e-8
    z = r * r
    s = r + r * z * ((-1.9515295891e-4 * z + 8.3321608736e-3) * z - 1.6666654611e-1)
    c = 1.0 + z * (((2.443315711809948e-5 * z - 1.388731625493765e-3) * z
                    + 4.166664568298827e-2) * z - 0.5)
    q = n.astype(I32)
    odd = (q & 1) == 1
    s, c = jnp.where(odd, c, s), jnp.where(odd, s, c)
    return jnp.where((q & 2) == 2, -s, s), jnp.where(((q + 1) & 2) == 2, -c, c)


def _pk(x):
    return pltpu.bitcast(x.astype(BF16), U32)


def _bf(words):
    return pltpu.bitcast(words, BF16)


def _layernorm(x):
    d = x - jnp.sum(x, axis=0, keepdims=True) * (1.0 / D)
    v = jnp.sum(d * d, axis=0, keepdims=True) * (1.0 / D)
    return (d * jax.lax.rsqrt(v + 1e-5)).astype(BF16)


def _rows(i, n):
    return slice(i * n, i * n + n)


def _ds(start, n):
    return pl.ds(start if isinstance(start, int) else pl.multiple_of(start, n), n)


def _pipeline(n, depth, step, bufs):
    def static(i):
        step(i, bufs[i % 2], bufs[1 - i % 2], [s for s in range(depth) if 0 <= i - s < n])

    def body(i, _):
        for par in range(2):
            pl.when(i % 2 == par)(lambda: step(i, bufs[par], bufs[1 - par], list(range(depth))))

    for i in range(depth - 1):
        static(i)
    jax.lax.fori_loop(depth - 1, n, body, None)
    for i in range(n, n + depth - 1):
        static(i)


def _kernel(u_hbm, are, aim, bre, bim, cre, cim, ldt, dsk, wqkv_hbm, wo_hbm, f_hbm, out_hbm,
            io, wq_in, wo_in, fm, wt, wot, wp, lam, dtc, k0s, ta, tb, kf,
            xs, xn, ca, cb, kx, vx, qs, ob, zs, sems):
    cp_u = [pltpu.make_async_copy(u_hbm.bitcast(U32).at[:, pl.ds(128 * j, 128)],
                                  io.at[j, pl.ds(0, L // 2)], sems.at[j]) for j in range(4)]
    cp_f = pltpu.make_async_copy(f_hbm, fm, sems.at[4])
    cp_wq = pltpu.make_async_copy(wqkv_hbm, wq_in, sems.at[5])
    cp_wo = pltpu.make_async_copy(wo_hbm, wo_in, sems.at[6])
    for cp in [cp_wq, cp_wo, cp_f] + cp_u:
        cp.start()

    lane = jax.lax.broadcasted_iota(I32, (8, T1), 1)
    zs[0] = 0

    def zero_rows(k):
        return pl.multiple_of((zs[0] >> k) * 8, 8)

    dt_row = jnp.exp(ldt[...].astype(F32)).astype(BF16).astype(F32)
    ds_row = dsk[...].astype(F32)
    for j in range(4):
        dtc[0, _rows(j, 128), :] = jnp.broadcast_to(dt_row[:, _rows(j, 128)], (128, 128)).T
        dtc[1, _rows(j, 128), :] = jnp.broadcast_to(ds_row[:, _rows(j, 128)], (128, 128)).T
    big = None
    for j in range(D // 16):
        r = _rows(j, 16)
        theta = dtc[0, r, :] * aim[r, :].astype(F32)
        mag = jnp.exp(dtc[0, r, :] * are[r, :].astype(F32))
        sn, cs = _sincos(theta)
        lam[0, r, :] = mag * cs
        lam[1, r, :] = mag * sn
        sc = dtc[0, r, :] * (2.0 / L)
        w = _cmul((cre[r, :].astype(F32), cim[r, :].astype(F32)),
                  (bre[r, :].astype(F32) * sc, bim[r, :].astype(F32) * sc))
        lam[2, r, :] = w[0]
        lam[3, r, :] = w[1]
        k0s[r, :] = jnp.sum(w[0], axis=1, keepdims=True) + dtc[1, r, :] * (2.0 / L)
        big = jnp.abs(theta) if big is None else jnp.maximum(big, jnp.abs(theta))

    @pl.when(jnp.logical_not(jnp.max(big) <= 8192.0))
    def _():
        def body(i, _):
            rows = pl.ds(pl.multiple_of(i * 16, 16), 16)
            th = dtc[0, rows, :] * aim[rows, :].astype(F32)
            mg = jnp.exp(dtc[0, rows, :] * are[rows, :].astype(F32))
            lam[0, rows, :] = mg * jnp.cos(th)
            lam[1, rows, :] = mg * jnp.sin(th)
        jax.lax.fori_loop(0, D // 16, body, None)

    def tap_tables(blk, e, dst, zero):
        rows = _ds(blk * 32 + 8 * e, 8)
        w = (lam[2, rows, :], lam[3, rows, :])

        def put(row, a, b):
            for z in range(2):
                dst[pl.ds(zero + TZ * z + row, 8, stride=QS), :] = pltpu.pack_elementwise(
                    [a[z], b[z]], packed_dtype=BF16)

        l1 = (lam[0, rows, :], lam[1, rows, :])
        l2 = _csq(l1)
        l16 = _csq(_csq(_csq(l2)))
        m1 = (l16[0], -l16[1])
        m2 = _csq(m1)
        a, b = _cmul(w, l1), _cmul(w, l2)
        c, d = m2, _cmul(m1, m2)
        put(16 * e, (jnp.ones_like(m1[0]), jnp.zeros_like(m1[0])), m1)
        keep = {}
        for j in range(1, 16):
            if j <= 8:
                put(64 + 12 * e + j - 1, a, b)
                keep[2 * j] = b
            if j < 8:
                a, b = _cmul(a, l2), _cmul(b, l2)
            put(16 * e + j, c, d)
            if j == 8:
                l512 = _csq((c[0], -c[1]))
                put(64 + 12 * e + 8, _cmul(keep[4], l512), _cmul(keep[12], l512))
                a, b = keep[8], keep[16]
            if j in (10, 12, 14):
                a, b = _cmul(a, l512), _cmul(b, l512)
                put(64 + 12 * e + 4 + j // 2, a, b)
            if j < 15:
                c, d = _cmul(c, m2), _cmul(d, m2)
            if j in (7, 15):
                yield

    def tap_sums(i, src, dst, zero):
        acc = None
        for z in range(2):
            rhs = _bf(src[pl.ds(TZ * z + QS * i, 64), :])
            lhs = _bf(src[pl.ds(TZ * z + QS * i + 64, 48), :])
            d = jax.lax.dot_general(lhs, rhs, NT, preferred_element_type=F32)
            acc = d if acc is None else acc + d
        for r in range(3):
            pc = [acc[_rows(3 * e + r, 8)] for e in range(4)]
            dst[pl.ds(zero + 2 * TZ + ZS * i + 8 * r, 8), :] = pltpu.bitcast(jnp.where(
                lane < 64, jnp.where(lane < 32, pc[0], pc[1]),
                jnp.where(lane < 96, pc[2], pc[3])), U32)

    def tap_blocks(blk, e, src):
        def at(r, g):
            z = pltpu.bitcast(src[pl.ds(2 * TZ + r, 8, stride=ZS), :], F32)
            return z if g == e else pltpu.roll(z, (32 * (g - e)) % 128, 1)

        def full(r, r1):
            return jnp.where(lane < 64, jnp.where(lane < 32, at(r, 0), at(r1, 1)),
                             jnp.where(lane < 96, at(r1 + 2, 2), at(r1 + 4, 3)))

        rows = _ds(blk * 32 + 8 * e, 8)
        e8, e16 = full(7, 18), full(15, 19)
        e0 = jnp.where(lane == 0, k0s[rows, :], pltpu.roll(e16, 1, 1))
        e4 = jnp.where(lane < 32, at(3, 0), at(16, 1))
        e12 = jnp.where(lane < 32, at(11, 0), at(17, 1))
        k4, k12 = jnp.where(lane < 64, e4, e0), jnp.where(lane < 64, e12, e16)
        far = {1: e0, 2: e0, 3: k4, 5: jnp.where(lane < 64, e4, e8), 6: e8, 7: e8, 9: e8,
               10: e8, 11: jnp.where(lane < 64, e12, e8), 13: k12, 14: e16, 15: e16}
        for p, v in ((0, e0), (4, k4), (8, e8), (12, k12)):
            kx[0, p, rows, :] = v
        for p, v in far.items():
            kx[0, p, rows, :] = jnp.where(lane < (16 if p % 2 else 32), at(p - 1, 0), v)

    def tap_step(i, src, dst, stages):
        z1, z2 = zero_rows(1), zero_rows(2)
        for e in range(4):
            tables = tap_tables(i, e, dst, z1) if 0 in stages else iter(())
            for h in range(2):
                next(tables, None)
                if 1 in stages:
                    tap_sums(2 * e + h, src, dst, z2)
            if 2 in stages:
                tap_blocks(i - 2, e, src)

    def lane_dft(load, q, dst, zero):
        x0, x1 = [jax.lax.dot_general(load(p), _bf(fm[p]), NN, preferred_element_type=F32)
                  for p in (q, q + 8)]
        for i in range(CB // 8):
            r = _rows(i, 8)
            dst[q, pl.ds(zero + 8 * i, 8), :] = x0[r] + x1[r]
            dst[q + 8, pl.ds(zero + 8 * i, 8), :] = x0[r] - x1[r]

    def tap_coefs(blk, u, src):
        i, odd = u // 2, u % 2
        r, ro = _rows(i, 8), _ds(blk * CB + 8 * i, 8)
        co = _conv_coefs([(src[8 * odd + c, r, :T1], src[8 * odd + c, r, T1:]) for c in range(8)],
                         4 * odd)
        for n, v in enumerate(co):
            kf[10 * odd + n, ro, :T1] = v[0]
            kf[10 * odd + n, ro, T1:] = v[1]

    ri = jax.lax.broadcasted_iota(I32, (128, 128), 0)
    ci = jax.lax.broadcasted_iota(I32, (128, 128), 1)
    hit = ci == (ri & 7) * 16 + (ri >> 3)

    def prep_weights(j):
        if j < 12:
            sel = jnp.where(hit, 0.25 if j < 4 else 1.0, 0.0).astype(BF16)
            wt[_rows(j, 64), :] = _pk(jax.lax.dot_general(
                sel, wq_in[:, _rows(j, 128)], NT, preferred_element_type=F32))
        elif j < 16:
            sel = jnp.where(hit, 1.0, 0.0).astype(BF16)
            wp[_rows(j - 12, 64), :] = _pk(jnp.dot(sel, wo_in[_rows(j - 12, 128), :],
                                                   preferred_element_type=F32))
        else:
            sel = jnp.where(ri == ci, 1.0, 0.0).astype(BF16)
            wot[_rows(j - 16, 64), :] = _pk(jax.lax.dot_general(
                sel, _bf(wp[:, _rows(j - 16, 128)]), NT, preferred_element_type=F32))

    def load_pair(h):
        for j in range(4):
            wds = io[j, pl.ds(h, T1, stride=8), :].T
            xs[2 * h, _rows(j, 128), :] = pltpu.bitcast(wds << 16, F32)
            xs[2 * h + 1, _rows(j, 128), :] = pltpu.bitcast(wds & jnp.uint32(0xFFFF0000), F32)
        for p in (2 * h, 2 * h + 1):
            xn[p] = _layernorm(xs[p])

    _pipeline(D // 32, 3, tap_step, (ta, tb))
    for cp in [cp_wq, cp_wo, cp_f] + cp_u:
        cp.wait()
    nc = D // CB

    def spec_step(i, src, dst, stages):
        for q in range(8):
            if 0 in stages:
                lane_dft(lambda p: kx[0, p, _ds(i * CB, CB), :], q, dst, 0)
            if 1 in stages:
                tap_coefs(i - 1, 2 * q, src)
                tap_coefs(i - 1, 2 * q + 1, src)

    _pipeline(nc, 2, spec_step, (ca, cb))
    for h in range(PH // 2):
        for j in range(20 * h // 8, 20 * (h + 1) // 8):
            prep_weights(j)
        load_pair(h)

    def phase_conv(blk, u, src, dst, zero):
        i, odd = u // 2, u % 2
        r, ro = _rows(i, 8), _ds(blk * CB + 8 * i, 8)
        ids = iter(range(10 * odd, NCOEF))

        def coef():
            n = next(ids)
            return kf[n, ro, :T1], kf[n, ro, T1:]

        y = _conv([(src[8 * odd + c, r, :T1], src[8 * odd + c, r, T1:]) for c in range(8)],
                  4 * odd, coef)
        for c in range(8):
            dst[PH + 8 * odd + c, pl.ds(zero + 8 * i, 8), :T1] = y[c][0]
            dst[PH + 8 * odd + c, pl.ds(zero + 8 * i, 8), T1:] = y[c][1]

    def lane_idft(blk, q, src):
        a, b = src[PH + q], src[PH + 8 + q]
        for p, v in ((q, a + b), (q + 8, a - b)):
            xs[p, _ds(blk * CB, CB), :] += jax.lax.dot_general(
                v, _bf(fm[p]), NT, preferred_element_type=F32)

    def conv_step(i, src, dst, stages):
        z1, z2 = zero_rows(1), zero_rows(2)
        for q in range(8):
            if 1 in stages:
                phase_conv(i - 1, 2 * q, src, dst, z2)
            if 0 in stages:
                lane_dft(lambda p: xn[p, _ds(i * CB, CB), :], q, dst, z1)
            if 1 in stages:
                phase_conv(i - 1, 2 * q + 1, src, dst, z2)
            if 2 in stages:
                lane_idft(i - 2, q, src)

    def norm(p):
        xn[p] = _layernorm(xs[p])

    def keys_values(p):
        par, m = p % 2, p // 2
        y = jnp.dot(_bf(wt[D // 2:, :]), xn[p], preferred_element_type=F32)
        for dst, part in ((kx, y[:D]), (vx, y[D:])):
            dst[par, WIN - 1 + m] = part
            if m:
                dst[par, m - 1] = pltpu.roll(part, 1, 1)

    def queries(p):
        qs[(p // 2) % 2] = jnp.dot(_bf(wt[:D // 2, :]), xn[p], preferred_element_type=F32)

    def attend(p):
        par, m = p % 2, p // 2
        for hg in range(4):
            lg = [None] * WIN
            for dh in range(16):
                r = _rows(16 * hg + dh, 8)
                q = qs[m % 2, r, :]
                for j in range(WIN):
                    t = q * kx[par, WIN - 1 + m - j, r, :]
                    lg[j] = t if dh == 0 else lg[j] + t
            for j in range(m + 1, WIN):
                lg[j] = jnp.where(lane == 0, -1e9, lg[j])
            mx = lg[0]
            for j in range(1, WIN):
                mx = jnp.maximum(mx, lg[j])
            ex = [jnp.exp(t - mx) for t in lg]
            den = ex[0]
            for j in range(1, WIN):
                den = den + ex[j]
            inv = 1.0 / den
            pr = [t * inv for t in ex]
            for d2 in range(8):
                o = []
                for s in range(2):
                    r = _rows(16 * hg + 2 * d2 + s, 8)
                    acc = pr[0] * vx[par, WIN - 1 + m, r, :]
                    for j in range(1, WIN):
                        acc = acc + pr[j] * vx[par, WIN - 1 + m - j, r, :]
                    o.append(acc)
                ob[m % 2, _rows(8 * hg + d2, 16), :] = jnp.concatenate(o, axis=0).astype(BF16)

    def project(p):
        xs[p] += jnp.dot(_bf(wot[...]), ob[(p // 2) % 2], preferred_element_type=F32)

    def layer(_, c):
        _pipeline(nc, 3, conv_step, (ca, cb))
        order = list(range(0, PH, 2)) + list(range(1, PH, 2))
        norm(0)
        for i in range(WIN):
            norm(order[i + 1])
            keys_values(order[i])
        queries(0)
        for i in range(PH + 2):
            if i < WIN:
                if i + 1 < WIN:
                    norm(order[WIN + i + 1])
                keys_values(order[WIN + i])
            if i + 1 < PH:
                queries(order[i + 1])
            if 1 <= i <= PH:
                project(order[i - 1])
            if i < PH:
                attend(order[i])
            if i >= 2:
                norm(order[i - 2])

    jax.lax.fori_loop(0, 2, layer, None)

    cp_o = [pltpu.make_async_copy(io.at[j, pl.ds(0, L // 2)],
                                  out_hbm.bitcast(U32).at[:, pl.ds(128 * j, 128)], sems.at[j])
            for j in range(4)]
    for j in range(4):
        for h in range(PH // 2):
            wds = pltpu.pack_elementwise(
                [xs[2 * h, _rows(j, 128), :], xs[2 * h + 1, _rows(j, 128), :]], packed_dtype=BF16)
            io[j, pl.ds(h, T1, stride=8), :] = wds.T
        cp_o[j].start()
    for cp in cp_o:
        cp.wait()


@jax.jit
def pallas_interleave_layers__ssm_conv_s4__sliding_local_dilated__prompt_kernel(
    A_u: jax.Array,
    A_A_re: jax.Array,
    A_A_im: jax.Array,
    A_B_re: jax.Array,
    A_B_im: jax.Array,
    A_C_re: jax.Array,
    A_C_im: jax.Array,
    A_log_dt: jax.Array,
    A_Dskip: jax.Array,
    B_x: jax.Array,
    B_wqkv: jax.Array,
    B_wo: jax.Array,
):
    del B_x
    hbm = pl.BlockSpec(memory_space=pl.ANY)
    vmem = pl.BlockSpec(memory_space=pltpu.VMEM)
    out = pl.pallas_call(
        _kernel,
        in_specs=[hbm] + [vmem] * 8 + [hbm] * 3,
        out_specs=hbm,
        out_shape=jax.ShapeDtypeStruct((L, D), BF16),
        scratch_shapes=[
            pltpu.VMEM((4, L // 2 + 8, 128), U32),
            pltpu.VMEM((D, 3 * D), BF16),
            pltpu.VMEM((D, D), BF16),
            pltpu.VMEM((PH, T1 // 2, 2 * T1), U32),
            pltpu.VMEM((3 * D // 2, D), U32),
            pltpu.VMEM((D // 2, D), U32),
            pltpu.VMEM((D // 2, D), U32),
            pltpu.VMEM((4, D, NS), F32),
            pltpu.VMEM((2, D, NS), F32),
            pltpu.VMEM((D, T1), F32),
            pltpu.VMEM((2 * TZ + 9 * ZS + 4, NS), U32),
            pltpu.VMEM((2 * TZ + 9 * ZS + 4, NS), U32),
            pltpu.VMEM((NCOEF, D, 2 * T1), F32),
            pltpu.VMEM((PH, D, T1), F32),
            pltpu.VMEM((PH, D, T1), BF16),
            pltpu.VMEM((2 * PH, CB, 2 * T1), F32),
            pltpu.VMEM((2 * PH, CB, 2 * T1), F32),
            pltpu.VMEM((2, 2 * WIN, D, T1), F32),
            pltpu.VMEM((2, 2 * WIN, D, T1), F32),
            pltpu.VMEM((2, D, T1), F32),
            pltpu.VMEM((2, D, T1), BF16),
            pltpu.SMEM((1,), I32),
            pltpu.SemaphoreType.DMA((7,)),
        ],
        compiler_params=pltpu.CompilerParams(vmem_limit_bytes=100 * 1024 * 1024),
    )(A_u.reshape(L, D), A_A_re, A_A_im, A_B_re, A_B_im, A_C_re, A_C_im,
      A_log_dt.reshape(1, D), A_Dskip.reshape(1, D), B_wqkv, B_wo,
      _dft_matrices())
    return out.reshape(1, L, D)
```

```python
import numpy as np

import jax
import jax.numpy as jnp
import jax.experimental.pallas as pl
import jax.experimental.pallas.tpu as pltpu

F32, BF16, U32, I32 = jnp.float32, jnp.bfloat16, jnp.uint32, jnp.int32
L, D, NS = 2048, 512, 128
PH, T1 = 16, 128
WIN = 8
NN = (((1,), (0,)), ((), ()))
NT = (((1,), (1,)), ((), ()))
QS = 116
TZ = 8 * QS
ZS = 28
_H = float(np.sqrt(0.5))
NCOEF = 22
HD = D // 2
RS = 64
LEAD = 1
RATE = 1.0
CB = 64


def _dft_matrices():
    t = 16 * np.arange(T1)[None, :, None] + np.arange(PH)[:, None, None]
    k = np.arange(T1)[None, None, :] + 0.5
    phi = 2.0 * np.pi * k * t / (2 * L)
    f = np.concatenate([np.cos(phi), -np.sin(phi)], axis=-1).astype(np.float32)
    bits = f.astype(BF16).view(np.uint16).astype(np.uint32)
    return bits[:, 0::2] | (bits[:, 1::2] << 16)


def _cmul(a, b):
    return a[0] * b[0] - a[1] * b[1], a[0] * b[1] + a[1] * b[0]


def _csq(a):
    t = a[0] * a[1]
    return a[0] * a[0] - a[1] * a[1], t + t


def _cadd(a, b):
    return a[0] + b[0], a[1] + b[1]


def _csub(a, b):
    return a[0] - b[0], a[1] - b[1]


def _rot8(x, e):
    s, d = x[0] + x[1], x[0] - x[1]
    return {1: (d * _H, s * _H), 3: (s * -_H, d * _H), 5: (d * -_H, s * -_H), 7: (s * _H, d * -_H)}[e]


def _split(x, e):
    n = len(x) // 2
    lo, hi = x[:n], x[n:]
    if e == 4:
        return ([(a[0] - b[1], a[1] + b[0]) for a, b in zip(lo, hi)],
                [(a[0] + b[1], a[1] - b[0]) for a, b in zip(lo, hi)])
    if e:
        hi = [_rot8(b, e // 2) for b in hi]
    return [_cadd(a, b) for a, b in zip(lo, hi)], [_csub(a, b) for a, b in zip(lo, hi)]


def _merge(p, m, e):
    lo = [_cadd(a, b) for a, b in zip(p, m)]
    if e == 4:
        return lo + [(a[1] - b[1], b[0] - a[0]) for a, b in zip(p, m)]
    hi = [_csub(a, b) for a, b in zip(p, m)]
    return lo + ([_rot8(b, 8 - e // 2) for b in hi] if e else hi)


def _conv_coefs(k, e):
    if len(k) == 1:
        return [(k[0][0] * 0.5, k[0][1] * 0.5)]
    if len(k) == 2 and e % 4:
        if e % 2:
            top = _csub(_rot8(k[1], e), k[0])
        elif e == 2:
            top = (-k[1][1] - k[0][0], k[1][0] - k[0][1])
        else:
            top = (k[1][1] - k[0][0], -k[1][0] - k[0][1])
        return [k[0], top, _csub(k[1], k[0])]
    p, m = _split(k, e)
    return _conv_coefs(p, e // 2) + _conv_coefs(m, e // 2 + 4)


def _conv(x, e, coef):
    if len(x) == 1:
        return [_cmul(x[0], coef())]
    if len(x) == 2 and e % 4:
        both = _cmul(_cadd(x[0], x[1]), coef())
        return [_cadd(both, _cmul(x[1], coef())), _cadd(both, _cmul(x[0], coef()))]
    p, m = _split(x, e)
    return _merge(_conv(p, e // 2, coef), _conv(m, e // 2 + 4, coef), e)


def _sincos(x):
    n = jnp.floor(x * float(2.0 / np.pi) + 0.5)
    r = ((x - n * 1.5703125) - n * 4.837512969970703125e-4) - n * 7.54978995489188216e-8
    z = r * r
    s = r + r * z * ((-1.9515295891e-4 * z + 8.3321608736e-3) * z - 1.6666654611e-1)
    c = 1.0 + z * (((2.443315711809948e-5 * z - 1.388731625493765e-3) * z
                    + 4.166664568298827e-2) * z - 0.5)
    q = n.astype(I32)
    odd = (q & 1) == 1
    s, c = jnp.where(odd, c, s), jnp.where(odd, s, c)
    return jnp.where((q & 2) == 2, -s, s), jnp.where(((q + 1) & 2) == 2, -c, c)


def _pk(x):
    return pltpu.bitcast(x.astype(BF16), U32)


def _bf(words):
    return pltpu.bitcast(words, BF16)


def _layernorm(load):
    def mean(term, every):
        acc = [term(load(i)) for i in range(4)]
        for i in range(4, D // 8):
            acc[i % 4] = acc[i % 4] + term(load(i))
            if i % every == every - 1:
                yield
        tot = jnp.sum((acc[0] + acc[1]) + (acc[2] + acc[3]), axis=0, keepdims=True)
        return jnp.broadcast_to(tot * (1.0 / D), (8, T1))

    mu = yield from mean(lambda x: x, 32)
    var = yield from mean(lambda x: (x - mu) * (x - mu), 10)
    rs = jax.lax.rsqrt(var + 1e-5)
    return lambda i: jnp.concatenate([(load(2 * i + s) - mu) * rs for s in range(2)], axis=0)


def _items(n):
    return lambda fn: lambda *args: (fn(*args), n)


def _interleave(mxu, vpu):
    (mg, mn), (vg, vn) = [((v for g, _ in w for v in g), sum(n for _, n in w)) for w in (mxu, vpu)]
    done = 0
    for i in range(mn):
        next(mg)
        while done < vn and done * mn < (i + LEAD) * vn * RATE:
            next(vg)
            done += 1
    for g in (mg, vg):
        for _ in g:
            pass


def _strassen_lhs(a11, a12, a21, a22):
    return a11 + a22, a22, a21 + a22, a11 + a12, a11, a12 - a22, a21 - a11


def _strassen_rhs(b11, b12, b21, b22):
    return b11 + b22, b21 - b11, b11, b22, b12 - b22, b21 + b22, b11 + b12


def _strassen(prod):
    m1, m4, m2 = prod(0), prod(1), prod(2)
    yield 1, 0, m2 + m4
    c11, c22 = m1 + m4, m1 - m2
    m5, m3 = prod(3), prod(4)
    yield 0, 1, m3 + m5
    c11, c22 = c11 - m5, c22 + m3
    yield 0, 0, c11 + prod(5)
    yield 1, 1, c22 + prod(6)


def _rows(i, n):
    return slice(i * n, i * n + n)


def _ds(start, n):
    return pl.ds(start if isinstance(start, int) else pl.multiple_of(start, n), n)


def _pipeline(n, depth, step, bufs):
    def static(i):
        step(i, bufs[i % 2], bufs[1 - i % 2], [s for s in range(depth) if 0 <= i - s < n])

    def body(i, _):
        for par in range(2):
            pl.when(i % 2 == par)(lambda: step(i, bufs[par], bufs[1 - par], list(range(depth))))

    for i in range(depth - 1):
        static(i)
    jax.lax.fori_loop(depth - 1, n, body, None)
    for i in range(n, n + depth - 1):
        static(i)


def _kernel(u_hbm, are, aim, bre, bim, cre, cim, ldt, dsk, wqkv_hbm, wo_hbm, f_hbm, out_hbm,
            io, wq_in, wo_in, fm, ws, wp, lam, dtc, k0s, ta, tb, kf,
            xr, xn, ca, cb, kv, xq, qs, oe, oo, ob, zs, sems):
    cp_u = [pltpu.make_async_copy(u_hbm.bitcast(U32).at[:, h, :], io.at[h], sems.at[3 + h])
            for h in range(PH // 2)]
    cp_o = [pltpu.make_async_copy(io.at[h], out_hbm.bitcast(U32).at[:, h, :], sems.at[3 + h])
            for h in range(PH // 2)]
    cp_f = pltpu.make_async_copy(f_hbm, fm, sems.at[0])
    cp_wq = pltpu.make_async_copy(wqkv_hbm, wq_in, sems.at[1])
    cp_wo = pltpu.make_async_copy(wo_hbm, wo_in, sems.at[2])
    for cp in [cp_wq, cp_wo, cp_f] + cp_u:
        cp.start()

    lane = jax.lax.broadcasted_iota(I32, (8, T1), 1)
    zs[0] = 0

    def zero_rows(k):
        return pl.multiple_of((zs[0] >> k) * 8, 8)

    def xs(p):
        return xr.at[p]

    def region(mxu, vpu):
        pl.when(zs[0] == 0)(lambda: _interleave(mxu, vpu))

    dt_row = jnp.exp(ldt[...].astype(F32).reshape(1, D)).astype(BF16).astype(F32)
    ds_row = dsk[...].astype(F32).reshape(1, D)
    for j in range(4):
        dtc[0, _rows(j, 128), :] = jnp.broadcast_to(dt_row[:, _rows(j, 128)], (128, 128)).T
        dtc[1, _rows(j, 128), :] = jnp.broadcast_to(ds_row[:, _rows(j, 128)], (128, 128)).T
    big = None
    for j in range(D // 16):
        r = _rows(j, 16)
        theta = dtc[0, r, :] * aim[r, :].astype(F32)
        mag = jnp.exp(dtc[0, r, :] * are[r, :].astype(F32))
        sn, cs = _sincos(theta)
        lam[0, r, :] = mag * cs
        lam[1, r, :] = mag * sn
        sc = dtc[0, r, :] * (2.0 / L)
        w = _cmul((cre[r, :].astype(F32), cim[r, :].astype(F32)),
                  (bre[r, :].astype(F32) * sc, bim[r, :].astype(F32) * sc))
        lam[2, r, :] = w[0]
        lam[3, r, :] = w[1]
        k0s[r, :] = jnp.sum(w[0], axis=1, keepdims=True) + dtc[1, r, :] * (2.0 / L)
        big = jnp.abs(theta) if big is None else jnp.maximum(big, jnp.abs(theta))

    @pl.when(jnp.logical_not(jnp.max(big) <= 8192.0))
    def _():
        def body(i, _):
            rows = pl.ds(pl.multiple_of(i * 16, 16), 16)
            th = dtc[0, rows, :] * aim[rows, :].astype(F32)
            mg = jnp.exp(dtc[0, rows, :] * are[rows, :].astype(F32))
            lam[0, rows, :] = mg * jnp.cos(th)
            lam[1, rows, :] = mg * jnp.sin(th)
        jax.lax.fori_loop(0, D // 16, body, None)

    def tap_tables(blk, e, dst, zero):
        rows = _ds(blk * 32 + 8 * e, 8)
        w = (lam[2, rows, :], lam[3, rows, :])

        def put(row, a, b):
            for z in range(2):
                dst[pl.ds(zero + TZ * z + row, 8, stride=QS), :] = pltpu.pack_elementwise(
                    [a[z], b[z]], packed_dtype=BF16)

        l1 = (lam[0, rows, :], lam[1, rows, :])
        l2 = _csq(l1)
        l16 = _csq(_csq(_csq(l2)))
        m1 = (l16[0], -l16[1])
        m2 = _csq(m1)
        a, b = _cmul(w, l1), _cmul(w, l2)
        c, d = m2, _cmul(m1, m2)
        put(16 * e, (jnp.ones_like(m1[0]), jnp.zeros_like(m1[0])), m1)
        keep = {}
        for j in range(1, 16):
            if j <= 8:
                put(64 + 12 * e + j - 1, a, b)
                keep[2 * j] = b
            if j < 8:
                a, b = _cmul(a, l2), _cmul(b, l2)
            put(16 * e + j, c, d)
            if j == 8:
                l512 = _csq((c[0], -c[1]))
                put(64 + 12 * e + 8, _cmul(keep[4], l512), _cmul(keep[12], l512))
                a, b = keep[8], keep[16]
            if j in (10, 12, 14):
                a, b = _cmul(a, l512), _cmul(b, l512)
                put(64 + 12 * e + 4 + j // 2, a, b)
            if j < 15:
                c, d = _cmul(c, m2), _cmul(d, m2)
            if j in (7, 15):
                yield

    def tap_sums(i, src, dst, zero):
        acc = None
        for z in range(2):
            rhs = _bf(src[pl.ds(TZ * z + QS * i, 64), :])
            lhs = _bf(src[pl.ds(TZ * z + QS * i + 64, 48), :])
            d = jax.lax.dot_general(lhs, rhs, NT, preferred_element_type=F32)
            acc = d if acc is None else acc + d
        for r in range(3):
            pc = [acc[_rows(3 * e + r, 8)] for e in range(4)]
            dst[pl.ds(zero + 2 * TZ + ZS * i + 8 * r, 8), :] = pltpu.bitcast(jnp.where(
                lane < 64, jnp.where(lane < 32, pc[0], pc[1]),
                jnp.where(lane < 96, pc[2], pc[3])), U32)

    def tap_blocks(blk, e, src):
        def at(r, g):
            z = pltpu.bitcast(src[pl.ds(2 * TZ + r, 8, stride=ZS), :], F32)
            return z if g == e else pltpu.roll(z, (32 * (g - e)) % 128, 1)

        def full(r, r1):
            return jnp.where(lane < 64, jnp.where(lane < 32, at(r, 0), at(r1, 1)),
                             jnp.where(lane < 96, at(r1 + 2, 2), at(r1 + 4, 3)))

        rows = _ds(blk * 32 + 8 * e, 8)
        e8, e16 = full(7, 18), full(15, 19)
        e0 = jnp.where(lane == 0, k0s[rows, :], pltpu.roll(e16, 1, 1))
        e4 = jnp.where(lane < 32, at(3, 0), at(16, 1))
        e12 = jnp.where(lane < 32, at(11, 0), at(17, 1))
        k4, k12 = jnp.where(lane < 64, e4, e0), jnp.where(lane < 64, e12, e16)
        far = {1: e0, 2: e0, 3: k4, 5: jnp.where(lane < 64, e4, e8), 6: e8, 7: e8, 9: e8,
               10: e8, 11: jnp.where(lane < 64, e12, e8), 13: k12, 14: e16, 15: e16}
        for p, v in ((0, e0), (4, k4), (8, e8), (12, k12)):
            kv[0, p, rows, :] = v
        for p, v in far.items():
            kv[0, p, rows, :] = jnp.where(lane < (16 if p % 2 else 32), at(p - 1, 0), v)

    def tap_step(i, src, dst, stages):
        z1, z2 = zero_rows(1), zero_rows(2)
        for e in range(4):
            tables = tap_tables(i, e, dst, z1) if 0 in stages else iter(())
            for h in range(2):
                next(tables, None)
                if 1 in stages:
                    tap_sums(2 * e + h, src, dst, z2)
            if 2 in stages:
                tap_blocks(i - 2, e, src)

    def lane_dft(load, q, dst, zero):
        x0, x1 = [jax.lax.dot_general(load(p), _bf(fm[p]), NN, preferred_element_type=F32)
                  for p in (q, q + 8)]
        for i in range(CB // 8):
            r = _rows(i, 8)
            dst[q, pl.ds(zero + 8 * i, 8), :] = x0[r] + x1[r]
            dst[q + 8, pl.ds(zero + 8 * i, 8), :] = x0[r] - x1[r]

    def tap_coefs(blk, u, src):
        i, odd = u // 2, u % 2
        r, ro = _rows(i, 8), _ds(blk * CB + 8 * i, 8)
        co = _conv_coefs([(src[8 * odd + c, r, :T1], src[8 * odd + c, r, T1:]) for c in range(8)],
                         4 * odd)
        for n, v in enumerate(co):
            kf[10 * odd + n, ro, :T1] = v[0]
            kf[10 * odd + n, ro, T1:] = v[1]

    ri = jax.lax.broadcasted_iota(I32, (128, 128), 0)
    ci = jax.lax.broadcasted_iota(I32, (128, 128), 1)
    hit = ci == (ri & 7) * 16 + (ri >> 3)

    def prep_weights(j):
        if j < 6:
            sel = jnp.where(hit, 1.0 if j < 4 else 0.25, 0.0).astype(BF16)
            src = [wq_in[:, _rows(c, 128)] for c in ((4 + j, 8 + j) if j < 4 else (j - 4, j - 2))]
        else:
            sel = jnp.where(ri == ci, 1.0, 0.0).astype(BF16)
            src = [_bf(wp[:, _rows(c, 128)]) for c in (j - 6, j - 4)]
        top, bot = [jax.lax.dot_general(sel, w, NT, preferred_element_type=F32) for w in src]
        for i, a in enumerate(_strassen_lhs(top[:, :HD], top[:, HD:], bot[:, :HD], bot[:, HD:])):
            ws[i, _rows(j, 64), :] = _pk(a)

    def permute_wo(j):
        sel = jnp.where(hit, 1.0, 0.0).astype(BF16)
        wp[_rows(j, 64), :] = _pk(jnp.dot(sel, wo_in[_rows(j, 128), :],
                                          preferred_element_type=F32))

    def load_pair(h):
        for j in range(4):
            wds = io[h, :, _rows(j, 128)].T
            xs(2 * h)[_rows(j, 128), :] = pltpu.bitcast(wds << 16, F32)
            xs(2 * h + 1)[_rows(j, 128), :] = pltpu.bitcast(wds & jnp.uint32(0xFFFF0000), F32)
        _interleave([], [norm(h)])

    @_items(24)
    def norm(h):
        for p in (2 * h, 2 * h + 1):
            normed = yield from _layernorm(lambda i: xs(p)[_rows(i, 8), :])
            for i in range(D // 16):
                xn[p, _rows(i, 16), :] = normed(i).astype(BF16)
                if i % 8 == 7:
                    yield

    _pipeline(D // 32, 3, tap_step, (ta, tb))
    for cp in [cp_wq, cp_wo, cp_f] + cp_u:
        cp.wait()
    nc = D // CB

    def spec_step(i, src, dst, stages):
        for q in range(8):
            if 0 in stages:
                lane_dft(lambda p: kv[0, p, _ds(i * CB, CB), :], q, dst, 0)
            if 1 in stages:
                tap_coefs(i - 1, 2 * q, src)
                tap_coefs(i - 1, 2 * q + 1, src)

    _pipeline(nc, 2, spec_step, (ca, cb))
    for h in range(PH // 2):
        if h < 4:
            permute_wo(h)
        prep_weights(h)
        load_pair(h)

    def phase_conv(blk, u, src, dst, zero):
        i, odd = u // 2, u % 2
        r, ro = _rows(i, 8), _ds(blk * CB + 8 * i, 8)
        ids = iter(range(10 * odd, NCOEF))

        def coef():
            n = next(ids)
            return kf[n, ro, :T1], kf[n, ro, T1:]

        y = _conv([(src[8 * odd + c, r, :T1], src[8 * odd + c, r, T1:]) for c in range(8)],
                  4 * odd, coef)
        for c in range(8):
            dst[PH + 8 * odd + c, pl.ds(zero + 8 * i, 8), :T1] = y[c][0]
            dst[PH + 8 * odd + c, pl.ds(zero + 8 * i, 8), T1:] = y[c][1]

    def lane_idft(blk, q, src):
        a, b = src[PH + q], src[PH + 8 + q]
        for p, v in ((q, a + b), (q + 8, a - b)):
            xs(p)[_ds(blk * CB, CB), :] += jax.lax.dot_general(
                v, _bf(fm[p]), NT, preferred_element_type=F32)

    def conv_step(i, src, dst, stages):
        z1, z2 = zero_rows(1), zero_rows(2)
        for q in range(8):
            if 1 in stages:
                phase_conv(i - 1, 2 * q, src, dst, z2)
            if 0 in stages:
                lane_dft(lambda p: xn[p, _ds(i * CB, CB), :], q, dst, z1)
            if 1 in stages:
                phase_conv(i - 1, 2 * q + 1, src, dst, z2)
            if 2 in stages:
                lane_idft(i - 2, q, src)

    @_items(32)
    def norm_pair(g):
        p = 4 * (g % 4) + g // 4
        a = yield from _layernorm(lambda i: xs(p)[_rows(i, 8), :])
        b = yield from _layernorm(lambda i: xs(p + 2)[_rows(i, 8), :])
        for r in range(HD // 16):
            xq[g, _rows(r, 8), :] = _pk(jnp.concatenate(
                _strassen_rhs(a(r), b(r), a(HD // 16 + r), b(HD // 16 + r)), axis=1))
            yield

    def block_product(row0, nrows, rhs):
        for r in range(nrows // RS):
            w = slice((row0 + r * RS) // 2, (row0 + r * RS + RS) // 2)
            for half, n, y in _strassen(lambda i: jnp.dot(
                    _bf(ws[i, w, :]), _bf(rhs[:, _rows(i, T1)]), preferred_element_type=F32)):
                yield half, n, r * RS, y

    @_items(4 * D // RS)
    def keys_values(g):
        for half, n, row, y in block_product(0, D, xq.at[g]):
            yield
            m = 2 * (g % 4) + n
            kv[g // 4, PH * half + WIN - 1 + m, pl.ds(row, RS), :] = y
            if m:
                kv[g // 4, PH * half + m - 1, pl.ds(row, RS), :] = pltpu.roll(y, 1, 1)

    @_items(4 * HD // RS)
    def queries(g):
        for half, n, row, y in block_product(D, HD, xq.at[g]):
            yield
            qs[g % 3, n, pl.ds(HD * half + row, RS), :] = y

    @_items(68)
    def attend(par, m):
        for hg in (0, 2, 1, 3):
            lg = []
            for j in range(WIN):
                acc = [None, None]
                for dh in range(16):
                    r = _rows(16 * hg + dh, 8)
                    t = qs[(4 * par + m // 2) % 3, m % 2, r, :] * kv[par, WIN - 1 + m - j, r, :]
                    acc[dh % 2] = t if dh < 2 else acc[dh % 2] + t
                lg.append(acc[0] + acc[1])
                yield
            for j in range(m + 1, WIN):
                lg[j] = jnp.where(lane == 0, -1e9, lg[j])
            mx = lg[0]
            for j in range(1, WIN):
                mx = jnp.maximum(mx, lg[j])
            ex = [jnp.exp(t - mx) for t in lg]
            den = ex[0]
            for j in range(1, WIN):
                den = den + ex[j]
            inv = 1.0 / den
            pr = [t * inv for t in ex]
            yield

            def out(dh):
                r = _rows(16 * hg + dh, 8)
                acc = pr[0] * kv[par, PH + WIN - 1 + m, r, :]
                for j in range(1, WIN):
                    acc = acc + pr[j] * kv[par, PH + WIN - 1 + m - j, r, :]
                return acc

            for d2 in range(8):
                o = jnp.concatenate([out(2 * d2), out(2 * d2 + 1)], axis=0)
                r = _rows(8 * hg + d2, 16)
                if par == 0:
                    oe[m, r, :] = o
                elif hg < 2:
                    oo[m % 2, r, :] = o
                else:
                    r1 = _rows(8 * (hg - 2) + d2, 16)
                    ob[m % 4, _rows(8 * (hg - 2) + d2, 8), :] = _pk(jnp.concatenate(
                        _strassen_rhs(oe[m, r1, :], oo[m % 2, r1, :], oe[m, r, :], o), axis=1))
                yield

    @_items(4 * HD // RS)
    def project(h):
        for half, n, row, y in block_product(D + HD, HD, ob.at[h % 4]):
            yield
            xs(2 * h + n)[pl.ds(HD * half + row, RS), :] += y

    @_items(4)
    def store_pair(h):
        for j in range(4):
            io[h, :, _rows(j, 128)] = pltpu.pack_elementwise(
                [xs(2 * h + n)[_rows(j, 128), :] for n in range(2)], packed_dtype=BF16).T
            yield

    def layer(it, c):
        def finish(hs, mxu, vpu):
            region(mxu, [fn(h) for h in hs for fn in (store_pair, norm)] + vpu)

            @pl.when(it == 1)
            def _():
                for h in hs:
                    cp_o[h].start()

        _pipeline(nc, 3, conv_step, (ca, cb))
        _interleave([], [norm_pair(0)])

        @pl.when(zs[0] == 0)
        def _():
            for g in range(3):
                _interleave([keys_values(g)], [norm_pair(g + 1), norm_pair(g + 5)])
            _interleave([keys_values(3), queries(0)], [norm_pair(4)])

        for g in range(4):
            region([keys_values(g + 4), queries(g + 1)], [attend(0, 2 * g), attend(0, 2 * g + 1)])
        region([queries(5), queries(6)], [attend(1, 0), attend(1, 1)])
        region([queries(7), project(0), project(1)], [attend(1, 2), attend(1, 3)])
        finish([0], [project(2), project(3)], [attend(1, 4), attend(1, 5)])
        finish([1], [project(4), project(5)], [attend(1, 6), attend(1, 7)])
        finish([2, 3, 4, 5], [project(6), project(7)], [])
        pl.when(it == 0)(lambda: _interleave([], [norm(6), norm(7)]))

    jax.lax.fori_loop(0, 2, layer, None)
    for h in (6, 7):
        _interleave([], [store_pair(h)])
        cp_o[h].start()
    for cp in cp_o:
        cp.wait()


@jax.jit
def pallas_interleave_layers__ssm_conv_s4__sliding_local_dilated__prompt_kernel(
    A_u: jax.Array,
    A_A_re: jax.Array,
    A_A_im: jax.Array,
    A_B_re: jax.Array,
    A_B_im: jax.Array,
    A_C_re: jax.Array,
    A_C_im: jax.Array,
    A_log_dt: jax.Array,
    A_Dskip: jax.Array,
    B_x: jax.Array,
    B_wqkv: jax.Array,
    B_wo: jax.Array,
):
    del B_x
    hbm = pl.BlockSpec(memory_space=pl.ANY)
    vmem = pl.BlockSpec(memory_space=pltpu.VMEM)
    out = pl.pallas_call(
        _kernel,
        in_specs=[hbm] + [vmem] * 8 + [hbm] * 3,
        out_specs=hbm,
        out_shape=jax.ShapeDtypeStruct((T1, PH, D), BF16),
        scratch_shapes=[
            pltpu.VMEM((PH // 2, T1, D), U32),
            pltpu.VMEM((D, 3 * D), BF16),
            pltpu.VMEM((D, D), BF16),
            pltpu.VMEM((PH, T1 // 2, 2 * T1), U32),
            pltpu.VMEM((7, D, HD), U32),
            pltpu.VMEM((D // 2, D), U32),
            pltpu.VMEM((4, D, NS), F32),
            pltpu.VMEM((2, D, NS), F32),
            pltpu.VMEM((D, T1), F32),
            pltpu.VMEM((2 * TZ + 9 * ZS + 4, NS), U32),
            pltpu.VMEM((2 * TZ + 9 * ZS + 4, NS), U32),
            pltpu.VMEM((NCOEF, D, 2 * T1), F32),
            pltpu.VMEM((PH, D, T1), F32),
            pltpu.VMEM((PH, D, T1), BF16),
            pltpu.VMEM((2 * PH, CB, 2 * T1), F32),
            pltpu.VMEM((2 * PH, CB, 2 * T1), F32),
            pltpu.VMEM((2, 2 * PH, D, T1), F32),
            pltpu.VMEM((PH // 2, HD // 2, 7 * T1), U32),
            pltpu.VMEM((3, 2, D, T1), F32),
            pltpu.VMEM((WIN, D, T1), F32),
            pltpu.VMEM((2, HD, T1), F32),
            pltpu.VMEM((4, HD // 2, 7 * T1), U32),
            pltpu.SMEM((1,), I32),
            pltpu.SemaphoreType.DMA((3 + PH // 2,)),
        ],
        compiler_params=pltpu.CompilerParams(vmem_limit_bytes=100 * 1024 * 1024),
    )(A_u.reshape(T1, PH, D), A_A_re, A_A_im, A_B_re, A_B_im, A_C_re, A_C_im,
      A_log_dt, A_Dskip, B_wqkv, B_wo,
      _dft_matrices())
    return out.reshape(1, L, D)
```

```python
import numpy as np

import jax
import jax.numpy as jnp
import jax.experimental.pallas as pl
import jax.experimental.pallas.tpu as pltpu

F32, BF16, U32, I32 = jnp.float32, jnp.bfloat16, jnp.uint32, jnp.int32
L, D, NS = 2048, 512, 128
PH, T1 = 16, 128
WIN = 8
NN = (((1,), (0,)), ((), ()))
NT = (((1,), (1,)), ((), ()))
QS = 116
TZ = 8 * QS
ZS = 28
_H = float(np.sqrt(0.5))
NCOEF = 22
HD = D // 2
RS = 64
JB = 4
LEAD = 1
RATE = 1.0
CB = 64


def _dft_matrices():
    t = 16 * np.arange(T1)[None, :, None] + np.arange(PH)[:, None, None]
    k = np.arange(T1)[None, None, :] + 0.5
    phi = 2.0 * np.pi * k * t / (2 * L)
    f = np.concatenate([np.cos(phi), -np.sin(phi)], axis=-1).astype(np.float32)
    bits = f.astype(BF16).view(np.uint16).astype(np.uint32)
    return bits[:, 0::2] | (bits[:, 1::2] << 16)


def _cmul(a, b):
    return a[0] * b[0] - a[1] * b[1], a[0] * b[1] + a[1] * b[0]


def _csq(a):
    t = a[0] * a[1]
    return a[0] * a[0] - a[1] * a[1], t + t


def _cadd(a, b):
    return a[0] + b[0], a[1] + b[1]


def _csub(a, b):
    return a[0] - b[0], a[1] - b[1]


def _rot8(x, e):
    s, d = x[0] + x[1], x[0] - x[1]
    return {1: (d * _H, s * _H), 3: (s * -_H, d * _H), 5: (d * -_H, s * -_H), 7: (s * _H, d * -_H)}[e]


def _split(x, e):
    n = len(x) // 2
    lo, hi = x[:n], x[n:]
    if e == 4:
        return ([(a[0] - b[1], a[1] + b[0]) for a, b in zip(lo, hi)],
                [(a[0] + b[1], a[1] - b[0]) for a, b in zip(lo, hi)])
    if e:
        hi = [_rot8(b, e // 2) for b in hi]
    return [_cadd(a, b) for a, b in zip(lo, hi)], [_csub(a, b) for a, b in zip(lo, hi)]


def _merge(p, m, e):
    lo = [_cadd(a, b) for a, b in zip(p, m)]
    if e == 4:
        return lo + [(a[1] - b[1], b[0] - a[0]) for a, b in zip(p, m)]
    hi = [_csub(a, b) for a, b in zip(p, m)]
    return lo + ([_rot8(b, 8 - e // 2) for b in hi] if e else hi)


def _conv_coefs(k, e):
    if len(k) == 1:
        return [(k[0][0] * 0.5, k[0][1] * 0.5)]
    if len(k) == 2 and e % 4:
        if e % 2:
            top = _csub(_rot8(k[1], e), k[0])
        elif e == 2:
            top = (-k[1][1] - k[0][0], k[1][0] - k[0][1])
        else:
            top = (k[1][1] - k[0][0], -k[1][0] - k[0][1])
        return [k[0], top, _csub(k[1], k[0])]
    p, m = _split(k, e)
    return _conv_coefs(p, e // 2) + _conv_coefs(m, e // 2 + 4)


def _conv(x, e, coef):
    if len(x) == 1:
        return [_cmul(x[0], coef())]
    if len(x) == 2 and e % 4:
        both = _cmul(_cadd(x[0], x[1]), coef())
        return [_cadd(both, _cmul(x[1], coef())), _cadd(both, _cmul(x[0], coef()))]
    p, m = _split(x, e)
    return _merge(_conv(p, e // 2, coef), _conv(m, e // 2 + 4, coef), e)


def _sincos(x):
    n = jnp.floor(x * float(2.0 / np.pi) + 0.5)
    r = ((x - n * 1.5703125) - n * 4.837512969970703125e-4) - n * 7.54978995489188216e-8
    z = r * r
    s = r + r * z * ((-1.9515295891e-4 * z + 8.3321608736e-3) * z - 1.6666654611e-1)
    c = 1.0 + z * (((2.443315711809948e-5 * z - 1.388731625493765e-3) * z
                    + 4.166664568298827e-2) * z - 0.5)
    q = n.astype(I32)
    odd = (q & 1) == 1
    s, c = jnp.where(odd, c, s), jnp.where(odd, s, c)
    return jnp.where((q & 2) == 2, -s, s), jnp.where(((q + 1) & 2) == 2, -c, c)


def _pk(x):
    return pltpu.bitcast(x.astype(BF16), U32)


def _zip(x):
    return jnp.concatenate(
        [pltpu.pack_elementwise([x[i:i + 8], x[i + 8:i + 16]], packed_dtype=BF16)
         for i in range(0, x.shape[0], 16)], axis=0)


def _bf(words):
    return pltpu.bitcast(words, BF16)


def _layernorm(load):
    def mean(term, every):
        acc = [term(load(i)) for i in range(4)]
        for i in range(4, D // 8):
            acc[i % 4] = acc[i % 4] + term(load(i))
            if i % every == every - 1:
                yield
        tot = jnp.sum((acc[0] + acc[1]) + (acc[2] + acc[3]), axis=0, keepdims=True)
        return jnp.broadcast_to(tot * (1.0 / D), (8, T1))

    mu = yield from mean(lambda x: x, 32)
    var = yield from mean(lambda x: (x - mu) * (x - mu), 10)
    rs = jax.lax.rsqrt(var + 1e-5)
    return lambda i: jnp.concatenate([(load(2 * i + s) - mu) * rs for s in range(2)], axis=0)


def _items(n):
    return lambda fn: lambda *args: (fn(*args), n)


def _interleave(mxu, vpu):
    (mg, mn), (vg, vn) = [((v for g, _ in w for v in g), sum(n for _, n in w)) for w in (mxu, vpu)]
    done = 0
    for i in range(mn):
        next(mg)
        while done < vn and done * mn < (i + LEAD) * vn * RATE:
            next(vg)
            done += 1
    for g in (mg, vg):
        for _ in g:
            pass


def _strassen_lhs(a11, a12, a21, a22):
    return a11 + a22, a22, a21 + a22, a11 + a12, a11, a12 - a22, a21 - a11


def _strassen_rhs(b11, b12, b21, b22):
    ops = (b11 + b22, b21 - b11, b11, b22, b12 - b22, b21 + b22, b11 + b12)
    return jnp.concatenate([_zip(v) for v in ops], axis=1)


def _strassen(prod, emit):
    m1 = prod(0)
    yield
    m4 = prod(1)
    c11 = m1 + m4
    yield
    m2 = prod(2)
    emit(1, 0, m2 + m4)
    c22 = m1 - m2
    yield
    m5 = prod(3)
    c11 = c11 - m5
    yield
    m3 = prod(4)
    emit(0, 1, m3 + m5)
    c22 = c22 + m3
    yield
    emit(0, 0, c11 + prod(5))
    yield
    emit(1, 1, c22 + prod(6))
    yield


def _rows(i, n):
    return slice(i * n, i * n + n)


def _ds(start, n):
    return pl.ds(start if isinstance(start, int) else pl.multiple_of(start, n), n)


def _pipeline(n, depth, step, bufs):
    def static(i):
        step(i, bufs[i % 2], bufs[1 - i % 2], [s for s in range(depth) if 0 <= i - s < n])

    def body(i, _):
        for par in range(2):
            pl.when(i % 2 == par)(lambda: step(i, bufs[par], bufs[1 - par], list(range(depth))))

    for i in range(depth - 1):
        static(i)
    jax.lax.fori_loop(depth - 1, n, body, None)
    for i in range(n, n + depth - 1):
        static(i)


def _kernel(u_hbm, are, aim, bre, bim, cre, cim, ldt, dsk, wqkv_hbm, wo_hbm, f_hbm, out_hbm,
            io, wq_in, wo_in, fm, ws, wp, lam, dtc, k0s, ta, tb, kf,
            xr, xn, ca, cb, kv, xq, qs, oe, oo, ob, zs, sems):
    cp_u = [pltpu.make_async_copy(u_hbm.bitcast(U32).at[:, h, :], io.at[h], sems.at[3 + h])
            for h in range(PH // 2)]
    cp_o = [pltpu.make_async_copy(io.at[h], out_hbm.bitcast(U32).at[:, h, :], sems.at[3 + h])
            for h in range(PH // 2)]
    cp_f = pltpu.make_async_copy(f_hbm, fm, sems.at[0])
    cp_wq = pltpu.make_async_copy(wqkv_hbm, wq_in, sems.at[1])
    cp_wo = pltpu.make_async_copy(wo_hbm, wo_in, sems.at[2])
    for cp in [cp_wq, cp_wo, cp_f] + cp_u:
        cp.start()

    lane = jax.lax.broadcasted_iota(I32, (8, T1), 1)
    zs[0] = 0

    def zero_rows(k):
        return pl.multiple_of((zs[0] >> k) * 8, 8)

    def xs(p):
        return xr.at[p]

    def region(mxu, vpu):
        pl.when(zs[0] == 0)(lambda: _interleave(mxu, vpu))

    dt_row = jnp.exp(ldt[...].astype(F32).reshape(1, D)).astype(BF16).astype(F32)
    ds_row = dsk[...].astype(F32).reshape(1, D)
    for j in range(4):
        dtc[0, _rows(j, 128), :] = jnp.broadcast_to(dt_row[:, _rows(j, 128)], (128, 128)).T
        dtc[1, _rows(j, 128), :] = jnp.broadcast_to(ds_row[:, _rows(j, 128)], (128, 128)).T
    big = None
    for j in range(D // 16):
        r = _rows(j, 16)
        theta = dtc[0, r, :] * aim[r, :].astype(F32)
        mag = jnp.exp(dtc[0, r, :] * are[r, :].astype(F32))
        sn, cs = _sincos(theta)
        lam[0, r, :] = mag * cs
        lam[1, r, :] = mag * sn
        sc = dtc[0, r, :] * (2.0 / L)
        w = _cmul((cre[r, :].astype(F32), cim[r, :].astype(F32)),
                  (bre[r, :].astype(F32) * sc, bim[r, :].astype(F32) * sc))
        lam[2, r, :] = w[0]
        lam[3, r, :] = w[1]
        k0s[r, :] = jnp.sum(w[0], axis=1, keepdims=True) + dtc[1, r, :] * (2.0 / L)
        big = jnp.abs(theta) if big is None else jnp.maximum(big, jnp.abs(theta))

    @pl.when(jnp.logical_not(jnp.max(big) <= 8192.0))
    def _():
        def body(i, _):
            rows = pl.ds(pl.multiple_of(i * 16, 16), 16)
            th = dtc[0, rows, :] * aim[rows, :].astype(F32)
            mg = jnp.exp(dtc[0, rows, :] * are[rows, :].astype(F32))
            lam[0, rows, :] = mg * jnp.cos(th)
            lam[1, rows, :] = mg * jnp.sin(th)
        jax.lax.fori_loop(0, D // 16, body, None)

    def tap_tables(blk, e, dst, zero):
        rows = _ds(blk * 32 + 8 * e, 8)
        w = (lam[2, rows, :], lam[3, rows, :])

        def put(row, a, b):
            for z in range(2):
                dst[pl.ds(zero + TZ * z + row, 8, stride=QS), :] = pltpu.pack_elementwise(
                    [a[z], b[z]], packed_dtype=BF16)

        l1 = (lam[0, rows, :], lam[1, rows, :])
        l2 = _csq(l1)
        l16 = _csq(_csq(_csq(l2)))
        m1 = (l16[0], -l16[1])
        m2 = _csq(m1)
        a, b = _cmul(w, l1), _cmul(w, l2)
        c, d = m2, _cmul(m1, m2)
        put(16 * e, (jnp.ones_like(m1[0]), jnp.zeros_like(m1[0])), m1)
        keep = {}
        for j in range(1, 16):
            if j <= 8:
                put(64 + 12 * e + j - 1, a, b)
                keep[2 * j] = b
            if j < 8:
                a, b = _cmul(a, l2), _cmul(b, l2)
            put(16 * e + j, c, d)
            if j == 8:
                l512 = _csq((c[0], -c[1]))
                put(64 + 12 * e + 8, _cmul(keep[4], l512), _cmul(keep[12], l512))
                a, b = keep[8], keep[16]
            if j in (10, 12, 14):
                a, b = _cmul(a, l512), _cmul(b, l512)
                put(64 + 12 * e + 4 + j // 2, a, b)
            if j < 15:
                c, d = _cmul(c, m2), _cmul(d, m2)
            if j in (7, 15):
                yield

    def tap_sums(i, src, dst, zero):
        acc = None
        for z in range(2):
            rhs = _bf(src[pl.ds(TZ * z + QS * i, 64), :])
            lhs = _bf(src[pl.ds(TZ * z + QS * i + 64, 48), :])
            d = jax.lax.dot_general(lhs, rhs, NT, preferred_element_type=F32)
            acc = d if acc is None else acc + d
        for r in range(3):
            pc = [acc[_rows(3 * e + r, 8)] for e in range(4)]
            dst[pl.ds(zero + 2 * TZ + ZS * i + 8 * r, 8), :] = pltpu.bitcast(jnp.where(
                lane < 64, jnp.where(lane < 32, pc[0], pc[1]),
                jnp.where(lane < 96, pc[2], pc[3])), U32)

    def tap_blocks(blk, e, src):
        def at(r, g):
            z = pltpu.bitcast(src[pl.ds(2 * TZ + r, 8, stride=ZS), :], F32)
            return z if g == e else pltpu.roll(z, (32 * (g - e)) % 128, 1)

        def full(r, r1):
            return jnp.where(lane < 64, jnp.where(lane < 32, at(r, 0), at(r1, 1)),
                             jnp.where(lane < 96, at(r1 + 2, 2), at(r1 + 4, 3)))

        rows = _ds(blk * 32 + 8 * e, 8)
        e8, e16 = full(7, 18), full(15, 19)
        e0 = jnp.where(lane == 0, k0s[rows, :], pltpu.roll(e16, 1, 1))
        e4 = jnp.where(lane < 32, at(3, 0), at(16, 1))
        e12 = jnp.where(lane < 32, at(11, 0), at(17, 1))
        k4, k12 = jnp.where(lane < 64, e4, e0), jnp.where(lane < 64, e12, e16)
        far = {1: e0, 2: e0, 3: k4, 5: jnp.where(lane < 64, e4, e8), 6: e8, 7: e8, 9: e8,
               10: e8, 11: jnp.where(lane < 64, e12, e8), 13: k12, 14: e16, 15: e16}
        for p, v in ((0, e0), (4, k4), (8, e8), (12, k12)):
            kv[0, p, rows, :] = v
        for p, v in far.items():
            kv[0, p, rows, :] = jnp.where(lane < (16 if p % 2 else 32), at(p - 1, 0), v)

    def tap_step(i, src, dst, stages):
        z1, z2 = zero_rows(1), zero_rows(2)
        for e in range(4):
            tables = tap_tables(i, e, dst, z1) if 0 in stages else iter(())
            for h in range(2):
                next(tables, None)
                if 1 in stages:
                    tap_sums(2 * e + h, src, dst, z2)
            if 2 in stages:
                tap_blocks(i - 2, e, src)

    def lane_dft(load, q, dst, zero):
        x0, x1 = [jax.lax.dot_general(load(p), _bf(fm[p]), NN, preferred_element_type=F32)
                  for p in (q, q + 8)]
        for i in range(CB // 8):
            r = _rows(i, 8)
            dst[q, pl.ds(zero + 8 * i, 8), :] = x0[r] + x1[r]
            dst[q + 8, pl.ds(zero + 8 * i, 8), :] = x0[r] - x1[r]

    def tap_coefs(blk, u, src):
        i, odd = u // 2, u % 2
        r, ro = _rows(i, 8), _ds(blk * CB + 8 * i, 8)
        co = _conv_coefs([(src[8 * odd + c, r, :T1], src[8 * odd + c, r, T1:]) for c in range(8)],
                         4 * odd)
        for n, v in enumerate(co):
            kf[10 * odd + n, ro, :T1] = v[0]
            kf[10 * odd + n, ro, T1:] = v[1]

    ri = jax.lax.broadcasted_iota(I32, (128, 128), 0)
    ci = jax.lax.broadcasted_iota(I32, (128, 128), 1)
    hit = ci == (ri & 7) * 16 + (ri >> 3)

    def prep_weights(j):
        if j < 6:
            sel = jnp.where(hit, 1.0 if j < 4 else 0.25, 0.0).astype(BF16)
            src = [_bf(_zip(wq_in[:, _rows(c, 128)].astype(F32)))
                   for c in ((4 + j, 8 + j) if j < 4 else (j - 4, j - 2))]
        else:
            sel = jnp.where(ri == ci, 1.0, 0.0).astype(BF16)
            src = [_bf(wp[:, _rows(c, 128)]) for c in (j - 6, j - 4)]
        top, bot = [jax.lax.dot_general(sel, w, NT, preferred_element_type=F32) for w in src]
        for i, a in enumerate(_strassen_lhs(top[:, :HD], top[:, HD:], bot[:, :HD], bot[:, HD:])):
            ws[i, _rows(j, 64), :] = _pk(a)

    def permute_wo(j):
        sel = jnp.where(hit, 1.0, 0.0).astype(BF16)
        wp[_rows(j, 64), :] = _zip(jnp.dot(sel, wo_in[_rows(j, 128), :],
                                           preferred_element_type=F32))

    def load_pair(h):
        for j in range(4):
            wds = io[h, :, _rows(j, 128)].T
            xs(2 * h)[_rows(j, 128), :] = pltpu.bitcast(wds << 16, F32)
            xs(2 * h + 1)[_rows(j, 128), :] = pltpu.bitcast(wds & jnp.uint32(0xFFFF0000), F32)
        _interleave([], [norm(h)])

    @_items(24)
    def norm(h):
        for p in (2 * h, 2 * h + 1):
            normed = yield from _layernorm(lambda i: xs(p)[_rows(i, 8), :])
            for i in range(D // 16):
                xn[p, _rows(i, 16), :] = normed(i).astype(BF16)
                if i % 8 == 7:
                    yield

    _pipeline(D // 32, 3, tap_step, (ta, tb))
    for cp in [cp_wq, cp_wo, cp_f] + cp_u:
        cp.wait()
    nc = D // CB

    def spec_step(i, src, dst, stages):
        for q in range(8):
            if 0 in stages:
                lane_dft(lambda p: kv[0, p, _ds(i * CB, CB), :], q, dst, 0)
            if 1 in stages:
                tap_coefs(i - 1, 2 * q, src)
                tap_coefs(i - 1, 2 * q + 1, src)

    _pipeline(nc, 2, spec_step, (ca, cb))
    for h in range(PH // 2):
        if h < 4:
            permute_wo(h)
        prep_weights(h)
        load_pair(h)

    def phase_conv(blk, u, src, dst, zero):
        i, odd = u // 2, u % 2
        r, ro = _rows(i, 8), _ds(blk * CB + 8 * i, 8)
        ids = iter(range(10 * odd, NCOEF))

        def coef():
            n = next(ids)
            return kf[n, ro, :T1], kf[n, ro, T1:]

        y = _conv([(src[8 * odd + c, r, :T1], src[8 * odd + c, r, T1:]) for c in range(8)],
                  4 * odd, coef)
        for c in range(8):
            dst[PH + 8 * odd + c, pl.ds(zero + 8 * i, 8), :T1] = y[c][0]
            dst[PH + 8 * odd + c, pl.ds(zero + 8 * i, 8), T1:] = y[c][1]

    def lane_idft(blk, q, src):
        a, b = src[PH + q], src[PH + 8 + q]
        for p, v in ((q, a + b), (q + 8, a - b)):
            xs(p)[_ds(blk * CB, CB), :] += jax.lax.dot_general(
                v, _bf(fm[p]), NT, preferred_element_type=F32)

    def conv_step(i, src, dst, stages):
        z1, z2 = zero_rows(1), zero_rows(2)
        for q in range(8):
            if 1 in stages:
                phase_conv(i - 1, 2 * q, src, dst, z2)
            if 0 in stages:
                lane_dft(lambda p: xn[p, _ds(i * CB, CB), :], q, dst, z1)
            if 1 in stages:
                phase_conv(i - 1, 2 * q + 1, src, dst, z2)
            if 2 in stages:
                lane_idft(i - 2, q, src)

    @_items(32)
    def norm_pair(g):
        p = 4 * (g % 4) + g // 4
        a = yield from _layernorm(lambda i: xs(p)[_rows(i, 8), :])
        b = yield from _layernorm(lambda i: xs(p + 2)[_rows(i, 8), :])
        for r in range(HD // 16):
            xq[g, _rows(r, 8), :] = _strassen_rhs(a(r), b(r), a(HD // 16 + r), b(HD // 16 + r))
            yield

    def block_product(row0, groups, rhs, emit):
        for r in [128 // RS * hg + i for hg in groups for i in range(128 // RS)]:
            w = slice((row0 + r * RS) // 2, (row0 + r * RS + RS) // 2)
            yield from _strassen(
                lambda i: jnp.dot(_bf(ws[i, w, :]), _bf(rhs[:, _rows(i, T1)]),
                                  preferred_element_type=F32),
                lambda half, n, y: emit(half, n, r * RS, y))

    @_items(7 * HD // RS)
    def keys_values(s, g):
        def emit(half, n, row, y):
            m = 2 * (g % 4) + n
            kv[g // 4, PH * half + WIN - 1 + m, pl.ds(row, RS), :] = y
            if m:
                kv[g // 4, PH * half + m - 1, pl.ds(row, RS), :] = pltpu.roll(y, 1, 1)

        return block_product(0, (s, s + 2), xq.at[g], emit)

    @_items(7 * 128 // RS)
    def queries(s, g):
        def emit(half, n, row, y):
            qs[g, n, pl.ds(HD * half + row, RS), :] = y

        return block_product(D, (s,), xq.at[g], emit)

    @_items(34)
    def attend(par, s, m):
        for hg in (s, s + 2):
            lg = [None] * WIN
            for j0 in range(0, WIN, JB):
                for dh in range(16):
                    r = _rows(16 * hg + dh, 8)
                    q = qs[4 * par + m // 2, m % 2, r, :]
                    for j in range(j0, j0 + JB):
                        t = q * kv[par, WIN - 1 + m - j, r, :]
                        lg[j] = t if dh == 0 else lg[j] + t
                    if (dh + 1) % (16 // JB) == 0:
                        yield
            for j in range(m + 1, WIN):
                lg[j] = jnp.where(lane == 0, -1e9, lg[j])
            mx = lg[0]
            for j in range(1, WIN):
                mx = jnp.maximum(mx, lg[j])
            ex = [jnp.exp(t - mx) for t in lg]
            den = ex[0]
            for j in range(1, WIN):
                den = den + ex[j]
            inv = pltpu.reciprocal(den, full_range=False)
            pr = [t * inv for t in ex]
            yield

            def out(dh):
                r = _rows(16 * hg + dh, 8)
                acc = pr[0] * kv[par, PH + WIN - 1 + m, r, :]
                for j in range(1, WIN):
                    acc = acc + pr[j] * kv[par, PH + WIN - 1 + m - j, r, :]
                return acc

            for d2 in range(8):
                o = jnp.concatenate([out(2 * d2), out(2 * d2 + 1)], axis=0)
                r = _rows(8 * hg + d2, 16)
                if par == 0:
                    oe[m, r, :] = o
                elif hg < 2:
                    oo[m % 4, r, :] = o
                else:
                    r1 = _rows(8 * (hg - 2) + d2, 16)
                    ob[m, _rows(8 * (hg - 2) + d2, 8), :] = _strassen_rhs(
                        oe[m, r1, :], oo[m % 4, r1, :], oe[m, r, :], o)
                yield

    @_items(7 * HD // RS)
    def project(h):
        def emit(half, n, row, y):
            xs(2 * h + n)[pl.ds(HD * half + row, RS), :] += y

        return block_product(D + HD, (0, 1), ob.at[h], emit)

    @_items(4)
    def store_pair(h):
        for j in range(4):
            io[h, :, _rows(j, 128)] = pltpu.pack_elementwise(
                [xs(2 * h + n)[_rows(j, 128), :] for n in range(2)], packed_dtype=BF16).T
            yield

    def layer(it, c):
        def finish(hs, mxu, vpu):
            region(mxu, [fn(h) for h in hs for fn in (store_pair, norm)] + vpu)

            @pl.when(it == 1)
            def _():
                for h in hs:
                    cp_o[h].start()

        _pipeline(nc, 3, conv_step, (ca, cb))
        _interleave([], [norm_pair(0)])

        @pl.when(zs[0] == 0)
        def _():
            for g in range(3):
                _interleave([keys_values(0, g)] + ([queries(0, g)] if g < 2 else []),
                            [norm_pair(g + 1)])
            _interleave([keys_values(0, 3)], [norm_pair(4)])

        for i in range(6):
            kvs, kvg = ((1, 0), (0, 4), (1, 4))[i // 2]
            qh, qg = ((0, 2), (1, 0), (1, 2), (0, 4), (0, 6), (1, 4))[i]
            region([keys_values(kvs, kvg + 2 * (i % 2) + n) for n in range(2)]
                   + [queries(qh, qg + n) for n in range(2 if i < 5 else 1)],
                   ([norm_pair(5 + i)] if i < 3 else [])
                   + [attend(i // 4, (i // 2) % 2, 4 * (i % 2) + n) for n in range(4)])
        region([queries(1, g) for g in (5, 6, 7)], [attend(1, 1, m) for m in (0, 1)])
        region([project(0), project(1)], [attend(1, 1, m) for m in (2, 3, 4)])
        finish([0, 1], [project(h) for h in (2, 3, 4)], [attend(1, 1, m) for m in (5, 6, 7)])
        finish([2, 3, 4], [project(5), project(6)], [])
        finish([5, 6], [project(7)], [])
        pl.when(it == 0)(lambda: _interleave([], [norm(7)]))

    jax.lax.fori_loop(0, 2, layer, None)
    _interleave([], [store_pair(7)])
    cp_o[7].start()
    for cp in cp_o:
        cp.wait()


@jax.jit
def pallas_interleave_layers__ssm_conv_s4__sliding_local_dilated__prompt_kernel(
    A_u: jax.Array,
    A_A_re: jax.Array,
    A_A_im: jax.Array,
    A_B_re: jax.Array,
    A_B_im: jax.Array,
    A_C_re: jax.Array,
    A_C_im: jax.Array,
    A_log_dt: jax.Array,
    A_Dskip: jax.Array,
    B_x: jax.Array,
    B_wqkv: jax.Array,
    B_wo: jax.Array,
):
    del B_x
    hbm = pl.BlockSpec(memory_space=pl.ANY)
    vmem = pl.BlockSpec(memory_space=pltpu.VMEM)
    out = pl.pallas_call(
        _kernel,
        in_specs=[hbm] + [vmem] * 8 + [hbm] * 3,
        out_specs=hbm,
        out_shape=jax.ShapeDtypeStruct((T1, PH, D), BF16),
        scratch_shapes=[
            pltpu.VMEM((PH // 2, T1, D), U32),
            pltpu.VMEM((D, 3 * D), BF16),
            pltpu.VMEM((D, D), BF16),
            pltpu.VMEM((PH, T1 // 2, 2 * T1), U32),
            pltpu.VMEM((7, D, HD), U32),
            pltpu.VMEM((D // 2, D), U32),
            pltpu.VMEM((4, D, NS), F32),
            pltpu.VMEM((2, D, NS), F32),
            pltpu.VMEM((D, T1), F32),
            pltpu.VMEM((2 * TZ + 9 * ZS + 4, NS), U32),
            pltpu.VMEM((2 * TZ + 9 * ZS + 4, NS), U32),
            pltpu.VMEM((NCOEF, D, 2 * T1), F32),
            pltpu.VMEM((PH, D, T1), F32),
            pltpu.VMEM((PH, D, T1), BF16),
            pltpu.VMEM((2 * PH, CB, 2 * T1), F32),
            pltpu.VMEM((2 * PH, CB, 2 * T1), F32),
            pltpu.VMEM((2, 2 * PH, D, T1), F32),
            pltpu.VMEM((PH // 2, HD // 2, 7 * T1), U32),
            pltpu.VMEM((PH // 2, 2, D, T1), F32),
            pltpu.VMEM((WIN, D, T1), F32),
            pltpu.VMEM((4, HD, T1), F32),
            pltpu.VMEM((WIN, HD // 2, 7 * T1), U32),
            pltpu.SMEM((1,), I32),
            pltpu.SemaphoreType.DMA((3 + PH // 2,)),
        ],
        compiler_params=pltpu.CompilerParams(vmem_limit_bytes=100 * 1024 * 1024),
    )(A_u.reshape(T1, PH, D), A_A_re, A_A_im, A_B_re, A_B_im, A_C_re, A_C_im,
      A_log_dt, A_Dskip, B_wqkv, B_wo,
      _dft_matrices())
    return out.reshape(1, L, D)
```

```python
import numpy as np

import jax
import jax.numpy as jnp
import jax.experimental.pallas as pl
import jax.experimental.pallas.tpu as pltpu

F32, BF16, U32, I32 = jnp.float32, jnp.bfloat16, jnp.uint32, jnp.int32
L, D, NS = 2048, 512, 128
PH, T1 = 16, 128
WIN = 8
NN = (((1,), (0,)), ((), ()))
NT = (((1,), (1,)), ((), ()))
QS = 116
ZS = 28
_H = float(np.sqrt(0.5))
NCOEF = 22
HD = D // 2
RS = 64
JB = 4
CB = 64


def _dft_matrices():
    t = 16 * np.arange(T1)[None, :, None] + np.arange(PH)[:, None, None]
    k = np.arange(T1)[None, None, :] + 0.5
    phi = 2.0 * np.pi * k * t / (2 * L)
    f = np.concatenate([np.cos(phi), -np.sin(phi)], axis=-1).astype(np.float32)
    bits = f.astype(BF16).view(np.uint16).astype(np.uint32)
    return bits[:, 0::2] | (bits[:, 1::2] << 16)


def _cmul(a, b):
    return a[0] * b[0] - a[1] * b[1], a[0] * b[1] + a[1] * b[0]


def _csq(a):
    t = a[0] * a[1]
    return a[0] * a[0] - a[1] * a[1], t + t


def _cadd(a, b):
    return a[0] + b[0], a[1] + b[1]


def _csub(a, b):
    return a[0] - b[0], a[1] - b[1]


def _rot8(x, e):
    s, d = x[0] + x[1], x[0] - x[1]
    return {1: (d * _H, s * _H), 3: (s * -_H, d * _H), 5: (d * -_H, s * -_H), 7: (s * _H, d * -_H)}[e]


def _split(x, e):
    n = len(x) // 2
    lo, hi = x[:n], x[n:]
    if e == 4:
        return ([(a[0] - b[1], a[1] + b[0]) for a, b in zip(lo, hi)],
                [(a[0] + b[1], a[1] - b[0]) for a, b in zip(lo, hi)])
    if e:
        hi = [_rot8(b, e // 2) for b in hi]
    return [_cadd(a, b) for a, b in zip(lo, hi)], [_csub(a, b) for a, b in zip(lo, hi)]


def _merge(p, m, e):
    lo = [_cadd(a, b) for a, b in zip(p, m)]
    if e == 4:
        return lo + [(a[1] - b[1], b[0] - a[0]) for a, b in zip(p, m)]
    hi = [_csub(a, b) for a, b in zip(p, m)]
    return lo + ([_rot8(b, 8 - e // 2) for b in hi] if e else hi)


def _conv_coefs(k, e):
    if len(k) == 1:
        return [(k[0][0] * 0.5, k[0][1] * 0.5)]
    if len(k) == 2 and e % 4:
        if e % 2:
            top = _csub(_rot8(k[1], e), k[0])
        elif e == 2:
            top = (-k[1][1] - k[0][0], k[1][0] - k[0][1])
        else:
            top = (k[1][1] - k[0][0], -k[1][0] - k[0][1])
        return [k[0], top, _csub(k[1], k[0])]
    p, m = _split(k, e)
    return _conv_coefs(p, e // 2) + _conv_coefs(m, e // 2 + 4)


def _conv(x, e, coef):
    if len(x) == 1:
        return [_cmul(x[0], coef())]
    if len(x) == 2 and e % 4:
        both = _cmul(_cadd(x[0], x[1]), coef())
        return [_cadd(both, _cmul(x[1], coef())), _cadd(both, _cmul(x[0], coef()))]
    p, m = _split(x, e)
    return _merge(_conv(p, e // 2, coef), _conv(m, e // 2 + 4, coef), e)


def _sincos(x):
    n = jnp.floor(x * float(2.0 / np.pi) + 0.5)
    r = ((x - n * 1.5703125) - n * 4.837512969970703125e-4) - n * 7.54978995489188216e-8
    z = r * r
    s = r + r * z * ((-1.9515295891e-4 * z + 8.3321608736e-3) * z - 1.6666654611e-1)
    c = 1.0 + z * (((2.443315711809948e-5 * z - 1.388731625493765e-3) * z
                    + 4.166664568298827e-2) * z - 0.5)
    q = n.astype(I32)
    odd = (q & 1) == 1
    s, c = jnp.where(odd, c, s), jnp.where(odd, s, c)
    return jnp.where((q & 2) == 2, -s, s), jnp.where(((q + 1) & 2) == 2, -c, c)


def _pk(x):
    return pltpu.bitcast(x.astype(BF16), U32)


def _zip(x):
    return jnp.concatenate(
        [pltpu.pack_elementwise([x[i:i + 8], x[i + 8:i + 16]], packed_dtype=BF16)
         for i in range(0, x.shape[0], 16)], axis=0)


def _bf(words):
    return pltpu.bitcast(words, BF16)


def _layernorm(load):
    def mean(term, every):
        acc = [term(load(i)) for i in range(4)]
        for i in range(4, D // 8):
            acc[i % 4] = acc[i % 4] + term(load(i))
            if i % every == every - 1:
                yield
        tot = jnp.sum((acc[0] + acc[1]) + (acc[2] + acc[3]), axis=0, keepdims=True)
        return jnp.broadcast_to(tot * (1.0 / D), (8, T1))

    mu = yield from mean(lambda x: x, 32)
    var = yield from mean(lambda x: (x - mu) * (x - mu), 10)
    rs = jax.lax.rsqrt(var + 1e-5)
    return lambda i: jnp.concatenate([(load(2 * i + s) - mu) * rs for s in range(2)], axis=0)


def _items(n):
    return lambda fn: lambda *args: (fn(*args), n)


def _interleave(*lists):
    gens = [(v for g, _ in w for v in g) for w in lists]
    sizes = [sum(n for _, n in w) for w in lists]
    for _, k in sorted((i / n, k) for k, n in enumerate(sizes) for i in range(n)):
        next(gens[k])
    for g in gens:
        for _ in g:
            pass


def _strassen_lhs(a11, a12, a21, a22):
    return a11 + a22, a22, a21 + a22, a11 + a12, a11, a12 - a22, a21 - a11


def _strassen_rhs(b11, b12, b21, b22):
    ops = (b11 + b22, b21 - b11, b11, b22, b12 - b22, b21 + b22, b11 + b12)
    return jnp.concatenate([_zip(v) for v in ops], axis=1)


def _strassen(prod, emit):
    m1 = prod(0)
    yield
    m4 = prod(1)
    c11 = m1 + m4
    yield
    m2 = prod(2)
    emit(1, 0, m2 + m4)
    c22 = m1 - m2
    yield
    m5 = prod(3)
    c11 = c11 - m5
    yield
    m3 = prod(4)
    emit(0, 1, m3 + m5)
    c22 = c22 + m3
    yield
    emit(0, 0, c11 + prod(5))
    yield
    emit(1, 1, c22 + prod(6))
    yield


def _rows(i, n):
    return slice(i * n, i * n + n)


def _ds(start, n):
    return pl.ds(start if isinstance(start, int) else pl.multiple_of(start, n), n)


def _pipeline(n, depth, step, bufs):
    def static(i):
        step(i, bufs[i % 2], bufs[1 - i % 2], [s for s in range(depth) if 0 <= i - s < n])

    def body(i, _):
        for par in range(2):
            pl.when(i % 2 == par)(lambda: step(i, bufs[par], bufs[1 - par], list(range(depth))))

    for i in range(depth - 1):
        static(i)
    jax.lax.fori_loop(depth - 1, n, body, None)
    for i in range(n, n + depth - 1):
        static(i)


def _kernel(u_hbm, are, aim, bre, bim, cre, cim, ldt, dsk, wqkv_hbm, wo_hbm, f_hbm, out_hbm,
            io, wq_in, wo_in, fm, ws, wp, lam, dtc, k0s, tab, ztab, kf,
            xr, xn, ca, cb, kv, xq, qs, oe, oo, ob, zs, sems):
    cp_u = [pltpu.make_async_copy(u_hbm.bitcast(U32).at[:, h, :], io.at[h], sems.at[3 + h])
            for h in range(PH // 2)]
    cp_o = [pltpu.make_async_copy(io.at[h], out_hbm.bitcast(U32).at[:, h, :], sems.at[3 + h])
            for h in range(PH // 2)]
    cp_f = pltpu.make_async_copy(f_hbm, fm, sems.at[0])
    cp_wq = pltpu.make_async_copy(wqkv_hbm, wq_in, sems.at[1])
    cp_wo = pltpu.make_async_copy(wo_hbm, wo_in, sems.at[2])
    for cp in [cp_f] + cp_u + [cp_wo, cp_wq]:
        cp.start()

    lane = jax.lax.broadcasted_iota(I32, (8, T1), 1)
    zs[0] = 0

    def zero_rows(k):
        return pl.multiple_of((zs[0] >> k) * 8, 8)

    def xs(p):
        return xr.at[p]

    def region(*lists):
        pl.when(zs[0] == 0)(lambda: _interleave(*lists))

    dt_row = jnp.exp(ldt[...].astype(F32).reshape(1, D)).astype(BF16).astype(F32)
    ds_row = dsk[...].astype(F32).reshape(1, D)
    for j in range(4):
        dtc[0, _rows(j, 128), :] = jnp.broadcast_to(dt_row[:, _rows(j, 128)], (128, 128)).T
        dtc[1, _rows(j, 128), :] = jnp.broadcast_to(ds_row[:, _rows(j, 128)], (128, 128)).T
    big = None
    for j in range(D // 16):
        r = _rows(j, 16)
        theta = dtc[0, r, :] * aim[r, :].astype(F32)
        mag = jnp.exp(dtc[0, r, :] * are[r, :].astype(F32))
        sn, cs = _sincos(theta)
        lam[0, r, :] = mag * cs
        lam[1, r, :] = mag * sn
        sc = dtc[0, r, :] * (2.0 / L)
        w = _cmul((cre[r, :].astype(F32), cim[r, :].astype(F32)),
                  (bre[r, :].astype(F32) * sc, bim[r, :].astype(F32) * sc))
        lam[2, r, :] = w[0]
        lam[3, r, :] = w[1]
        k0s[r, :] = jnp.sum(w[0], axis=1, keepdims=True) + dtc[1, r, :] * (2.0 / L)
        big = jnp.abs(theta) if big is None else jnp.maximum(big, jnp.abs(theta))

    @pl.when(jnp.logical_not(jnp.max(big) <= 8192.0))
    def _():
        def body(i, _):
            rows = pl.ds(pl.multiple_of(i * 16, 16), 16)
            th = dtc[0, rows, :] * aim[rows, :].astype(F32)
            mg = jnp.exp(dtc[0, rows, :] * are[rows, :].astype(F32))
            lam[0, rows, :] = mg * jnp.cos(th)
            lam[1, rows, :] = mg * jnp.sin(th)
        jax.lax.fori_loop(0, D // 16, body, None)

    @_items(5)
    def tap_tables(blk, e):
        rows = _rows(4 * blk + e, 8)
        w = (lam[2, rows, :], lam[3, rows, :])

        def put(row, a, b):
            for z in range(2):
                tab[blk % 4, z, pl.ds(row, 8, stride=QS), :] = pltpu.pack_elementwise(
                    [a[z], b[z]], packed_dtype=BF16)

        l1 = (lam[0, rows, :], lam[1, rows, :])
        l2 = _csq(l1)
        l16 = _csq(_csq(_csq(l2)))
        m1 = (l16[0], -l16[1])
        m2 = _csq(m1)
        a, b = _cmul(w, l1), _cmul(w, l2)
        c, d = m2, _cmul(m1, m2)
        put(16 * e, (jnp.ones_like(m1[0]), jnp.zeros_like(m1[0])), m1)
        keep = {}
        for j in range(1, 16):
            if j <= 8:
                put(64 + 12 * e + j - 1, a, b)
                keep[2 * j] = b
            if j < 8:
                a, b = _cmul(a, l2), _cmul(b, l2)
            put(16 * e + j, c, d)
            if j == 8:
                l512 = _csq((c[0], -c[1]))
                put(64 + 12 * e + 8, _cmul(keep[4], l512), _cmul(keep[12], l512))
                a, b = keep[8], keep[16]
            if j in (10, 12, 14):
                a, b = _cmul(a, l512), _cmul(b, l512)
                put(64 + 12 * e + 4 + j // 2, a, b)
            if j < 15:
                c, d = _cmul(c, m2), _cmul(d, m2)
            if j % 3 == 0:
                yield

    @_items(8)
    def tap_sums(blk):
        for i in range(8):
            acc = None
            for z in range(2):
                rhs = _bf(tab[blk % 4, z, pl.ds(QS * i, 64), :])
                lhs = _bf(tab[blk % 4, z, pl.ds(QS * i + 64, 48), :])
                d = jax.lax.dot_general(lhs, rhs, NT, preferred_element_type=F32)
                acc = d if acc is None else acc + d
            for r in range(3):
                pc = [acc[_rows(3 * e + r, 8)] for e in range(4)]
                ztab[blk % 4, pl.ds(ZS * i + 8 * r, 8), :] = jnp.where(
                    lane < 64, jnp.where(lane < 32, pc[0], pc[1]),
                    jnp.where(lane < 96, pc[2], pc[3]))
            yield

    @_items(1)
    def tap_blocks(blk, e):
        def at(r, g):
            z = ztab[blk % 4, pl.ds(r, 8, stride=ZS), :]
            return z if g == e else pltpu.roll(z, (32 * (g - e)) % 128, 1)

        def full(r, r1):
            return jnp.where(lane < 64, jnp.where(lane < 32, at(r, 0), at(r1, 1)),
                             jnp.where(lane < 96, at(r1 + 2, 2), at(r1 + 4, 3)))

        rows = _rows(4 * blk + e, 8)
        e8, e16 = full(7, 18), full(15, 19)
        e0 = jnp.where(lane == 0, k0s[rows, :], pltpu.roll(e16, 1, 1))
        e4 = jnp.where(lane < 32, at(3, 0), at(16, 1))
        e12 = jnp.where(lane < 32, at(11, 0), at(17, 1))
        k4, k12 = jnp.where(lane < 64, e4, e0), jnp.where(lane < 64, e12, e16)
        far = {1: e0, 2: e0, 3: k4, 5: jnp.where(lane < 64, e4, e8), 6: e8, 7: e8, 9: e8,
               10: e8, 11: jnp.where(lane < 64, e12, e8), 13: k12, 14: e16, 15: e16}
        for p, v in ((0, e0), (4, k4), (8, e8), (12, k12)):
            kv[0, p, rows, :] = v
        for p, v in far.items():
            kv[0, p, rows, :] = jnp.where(lane < (16 if p % 2 else 32), at(p - 1, 0), v)
        yield

    def lane_dft(load, q, dst, zero):
        x0, x1 = [jax.lax.dot_general(load(p), _bf(fm[p]), NN, preferred_element_type=F32)
                  for p in (q, q + 8)]
        for i in range(CB // 8):
            r = _rows(i, 8)
            dst[q, pl.ds(zero + 8 * i, 8), :] = x0[r] + x1[r]
            dst[q + 8, pl.ds(zero + 8 * i, 8), :] = x0[r] - x1[r]

    @_items(8)
    def tap_dft(blk):
        for q in range(8):
            lane_dft(lambda p: kv[0, p, _rows(blk, CB), :], q, (ca, cb)[blk % 2], 0)
            yield

    @_items(CB // 4)
    def tap_coefs(blk):
        src = (ca, cb)[blk % 2]
        for i in range(CB // 8):
            r, ro = _rows(i, 8), _rows(blk * CB // 8 + i, 8)
            for odd in range(2):
                co = _conv_coefs([(src[8 * odd + c, r, :T1], src[8 * odd + c, r, T1:])
                                  for c in range(8)], 4 * odd)
                for n, v in enumerate(co):
                    kf[10 * odd + n, ro, :T1] = v[0]
                    kf[10 * odd + n, ro, T1:] = v[1]
                yield

    r0 = jax.lax.broadcasted_iota(I32, (128, 128), 0)
    ri = (r0 & ~15) + (r0 & 7) * 2 + ((r0 >> 3) & 1)
    ci = jax.lax.broadcasted_iota(I32, (128, 128), 1)
    hit = ci == (ri & 7) * 16 + (ri >> 3)

    @_items(2)
    def prep_weights(j):
        def block(c, k):
            if j < 6:
                sel = jnp.where(hit, 1.0 if j < 4 else 0.25, 0.0)
                w = _bf(_zip(wq_in[_rows(k, 128), _rows(c, 128)].astype(F32)))
            else:
                sel = jnp.where(ri == ci, 1.0, 0.0)
                w = _bf(wp[_rows(k, 64), _rows(c, 128)])
            return jax.lax.dot_general(sel.astype(BF16), w, NT, preferred_element_type=F32)

        top, bot = (4 + j, 8 + j) if j < 4 else (j % 2, j % 2 + 2)
        for k in range(2):
            for i, a in enumerate(_strassen_lhs(block(top, k), block(top, k + 2),
                                                block(bot, k), block(bot, k + 2))):
                ws[i, _rows(j, 64), _rows(k, 128)] = _zip(a)
            yield

    @_items(1)
    def permute_wo(j):
        sel = jnp.where(ci == (r0 & 7) * 16 + (r0 >> 3), 1.0, 0.0).astype(BF16)
        wp[_rows(j, 64), :] = _zip(jnp.dot(sel, wo_in[_rows(j, 128), :],
                                           preferred_element_type=F32))
        yield

    @_items(4)
    def load_pair(h):
        for j in range(4):
            wds = io[h, :, _rows(j, 128)].T
            xs(2 * h)[_rows(j, 128), :] = pltpu.bitcast(wds << 16, F32)
            xs(2 * h + 1)[_rows(j, 128), :] = pltpu.bitcast(wds & jnp.uint32(0xFFFF0000), F32)
            yield

    @_items(24)
    def norm(h):
        for p in (2 * h, 2 * h + 1):
            normed = yield from _layernorm(lambda i: xs(p)[_rows(i, 8), :])
            for i in range(D // 16):
                xn[p, _rows(i, 16), :] = normed(i).astype(BF16)
                if i % 8 == 7:
                    yield

    nc = D // CB
    for i in range(nc + 4):
        def subs(s):
            return [2 * (i - s), 2 * (i - s) + 1] if 0 <= i - s < nc else []

        if i == 3:
            cp_f.wait()
        if i == nc - 1:
            for cp in cp_u:
                cp.wait()
        if i == nc:
            cp_wq.wait()
            cp_wo.wait()
        k = i - nc
        region([tap_sums(b) for b in subs(1)] + ([tap_dft(i - 3)] if subs(3) else [])
               + ([permute_wo(j) for j in range(4)] if k == 0 else [])
               + [prep_weights(j) for j in {1: (0, 1), 2: (2, 3), 3: (4, 5, 6, 7)}.get(k, ())],
               [tap_tables(b, e) for b in subs(0) for e in range(4)]
               + ([norm(2 * k), norm(2 * k + 1)] if k >= 0 else []),
               [tap_blocks(b, e) for b in subs(2) for e in range(4)],
               [tap_coefs(i - 4)] if subs(4) else [],
               [load_pair(2 * k + 2), load_pair(2 * k + 3)] if -1 <= k < 3 else [])

    def phase_conv(blk, u, src, dst, zero):
        i, odd = u // 2, u % 2
        r, ro = _rows(i, 8), _ds(blk * CB + 8 * i, 8)
        ids = iter(range(10 * odd, NCOEF))

        def coef():
            n = next(ids)
            return kf[n, ro, :T1], kf[n, ro, T1:]

        y = _conv([(src[8 * odd + c, r, :T1], src[8 * odd + c, r, T1:]) for c in range(8)],
                  4 * odd, coef)
        for c in range(8):
            dst[PH + 8 * odd + c, pl.ds(zero + 8 * i, 8), :T1] = y[c][0]
            dst[PH + 8 * odd + c, pl.ds(zero + 8 * i, 8), T1:] = y[c][1]

    def lane_idft(blk, q, src):
        a, b = src[PH + q], src[PH + 8 + q]
        for p, v in ((q, a + b), (q + 8, a - b)):
            xs(p)[_ds(blk * CB, CB), :] += jax.lax.dot_general(
                v, _bf(fm[p]), NT, preferred_element_type=F32)

    def conv_step(i, src, dst, stages):
        z1, z2 = zero_rows(1), zero_rows(2)
        for q in range(8):
            if 1 in stages:
                phase_conv(i - 1, 2 * q, src, dst, z2)
            if 0 in stages:
                lane_dft(lambda p: xn[p, _ds(i * CB, CB), :], q, dst, z1)
            if 1 in stages:
                phase_conv(i - 1, 2 * q + 1, src, dst, z2)
            if 2 in stages:
                lane_idft(i - 2, q, src)

    @_items(32)
    def norm_pair(g):
        p = 4 * (g % 4) + g // 4
        a = yield from _layernorm(lambda i: xs(p)[_rows(i, 8), :])
        b = yield from _layernorm(lambda i: xs(p + 2)[_rows(i, 8), :])
        for r in range(HD // 16):
            xq[g, _rows(r, 8), :] = _strassen_rhs(a(r), b(r), a(HD // 16 + r), b(HD // 16 + r))
            yield

    def block_product(row0, groups, rhs, emit):
        for r in [128 // RS * hg + i for hg in groups for i in range(128 // RS)]:
            w = slice((row0 + r * RS) // 2, (row0 + r * RS + RS) // 2)
            yield from _strassen(
                lambda i: jnp.dot(_bf(ws[i, w, :]), _bf(rhs[:, _rows(i, T1)]),
                                  preferred_element_type=F32),
                lambda half, n, y: emit(half, n, r * RS, y))

    @_items(7 * HD // RS)
    def keys_values(s, g):
        def emit(half, n, row, y):
            m = 2 * (g % 4) + n
            kv[g // 4, PH * half + WIN - 1 + m, pl.ds(row, RS), :] = y
            if m:
                kv[g // 4, PH * half + m - 1, pl.ds(row, RS), :] = pltpu.roll(y, 1, 1)

        return block_product(0, (s, s + 2), xq.at[g], emit)

    @_items(7 * 128 // RS)
    def queries(s, g):
        def emit(half, n, row, y):
            qs[g, n, pl.ds(HD * half + row, RS), :] = y

        return block_product(D, (s,), xq.at[g], emit)

    @_items(34)
    def attend(par, s, m):
        for hg in (s, s + 2):
            lg = [None] * WIN
            for j0 in range(0, WIN, JB):
                for dh in range(16):
                    r = _rows(16 * hg + dh, 8)
                    q = qs[4 * par + m // 2, m % 2, r, :]
                    for j in range(j0, j0 + JB):
                        t = q * kv[par, WIN - 1 + m - j, r, :]
                        lg[j] = t if dh == 0 else lg[j] + t
                    if (dh + 1) % (16 // JB) == 0:
                        yield
            for j in range(m + 1, WIN):
                lg[j] = jnp.where(lane == 0, -1e9, lg[j])
            mx = lg[0]
            for j in range(1, WIN):
                mx = jnp.maximum(mx, lg[j])
            ex = [jnp.exp(t - mx) for t in lg]
            den = ex[0]
            for j in range(1, WIN):
                den = den + ex[j]
            inv = pltpu.reciprocal(den, full_range=False)
            pr = [t * inv for t in ex]
            yield

            def out(dh):
                r = _rows(16 * hg + dh, 8)
                acc = pr[0] * kv[par, PH + WIN - 1 + m, r, :]
                for j in range(1, WIN):
                    acc = acc + pr[j] * kv[par, PH + WIN - 1 + m - j, r, :]
                return acc

            for d2 in range(8):
                o = jnp.concatenate([out(2 * d2), out(2 * d2 + 1)], axis=0)
                r = _rows(8 * hg + d2, 16)
                if par == 0:
                    oe[m, r, :] = o
                elif hg < 2:
                    oo[m % 4, r, :] = o
                else:
                    r1 = _rows(8 * (hg - 2) + d2, 16)
                    ob[m, _rows(8 * (hg - 2) + d2, 8), :] = _strassen_rhs(
                        oe[m, r1, :], oo[m % 4, r1, :], oe[m, r, :], o)
                yield

    @_items(7 * HD // RS)
    def project(h):
        def emit(half, n, row, y):
            xs(2 * h + n)[pl.ds(HD * half + row, RS), :] += y

        return block_product(D + HD, (0, 1), ob.at[h], emit)

    @_items(4)
    def store_pair(h):
        for j in range(4):
            io[h, :, _rows(j, 128)] = pltpu.pack_elementwise(
                [xs(2 * h + n)[_rows(j, 128), :] for n in range(2)], packed_dtype=BF16).T
            yield

    def layer(it, c):
        def finish(hs, mxu, vpu):
            region(mxu, [fn(h) for h in hs for fn in (store_pair, norm)] + vpu)

            @pl.when(it == 1)
            def _():
                for h in hs:
                    cp_o[h].start()

        _pipeline(nc, 3, conv_step, (ca, cb))
        _interleave([], [norm_pair(0)])

        @pl.when(zs[0] == 0)
        def _():
            for g in range(3):
                _interleave([keys_values(0, g)] + ([queries(0, g)] if g < 2 else []),
                            [norm_pair(g + 1)])
            _interleave([keys_values(0, 3)], [norm_pair(4)])

        for i in range(6):
            kvs, kvg = ((1, 0), (0, 4), (1, 4))[i // 2]
            qh, qg = ((0, 2), (1, 0), (1, 2), (0, 4), (0, 6), (1, 4))[i]
            region([keys_values(kvs, kvg + 2 * (i % 2) + n) for n in range(2)]
                   + [queries(qh, qg + n) for n in range(2 if i < 5 else 1)],
                   ([norm_pair(5 + i)] if i < 3 else [])
                   + [attend(i // 4, (i // 2) % 2, 4 * (i % 2) + n) for n in range(4)])
        region([queries(1, g) for g in (5, 6, 7)], [attend(1, 1, m) for m in (0, 1)])
        region([project(0), project(1)], [attend(1, 1, m) for m in (2, 3, 4)])
        finish([0, 1], [project(h) for h in (2, 3, 4)], [attend(1, 1, m) for m in (5, 6, 7)])
        finish([2, 3, 4], [project(5), project(6)], [])
        finish([5, 6], [project(7)], [])
        pl.when(it == 0)(lambda: _interleave([], [norm(7)]))

    jax.lax.fori_loop(0, 2, layer, None)
    _interleave([], [store_pair(7)])
    cp_o[7].start()
    for cp in cp_o:
        cp.wait()


@jax.jit
def pallas_interleave_layers__ssm_conv_s4__sliding_local_dilated__prompt_kernel(
    A_u: jax.Array,
    A_A_re: jax.Array,
    A_A_im: jax.Array,
    A_B_re: jax.Array,
    A_B_im: jax.Array,
    A_C_re: jax.Array,
    A_C_im: jax.Array,
    A_log_dt: jax.Array,
    A_Dskip: jax.Array,
    B_x: jax.Array,
    B_wqkv: jax.Array,
    B_wo: jax.Array,
):
    del B_x
    hbm = pl.BlockSpec(memory_space=pl.ANY)
    vmem = pl.BlockSpec(memory_space=pltpu.VMEM)
    out = pl.pallas_call(
        _kernel,
        in_specs=[hbm] + [vmem] * 8 + [hbm] * 3,
        out_specs=hbm,
        out_shape=jax.ShapeDtypeStruct((T1, PH, D), BF16),
        scratch_shapes=[
            pltpu.VMEM((PH // 2, T1, D), U32),
            pltpu.VMEM((D, 3 * D), BF16),
            pltpu.VMEM((D, D), BF16),
            pltpu.VMEM((PH, T1 // 2, 2 * T1), U32),
            pltpu.VMEM((7, D, HD), U32),
            pltpu.VMEM((D // 2, D), U32),
            pltpu.VMEM((4, D, NS), F32),
            pltpu.VMEM((2, D, NS), F32),
            pltpu.VMEM((D, T1), F32),
            pltpu.VMEM((4, 2, 9 * QS + 4, NS), U32),
            pltpu.VMEM((4, 9 * ZS + 4, T1), F32),
            pltpu.VMEM((NCOEF, D, 2 * T1), F32),
            pltpu.VMEM((PH, D, T1), F32),
            pltpu.VMEM((PH, D, T1), BF16),
            pltpu.VMEM((2 * PH, CB, 2 * T1), F32),
            pltpu.VMEM((2 * PH, CB, 2 * T1), F32),
            pltpu.VMEM((2, 2 * PH, D, T1), F32),
            pltpu.VMEM((PH // 2, HD // 2, 7 * T1), U32),
            pltpu.VMEM((PH // 2, 2, D, T1), F32),
            pltpu.VMEM((WIN, D, T1), F32),
            pltpu.VMEM((4, HD, T1), F32),
            pltpu.VMEM((WIN, HD // 2, 7 * T1), U32),
            pltpu.SMEM((1,), I32),
            pltpu.SemaphoreType.DMA((3 + PH // 2,)),
        ],
        compiler_params=pltpu.CompilerParams(vmem_limit_bytes=100 * 1024 * 1024),
    )(A_u.reshape(T1, PH, D), A_A_re, A_A_im, A_B_re, A_B_im, A_C_re, A_C_im,
      A_log_dt, A_Dskip, B_wqkv, B_wo,
      _dft_matrices())
    return out.reshape(1, L, D)
```

```python
import numpy as np

import jax
import jax.numpy as jnp
import jax.experimental.pallas as pl
import jax.experimental.pallas.tpu as pltpu

F32, BF16, U32, I32 = jnp.float32, jnp.bfloat16, jnp.uint32, jnp.int32
L, D, NS = 2048, 512, 128
PH, T1 = 16, 128
WIN = 8
NN = (((1,), (0,)), ((), ()))
NT = (((1,), (1,)), ((), ()))
QS = 116
ZS = 28
_H = float(np.sqrt(0.5))
NCOEF = 22
HD = D // 2
RS = 64
JB = 4
CUTS = ((0, 64, 192, 384, D, D, D, D),
        (0, 0, 64, 192, 352, 448, D, D),
        (0, 0, 0, 64, 192, 352, 448, D))
CB = 64


def _dft_matrices():
    t = 16 * np.arange(T1)[None, :, None] + np.arange(PH)[:, None, None]
    k = np.arange(T1)[None, None, :] + 0.5
    phi = 2.0 * np.pi * k * t / (2 * L)
    f = np.concatenate([np.cos(phi), -np.sin(phi)], axis=-1).astype(np.float32)
    bits = f.astype(BF16).view(np.uint16).astype(np.uint32)
    return bits[:, 0::2] | (bits[:, 1::2] << 16)


def _cmul(a, b):
    return a[0] * b[0] - a[1] * b[1], a[0] * b[1] + a[1] * b[0]


def _csq(a):
    t = a[0] * a[1]
    return a[0] * a[0] - a[1] * a[1], t + t


def _cadd(a, b):
    return a[0] + b[0], a[1] + b[1]


def _csub(a, b):
    return a[0] - b[0], a[1] - b[1]


def _rot8(x, e):
    s, d = x[0] + x[1], x[0] - x[1]
    return {1: (d * _H, s * _H), 3: (s * -_H, d * _H), 5: (d * -_H, s * -_H), 7: (s * _H, d * -_H)}[e]


def _split(x, e):
    n = len(x) // 2
    lo, hi = x[:n], x[n:]
    if e == 4:
        return ([(a[0] - b[1], a[1] + b[0]) for a, b in zip(lo, hi)],
                [(a[0] + b[1], a[1] - b[0]) for a, b in zip(lo, hi)])
    if e:
        hi = [_rot8(b, e // 2) for b in hi]
    return [_cadd(a, b) for a, b in zip(lo, hi)], [_csub(a, b) for a, b in zip(lo, hi)]


def _merge(p, m, e):
    lo = [_cadd(a, b) for a, b in zip(p, m)]
    if e == 4:
        return lo + [(a[1] - b[1], b[0] - a[0]) for a, b in zip(p, m)]
    hi = [_csub(a, b) for a, b in zip(p, m)]
    return lo + ([_rot8(b, 8 - e // 2) for b in hi] if e else hi)


def _conv_coefs(k, e):
    if len(k) == 1:
        return [(k[0][0] * 0.5, k[0][1] * 0.5)]
    if len(k) == 2 and e % 4:
        if e % 2:
            top = _csub(_rot8(k[1], e), k[0])
        elif e == 2:
            top = (-k[1][1] - k[0][0], k[1][0] - k[0][1])
        else:
            top = (k[1][1] - k[0][0], -k[1][0] - k[0][1])
        return [k[0], top, _csub(k[1], k[0])]
    p, m = _split(k, e)
    return _conv_coefs(p, e // 2) + _conv_coefs(m, e // 2 + 4)


def _conv(x, e, coef):
    if len(x) == 1:
        return [_cmul(x[0], coef())]
    if len(x) == 2 and e % 4:
        both = _cmul(_cadd(x[0], x[1]), coef())
        return [_cadd(both, _cmul(x[1], coef())), _cadd(both, _cmul(x[0], coef()))]
    p, m = _split(x, e)
    return _merge(_conv(p, e // 2, coef), _conv(m, e // 2 + 4, coef), e)


def _sincos(x):
    n = jnp.floor(x * float(2.0 / np.pi) + 0.5)
    r = ((x - n * 1.5703125) - n * 4.837512969970703125e-4) - n * 7.54978995489188216e-8
    z = r * r
    s = r + r * z * ((-1.9515295891e-4 * z + 8.3321608736e-3) * z - 1.6666654611e-1)
    c = 1.0 + z * (((2.443315711809948e-5 * z - 1.388731625493765e-3) * z
                    + 4.166664568298827e-2) * z - 0.5)
    q = n.astype(I32)
    odd = (q & 1) == 1
    s, c = jnp.where(odd, c, s), jnp.where(odd, s, c)
    return jnp.where((q & 2) == 2, -s, s), jnp.where(((q + 1) & 2) == 2, -c, c)


def _pk(x):
    return pltpu.bitcast(x.astype(BF16), U32)


def _zip(x):
    return jnp.concatenate(
        [pltpu.pack_elementwise([x[i:i + 8], x[i + 8:i + 16]], packed_dtype=BF16)
         for i in range(0, x.shape[0], 16)], axis=0)


def _bf(words):
    return pltpu.bitcast(words, BF16)


def _layernorm(load):
    def mean(term, every):
        acc = [term(load(i)) for i in range(4)]
        for i in range(4, D // 8):
            acc[i % 4] = acc[i % 4] + term(load(i))
            if i % every == every - 1:
                yield
        tot = jnp.sum((acc[0] + acc[1]) + (acc[2] + acc[3]), axis=0, keepdims=True)
        return jnp.broadcast_to(tot * (1.0 / D), (8, T1))

    mu = yield from mean(lambda x: x, 32)
    var = yield from mean(lambda x: (x - mu) * (x - mu), 10)
    rs = jax.lax.rsqrt(var + 1e-5)
    return lambda i: jnp.concatenate([(load(2 * i + s) - mu) * rs for s in range(2)], axis=0)


def _items(n):
    return lambda fn: lambda *args: (fn(*args), n)


def _interleave(*lists, lead=0.0, span=1.0):
    gens = [(v for g, _ in w for v in g) for w in lists]
    sizes = [sum(n for _, n in w) for w in lists]
    for _, k in sorted((i / n if k else i / n * span - lead, k)
                       for k, n in enumerate(sizes) for i in range(n)):
        next(gens[k])
    for g in gens:
        for _ in g:
            pass


def _strassen_lhs(a11, a12, a21, a22):
    return a11 + a22, a22, a21 + a22, a11 + a12, a11, a12 - a22, a21 - a11


def _strassen_rhs(b11, b12, b21, b22):
    ops = (b11 + b22, b21 - b11, b11, b22, b12 - b22, b21 + b22, b11 + b12)
    return jnp.concatenate([_zip(v) for v in ops], axis=1)


def _strassen(prod, emit):
    m1 = prod(0)
    yield
    m4 = prod(1)
    c11 = m1 + m4
    yield
    m2 = prod(2)
    emit(1, 0, m2 + m4)
    c22 = m1 - m2
    yield
    m5 = prod(3)
    c11 = c11 - m5
    yield
    m3 = prod(4)
    emit(0, 1, m3 + m5)
    c22 = c22 + m3
    yield
    emit(0, 0, c11 + prod(5))
    yield
    emit(1, 1, c22 + prod(6))
    yield


def _rows(i, n):
    return slice(i * n, i * n + n)


def _kernel(u_hbm, are_hbm, aim_hbm, bre_hbm, bim_hbm, cre_hbm, cim_hbm, ldt, dsk, wqkv_hbm, wo_hbm, f_hbm, out_hbm,
            are, aim, bre, bim, cre, cim, io, wq_in, wo_in, fm, ws, wp, lam, dtc, k0s, tab, ztab, kf,
            xr, xn, kv, xq, qs, oe, oo, ob, zs, sems):
    cp_u = [pltpu.make_async_copy(u_hbm.bitcast(U32).at[:, h, :], io.at[h], sems.at[3 + h])
            for h in range(PH // 2)]
    cp_o = [pltpu.make_async_copy(io.at[h], out_hbm.bitcast(U32).at[:, h, :], sems.at[3 + h])
            for h in range(PH // 2)]
    cp_f = pltpu.make_async_copy(f_hbm, fm, sems.at[0])
    cp_wq = pltpu.make_async_copy(wqkv_hbm, wq_in, sems.at[1])
    cp_wo = pltpu.make_async_copy(wo_hbm, wo_in, sems.at[2])
    cp_p = [pltpu.make_async_copy(src, dst, sems.at[3 + PH // 2 + i]) for i, (src, dst) in enumerate(
        ((aim_hbm, aim), (are_hbm, are), (bre_hbm, bre), (bim_hbm, bim), (cre_hbm, cre),
         (cim_hbm, cim)))]
    for cp in cp_p:
        cp.start()

    lane = jax.lax.broadcasted_iota(I32, (8, T1), 1)
    zs[0] = 0

    def xs(p):
        return xr.at[p]

    def region(*lists, **pace):
        pl.when(zs[0] == 0)(lambda: _interleave(*lists, **pace))

    dt_row = jnp.exp(ldt[...].astype(F32).reshape(1, D)).astype(BF16).astype(F32)
    ds_row = dsk[...].astype(F32).reshape(1, D)
    for j in range(4):
        dtc[0, _rows(j, 128), :] = jnp.broadcast_to(dt_row[:, _rows(j, 128)], (128, 128)).T
        dtc[1, _rows(j, 128), :] = jnp.broadcast_to(ds_row[:, _rows(j, 128)], (128, 128)).T
    cp_p[0].wait()
    cp_p[1].wait()
    for cp in [cp_f] + cp_u + [cp_wo, cp_wq]:
        cp.start()
    big = None
    for j in range(D // 16):
        r = _rows(j, 16)
        theta = dtc[0, r, :] * aim[r, :].astype(F32)
        mag = jnp.exp(dtc[0, r, :] * are[r, :].astype(F32))
        sn, cs = _sincos(theta)
        lam[0, r, :] = mag * cs
        lam[1, r, :] = mag * sn
        big = jnp.abs(theta) if big is None else jnp.maximum(big, jnp.abs(theta))

    @pl.when(jnp.logical_not(jnp.max(big) <= 8192.0))
    def _():
        def body(i, _):
            rows = pl.ds(pl.multiple_of(i * 16, 16), 16)
            th = dtc[0, rows, :] * aim[rows, :].astype(F32)
            mg = jnp.exp(dtc[0, rows, :] * are[rows, :].astype(F32))
            lam[0, rows, :] = mg * jnp.cos(th)
            lam[1, rows, :] = mg * jnp.sin(th)
        jax.lax.fori_loop(0, D // 16, body, None)

    for cp in cp_p[2:]:
        cp.wait()

    @_items(15)
    def tap_tables(blk, e):
        rows = _rows(4 * blk + e, 8)

        def part(ref):
            return ref[_rows(2 * blk + e // 2, 16), :].astype(F32)[_rows(e % 2, 8)]

        sc = dtc[0, rows, :] * (2.0 / L)
        w = _cmul((part(cre), part(cim)), (part(bre) * sc, part(bim) * sc))
        k0s[rows, :] = w[0]

        def put(row, a, b):
            for z in range(2):
                tab[blk % 4, z, pl.ds(row, 8, stride=QS), :] = pltpu.pack_elementwise(
                    [a[z], b[z]], packed_dtype=BF16)

        l1 = (lam[0, rows, :], lam[1, rows, :])
        l2 = _csq(l1)
        l16 = _csq(_csq(_csq(l2)))
        m1 = (l16[0], -l16[1])
        m2 = _csq(m1)
        a, b = _cmul(w, l1), _cmul(w, l2)
        c, d = m2, _cmul(m1, m2)
        put(16 * e, (jnp.ones_like(m1[0]), jnp.zeros_like(m1[0])), m1)
        keep = {}
        for j in range(1, 16):
            if j <= 8:
                put(64 + 12 * e + j - 1, a, b)
                keep[2 * j] = b
            if j < 8:
                a, b = _cmul(a, l2), _cmul(b, l2)
            put(16 * e + j, c, d)
            if j == 8:
                l512 = _csq((c[0], -c[1]))
                put(64 + 12 * e + 8, _cmul(keep[4], l512), _cmul(keep[12], l512))
                a, b = keep[8], keep[16]
            if j in (10, 12, 14):
                a, b = _cmul(a, l512), _cmul(b, l512)
                put(64 + 12 * e + 4 + j // 2, a, b)
            if j < 15:
                c, d = _cmul(c, m2), _cmul(d, m2)
            yield

    @_items(8)
    def tap_sums(blk):
        for i in range(8):
            re, im = [jax.lax.dot_general(_bf(tab[blk % 4, z, pl.ds(QS * i + 64, 48), :]),
                                          _bf(tab[blk % 4, z, pl.ds(QS * i, 64), :]),
                                          NT, preferred_element_type=F32) for z in range(2)]
            yield
            acc = re + im
            for r in range(3):
                pc = [acc[_rows(3 * e + r, 8)] for e in range(4)]
                ztab[blk % 4, pl.ds(ZS * i + 8 * r, 8), :] = jnp.where(
                    lane < 64, jnp.where(lane < 32, pc[0], pc[1]),
                    jnp.where(lane < 96, pc[2], pc[3]))

    @_items(1)
    def tap_blocks(blk, e):
        def at(r, g):
            z = ztab[blk % 4, pl.ds(r, 8, stride=ZS), :]
            return z if g == e else pltpu.roll(z, (32 * (g - e)) % 128, 1)

        def full(r, r1):
            return jnp.where(lane < 64, jnp.where(lane < 32, at(r, 0), at(r1, 1)),
                             jnp.where(lane < 96, at(r1 + 2, 2), at(r1 + 4, 3)))

        rows = _rows(4 * blk + e, 8)
        e8, e16 = full(7, 18), full(15, 19)
        k0 = jnp.sum(k0s[rows, :], axis=1, keepdims=True) + dtc[1, rows, :] * (2.0 / L)
        e0 = jnp.where(lane == 0, k0, pltpu.roll(e16, 1, 1))
        e4 = jnp.where(lane < 32, at(3, 0), at(16, 1))
        e12 = jnp.where(lane < 32, at(11, 0), at(17, 1))
        k4, k12 = jnp.where(lane < 64, e4, e0), jnp.where(lane < 64, e12, e16)
        far = {1: e0, 2: e0, 3: k4, 5: jnp.where(lane < 64, e4, e8), 6: e8, 7: e8, 9: e8,
               10: e8, 11: jnp.where(lane < 64, e12, e8), 13: k12, 14: e16, 15: e16}
        for p, v in ((0, e0), (4, k4), (8, e8), (12, k12)):
            kv[1, p, rows, :] = v
        for p, v in far.items():
            kv[1, p, rows, :] = jnp.where(lane < (16 if p % 2 else 32), at(p - 1, 0), v)
        yield

    @_items(8)
    def lane_dft(src, lo, hi):
        for q in range(8):
            x0, x1 = [jax.lax.dot_general(src[p, lo:hi, :], _bf(fm[p]), NN,
                                          preferred_element_type=F32) for p in (q, q + 8)]
            for i in range((hi - lo) // 8):
                r = _rows(i, 8)
                for c, v in ((q, x0[r] + x1[r]), (q + 8, x0[r] - x1[r])):
                    for z in range(2):
                        kv[0, 2 * c + z, _rows(lo // 8 + i, 8), :] = v[:, _rows(z, T1)]
            yield

    def residues(r, odd):
        return [(kv[0, 2 * c, r, :], kv[0, 2 * c + 1, r, :]) for c in range(8 * odd, 8 * odd + 8)]

    @_items(CB // 4)
    def tap_coefs(blk):
        for i in range(CB // 8):
            r = _rows(blk * CB // 8 + i, 8)
            for odd in range(2):
                for n, v in enumerate(_conv_coefs(residues(r, odd), 4 * odd)):
                    kf[10 * odd + n, r, :T1] = v[0]
                    kf[10 * odd + n, r, T1:] = v[1]
                yield

    r0 = jax.lax.broadcasted_iota(I32, (128, 128), 0)
    ri = (r0 & ~15) + (r0 & 7) * 2 + ((r0 >> 3) & 1)
    ci = jax.lax.broadcasted_iota(I32, (128, 128), 1)
    hit = ci == (ri & 7) * 16 + (ri >> 3)

    @_items(2)
    def prep_weights(j):
        def block(c, k):
            if j < 6:
                sel = jnp.where(hit, 1.0 if j < 4 else 0.25, 0.0)
                w = _bf(_zip(wq_in[_rows(k, 128), _rows(c, 128)].astype(F32)))
            else:
                sel = jnp.where(ri == ci, 1.0, 0.0)
                w = _bf(wp[_rows(k, 64), _rows(c, 128)])
            return jax.lax.dot_general(sel.astype(BF16), w, NT, preferred_element_type=F32)

        top, bot = (4 + j, 8 + j) if j < 4 else (j % 2, j % 2 + 2)
        for k in range(2):
            for i, a in enumerate(_strassen_lhs(block(top, k), block(top, k + 2),
                                                block(bot, k), block(bot, k + 2))):
                ws[i, _rows(j, 64), _rows(k, 128)] = _zip(a)
            yield

    @_items(1)
    def permute_wo(j):
        sel = jnp.where(ci == (r0 & 7) * 16 + (r0 >> 3), 1.0, 0.0).astype(BF16)
        wp[_rows(j, 64), :] = _zip(jnp.dot(sel, wo_in[_rows(j, 128), :],
                                           preferred_element_type=F32))
        yield

    @_items(4)
    def load_pair(h):
        for j in range(4):
            wds = io[h, :, _rows(j, 128)].T
            xs(2 * h)[_rows(j, 128), :] = pltpu.bitcast(wds << 16, F32)
            xs(2 * h + 1)[_rows(j, 128), :] = pltpu.bitcast(wds & jnp.uint32(0xFFFF0000), F32)
            yield

    @_items(24)
    def norm(h):
        for p in (2 * h, 2 * h + 1):
            normed = yield from _layernorm(lambda i: xs(p)[_rows(i, 8), :])
            for i in range(D // 16):
                xn[p, _rows(i, 16), :] = normed(i).astype(BF16)
                if i % 8 == 7:
                    yield

    nc = D // CB
    for i in range(nc + 4):
        def subs(s):
            return [2 * (i - s), 2 * (i - s) + 1] if 0 <= i - s < nc else []

        if i == 3:
            cp_f.wait()
        if i == nc - 1:
            for cp in cp_u:
                cp.wait()
        if i == nc:
            cp_wq.wait()
            cp_wo.wait()
        k = i - nc
        region([tap_sums(b) for b in subs(1)] + ([lane_dft(kv.at[1], CB * (i - 3), CB * (i - 2))] if subs(3) else [])
               + ([permute_wo(j) for j in range(4)] if k == 0 else [])
               + [prep_weights(j) for j in {1: (0, 1), 2: (2, 3), 3: (4, 5, 6, 7)}.get(k, ())],
               [tap_tables(b, e) for b in subs(0) for e in range(4)]
               + [norm(h) for h in (2 * k, 2 * k + 1) if 0 <= h < 7],
               [tap_blocks(b, e) for b in subs(2) for e in range(4)],
               [tap_coefs(i - 4)] if subs(4) else [],
               [load_pair(2 * k + 2), load_pair(2 * k + 3)] if -1 <= k < 3 else [])

    @_items(2)
    def phase_conv(i):
        r = _rows(i, 8)
        coefs = ((kf[n, r, :T1], kf[n, r, T1:]) for n in range(NCOEF))
        for odd in range(2):
            for c, v in enumerate(_conv(residues(r, odd), 4 * odd, lambda: next(coefs))):
                for z in range(2):
                    kv[1, 16 * odd + 2 * c + z, r, :] = v[z]
            yield

    @_items(8)
    def lane_idft(lo, hi):
        for q in (0, 2, 4, 6, 1, 3, 5, 7):
            a, b = [jnp.concatenate([kv[1, 2 * c + z, lo:hi, :] for z in range(2)], axis=1)
                    for c in (q, q + 8)]
            for p, v in ((q, a + b), (q + 8, a - b)):
                xs(p)[lo:hi, :] += jax.lax.dot_general(v, _bf(fm[p]), NT,
                                                       preferred_element_type=F32)
            yield

    @_items(32)
    def norm_pair(g):
        p = 4 * (g % 4) + g // 4
        a = yield from _layernorm(lambda i: xs(p)[_rows(i, 8), :])
        b = yield from _layernorm(lambda i: xs(p + 2)[_rows(i, 8), :])
        for r in range(HD // 16):
            xq[g, _rows(r, 8), :] = _strassen_rhs(a(r), b(r), a(HD // 16 + r), b(HD // 16 + r))
            yield

    def block_product(row0, groups, rhs, emit):
        for r in [128 // RS * hg + i for hg in groups for i in range(128 // RS)]:
            w = slice((row0 + r * RS) // 2, (row0 + r * RS + RS) // 2)
            yield from _strassen(
                lambda i: jnp.dot(_bf(ws[i, w, :]), _bf(rhs[:, _rows(i, T1)]),
                                  preferred_element_type=F32),
                lambda half, n, y: emit(half, n, r * RS, y))

    @_items(7 * HD // RS)
    def keys_values(s, g):
        def emit(half, n, row, y):
            m = 2 * (g % 4) + n
            kv[g // 4, PH * half + WIN - 1 + m, pl.ds(row, RS), :] = y
            if m:
                kv[g // 4, PH * half + m - 1, pl.ds(row, RS), :] = pltpu.roll(y, 1, 1)

        return block_product(0, (s, s + 2), xq.at[g], emit)

    @_items(7 * 128 // RS)
    def queries(s, g):
        def emit(half, n, row, y):
            qs[g, n, pl.ds(HD * half + row, RS), :] = y

        return block_product(D, (s,), xq.at[g], emit)

    @_items(34)
    def attend(par, s, m):
        for hg in (s, s + 2):
            lg = [None] * WIN
            for j0 in range(0, WIN, JB):
                for dh in range(16):
                    r = _rows(16 * hg + dh, 8)
                    q = qs[4 * par + m // 2, m % 2, r, :]
                    for j in range(j0, j0 + JB):
                        t = q * kv[par, WIN - 1 + m - j, r, :]
                        lg[j] = t if dh == 0 else lg[j] + t
                    if (dh + 1) % (16 // JB) == 0:
                        yield
            for j in range(m + 1, WIN):
                lg[j] = jnp.where(lane == 0, -1e9, lg[j])
            mx = lg[0]
            for j in range(1, WIN):
                mx = jnp.maximum(mx, lg[j])
            ex = [jnp.exp(t - mx) for t in lg]
            den = ex[0]
            for j in range(1, WIN):
                den = den + ex[j]
            inv = pltpu.reciprocal(den, full_range=False)
            pr = [t * inv for t in ex]
            yield

            def out(dh):
                r = _rows(16 * hg + dh, 8)
                acc = pr[0] * kv[par, PH + WIN - 1 + m, r, :]
                for j in range(1, WIN):
                    acc = acc + pr[j] * kv[par, PH + WIN - 1 + m - j, r, :]
                return acc

            for d2 in range(8):
                o = jnp.concatenate([out(2 * d2), out(2 * d2 + 1)], axis=0)
                r = _rows(8 * hg + d2, 16)
                if par == 0:
                    oe[m, r, :] = o
                elif hg < 2:
                    oo[m, r, :] = o
                else:
                    r1 = _rows(8 * (hg - 2) + d2, 16)
                    ob[m, _rows(8 * (hg - 2) + d2, 8), :] = _strassen_rhs(
                        oe[m, r1, :], oo[m, r1, :], oe[m, r, :], o)
                yield

    late = (1, 4)

    @_items(7 * HD // RS)
    def project(h):
        def emit(half, n, row, y):
            xs(2 * h + n)[pl.ds(HD * half + row, RS), :] += y

        for s in range(2):
            yield from block_product(D + HD, (s,), ob.at[h], emit)
            if h not in late:
                for _ in store_pair(h, (s, s + 2))[0]:
                    pass

    @_items(4)
    def store_pair(h, groups):
        for j in groups:
            io[h, :, _rows(j, 128)] = pltpu.pack_elementwise(
                [xs(2 * h + n)[_rows(j, 128), :] for n in range(2)], packed_dtype=BF16).T
            yield

    def layer(it, c):
        def send(hs):
            @pl.when(it == 1)
            def _():
                for h in hs:
                    cp_o[h].start()

        for i in range(len(CUTS[0]) - 1):
            (f0, f1), (c0, c1), (i0, i1) = [c[i:i + 2] for c in CUTS]
            last = i0 < i1 == D
            region([lane_dft(xn, c, min(c + CB, f1)) for c in range(f0, f1, CB)]
                   + [lane_idft(c, min(c + CB, i1)) for c in range(i0, i1, CB)],
                   [phase_conv(r) for r in range(c0 // 8, c1 // 8)]
                   + ([norm(7)] if i == 0 else []) + ([norm_pair(0)] if last else []),
                   lead=0.4 if last else 0.0, span=1.5 if i == 0 else 1.0)
        region([fn(0, g) for g in range(4) for fn in (keys_values, queries)],
               [norm_pair(g) for g in range(1, 8)])
        for par, s in ((0, 0), (0, 1), (1, 0)):
            g0 = 4 * (par + s)
            region([keys_values(1 - s, g0 + g) for g in range(4)]
                   + [queries(1 - s, g0 + g) for g in range(1 if par else 4)],
                   [attend(par, s, m) for m in range(WIN)])
        region([queries(1, g) for g in (5, 6, 7)], [attend(1, 1, m) for m in (0, 1)])
        done = ()
        for hs, ms in (((0, 1), (2, 3, 4)), ((2, 3, 4), (5, 6, 7)), ((5, 6), ()), ((7,), ())):
            region([project(h) for h in hs],
                   [store_pair(h, range(4)) for h in done if h in late]
                   + [norm(h) for h in done] + [attend(1, 1, m) for m in ms])
            send([h for h in done if h in late] + [h for h in hs if h not in late])
            done = hs

    jax.lax.fori_loop(0, 2, layer, None)
    for cp in cp_o:
        cp.wait()


@jax.jit
def pallas_interleave_layers__ssm_conv_s4__sliding_local_dilated__prompt_kernel(
    A_u: jax.Array,
    A_A_re: jax.Array,
    A_A_im: jax.Array,
    A_B_re: jax.Array,
    A_B_im: jax.Array,
    A_C_re: jax.Array,
    A_C_im: jax.Array,
    A_log_dt: jax.Array,
    A_Dskip: jax.Array,
    B_x: jax.Array,
    B_wqkv: jax.Array,
    B_wo: jax.Array,
):
    del B_x
    hbm = pl.BlockSpec(memory_space=pl.ANY)
    vmem = pl.BlockSpec(memory_space=pltpu.VMEM)
    out = pl.pallas_call(
        _kernel,
        in_specs=[hbm] * 7 + [vmem] * 2 + [hbm] * 3,
        out_specs=hbm,
        out_shape=jax.ShapeDtypeStruct((T1, PH, D), BF16),
        scratch_shapes=[pltpu.VMEM((D, NS), BF16)] * 6 + [
            pltpu.VMEM((PH // 2, T1, D), U32),
            pltpu.VMEM((D, 3 * D), BF16),
            pltpu.VMEM((D, D), BF16),
            pltpu.VMEM((PH, T1 // 2, 2 * T1), U32),
            pltpu.VMEM((7, D, HD), U32),
            pltpu.VMEM((D // 2, D), U32),
            pltpu.VMEM((2, D, NS), F32),
            pltpu.VMEM((2, D, NS), F32),
            pltpu.VMEM((D, T1), F32),
            pltpu.VMEM((4, 2, 9 * QS + 4, NS), U32),
            pltpu.VMEM((4, 9 * ZS + 4, T1), F32),
            pltpu.VMEM((NCOEF, D, 2 * T1), F32),
            pltpu.VMEM((PH, D, T1), F32),
            pltpu.VMEM((PH, D, T1), BF16),
            pltpu.VMEM((2, 2 * PH, D, T1), F32),
            pltpu.VMEM((PH // 2, HD // 2, 7 * T1), U32),
            pltpu.VMEM((PH // 2, 2, D, T1), F32),
            pltpu.VMEM((WIN, D, T1), F32),
            pltpu.VMEM((WIN, HD, T1), F32),
            pltpu.VMEM((WIN, HD // 2, 7 * T1), U32),
            pltpu.SMEM((1,), I32),
            pltpu.SemaphoreType.DMA((9 + PH // 2,)),
        ],
        compiler_params=pltpu.CompilerParams(vmem_limit_bytes=100 * 1024 * 1024),
    )(A_u.reshape(T1, PH, D), A_A_re, A_A_im, A_B_re, A_B_im, A_C_re, A_C_im,
      A_log_dt, A_Dskip, B_wqkv, B_wo,
      _dft_matrices())
    return out.reshape(1, L, D)
```

```python
import numpy as np

import jax
import jax.numpy as jnp
import jax.experimental.pallas as pl
import jax.experimental.pallas.tpu as pltpu

F32, BF16, U32, I32 = jnp.float32, jnp.bfloat16, jnp.uint32, jnp.int32
L, D, NS = 2048, 512, 128
PH, T1 = 16, 128
WIN = 8
NN = (((1,), (0,)), ((), ()))
NT = (((1,), (1,)), ((), ()))
QS = 116
ZS = 28
_H = float(np.sqrt(0.5))
NCOEF = 22
HD = D // 2
RS = 64
JB = 4
CUTS = ((0, 64, 192, 320, 448, D, D, D),
        (0, 0, 64, 192, 320, 448, D, D),
        (0, 0, 0, 64, 192, 320, 448, D))
PROLOGUE = ((1, 0, 0, 0, 0, 0, 0, 0, 0),
            (3, 1, 0, 0, 0, 2, 0, 0, 0),
            (5, 3, 1, 0, 0, 5, 0, 0, 0),
            (7, 5, 3, 1, 0, 8, 0, 0, 0),
            (8, 7, 5, 3, 1, 8, 0, 4, 0),
            (8, 8, 7, 5, 3, 8, 2, 4, 2),
            (8, 8, 8, 7, 5, 8, 5, 4, 4),
            (8, 8, 8, 8, 8, 8, 7, 4, 8))
CB = 64


def _dft_matrices():
    t = 16 * np.arange(T1)[None, :, None] + np.arange(PH)[:, None, None]
    k = np.arange(T1)[None, None, :] + 0.5
    phi = 2.0 * np.pi * k * t / (2 * L)
    f = np.concatenate([np.cos(phi), -np.sin(phi)], axis=-1).astype(np.float32)
    bits = f.astype(BF16).view(np.uint16).astype(np.uint32)
    return bits[:, 0::2] | (bits[:, 1::2] << 16)


def _cmul(a, b):
    return a[0] * b[0] - a[1] * b[1], a[0] * b[1] + a[1] * b[0]


def _csq(a):
    t = a[0] * a[1]
    return a[0] * a[0] - a[1] * a[1], t + t


def _cadd(a, b):
    return a[0] + b[0], a[1] + b[1]


def _csub(a, b):
    return a[0] - b[0], a[1] - b[1]


def _rot8(x, e):
    s, d = x[0] + x[1], x[0] - x[1]
    return {1: (d * _H, s * _H), 3: (s * -_H, d * _H), 5: (d * -_H, s * -_H), 7: (s * _H, d * -_H)}[e]


def _split(x, e):
    n = len(x) // 2
    lo, hi = x[:n], x[n:]
    if e == 4:
        return ([(a[0] - b[1], a[1] + b[0]) for a, b in zip(lo, hi)],
                [(a[0] + b[1], a[1] - b[0]) for a, b in zip(lo, hi)])
    if e:
        hi = [_rot8(b, e // 2) for b in hi]
    return [_cadd(a, b) for a, b in zip(lo, hi)], [_csub(a, b) for a, b in zip(lo, hi)]


def _merge(p, m, e):
    lo = [_cadd(a, b) for a, b in zip(p, m)]
    if e == 4:
        return lo + [(a[1] - b[1], b[0] - a[0]) for a, b in zip(p, m)]
    hi = [_csub(a, b) for a, b in zip(p, m)]
    return lo + ([_rot8(b, 8 - e // 2) for b in hi] if e else hi)


def _conv_coefs(k, e):
    if len(k) == 1:
        return [(k[0][0] * 0.5, k[0][1] * 0.5)]
    if len(k) == 2 and e % 4:
        if e % 2:
            top = _csub(_rot8(k[1], e), k[0])
        elif e == 2:
            top = (-k[1][1] - k[0][0], k[1][0] - k[0][1])
        else:
            top = (k[1][1] - k[0][0], -k[1][0] - k[0][1])
        return [k[0], top, _csub(k[1], k[0])]
    p, m = _split(k, e)
    return _conv_coefs(p, e // 2) + _conv_coefs(m, e // 2 + 4)


def _conv(x, e, coef):
    if len(x) == 1:
        return [_cmul(x[0], coef())]
    if len(x) == 2 and e % 4:
        both = _cmul(_cadd(x[0], x[1]), coef())
        return [_cadd(both, _cmul(x[1], coef())), _cadd(both, _cmul(x[0], coef()))]
    p, m = _split(x, e)
    return _merge(_conv(p, e // 2, coef), _conv(m, e // 2 + 4, coef), e)


def _sincos(x):
    n = jnp.floor(x * float(2.0 / np.pi) + 0.5)
    r = ((x - n * 1.5703125) - n * 4.837512969970703125e-4) - n * 7.54978995489188216e-8
    z = r * r
    s = r + r * z * ((-1.9515295891e-4 * z + 8.3321608736e-3) * z - 1.6666654611e-1)
    c = 1.0 + z * (((2.443315711809948e-5 * z - 1.388731625493765e-3) * z
                    + 4.166664568298827e-2) * z - 0.5)
    q = n.astype(I32)
    odd = (q & 1) == 1
    s, c = jnp.where(odd, c, s), jnp.where(odd, s, c)
    return jnp.where((q & 2) == 2, -s, s), jnp.where(((q + 1) & 2) == 2, -c, c)


def _pk(x):
    return pltpu.bitcast(x.astype(BF16), U32)


def _zip(x):
    return jnp.concatenate(
        [pltpu.pack_elementwise([x[i:i + 8], x[i + 8:i + 16]], packed_dtype=BF16)
         for i in range(0, x.shape[0], 16)], axis=0)


def _bf(words):
    return pltpu.bitcast(words, BF16)


def _layernorm(load):
    def mean(term, every):
        acc = [term(load(i)) for i in range(4)]
        for i in range(4, D // 8):
            acc[i % 4] = acc[i % 4] + term(load(i))
            if i % every == every - 1:
                yield
        tot = jnp.sum((acc[0] + acc[1]) + (acc[2] + acc[3]), axis=0, keepdims=True)
        return jnp.broadcast_to(tot * (1.0 / D), (8, T1))

    mu = yield from mean(lambda x: x, 32)
    var = yield from mean(lambda x: (x - mu) * (x - mu), 10)
    rs = jax.lax.rsqrt(var + 1e-5)
    return lambda i: jnp.concatenate([(load(2 * i + s) - mu) * rs for s in range(2)], axis=0)


def _items(n):
    return lambda fn: lambda *args: (fn(*args), n)


def _interleave(*lists, lead=0.0, span=1.0):
    gens = [(v for g, _ in w for v in g) for w in lists]
    sizes = [sum(n for _, n in w) for w in lists]
    for _, k in sorted((i / n if k else i / n * span - lead, k)
                       for k, n in enumerate(sizes) for i in range(n)):
        next(gens[k])
    for g in gens:
        for _ in g:
            pass


def _strassen_lhs(a11, a12, a21, a22):
    return a11 + a22, a22, a21 + a22, a11 + a12, a11, a12 - a22, a21 - a11


def _strassen_rhs(b11, b12, b21, b22):
    ops = (b11 + b22, b21 - b11, b11, b22, b12 - b22, b21 + b22, b11 + b12)
    return jnp.concatenate([_zip(v) for v in ops], axis=1)


def _strassen(prod, emit):
    m1 = prod(0)
    yield
    m4 = prod(1)
    c11 = m1 + m4
    yield
    m2 = prod(2)
    emit(1, 0, m2 + m4)
    c22 = m1 - m2
    yield
    m5 = prod(3)
    c11 = c11 - m5
    yield
    m3 = prod(4)
    emit(0, 1, m3 + m5)
    c22 = c22 + m3
    yield
    emit(0, 0, c11 + prod(5))
    yield
    emit(1, 1, c22 + prod(6))
    yield


def _rows(i, n):
    return slice(i * n, i * n + n)


def _kernel(u_hbm, are_hbm, aim_hbm, bre_hbm, bim_hbm, cre_hbm, cim_hbm, ldt, dsk, wqkv_hbm, wo_hbm, f_hbm, out_hbm,
            are, aim, bre, bim, cre, cim, io, wq_in, wo_in, fm, ws, wp, lam, dtc, k0s, tab, ztab, kb, kf,
            xr, xn, kv, xq, qs, oe, oo, ob, zs, sems):
    cp_u = [pltpu.make_async_copy(u_hbm.bitcast(U32).at[:, h, :], io.at[h], sems.at[3 + h])
            for h in range(PH // 2)]
    cp_o = [pltpu.make_async_copy(io.at[h], out_hbm.bitcast(U32).at[:, h, :], sems.at[3 + h])
            for h in range(PH // 2)]
    cp_f = pltpu.make_async_copy(f_hbm, fm, sems.at[0])
    cp_wq = pltpu.make_async_copy(wqkv_hbm, wq_in, sems.at[1])
    cp_wo = pltpu.make_async_copy(wo_hbm, wo_in, sems.at[2])
    cp_p = [pltpu.make_async_copy(src, dst, sems.at[3 + PH // 2 + i]) for i, (src, dst) in enumerate(
        ((aim_hbm, aim), (are_hbm, are), (bre_hbm, bre), (bim_hbm, bim), (cre_hbm, cre),
         (cim_hbm, cim)))]
    for cp in cp_p:
        cp.start()

    lane = jax.lax.broadcasted_iota(I32, (8, T1), 1)
    zs[0] = 0

    def xs(p):
        return xr.at[p]

    def region(*lists, **pace):
        pl.when(zs[0] == 0)(lambda: _interleave(*lists, **pace))

    dt_row = jnp.exp(ldt[...].astype(F32).reshape(1, D)).astype(BF16).astype(F32)
    ds_row = dsk[...].astype(F32).reshape(1, D)
    for j in range(4):
        dtc[0, _rows(j, 128), :] = jnp.broadcast_to(dt_row[:, _rows(j, 128)], (128, 128)).T
        dtc[1, _rows(j, 128), :] = jnp.broadcast_to(ds_row[:, _rows(j, 128)], (128, 128)).T
    cp_p[0].wait()
    cp_p[1].wait()
    for cp in cp_u[:2]:
        cp.start()
    big = None
    for j in range(D // 16):
        r = _rows(j, 16)
        theta = dtc[0, r, :] * aim[r, :].astype(F32)
        mag = jnp.exp(dtc[0, r, :] * are[r, :].astype(F32))
        sn, cs = _sincos(theta)
        lam[0, r, :] = mag * cs
        lam[1, r, :] = mag * sn
        big = jnp.abs(theta) if big is None else jnp.maximum(big, jnp.abs(theta))

    @pl.when(jnp.logical_not(jnp.max(big) <= 8192.0))
    def _():
        def body(i, _):
            rows = pl.ds(pl.multiple_of(i * 16, 16), 16)
            th = dtc[0, rows, :] * aim[rows, :].astype(F32)
            mg = jnp.exp(dtc[0, rows, :] * are[rows, :].astype(F32))
            lam[0, rows, :] = mg * jnp.cos(th)
            lam[1, rows, :] = mg * jnp.sin(th)
        jax.lax.fori_loop(0, D // 16, body, None)

    for cp in cp_p[2:]:
        cp.wait()

    @_items(15)
    def tap_tables(blk, e):
        rows = _rows(4 * blk + e, 8)

        def part(ref):
            return ref[_rows(2 * blk + e // 2, 16), :].astype(F32)[_rows(e % 2, 8)]

        sc = dtc[0, rows, :] * (2.0 / L)
        w = _cmul((part(cre), part(cim)), (part(bre) * sc, part(bim) * sc))
        k0s[rows, :] = w[0]

        def put(row, a, b):
            for z in range(2):
                tab[blk % 8, z, pl.ds(row, 8, stride=QS), :] = pltpu.pack_elementwise(
                    [a[z], b[z]], packed_dtype=BF16)

        l1 = (lam[0, rows, :], lam[1, rows, :])
        l2 = _csq(l1)
        l16 = _csq(_csq(_csq(l2)))
        m1 = (l16[0], -l16[1])
        m2 = _csq(m1)
        a, b = _cmul(w, l1), _cmul(w, l2)
        c, d = m2, _cmul(m1, m2)
        put(16 * e, (jnp.ones_like(m1[0]), jnp.zeros_like(m1[0])), m1)
        keep = {}
        for j in range(1, 16):
            if j <= 8:
                put(64 + 12 * e + j - 1, a, b)
                keep[2 * j] = b
            if j < 8:
                a, b = _cmul(a, l2), _cmul(b, l2)
            put(16 * e + j, c, d)
            if j == 8:
                l512 = _csq((c[0], -c[1]))
                put(64 + 12 * e + 8, _cmul(keep[4], l512), _cmul(keep[12], l512))
                a, b = keep[8], keep[16]
            if j in (10, 12, 14):
                a, b = _cmul(a, l512), _cmul(b, l512)
                put(64 + 12 * e + 4 + j // 2, a, b)
            if j < 15:
                c, d = _cmul(c, m2), _cmul(d, m2)
            yield

    @_items(8)
    def tap_sums(blk):
        for i in range(8):
            re, im = [jax.lax.dot_general(_bf(tab[blk % 8, z, pl.ds(QS * i + 64, 48), :]),
                                          _bf(tab[blk % 8, z, pl.ds(QS * i, 64), :]),
                                          NT, preferred_element_type=F32) for z in range(2)]
            yield
            acc = re + im
            for r in range(3):
                pc = [acc[_rows(3 * e + r, 8)] for e in range(4)]
                ztab[blk % 8, pl.ds(ZS * i + 8 * r, 8), :] = jnp.where(
                    lane < 64, jnp.where(lane < 32, pc[0], pc[1]),
                    jnp.where(lane < 96, pc[2], pc[3]))

    def tap_rows(blk, e):
        def at(r, g):
            z = ztab[blk % 8, pl.ds(r, 8, stride=ZS), :]
            return z if g == e else pltpu.roll(z, (32 * (g - e)) % 128, 1)

        def full(r, r1):
            return jnp.where(lane < 64, jnp.where(lane < 32, at(r, 0), at(r1, 1)),
                             jnp.where(lane < 96, at(r1 + 2, 2), at(r1 + 4, 3)))

        rows = _rows(4 * blk + e, 8)
        e8, e16 = full(7, 18), full(15, 19)
        k0 = jnp.sum(k0s[rows, :], axis=1, keepdims=True) + dtc[1, rows, :] * (2.0 / L)
        e0 = jnp.where(lane == 0, k0, pltpu.roll(e16, 1, 1))
        e4 = jnp.where(lane < 32, at(3, 0), at(16, 1))
        e12 = jnp.where(lane < 32, at(11, 0), at(17, 1))
        k4, k12 = jnp.where(lane < 64, e4, e0), jnp.where(lane < 64, e12, e16)
        far = {1: e0, 2: e0, 3: k4, 5: jnp.where(lane < 64, e4, e8), 6: e8, 7: e8, 9: e8,
               10: e8, 11: jnp.where(lane < 64, e12, e8), 13: k12, 14: e16, 15: e16}
        taps = {0: e0, 4: k4, 8: e8, 12: k12}
        return lambda p: taps[p] if p in taps else jnp.where(
            lane < (16 if p % 2 else 32), at(p - 1, 0), far[p])

    @_items(2)
    def tap_blocks(blk, e2):
        a, b = tap_rows(blk, 2 * e2), tap_rows(blk, 2 * e2 + 1)
        yield
        for p in range(PH):
            kb[p, _rows(2 * blk + e2, 16), :] = jnp.concatenate([a(p), b(p)], axis=0).astype(BF16)
        yield

    @_items(8)
    def lane_dft(src, lo, hi):
        for q in range(8):
            x0, x1 = [jax.lax.dot_general(src[p, lo:hi, :], _bf(fm[p]), NN,
                                          preferred_element_type=F32) for p in (q, q + 8)]
            for i in range((hi - lo) // 8):
                r = _rows(i, 8)
                for c, v in ((q, x0[r] + x1[r]), (q + 8, x0[r] - x1[r])):
                    for z in range(2):
                        kv[0, 2 * c + z, _rows(lo // 8 + i, 8), :] = v[:, _rows(z, T1)]
            yield

    def residues(r, odd):
        return [(kv[0, 2 * c, r, :], kv[0, 2 * c + 1, r, :]) for c in range(8 * odd, 8 * odd + 8)]

    @_items(CB // 4)
    def tap_coefs(blk):
        for i in range(CB // 8):
            r = _rows(blk * CB // 8 + i, 8)
            for odd in range(2):
                for n, v in enumerate(_conv_coefs(residues(r, odd), 4 * odd)):
                    kf[10 * odd + n, r, :T1] = v[0]
                    kf[10 * odd + n, r, T1:] = v[1]
                yield

    r0 = jax.lax.broadcasted_iota(I32, (128, 128), 0)
    ri = (r0 & ~15) + (r0 & 7) * 2 + ((r0 >> 3) & 1)
    ci = jax.lax.broadcasted_iota(I32, (128, 128), 1)
    hit = ci == (ri & 7) * 16 + (ri >> 3)

    @_items(2)
    def prep_weights(j):
        def block(c, k):
            if j < 6:
                sel = jnp.where(hit, 1.0 if j < 4 else 0.25, 0.0)
                w = wq_in[_rows(k, 128), _rows(c, 128)]
            else:
                sel = jnp.where(ri == ci, 1.0, 0.0)
                w = _bf(wp[_rows(k, 64), _rows(c, 128)])
            return jax.lax.dot_general(sel.astype(BF16), w, NT, preferred_element_type=F32)

        top, bot = (4 + j, 8 + j) if j < 4 else (j % 2, j % 2 + 2)
        for k in range(2):
            for i, a in enumerate(_strassen_lhs(block(top, k), block(top, k + 2),
                                                block(bot, k), block(bot, k + 2))):
                ws[i, _rows(j, 64), _rows(k, 128)] = _zip(a)
            yield

    @_items(1)
    def permute_wo(j):
        sel = jnp.where(ci == (r0 & 7) * 16 + (r0 >> 3), 1.0, 0.0).astype(BF16)
        wp[_rows(j, 64), :] = _zip(jnp.dot(sel, wo_in[_rows(j, 128), :],
                                           preferred_element_type=F32))
        yield

    @_items(4)
    def load_pair(h):
        for j in range(4):
            wds = io[h, :, _rows(j, 128)].T
            xs(2 * h)[_rows(j, 128), :] = pltpu.bitcast(wds << 16, F32)
            xs(2 * h + 1)[_rows(j, 128), :] = pltpu.bitcast(wds & jnp.uint32(0xFFFF0000), F32)
            yield

    @_items(24)
    def norm(h):
        for p in (2 * h, 2 * h + 1):
            normed = yield from _layernorm(lambda i: xs(p)[_rows(i, 8), :])
            for i in range(D // 16):
                xn[p, _rows(i, 16), :] = normed(i).astype(BF16)
                if i % 8 == 7:
                    yield

    for i, step in enumerate(PROLOGUE):
        tables, sums, blocks, dft, coefs, loads, norms, perms, preps = [
            range(a, b) for a, b in zip(PROLOGUE[i - 1] if i else (0,) * 9, step)]
        for cp in {0: cp_u[2:5], 1: [cp_f], 2: cp_u[5:], 3: [cp_wo, cp_wq]}.get(i, ()):
            cp.start()
        for cp, users in ((cp_f, dft), (cp_wo, perms), (cp_wq, preps)):
            if 0 in users:
                cp.wait()
        for h in loads:
            cp_u[h].wait()
        region([tap_sums(2 * b + s) for b in sums for s in range(2)]
               + [lane_dft(kb, CB * b, CB * b + CB) for b in dft]
               + [permute_wo(j) for j in perms] + [prep_weights(j) for j in preps],
               [tap_tables(2 * b + s, e) for b in tables for s in range(2) for e in range(4)]
               + [norm(h) for h in norms],
               [tap_blocks(2 * b + s, e) for b in blocks for s in range(2) for e in range(2)],
               [tap_coefs(b) for b in coefs],
               [load_pair(h) for h in loads])

    @_items(2)
    def phase_conv(i):
        r = _rows(i, 8)
        coefs = ((kf[n, r, :T1], kf[n, r, T1:]) for n in range(NCOEF))
        for odd in range(2):
            for c, v in enumerate(_conv(residues(r, odd), 4 * odd, lambda: next(coefs))):
                for z in range(2):
                    kv[1, 16 * odd + 2 * c + z, r, :] = v[z]
            yield

    @_items(8)
    def lane_idft(lo, hi):
        for q in (0, 2, 4, 6, 1, 3, 5, 7):
            a, b = [jnp.concatenate([kv[1, 2 * c + z, lo:hi, :] for z in range(2)], axis=1)
                    for c in (q, q + 8)]
            for p, v in ((q, a + b), (q + 8, a - b)):
                xs(p)[lo:hi, :] += jax.lax.dot_general(v, _bf(fm[p]), NT,
                                                       preferred_element_type=F32)
            yield

    @_items(32)
    def norm_pair(g):
        def unzipped(i):
            return pl.ds(16 * (i // 2) + i % 2, 8, stride=2)

        p = 4 * (g % 4) + g // 4
        a = yield from _layernorm(lambda i: xr[p, unzipped(i), :])
        b = yield from _layernorm(lambda i: xr[p + 2, unzipped(i), :])
        for r in range(HD // 16):
            xq[g, _rows(r, 8), :] = _strassen_rhs(a(r), b(r), a(HD // 16 + r), b(HD // 16 + r))
            yield

    def block_product(row0, groups, rhs, emit):
        for r in [128 // RS * hg + i for hg in groups for i in range(128 // RS)]:
            w = slice((row0 + r * RS) // 2, (row0 + r * RS + RS) // 2)
            yield from _strassen(
                lambda i: jnp.dot(_bf(ws[i, w, :]), _bf(rhs[:, _rows(i, T1)]),
                                  preferred_element_type=F32),
                lambda half, n, y: emit(half, n, r * RS, y))

    @_items(7 * HD // RS)
    def keys_values(s, g):
        def emit(half, n, row, y):
            m = 2 * (g % 4) + n
            kv[g // 4, PH * half + WIN - 1 + m, pl.ds(row, RS), :] = y
            if m:
                kv[g // 4, PH * half + m - 1, pl.ds(row, RS), :] = pltpu.roll(y, 1, 1)

        return block_product(0, (s, s + 2), xq.at[g], emit)

    @_items(7 * 128 // RS)
    def queries(s, g):
        def emit(half, n, row, y):
            qs[g, n, pl.ds(HD * half + row, RS), :] = y

        return block_product(D, (s,), xq.at[g], emit)

    @_items(34)
    def attend(par, s, m):
        for hg in (s, s + 2):
            lg = [None] * WIN
            for j0 in range(0, WIN, JB):
                for dh in range(16):
                    r = _rows(16 * hg + dh, 8)
                    q = qs[4 * par + m // 2, m % 2, r, :]
                    for j in range(j0, j0 + JB):
                        t = q * kv[par, WIN - 1 + m - j, r, :]
                        lg[j] = t if dh == 0 else lg[j] + t
                    if (dh + 1) % (16 // JB) == 0:
                        yield
            for j in range(m + 1, WIN):
                lg[j] = jnp.where(lane == 0, -1e9, lg[j])
            mx = lg[0]
            for j in range(1, WIN):
                mx = jnp.maximum(mx, lg[j])
            ex = [jnp.exp(t - mx) for t in lg]
            den = ex[0]
            for j in range(1, WIN):
                den = den + ex[j]
            inv = pltpu.reciprocal(den, full_range=False)
            pr = [t * inv for t in ex]
            yield

            def out(dh):
                r = _rows(16 * hg + dh, 8)
                acc = pr[0] * kv[par, PH + WIN - 1 + m, r, :]
                for j in range(1, WIN):
                    acc = acc + pr[j] * kv[par, PH + WIN - 1 + m - j, r, :]
                return acc

            for d2 in range(8):
                o = jnp.concatenate([out(2 * d2), out(2 * d2 + 1)], axis=0)
                r = _rows(8 * hg + d2, 16)
                if par == 0:
                    oe[m, r, :] = o
                elif hg < 2:
                    oo[m, r, :] = o
                else:
                    r1 = _rows(8 * (hg - 2) + d2, 16)
                    ob[m, _rows(8 * (hg - 2) + d2, 8), :] = _strassen_rhs(
                        oe[m, r1, :], oo[m, r1, :], oe[m, r, :], o)
                yield

    late = (1, 4)

    @_items(7 * HD // RS)
    def project(h):
        def emit(half, n, row, y):
            xs(2 * h + n)[pl.ds(HD * half + row, RS), :] += y

        for s in range(2):
            yield from block_product(D + HD, (s,), ob.at[h], emit)
            if h not in late:
                for _ in store_pair(h, (s, s + 2))[0]:
                    pass

    @_items(4)
    def store_pair(h, groups):
        for j in groups:
            io[h, :, _rows(j, 128)] = pltpu.pack_elementwise(
                [xs(2 * h + n)[_rows(j, 128), :] for n in range(2)], packed_dtype=BF16).T
            yield

    def layer(it, c):
        def send(hs):
            @pl.when(it == 1)
            def _():
                for h in hs:
                    cp_o[h].start()

        for i in range(len(CUTS[0]) - 1):
            (f0, f1), (c0, c1), (i0, i1) = [c[i:i + 2] for c in CUTS]
            last = i0 < i1 == D
            region([lane_dft(xn, c, min(c + CB, f1)) for c in range(f0, f1, CB)]
                   + [lane_idft(c, min(c + CB, i1)) for c in range(i0, i1, CB)],
                   [phase_conv(r) for r in range(c0 // 8, c1 // 8)]
                   + ([norm(7)] if i == 0 else []) + ([norm_pair(0)] if last else []),
                   lead=0.4 if last else 0.0, span=1.5 if i == 0 else 1.0)
        region([keys_values(0, 0), queries(0, 0), keys_values(1, 0), queries(1, 0)],
               [norm_pair(g) for g in (1, 2, 3, 4)])
        region([fn(0, g) for fn in (keys_values, queries) for g in (1, 2, 3)],
               [norm_pair(g) for g in (5, 6, 7)])
        for par, s in ((0, 0), (0, 1), (1, 0)):
            gs = (4, 5, 6, 7) if par + s else (1, 2, 3)
            region([keys_values(1 - s, g) for g in gs]
                   + [queries(1 - s, g) for g in (gs[:1] if par else gs)],
                   [attend(par, s, m) for m in range(WIN)])
        region([queries(1, g) for g in (5, 6, 7)], [attend(1, 1, m) for m in (0, 1)])
        done = ()
        for hs, ms in (((0, 1), (2, 3, 4)), ((2, 3, 4), (5, 6, 7)), ((5, 6), ()), ((7,), ())):
            region([project(h) for h in hs],
                   [store_pair(h, range(4)) for h in done if h in late]
                   + [norm(h) for h in done] + [attend(1, 1, m) for m in ms])
            send([h for h in done if h in late] + [h for h in hs if h not in late])
            done = hs

    jax.lax.fori_loop(0, 2, layer, None)
    for cp in cp_o:
        cp.wait()


@jax.jit
def pallas_interleave_layers__ssm_conv_s4__sliding_local_dilated__prompt_kernel(
    A_u: jax.Array,
    A_A_re: jax.Array,
    A_A_im: jax.Array,
    A_B_re: jax.Array,
    A_B_im: jax.Array,
    A_C_re: jax.Array,
    A_C_im: jax.Array,
    A_log_dt: jax.Array,
    A_Dskip: jax.Array,
    B_x: jax.Array,
    B_wqkv: jax.Array,
    B_wo: jax.Array,
):
    del B_x
    hbm = pl.BlockSpec(memory_space=pl.ANY)
    vmem = pl.BlockSpec(memory_space=pltpu.VMEM)
    out = pl.pallas_call(
        _kernel,
        in_specs=[hbm] * 7 + [vmem] * 2 + [hbm] * 3,
        out_specs=hbm,
        out_shape=jax.ShapeDtypeStruct((T1, PH, D), BF16),
        scratch_shapes=[pltpu.VMEM((D, NS), BF16)] * 6 + [
            pltpu.VMEM((PH // 2, T1, D), U32),
            pltpu.VMEM((D, 3 * D), BF16),
            pltpu.VMEM((D, D), BF16),
            pltpu.VMEM((PH, T1 // 2, 2 * T1), U32),
            pltpu.VMEM((7, D, HD), U32),
            pltpu.VMEM((D // 2, D), U32),
            pltpu.VMEM((2, D, NS), F32),
            pltpu.VMEM((2, D, NS), F32),
            pltpu.VMEM((D, T1), F32),
            pltpu.VMEM((8, 2, 9 * QS + 4, NS), U32),
            pltpu.VMEM((8, 9 * ZS + 4, T1), F32),
            pltpu.VMEM((PH, D, T1), BF16),
            pltpu.VMEM((NCOEF, D, 2 * T1), F32),
            pltpu.VMEM((PH, D + 8, T1), F32),
            pltpu.VMEM((PH, D, T1), BF16),
            pltpu.VMEM((2, 2 * PH, D, T1), F32),
            pltpu.VMEM((PH // 2, HD // 2, 7 * T1), U32),
            pltpu.VMEM((PH // 2, 2, D, T1), F32),
            pltpu.VMEM((WIN, D, T1), F32),
            pltpu.VMEM((WIN, HD, T1), F32),
            pltpu.VMEM((WIN, HD // 2, 7 * T1), U32),
            pltpu.SMEM((1,), I32),
            pltpu.SemaphoreType.DMA((9 + PH // 2,)),
        ],
        compiler_params=pltpu.CompilerParams(vmem_limit_bytes=100 * 1024 * 1024),
    )(A_u.reshape(T1, PH, D), A_A_re, A_A_im, A_B_re, A_B_im, A_C_re, A_C_im,
      A_log_dt, A_Dskip, B_wqkv, B_wo,
      _dft_matrices())
    return out.reshape(1, L, D)
```

```python
import numpy as np

import jax
import jax.numpy as jnp
import jax.experimental.pallas as pl
import jax.experimental.pallas.tpu as pltpu

F32, BF16, U32, I32 = jnp.float32, jnp.bfloat16, jnp.uint32, jnp.int32
L, D, NS = 2048, 512, 128
PH, T1 = 16, 128
WIN = 8
NN = (((1,), (0,)), ((), ()))
NT = (((1,), (1,)), ((), ()))
QS = 116
ZS = 28
_H = float(np.sqrt(0.5))
NCOEF = 22
HD = D // 2
RS = 64
JB = 4
CUTS = ((0, 64, 192, 320, 448, D, D, D),
        (0, 0, 64, 192, 320, 448, D, D),
        (0, 0, 0, 64, 192, 320, 448, D))
PROLOGUE = ((1, 0, 0, 0, 0, 0, 0, 0, 0),
            (3, 1, 0, 0, 0, 2, 0, 0, 0),
            (5, 3, 1, 0, 0, 5, 0, 0, 0),
            (7, 5, 3, 1, 0, 8, 0, 0, 0),
            (8, 7, 5, 3, 1, 8, 0, 4, 0),
            (8, 8, 7, 5, 3, 8, 2, 4, 2),
            (8, 8, 8, 7, 5, 8, 5, 4, 4),
            (8, 8, 8, 8, 8, 8, 7, 4, 8))
CB = 64


def _dft_matrices():
    t = 16 * np.arange(T1)[None, :, None] + np.arange(PH)[:, None, None]
    k = np.arange(T1)[None, None, :] + 0.5
    phi = 2.0 * np.pi * k * t / (2 * L)
    phi = np.concatenate([phi, phi.transpose(0, 2, 1)])
    f = np.concatenate([np.cos(phi), -np.sin(phi)], axis=-1).astype(np.float32)
    bits = f.astype(BF16).view(np.uint16).astype(np.uint32)
    return bits[:, 0::2] | (bits[:, 1::2] << 16)


def _cmul(a, b):
    return a[0] * b[0] - a[1] * b[1], a[0] * b[1] + a[1] * b[0]


def _csq(a):
    t = a[0] * a[1]
    return a[0] * a[0] - a[1] * a[1], t + t


def _cadd(a, b):
    return a[0] + b[0], a[1] + b[1]


def _csub(a, b):
    return a[0] - b[0], a[1] - b[1]


def _rot8(x, e):
    s, d = x[0] + x[1], x[0] - x[1]
    return {1: (d * _H, s * _H), 3: (s * -_H, d * _H), 5: (d * -_H, s * -_H), 7: (s * _H, d * -_H)}[e]


def _split(x, e):
    n = len(x) // 2
    lo, hi = x[:n], x[n:]
    if e == 4:
        return ([(a[0] - b[1], a[1] + b[0]) for a, b in zip(lo, hi)],
                [(a[0] + b[1], a[1] - b[0]) for a, b in zip(lo, hi)])
    if e:
        hi = [_rot8(b, e // 2) for b in hi]
    return [_cadd(a, b) for a, b in zip(lo, hi)], [_csub(a, b) for a, b in zip(lo, hi)]


def _merge(p, m, e):
    lo = [_cadd(a, b) for a, b in zip(p, m)]
    if e == 4:
        return lo + [(a[1] - b[1], b[0] - a[0]) for a, b in zip(p, m)]
    hi = [_csub(a, b) for a, b in zip(p, m)]
    return lo + ([_rot8(b, 8 - e // 2) for b in hi] if e else hi)


def _conv_coefs(k, e):
    if len(k) == 1:
        return [(k[0][0] * 0.5, k[0][1] * 0.5)]
    if len(k) == 2 and e % 4:
        if e % 2:
            top = _csub(_rot8(k[1], e), k[0])
        elif e == 2:
            top = (-k[1][1] - k[0][0], k[1][0] - k[0][1])
        else:
            top = (k[1][1] - k[0][0], -k[1][0] - k[0][1])
        return [k[0], top, _csub(k[1], k[0])]
    p, m = _split(k, e)
    return _conv_coefs(p, e // 2) + _conv_coefs(m, e // 2 + 4)


def _conv(x, e, coef):
    if len(x) == 1:
        return [_cmul(x[0], coef())]
    if len(x) == 2:
        yield
    if len(x) == 2 and e % 4:
        both = _cmul(_cadd(x[0], x[1]), coef())
        return [_cadd(both, _cmul(x[1], coef())), _cadd(both, _cmul(x[0], coef()))]
    p, m = _split(x, e)
    p = yield from _conv(p, e // 2, coef)
    m = yield from _conv(m, e // 2 + 4, coef)
    return _merge(p, m, e)


def _sincos(x):
    n = jnp.floor(x * float(2.0 / np.pi) + 0.5)
    r = ((x - n * 1.5703125) - n * 4.837512969970703125e-4) - n * 7.54978995489188216e-8
    z = r * r
    s = r + r * z * ((-1.9515295891e-4 * z + 8.3321608736e-3) * z - 1.6666654611e-1)
    c = 1.0 + z * (((2.443315711809948e-5 * z - 1.388731625493765e-3) * z
                    + 4.166664568298827e-2) * z - 0.5)
    q = n.astype(I32)
    odd = (q & 1) == 1
    s, c = jnp.where(odd, c, s), jnp.where(odd, s, c)
    return jnp.where((q & 2) == 2, -s, s), jnp.where(((q + 1) & 2) == 2, -c, c)


def _pk(x):
    return pltpu.bitcast(x.astype(BF16), U32)


def _zip(x):
    return jnp.concatenate(
        [pltpu.pack_elementwise([x[i:i + 8], x[i + 8:i + 16]], packed_dtype=BF16)
         for i in range(0, x.shape[0], 16)], axis=0)


def _bf(words):
    return pltpu.bitcast(words, BF16)


def _layernorm(load):
    def mean(term, every):
        acc = [term(load(i)) for i in range(4)]
        for i in range(4, D // 8):
            acc[i % 4] = acc[i % 4] + term(load(i))
            if i % every == every - 1:
                yield
        tot = jnp.sum((acc[0] + acc[1]) + (acc[2] + acc[3]), axis=0, keepdims=True)
        return jnp.broadcast_to(tot * (1.0 / D), (8, T1))

    mu = yield from mean(lambda x: x, 32)
    var = yield from mean(lambda x: (x - mu) * (x - mu), 10)
    rs = jax.lax.rsqrt(var + 1e-5)
    return lambda i: jnp.concatenate([(load(2 * i + s) - mu) * rs for s in range(2)], axis=0)


def _items(n):
    return lambda fn: lambda *args: (fn(*args), n)


def _interleave(*lists, lead=0.0, span=1.0):
    gens = [(v for g, _ in w for v in g) for w in lists]
    sizes = [sum(n for _, n in w) for w in lists]
    for _, k in sorted((i / n if k else i / n * span - lead, k)
                       for k, n in enumerate(sizes) for i in range(n)):
        next(gens[k])
    for g in gens:
        for _ in g:
            pass


def _strassen_lhs(a11, a12, a21, a22):
    return a11 + a22, a22, a21 + a22, a11 + a12, a11, a12 - a22, a21 - a11


def _strassen_rhs(b11, b12, b21, b22):
    ops = (b11 + b22, b21 - b11, b11, b22, b12 - b22, b21 + b22, b11 + b12)
    return jnp.concatenate([_zip(v) for v in ops], axis=1)


def _strassen(prod, emit):
    m4 = prod(1)
    yield
    m2 = prod(2)
    emit(1, 0, m2 + m4)
    yield
    m1 = prod(0)
    c11, c22 = m1 + m4, m1 - m2
    yield
    c11 = c11 + prod(5)
    yield
    m5 = prod(3)
    emit(0, 0, c11 - m5)
    yield
    m3 = prod(4)
    emit(0, 1, m3 + m5)
    c22 = c22 + m3
    yield
    emit(1, 1, c22 + prod(6))
    yield


def _rows(i, n):
    return slice(i * n, i * n + n)


def _kernel(u_hbm, are_hbm, aim_hbm, bre_hbm, bim_hbm, cre_hbm, cim_hbm, ldt, dsk, wqkv_hbm, wo_hbm, f_hbm, out_hbm,
            are, aim, bre, bim, cre, cim, io, wq_in, wo_in, fm, ws, wp, lam, dtc, k0s, tab, ztab, kb, kf,
            xr, xn, kv, xq, qs, oe, oo, ob, zs, sems):
    cp_u = [pltpu.make_async_copy(u_hbm.bitcast(U32).at[:, h, :], io.at[h], sems.at[3 + h])
            for h in range(PH // 2)]
    cp_o = [pltpu.make_async_copy(io.at[h], out_hbm.bitcast(U32).at[:, h, :], sems.at[3 + h])
            for h in range(PH // 2)]
    cp_f, cp_g = [pltpu.make_async_copy(f_hbm.at[_rows(i, PH)], fm.at[_rows(i, PH)], sems.at[0])
                  for i in range(2)]
    cp_wq = pltpu.make_async_copy(wqkv_hbm, wq_in, sems.at[1])
    cp_wo = pltpu.make_async_copy(wo_hbm, wo_in, sems.at[2])
    cp_p = [pltpu.make_async_copy(src, dst, sems.at[3 + PH // 2 + i]) for i, (src, dst) in enumerate(
        ((aim_hbm, aim), (are_hbm, are), (bre_hbm, bre), (bim_hbm, bim), (cre_hbm, cre),
         (cim_hbm, cim)))]
    for cp in cp_p:
        cp.start()

    lane = jax.lax.broadcasted_iota(I32, (8, T1), 1)
    zs[0] = 0

    def xs(p):
        return xr.at[p]

    def region(*lists, **pace):
        pl.when(zs[0] == 0)(lambda: _interleave(*lists, **pace))

    dt_row = jnp.exp(ldt[...].astype(F32).reshape(1, D)).astype(BF16).astype(F32)
    ds_row = dsk[...].astype(F32).reshape(1, D)
    for j in range(4):
        dtc[0, _rows(j, 128), :] = jnp.broadcast_to(dt_row[:, _rows(j, 128)], (128, 128)).T
        dtc[1, _rows(j, 128), :] = jnp.broadcast_to(ds_row[:, _rows(j, 128)], (128, 128)).T
    cp_p[0].wait()
    cp_p[1].wait()
    for cp in cp_u[:2]:
        cp.start()
    big = None
    for j in range(D // 16):
        r = _rows(j, 16)
        theta = dtc[0, r, :] * aim[r, :].astype(F32)
        mag = jnp.exp(dtc[0, r, :] * are[r, :].astype(F32))
        sn, cs = _sincos(theta)
        lam[0, r, :] = mag * cs
        lam[1, r, :] = mag * sn
        big = jnp.abs(theta) if big is None else jnp.maximum(big, jnp.abs(theta))

    @pl.when(jnp.logical_not(jnp.max(big) <= 8192.0))
    def _():
        def body(i, _):
            rows = pl.ds(pl.multiple_of(i * 16, 16), 16)
            th = dtc[0, rows, :] * aim[rows, :].astype(F32)
            mg = jnp.exp(dtc[0, rows, :] * are[rows, :].astype(F32))
            lam[0, rows, :] = mg * jnp.cos(th)
            lam[1, rows, :] = mg * jnp.sin(th)
        jax.lax.fori_loop(0, D // 16, body, None)

    for cp in cp_p[2:]:
        cp.wait()

    @_items(15)
    def tap_tables(blk, e):
        rows = _rows(4 * blk + e, 8)

        def part(ref):
            return ref[_rows(2 * blk + e // 2, 16), :].astype(F32)[_rows(e % 2, 8)]

        sc = dtc[0, rows, :] * (2.0 / L)
        w = _cmul((part(cre), part(cim)), (part(bre) * sc, part(bim) * sc))
        k0s[rows, :] = w[0]

        def put(row, a, b):
            for z in range(2):
                tab[blk % 8, z, pl.ds(row, 8, stride=QS), :] = pltpu.pack_elementwise(
                    [a[z], b[z]], packed_dtype=BF16)

        l1 = (lam[0, rows, :], lam[1, rows, :])
        l2 = _csq(l1)
        l16 = _csq(_csq(_csq(l2)))
        m1 = (l16[0], -l16[1])
        m2 = _csq(m1)
        a, b = _cmul(w, l1), _cmul(w, l2)
        c, d = m2, _cmul(m1, m2)
        put(16 * e, (jnp.ones_like(m1[0]), jnp.zeros_like(m1[0])), m1)
        keep = {}
        for j in range(1, 16):
            if j <= 8:
                put(64 + 12 * e + j - 1, a, b)
                keep[2 * j] = b
            if j < 8:
                a, b = _cmul(a, l2), _cmul(b, l2)
            put(16 * e + j, c, d)
            if j == 8:
                l512 = _csq((c[0], -c[1]))
                put(64 + 12 * e + 8, _cmul(keep[4], l512), _cmul(keep[12], l512))
                a, b = keep[8], keep[16]
            if j in (10, 12, 14):
                a, b = _cmul(a, l512), _cmul(b, l512)
                put(64 + 12 * e + 4 + j // 2, a, b)
            if j < 15:
                c, d = _cmul(c, m2), _cmul(d, m2)
            yield

    @_items(24)
    def tap_sums(blk):
        for i in range(8):
            re, im = [jax.lax.dot_general(_bf(tab[blk % 8, z, pl.ds(QS * i + 64, 48), :]),
                                          _bf(tab[blk % 8, z, pl.ds(QS * i, 64), :]),
                                          NT, preferred_element_type=F32) for z in range(2)]
            acc = re + im
            for r in range(3):
                pc = [acc[_rows(3 * e + r, 8)] for e in range(4)]
                ztab[blk % 8, pl.ds(ZS * i + 8 * r, 8), :] = jnp.where(
                    lane < 64, jnp.where(lane < 32, pc[0], pc[1]),
                    jnp.where(lane < 96, pc[2], pc[3]))
                yield

    def tap_rows(blk, e):
        def at(r, g):
            z = ztab[blk % 8, pl.ds(r, 8, stride=ZS), :]
            return z if g == e else pltpu.roll(z, (32 * (g - e)) % 128, 1)

        def full(r, r1):
            return jnp.where(lane < 64, jnp.where(lane < 32, at(r, 0), at(r1, 1)),
                             jnp.where(lane < 96, at(r1 + 2, 2), at(r1 + 4, 3)))

        rows = _rows(4 * blk + e, 8)
        e8, e16 = full(7, 18), full(15, 19)
        k0 = jnp.sum(k0s[rows, :], axis=1, keepdims=True) + dtc[1, rows, :] * (2.0 / L)
        e0 = jnp.where(lane == 0, k0, pltpu.roll(e16, 1, 1))
        e4 = jnp.where(lane < 32, at(3, 0), at(16, 1))
        e12 = jnp.where(lane < 32, at(11, 0), at(17, 1))
        k4, k12 = jnp.where(lane < 64, e4, e0), jnp.where(lane < 64, e12, e16)
        far = {1: e0, 2: e0, 3: k4, 5: jnp.where(lane < 64, e4, e8), 6: e8, 7: e8, 9: e8,
               10: e8, 11: jnp.where(lane < 64, e12, e8), 13: k12, 14: e16, 15: e16}
        taps = {0: e0, 4: k4, 8: e8, 12: k12}
        return lambda p: taps[p] if p in taps else jnp.where(
            lane < (16 if p % 2 else 32), at(p - 1, 0), far[p])

    @_items(2)
    def tap_blocks(blk, e2):
        a, b = tap_rows(blk, 2 * e2), tap_rows(blk, 2 * e2 + 1)
        yield
        for p in range(PH):
            kb[p, _rows(2 * blk + e2, 16), :] = jnp.concatenate([a(p), b(p)], axis=0).astype(BF16)
        yield

    @_items(CB // 2)
    def lane_dft(src, lo, hi):
        for q in range(8):
            x0, x1 = [jax.lax.dot_general(src[p, lo:hi, :], _bf(fm[p]), NN,
                                          preferred_element_type=F32) for p in (q, q + 8)]
            for i in range((hi - lo) // 8):
                r = _rows(i, 8)
                for c, v in ((q, x0[r] + x1[r]), (q + 8, x0[r] - x1[r])):
                    for z in range(2):
                        kv[0, 2 * c + z, _rows(lo // 8 + i, 8), :] = v[:, _rows(z, T1)]
                if i % 2:
                    yield

    def residues(r, odd):
        return [(kv[0, 2 * c, r, :], kv[0, 2 * c + 1, r, :]) for c in range(8 * odd, 8 * odd + 8)]

    @_items(CB // 4)
    def tap_coefs(blk):
        for i in range(CB // 8):
            r = _rows(blk * CB // 8 + i, 8)
            for odd in range(2):
                for n, v in enumerate(_conv_coefs(residues(r, odd), 4 * odd)):
                    kf[10 * odd + n, r, :T1] = v[0]
                    kf[10 * odd + n, r, T1:] = v[1]
                yield

    r0 = jax.lax.broadcasted_iota(I32, (128, 128), 0)
    ri = (r0 & ~15) + (r0 & 7) * 2 + ((r0 >> 3) & 1)
    ci = jax.lax.broadcasted_iota(I32, (128, 128), 1)
    hit = ci == (ri & 7) * 16 + (ri >> 3)

    @_items(14)
    def prep_weights(j):
        def block(c, k):
            if j < 6:
                sel = jnp.where(hit, 1.0 if j < 4 else 0.25, 0.0)
                w = wq_in[_rows(k, 128), _rows(c, 128)]
            else:
                sel = jnp.where(ri == ci, 1.0, 0.0)
                w = _bf(wp[_rows(k, 64), _rows(c, 128)])
            return jax.lax.dot_general(sel.astype(BF16), w, NT, preferred_element_type=F32)

        top, bot = (4 + j, 8 + j) if j < 4 else (j % 2, j % 2 + 2)
        for k in range(2):
            for i, a in enumerate(_strassen_lhs(block(top, k), block(top, k + 2),
                                                block(bot, k), block(bot, k + 2))):
                ws[i, _rows(j, 64), _rows(k, 128)] = _zip(a)
                yield

    @_items(8)
    def permute_wo(j):
        sel = jnp.where(ci == (r0 & 7) * 16 + (r0 >> 3), 1.0, 0.0).astype(BF16)
        wp[_rows(j, 64), :] = _zip(jnp.dot(sel, wo_in[_rows(j, 128), :],
                                           preferred_element_type=F32))
        yield from range(8)

    @_items(4)
    def load_pair(h):
        for j in range(4):
            wds = io[h, :, _rows(j, 128)].T
            xs(2 * h)[_rows(j, 128), :] = pltpu.bitcast(wds << 16, F32)
            xs(2 * h + 1)[_rows(j, 128), :] = pltpu.bitcast(wds & jnp.uint32(0xFFFF0000), F32)
            yield

    @_items(24)
    def norm(h):
        for p in (2 * h, 2 * h + 1):
            normed = yield from _layernorm(lambda i: xs(p)[_rows(i, 8), :])
            for i in range(D // 16):
                xn[p, _rows(i, 16), :] = normed(i).astype(BF16)
                if i % 8 == 7:
                    yield

    for i, step in enumerate(PROLOGUE):
        tables, sums, blocks, dft, coefs, loads, norms, perms, preps = [
            range(a, b) for a, b in zip(PROLOGUE[i - 1] if i else (0,) * 9, step)]
        for cp in {0: cp_u[2:5], 1: [cp_f], 2: cp_u[5:], 3: [cp_wo, cp_wq], 5: [cp_g]}.get(i, ()):
            cp.start()
        for cp, users in ((cp_f, dft), (cp_wo, perms), (cp_wq, preps)):
            if 0 in users:
                cp.wait()
        for h in loads:
            cp_u[h].wait()
        region([tap_sums(2 * b + s) for b in sums for s in range(2)]
               + [lane_dft(kb, CB * b, CB * b + CB) for b in dft]
               + [permute_wo(j) for j in perms] + [prep_weights(j) for j in preps],
               [tap_tables(2 * b + s, e) for b in tables for s in range(2) for e in range(4)]
               + [norm(h) for h in norms],
               [tap_blocks(2 * b + s, e) for b in blocks for s in range(2) for e in range(2)],
               [tap_coefs(b) for b in coefs],
               [load_pair(h) for h in loads])

    cp_g.wait()

    @_items(10)
    def phase_conv(i):
        r = _rows(i, 8)
        coefs = ((kf[n, r, :T1], kf[n, r, T1:]) for n in range(NCOEF))
        for odd in range(2):
            y = yield from _conv(residues(r, odd), 4 * odd, lambda: next(coefs))
            for c, v in enumerate(y):
                for z in range(2):
                    kv[1, 16 * odd + 2 * c + z, r, :] = v[z]
            yield

    @_items(32)
    def lane_idft(lo, hi):
        for q in (0, 2, 4, 6, 1, 3, 5, 7):
            a, b = [jnp.concatenate([kv[1, 2 * c + z, lo:hi, :] for z in range(2)], axis=1)
                    for c in (q, q + 8)]
            for p, v in ((q, a + b), (q + 8, a - b)):
                inv = jnp.concatenate([fm[PH + p, :, :T1], fm[PH + p, :, T1:]], axis=0)
                d = jax.lax.dot_general(v, _bf(inv), NN, preferred_element_type=F32)
                yield
                xs(p)[lo:hi, :] += d
                yield

    @_items(32)
    def norm_pair(g):
        def unzipped(i):
            return pl.ds(16 * (i // 2) + i % 2, 8, stride=2)

        p = 4 * (g % 4) + g // 4
        a = yield from _layernorm(lambda i: xr[p, unzipped(i), :])
        b = yield from _layernorm(lambda i: xr[p + 2, unzipped(i), :])
        for r in range(HD // 16):
            xq[g, _rows(r, 8), :] = _strassen_rhs(a(r), b(r), a(HD // 16 + r), b(HD // 16 + r))
            yield

    def block_product(row0, groups, rhs, emit):
        for r in [128 // RS * hg + i for hg in groups for i in range(128 // RS)]:
            w = slice((row0 + r * RS) // 2, (row0 + r * RS + RS) // 2)
            yield from _strassen(
                lambda i: jnp.dot(_bf(ws[i, w, :]), _bf(rhs[:, _rows(i, T1)]),
                                  preferred_element_type=F32),
                lambda half, n, y: emit(half, n, r * RS, y))

    @_items(7 * HD // RS)
    def keys_values(s, g):
        def emit(half, n, row, y):
            m = 2 * (g % 4) + n
            kv[g // 4, PH * half + WIN - 1 + m, pl.ds(row, RS), :] = y
            if m:
                kv[g // 4, PH * half + m - 1, pl.ds(row, RS), :] = pltpu.roll(y, 1, 1)

        return block_product(0, (s, s + 2), xq.at[g], emit)

    @_items(7 * 128 // RS)
    def queries(s, g):
        def emit(half, n, row, y):
            qs[g, n, pl.ds(HD * half + row, RS), :] = y

        return block_product(D, (s,), xq.at[g], emit)

    @_items(34)
    def attend(par, s, m):
        for hg in (s, s + 2):
            lg = [None] * WIN
            for j0 in range(0, WIN, JB):
                for dh in range(16):
                    r = _rows(16 * hg + dh, 8)
                    q = qs[4 * par + m // 2, m % 2, r, :]
                    for j in range(j0, j0 + JB):
                        t = q * kv[par, WIN - 1 + m - j, r, :]
                        lg[j] = t if dh == 0 else lg[j] + t
                    if (dh + 1) % (16 // JB) == 0:
                        yield
            for j in range(m + 1, WIN):
                lg[j] = jnp.where(lane == 0, -1e9, lg[j])
            mx = lg[0]
            for j in range(1, WIN):
                mx = jnp.maximum(mx, lg[j])
            ex = [jnp.exp(t - mx) for t in lg]
            den = ex[0]
            for j in range(1, WIN):
                den = den + ex[j]
            inv = pltpu.reciprocal(den, full_range=False)
            pr = [t * inv for t in ex]
            yield

            def out(dh):
                r = _rows(16 * hg + dh, 8)
                acc = pr[0] * kv[par, PH + WIN - 1 + m, r, :]
                for j in range(1, WIN):
                    acc = acc + pr[j] * kv[par, PH + WIN - 1 + m - j, r, :]
                return acc

            for d2 in range(8):
                o = jnp.concatenate([out(2 * d2), out(2 * d2 + 1)], axis=0)
                r = _rows(8 * hg + d2, 16)
                if par == 0:
                    oe[m, r, :] = o
                elif hg < 2:
                    oo[m, r, :] = o
                else:
                    r1 = _rows(8 * (hg - 2) + d2, 16)
                    ob[m, _rows(8 * (hg - 2) + d2, 8), :] = _strassen_rhs(
                        oe[m, r1, :], oo[m, r1, :], oe[m, r, :], o)
                yield

    late = (1, 4)

    @_items(7 * HD // RS)
    def project(h):
        def emit(half, n, row, y):
            xs(2 * h + n)[pl.ds(HD * half + row, RS), :] += y

        for s in range(2):
            yield from block_product(D + HD, (s,), ob.at[h], emit)
            if h not in late:
                for _ in store_pair(h, (s, s + 2))[0]:
                    pass

    @_items(4)
    def store_pair(h, groups):
        for j in groups:
            io[h, :, _rows(j, 128)] = pltpu.pack_elementwise(
                [xs(2 * h + n)[_rows(j, 128), :] for n in range(2)], packed_dtype=BF16).T
            yield

    def layer(it, c):
        def send(hs):
            @pl.when(it == 1)
            def _():
                for h in hs:
                    cp_o[h].start()

        for i in range(len(CUTS[0]) - 1):
            (f0, f1), (c0, c1), (i0, i1) = [c[i:i + 2] for c in CUTS]
            last = i0 < i1 == D
            region([lane_dft(xn, c, min(c + CB, f1)) for c in range(f0, f1, CB)]
                   + [lane_idft(c, min(c + CB, i1)) for c in range(i0, i1, CB)],
                   [phase_conv(r) for r in range(c0 // 8, c1 // 8)]
                   + ([norm(7)] if i == 0 else []) + ([norm_pair(0)] if last else []),
                   lead=0.4 if last else 0.0, span=1.5 if i == 0 else 1.0)
        region([keys_values(0, 0), keys_values(1, 0), queries(0, 0)],
               [norm_pair(g) for g in (1, 2, 3)])
        region([fn(0, g) for fn in (keys_values, queries) for g in (1, 2, 3)],
               [norm_pair(g) for g in (4, 5, 6, 7)])
        for par, s, kvg, qg in ((0, 0, (1, 2, 3), (0, 1, 2, 3)), (0, 1, (4, 5, 6, 7), (4, 5, 6, 7)),
                                (1, 0, (4, 5, 6, 7), (4, 5))):
            region([keys_values(1 - s, g) for g in kvg] + [queries(1 - s, g) for g in qg],
                   [attend(par, s, m) for m in range(WIN)])
        region([queries(1, g) for g in (6, 7)], [attend(1, 1, m) for m in (0, 1)])
        done = ()
        for hs, ms in (((0, 1), (2, 3, 4)), ((2, 3, 4), (5, 6, 7)), ((5, 6), ()), ((7,), ())):
            region([project(h) for h in hs],
                   [store_pair(h, range(4)) for h in done if h in late]
                   + [norm(h) for h in done] + [attend(1, 1, m) for m in ms])
            send([h for h in done if h in late] + [h for h in hs if h not in late])
            done = hs

    jax.lax.fori_loop(0, 2, layer, None)
    for cp in cp_o:
        cp.wait()


@jax.jit
def pallas_interleave_layers__ssm_conv_s4__sliding_local_dilated__prompt_kernel(
    A_u: jax.Array,
    A_A_re: jax.Array,
    A_A_im: jax.Array,
    A_B_re: jax.Array,
    A_B_im: jax.Array,
    A_C_re: jax.Array,
    A_C_im: jax.Array,
    A_log_dt: jax.Array,
    A_Dskip: jax.Array,
    B_x: jax.Array,
    B_wqkv: jax.Array,
    B_wo: jax.Array,
):
    del B_x
    hbm = pl.BlockSpec(memory_space=pl.ANY)
    vmem = pl.BlockSpec(memory_space=pltpu.VMEM)
    out = pl.pallas_call(
        _kernel,
        in_specs=[hbm] * 7 + [vmem] * 2 + [hbm] * 3,
        out_specs=hbm,
        out_shape=jax.ShapeDtypeStruct((T1, PH, D), BF16),
        scratch_shapes=[pltpu.VMEM((D, NS), BF16)] * 6 + [
            pltpu.VMEM((PH // 2, T1, D), U32),
            pltpu.VMEM((D, 3 * D), BF16),
            pltpu.VMEM((D, D), BF16),
            pltpu.VMEM((2 * PH, T1 // 2, 2 * T1), U32),
            pltpu.VMEM((7, D, HD), U32),
            pltpu.VMEM((D // 2, D), U32),
            pltpu.VMEM((2, D, NS), F32),
            pltpu.VMEM((2, D, NS), F32),
            pltpu.VMEM((D, T1), F32),
            pltpu.VMEM((8, 2, 9 * QS + 4, NS), U32),
            pltpu.VMEM((8, 9 * ZS + 4, T1), F32),
            pltpu.VMEM((PH, D, T1), BF16),
            pltpu.VMEM((NCOEF, D, 2 * T1), F32),
            pltpu.VMEM((PH, D + 8, T1), F32),
            pltpu.VMEM((PH, D, T1), BF16),
            pltpu.VMEM((2, 2 * PH, D, T1), F32),
            pltpu.VMEM((PH // 2, HD // 2, 7 * T1), U32),
            pltpu.VMEM((PH // 2, 2, D, T1), F32),
            pltpu.VMEM((WIN, D, T1), F32),
            pltpu.VMEM((WIN, HD, T1), F32),
            pltpu.VMEM((WIN, HD // 2, 7 * T1), U32),
            pltpu.SMEM((1,), I32),
            pltpu.SemaphoreType.DMA((9 + PH // 2,)),
        ],
        compiler_params=pltpu.CompilerParams(vmem_limit_bytes=100 * 1024 * 1024),
    )(A_u.reshape(T1, PH, D), A_A_re, A_A_im, A_B_re, A_B_im, A_C_re, A_C_im,
      A_log_dt, A_Dskip, B_wqkv, B_wo,
      _dft_matrices())
    return out.reshape(1, L, D)
```

```python
import numpy as np

import jax
import jax.numpy as jnp
import jax.experimental.pallas as pl
import jax.experimental.pallas.tpu as pltpu

F32, BF16, U32, I32 = jnp.float32, jnp.bfloat16, jnp.uint32, jnp.int32
L, D, NS = 2048, 512, 128
PH, T1 = 16, 128
WIN = 8
NN = (((1,), (0,)), ((), ()))
NT = (((1,), (1,)), ((), ()))
QS = 116
ZS = 28
_H = float(np.sqrt(0.5))
NCOEF = 22
HD = D // 2
RS = 64
JB = 4
CUTS = ((0, 64, 192, 320, 448, D, D, D),
        (0, 0, 64, 192, 320, 448, D, D),
        (0, 0, 0, 64, 192, 320, 448, D))
PROLOGUE = ((1, 0, 0, 0, 0, 0, 0, 0, 0),
            (3, 1, 0, 0, 0, 2, 0, 0, 0),
            (5, 3, 1, 0, 0, 5, 0, 0, 0),
            (7, 5, 3, 1, 0, 8, 0, 0, 0),
            (8, 7, 5, 3, 1, 8, 0, 4, 0),
            (8, 8, 7, 5, 3, 8, 2, 4, 2),
            (8, 8, 8, 7, 5, 8, 5, 4, 4),
            (8, 8, 8, 8, 8, 8, 7, 4, 8))
CB = 64


def _dft_matrices():
    t = 16 * np.arange(T1)[None, :, None] + np.arange(PH)[:, None, None]
    k = np.arange(T1)[None, None, :] + 0.5
    phi = 2.0 * np.pi * k * t / (2 * L)
    phi = np.concatenate([phi, phi.transpose(0, 2, 1)])
    f = np.concatenate([np.cos(phi), -np.sin(phi)], axis=-1).astype(np.float32)
    bits = f.astype(BF16).view(np.uint16).astype(np.uint32)
    return bits[:, 0::2] | (bits[:, 1::2] << 16)


def _cmul(a, b):
    return a[0] * b[0] - a[1] * b[1], a[0] * b[1] + a[1] * b[0]


def _csq(a):
    t = a[0] * a[1]
    return a[0] * a[0] - a[1] * a[1], t + t


def _cadd(a, b):
    return a[0] + b[0], a[1] + b[1]


def _csub(a, b):
    return a[0] - b[0], a[1] - b[1]


def _rot8(x, e):
    s, d = x[0] + x[1], x[0] - x[1]
    return {1: (d * _H, s * _H), 3: (s * -_H, d * _H), 5: (d * -_H, s * -_H), 7: (s * _H, d * -_H)}[e]


def _split(x, e):
    n = len(x) // 2
    lo, hi = x[:n], x[n:]
    if e == 4:
        return ([(a[0] - b[1], a[1] + b[0]) for a, b in zip(lo, hi)],
                [(a[0] + b[1], a[1] - b[0]) for a, b in zip(lo, hi)])
    if e:
        hi = [_rot8(b, e // 2) for b in hi]
    return [_cadd(a, b) for a, b in zip(lo, hi)], [_csub(a, b) for a, b in zip(lo, hi)]


def _merge(p, m, e):
    lo = [_cadd(a, b) for a, b in zip(p, m)]
    if e == 4:
        return lo + [(a[1] - b[1], b[0] - a[0]) for a, b in zip(p, m)]
    hi = [_csub(a, b) for a, b in zip(p, m)]
    return lo + ([_rot8(b, 8 - e // 2) for b in hi] if e else hi)


def _conv_coefs(k, e):
    if len(k) == 1:
        return [(k[0][0] * 0.5, k[0][1] * 0.5)]
    if len(k) == 2 and e % 4:
        if e % 2:
            top = _csub(_rot8(k[1], e), k[0])
        elif e == 2:
            top = (-k[1][1] - k[0][0], k[1][0] - k[0][1])
        else:
            top = (k[1][1] - k[0][0], -k[1][0] - k[0][1])
        return [k[0], top, _csub(k[1], k[0])]
    p, m = _split(k, e)
    return _conv_coefs(p, e // 2) + _conv_coefs(m, e // 2 + 4)


def _conv(x, e, coef):
    if len(x) == 1:
        return [_cmul(x[0], coef())]
    if len(x) == 2:
        yield
    if len(x) == 2 and e % 4:
        both = _cmul(_cadd(x[0], x[1]), coef())
        return [_cadd(both, _cmul(x[1], coef())), _cadd(both, _cmul(x[0], coef()))]
    p, m = _split(x, e)
    p = yield from _conv(p, e // 2, coef)
    m = yield from _conv(m, e // 2 + 4, coef)
    return _merge(p, m, e)


def _sincos(x):
    n = jnp.floor(x * float(2.0 / np.pi) + 0.5)
    r = ((x - n * 1.5703125) - n * 4.837512969970703125e-4) - n * 7.54978995489188216e-8
    z = r * r
    s = r + r * z * ((-1.9515295891e-4 * z + 8.3321608736e-3) * z - 1.6666654611e-1)
    c = 1.0 + z * (((2.443315711809948e-5 * z - 1.388731625493765e-3) * z
                    + 4.166664568298827e-2) * z - 0.5)
    q = n.astype(I32)
    odd = (q & 1) == 1
    s, c = jnp.where(odd, c, s), jnp.where(odd, s, c)
    return jnp.where((q & 2) == 2, -s, s), jnp.where(((q + 1) & 2) == 2, -c, c)


def _pk(x):
    return pltpu.bitcast(x.astype(BF16), U32)


def _zip(x):
    return jnp.concatenate(
        [pltpu.pack_elementwise([x[i:i + 8], x[i + 8:i + 16]], packed_dtype=BF16)
         for i in range(0, x.shape[0], 16)], axis=0)


def _bf(words):
    return pltpu.bitcast(words, BF16)


def _layernorm(load):
    def mean(term, every):
        acc = [term(load(i)) for i in range(4)]
        for i in range(4, D // 8):
            acc[i % 4] = acc[i % 4] + term(load(i))
            if i % every == every - 1:
                yield
        tot = jnp.sum((acc[0] + acc[1]) + (acc[2] + acc[3]), axis=0, keepdims=True)
        return jnp.broadcast_to(tot * (1.0 / D), (8, T1))

    mu = yield from mean(lambda x: x, 32)
    var = yield from mean(lambda x: (x - mu) * (x - mu), 10)
    rs = jax.lax.rsqrt(var + 1e-5)
    return lambda i: jnp.concatenate([(load(2 * i + s) - mu) * rs for s in range(2)], axis=0)


def _items(n):
    return lambda fn: lambda *args: (fn(*args), n)


def _interleave(*lists, lead=0.0, span=1.0):
    gens = [(v for g, _ in w for v in g) for w in lists]
    sizes = [sum(n for _, n in w) for w in lists]
    for _, k in sorted((i / n if k else i / n * span - lead, k)
                       for k, n in enumerate(sizes) for i in range(n)):
        next(gens[k])
    for g in gens:
        for _ in g:
            pass


def _strassen_lhs(a11, a12, a21, a22):
    return a11 + a22, a22, a21 + a22, a11 + a12, a11, a12 - a22, a21 - a11


def _strassen_rhs(b11, b12, b21, b22):
    ops = (b11 + b22, b21 - b11, b11, b22, b12 - b22, b21 + b22, b11 + b12)
    return jnp.concatenate([_zip(v) for v in ops], axis=1)


def _strassen(prod, emit):
    m4 = prod(1)
    yield
    m2 = prod(2)
    emit(1, 0, m2 + m4)
    yield
    m1 = prod(0)
    c11, c22 = m1 + m4, m1 - m2
    yield
    c11 = c11 + prod(5)
    yield
    m5 = prod(3)
    emit(0, 0, c11 - m5)
    yield
    m3 = prod(4)
    emit(0, 1, m3 + m5)
    c22 = c22 + m3
    yield
    emit(1, 1, c22 + prod(6))
    yield


def _rows(i, n):
    return slice(i * n, i * n + n)


def _kernel(u_hbm, are_hbm, aim_hbm, bre_hbm, bim_hbm, cre_hbm, cim_hbm, ldt_hbm, dsk_hbm, wqkv_hbm, wo_hbm, f_hbm, out_hbm,
            are, aim, bre, bim, cre, cim, ldt, dsk, io, wq_in, wo_in, fm, ws, wp, lam, dtc, k0s, tab, ztab, kb, kf,
            xr, xn, kv, xq, qs, oe, oo, ob, zs, sems):
    cp_u = [pltpu.make_async_copy(u_hbm.bitcast(U32).at[:, h, :], io.at[h], sems.at[3 + h])
            for h in range(PH // 2)]
    cp_o = [pltpu.make_async_copy(io.at[h], out_hbm.bitcast(U32).at[:, h, :], sems.at[3 + h])
            for h in range(PH // 2)]
    cp_f, cp_g = [pltpu.make_async_copy(f_hbm.at[_rows(i, PH)], fm.at[_rows(i, PH)], sems.at[0])
                  for i in range(2)]
    cp_wq = pltpu.make_async_copy(wqkv_hbm, wq_in, sems.at[1])
    cp_wo = pltpu.make_async_copy(wo_hbm, wo_in, sems.at[2])
    cp_p = [pltpu.make_async_copy(src, dst, sems.at[3 + PH // 2 + i]) for i, (src, dst) in enumerate(
        ((ldt_hbm, ldt), (dsk_hbm, dsk), (aim_hbm, aim), (are_hbm, are), (bre_hbm, bre), (bim_hbm, bim), (cre_hbm, cre),
         (cim_hbm, cim)))]
    for cp in cp_p:
        cp.start()

    lane = jax.lax.broadcasted_iota(I32, (8, T1), 1)
    zs[0] = 0

    def xs(p):
        return xr.at[p]

    def region(*lists, **pace):
        pl.when(zs[0] == 0)(lambda: _interleave(*lists, **pace))

    cp_p[0].wait()
    cp_p[1].wait()
    dt_row = jnp.exp(ldt[...].astype(F32).reshape(1, D)).astype(BF16).astype(F32)
    ds_row = dsk[...].astype(F32).reshape(1, D)
    for j in range(4):
        dtc[0, _rows(j, 128), :] = jnp.broadcast_to(dt_row[:, _rows(j, 128)], (128, 128)).T
        dtc[1, _rows(j, 128), :] = jnp.broadcast_to(ds_row[:, _rows(j, 128)], (128, 128)).T
    cp_p[2].wait()
    cp_p[3].wait()
    for cp in cp_u[:2]:
        cp.start()
    big = None
    for j in range(D // 16):
        r = _rows(j, 16)
        theta = dtc[0, r, :] * aim[r, :].astype(F32)
        mag = jnp.exp(dtc[0, r, :] * are[r, :].astype(F32))
        sn, cs = _sincos(theta)
        lam[0, r, :] = mag * cs
        lam[1, r, :] = mag * sn
        big = jnp.abs(theta) if big is None else jnp.maximum(big, jnp.abs(theta))

    @pl.when(jnp.logical_not(jnp.max(big) <= 8192.0))
    def _():
        def body(i, _):
            rows = pl.ds(pl.multiple_of(i * 16, 16), 16)
            th = dtc[0, rows, :] * aim[rows, :].astype(F32)
            mg = jnp.exp(dtc[0, rows, :] * are[rows, :].astype(F32))
            lam[0, rows, :] = mg * jnp.cos(th)
            lam[1, rows, :] = mg * jnp.sin(th)
        jax.lax.fori_loop(0, D // 16, body, None)

    for cp in cp_p[4:]:
        cp.wait()

    @_items(15)
    def tap_tables(blk, e):
        rows = _rows(4 * blk + e, 8)

        def part(ref):
            return ref[_rows(2 * blk + e // 2, 16), :].astype(F32)[_rows(e % 2, 8)]

        sc = dtc[0, rows, :] * (2.0 / L)
        w = _cmul((part(cre), part(cim)), (part(bre) * sc, part(bim) * sc))
        k0s[rows, :] = w[0]

        def put(row, a, b):
            for z in range(2):
                tab[blk % 8, z, pl.ds(row, 8, stride=QS), :] = pltpu.pack_elementwise(
                    [a[z], b[z]], packed_dtype=BF16)

        l1 = (lam[0, rows, :], lam[1, rows, :])
        l2 = _csq(l1)
        l16 = _csq(_csq(_csq(l2)))
        m1 = (l16[0], -l16[1])
        m2 = _csq(m1)
        a, b = _cmul(w, l1), _cmul(w, l2)
        c, d = m2, _cmul(m1, m2)
        put(16 * e, (jnp.ones_like(m1[0]), jnp.zeros_like(m1[0])), m1)
        keep = {}
        for j in range(1, 16):
            if j <= 8:
                put(64 + 12 * e + j - 1, a, b)
                keep[2 * j] = b
            if j < 8:
                a, b = _cmul(a, l2), _cmul(b, l2)
            put(16 * e + j, c, d)
            if j == 8:
                l512 = _csq((c[0], -c[1]))
                put(64 + 12 * e + 8, _cmul(keep[4], l512), _cmul(keep[12], l512))
                a, b = keep[8], keep[16]
            if j in (10, 12, 14):
                a, b = _cmul(a, l512), _cmul(b, l512)
                put(64 + 12 * e + 4 + j // 2, a, b)
            if j < 15:
                c, d = _cmul(c, m2), _cmul(d, m2)
            yield

    @_items(24)
    def tap_sums(blk):
        for i in range(8):
            re, im = [jax.lax.dot_general(_bf(tab[blk % 8, z, pl.ds(QS * i + 64, 48), :]),
                                          _bf(tab[blk % 8, z, pl.ds(QS * i, 64), :]),
                                          NT, preferred_element_type=F32) for z in range(2)]
            acc = re + im
            for r in range(3):
                pc = [acc[_rows(3 * e + r, 8)] for e in range(4)]
                ztab[blk % 8, pl.ds(ZS * i + 8 * r, 8), :] = jnp.where(
                    lane < 64, jnp.where(lane < 32, pc[0], pc[1]),
                    jnp.where(lane < 96, pc[2], pc[3]))
                yield

    def tap_rows(blk, e):
        def at(r, g):
            z = ztab[blk % 8, pl.ds(r, 8, stride=ZS), :]
            return z if g == e else pltpu.roll(z, (32 * (g - e)) % 128, 1)

        def full(r, r1):
            return jnp.where(lane < 64, jnp.where(lane < 32, at(r, 0), at(r1, 1)),
                             jnp.where(lane < 96, at(r1 + 2, 2), at(r1 + 4, 3)))

        rows = _rows(4 * blk + e, 8)
        e8, e16 = full(7, 18), full(15, 19)
        k0 = jnp.sum(k0s[rows, :], axis=1, keepdims=True) + dtc[1, rows, :] * (2.0 / L)
        e0 = jnp.where(lane == 0, k0, pltpu.roll(e16, 1, 1))
        e4 = jnp.where(lane < 32, at(3, 0), at(16, 1))
        e12 = jnp.where(lane < 32, at(11, 0), at(17, 1))
        k4, k12 = jnp.where(lane < 64, e4, e0), jnp.where(lane < 64, e12, e16)
        far = {1: e0, 2: e0, 3: k4, 5: jnp.where(lane < 64, e4, e8), 6: e8, 7: e8, 9: e8,
               10: e8, 11: jnp.where(lane < 64, e12, e8), 13: k12, 14: e16, 15: e16}
        taps = {0: e0, 4: k4, 8: e8, 12: k12}
        return lambda p: taps[p] if p in taps else jnp.where(
            lane < (16 if p % 2 else 32), at(p - 1, 0), far[p])

    @_items(2)
    def tap_blocks(blk, e2):
        a, b = tap_rows(blk, 2 * e2), tap_rows(blk, 2 * e2 + 1)
        yield
        for p in range(PH):
            kb[p, _rows(2 * blk + e2, 16), :] = jnp.concatenate([a(p), b(p)], axis=0).astype(BF16)
        yield

    @_items(CB // 2)
    def lane_dft(src, lo, hi):
        for q in range(8):
            x0, x1 = [jax.lax.dot_general(src[p, lo:hi, :], _bf(fm[p]), NN,
                                          preferred_element_type=F32) for p in (q, q + 8)]
            for i in range((hi - lo) // 8):
                r = _rows(i, 8)
                for c, v in ((q, x0[r] + x1[r]), (q + 8, x0[r] - x1[r])):
                    for z in range(2):
                        kv[0, 2 * c + z, _rows(lo // 8 + i, 8), :] = v[:, _rows(z, T1)]
                if i % 2:
                    yield

    def residues(r, odd):
        return [(kv[0, 2 * c, r, :], kv[0, 2 * c + 1, r, :]) for c in range(8 * odd, 8 * odd + 8)]

    @_items(CB // 4)
    def tap_coefs(blk):
        for i in range(CB // 8):
            r = _rows(blk * CB // 8 + i, 8)
            for odd in range(2):
                for n, v in enumerate(_conv_coefs(residues(r, odd), 4 * odd)):
                    kf[10 * odd + n, r, :T1] = v[0]
                    kf[10 * odd + n, r, T1:] = v[1]
                yield

    r0 = jax.lax.broadcasted_iota(I32, (128, 128), 0)
    ri = (r0 & ~15) + (r0 & 7) * 2 + ((r0 >> 3) & 1)
    ci = jax.lax.broadcasted_iota(I32, (128, 128), 1)
    hit = ci == (ri & 7) * 16 + (ri >> 3)

    @_items(14)
    def prep_weights(j):
        def block(c, k):
            if j < 6:
                sel = jnp.where(hit, 1.0 if j < 4 else 0.25, 0.0)
                w = wq_in[_rows(k, 128), _rows(c, 128)]
            else:
                sel = jnp.where(ri == ci, 1.0, 0.0)
                w = _bf(wp[_rows(k, 64), _rows(c, 128)])
            return jax.lax.dot_general(sel.astype(BF16), w, NT, preferred_element_type=F32)

        top, bot = (4 + j, 8 + j) if j < 4 else (j % 2, j % 2 + 2)
        for k in range(2):
            for i, a in enumerate(_strassen_lhs(block(top, k), block(top, k + 2),
                                                block(bot, k), block(bot, k + 2))):
                ws[i, _rows(j, 64), _rows(k, 128)] = _zip(a)
                yield

    @_items(8)
    def permute_wo(j):
        sel = jnp.where(ci == (r0 & 7) * 16 + (r0 >> 3), 1.0, 0.0).astype(BF16)
        wp[_rows(j, 64), :] = _zip(jnp.dot(sel, wo_in[_rows(j, 128), :],
                                           preferred_element_type=F32))
        yield from range(8)

    @_items(4)
    def load_pair(h):
        for j in range(4):
            wds = io[h, :, _rows(j, 128)].T
            xs(2 * h)[_rows(j, 128), :] = pltpu.bitcast(wds << 16, F32)
            xs(2 * h + 1)[_rows(j, 128), :] = pltpu.bitcast(wds & jnp.uint32(0xFFFF0000), F32)
            yield

    @_items(24)
    def norm(h):
        for p in (2 * h, 2 * h + 1):
            normed = yield from _layernorm(lambda i: xs(p)[_rows(i, 8), :])
            for i in range(D // 16):
                xn[p, _rows(i, 16), :] = normed(i).astype(BF16)
                if i % 8 == 7:
                    yield

    for i, step in enumerate(PROLOGUE):
        tables, sums, blocks, dft, coefs, loads, norms, perms, preps = [
            range(a, b) for a, b in zip(PROLOGUE[i - 1] if i else (0,) * 9, step)]
        for cp in {0: cp_u[2:5], 1: [cp_f], 2: cp_u[5:], 3: [cp_wo, cp_wq], 5: [cp_g]}.get(i, ()):
            cp.start()
        for cp, users in ((cp_f, dft), (cp_wo, perms), (cp_wq, preps)):
            if 0 in users:
                cp.wait()
        for h in loads:
            cp_u[h].wait()
        region([tap_sums(2 * b + s) for b in sums for s in range(2)]
               + [lane_dft(kb, CB * b, CB * b + CB) for b in dft]
               + [permute_wo(j) for j in perms] + [prep_weights(j) for j in preps],
               [tap_tables(2 * b + s, e) for b in tables for s in range(2) for e in range(4)]
               + [norm(h) for h in norms],
               [tap_blocks(2 * b + s, e) for b in blocks for s in range(2) for e in range(2)],
               [tap_coefs(b) for b in coefs],
               [load_pair(h) for h in loads])

    cp_g.wait()

    @_items(10)
    def phase_conv(i):
        r = _rows(i, 8)
        coefs = ((kf[n, r, :T1], kf[n, r, T1:]) for n in range(NCOEF))
        for odd in range(2):
            y = yield from _conv(residues(r, odd), 4 * odd, lambda: next(coefs))
            for c, v in enumerate(y):
                for z in range(2):
                    kv[1, 16 * odd + 2 * c + z, r, :] = v[z]
            yield

    @_items(32)
    def lane_idft(lo, hi):
        for q in (0, 2, 4, 6, 1, 3, 5, 7):
            a, b = [jnp.concatenate([kv[1, 2 * c + z, lo:hi, :] for z in range(2)], axis=1)
                    for c in (q, q + 8)]
            for p, v in ((q, a + b), (q + 8, a - b)):
                inv = jnp.concatenate([fm[PH + p, :, :T1], fm[PH + p, :, T1:]], axis=0)
                d = jax.lax.dot_general(v, _bf(inv), NN, preferred_element_type=F32)
                yield
                xs(p)[lo:hi, :] += d
                yield

    @_items(32)
    def norm_pair(g):
        def unzipped(i):
            return pl.ds(16 * (i // 2) + i % 2, 8, stride=2)

        p = 4 * (g % 4) + g // 4
        a = yield from _layernorm(lambda i: xr[p, unzipped(i), :])
        b = yield from _layernorm(lambda i: xr[p + 2, unzipped(i), :])
        for r in range(HD // 16):
            xq[g, _rows(r, 8), :] = _strassen_rhs(a(r), b(r), a(HD // 16 + r), b(HD // 16 + r))
            yield

    def block_product(row0, groups, rhs, emit):
        for r in [128 // RS * hg + i for hg in groups for i in range(128 // RS)]:
            w = slice((row0 + r * RS) // 2, (row0 + r * RS + RS) // 2)
            yield from _strassen(
                lambda i: jnp.dot(_bf(ws[i, w, :]), _bf(rhs[:, _rows(i, T1)]),
                                  preferred_element_type=F32),
                lambda half, n, y: emit(half, n, r * RS, y))

    @_items(7 * HD // RS)
    def keys_values(s, g):
        def emit(half, n, row, y):
            m = 2 * (g % 4) + n
            kv[g // 4, PH * half + WIN - 1 + m, pl.ds(row, RS), :] = y
            if m:
                kv[g // 4, PH * half + m - 1, pl.ds(row, RS), :] = pltpu.roll(y, 1, 1)

        return block_product(0, (s, s + 2), xq.at[g], emit)

    @_items(7 * 128 // RS)
    def queries(s, g):
        def emit(half, n, row, y):
            qs[g, n, pl.ds(HD * half + row, RS), :] = y

        return block_product(D, (s,), xq.at[g], emit)

    @_items(34)
    def attend(par, s, m):
        for hg in (s, s + 2):
            lg = [None] * WIN
            for j0 in range(0, WIN, JB):
                for dh in range(16):
                    r = _rows(16 * hg + dh, 8)
                    q = qs[4 * par + m // 2, m % 2, r, :]
                    for j in range(j0, j0 + JB):
                        t = q * kv[par, WIN - 1 + m - j, r, :]
                        lg[j] = t if dh == 0 else lg[j] + t
                    if (dh + 1) % (16 // JB) == 0:
                        yield
            for j in range(m + 1, WIN):
                lg[j] = jnp.where(lane == 0, -1e9, lg[j])
            mx = lg[0]
            for j in range(1, WIN):
                mx = jnp.maximum(mx, lg[j])
            ex = [jnp.exp(t - mx) for t in lg]
            den = ex[0]
            for j in range(1, WIN):
                den = den + ex[j]
            inv = pltpu.reciprocal(den, full_range=False)
            pr = [t * inv for t in ex]
            yield

            def out(dh):
                r = _rows(16 * hg + dh, 8)
                acc = pr[0] * kv[par, PH + WIN - 1 + m, r, :]
                for j in range(1, WIN):
                    acc = acc + pr[j] * kv[par, PH + WIN - 1 + m - j, r, :]
                return acc

            for d2 in range(8):
                o = jnp.concatenate([out(2 * d2), out(2 * d2 + 1)], axis=0)
                r = _rows(8 * hg + d2, 16)
                if par == 0:
                    oe[m, r, :] = o
                elif hg < 2:
                    oo[m, r, :] = o
                else:
                    r1 = _rows(8 * (hg - 2) + d2, 16)
                    ob[m, _rows(8 * (hg - 2) + d2, 8), :] = _strassen_rhs(
                        oe[m, r1, :], oo[m, r1, :], oe[m, r, :], o)
                yield

    late = (1, 4)

    @_items(7 * HD // RS)
    def project(h):
        def emit(half, n, row, y):
            xs(2 * h + n)[pl.ds(HD * half + row, RS), :] += y

        for s in range(2):
            yield from block_product(D + HD, (s,), ob.at[h], emit)
            if h not in late:
                for _ in store_pair(h, (s, s + 2))[0]:
                    pass

    @_items(4)
    def store_pair(h, groups):
        for j in groups:
            io[h, :, _rows(j, 128)] = pltpu.pack_elementwise(
                [xs(2 * h + n)[_rows(j, 128), :] for n in range(2)], packed_dtype=BF16).T
            yield

    def layer(it, c):
        def send(hs):
            @pl.when(it == 1)
            def _():
                for h in hs:
                    cp_o[h].start()

        for i in range(len(CUTS[0]) - 1):
            (f0, f1), (c0, c1), (i0, i1) = [c[i:i + 2] for c in CUTS]
            last = i0 < i1 == D
            region([lane_dft(xn, c, min(c + CB, f1)) for c in range(f0, f1, CB)]
                   + [lane_idft(c, min(c + CB, i1)) for c in range(i0, i1, CB)],
                   [phase_conv(r) for r in range(c0 // 8, c1 // 8)]
                   + ([norm(7)] if i == 0 else []) + ([norm_pair(0)] if last else []),
                   lead=0.4 if last else 0.0, span=1.5 if i == 0 else 1.0)
        region([keys_values(0, 0), keys_values(1, 0), queries(0, 0)],
               [norm_pair(g) for g in (1, 2, 3)])
        region([fn(0, g) for fn in (keys_values, queries) for g in (1, 2, 3)],
               [norm_pair(g) for g in (4, 5, 6, 7)])
        for par, s, kvg, qg in ((0, 0, (1, 2, 3), (0, 1, 2, 3)), (0, 1, (4, 5, 6, 7), (4, 5, 6, 7)),
                                (1, 0, (4, 5, 6, 7), (4, 5))):
            region([keys_values(1 - s, g) for g in kvg] + [queries(1 - s, g) for g in qg],
                   [attend(par, s, m) for m in range(WIN)])
        region([queries(1, g) for g in (6, 7)], [attend(1, 1, m) for m in (0, 1)])
        done = ()
        for hs, ms in (((0, 1), (2, 3, 4)), ((2, 3, 4), (5, 6, 7)), ((5, 6), ()), ((7,), ())):
            region([project(h) for h in hs],
                   [store_pair(h, range(4)) for h in done if h in late]
                   + [norm(h) for h in done] + [attend(1, 1, m) for m in ms])
            send([h for h in done if h in late] + [h for h in hs if h not in late])
            done = hs

    jax.lax.fori_loop(0, 2, layer, None)
    for cp in cp_o:
        cp.wait()


@jax.jit
def pallas_interleave_layers__ssm_conv_s4__sliding_local_dilated__prompt_kernel(
    A_u: jax.Array,
    A_A_re: jax.Array,
    A_A_im: jax.Array,
    A_B_re: jax.Array,
    A_B_im: jax.Array,
    A_C_re: jax.Array,
    A_C_im: jax.Array,
    A_log_dt: jax.Array,
    A_Dskip: jax.Array,
    B_x: jax.Array,
    B_wqkv: jax.Array,
    B_wo: jax.Array,
):
    del B_x
    hbm = pl.BlockSpec(memory_space=pl.ANY)
    out = pl.pallas_call(
        _kernel,
        in_specs=[hbm] * 12,
        out_specs=hbm,
        out_shape=jax.ShapeDtypeStruct((T1, PH, D), BF16),
        scratch_shapes=[pltpu.VMEM((D, NS), BF16)] * 6 + [pltpu.VMEM((D,), BF16)] * 2 + [
            pltpu.VMEM((PH // 2, T1, D), U32),
            pltpu.VMEM((D, 3 * D), BF16),
            pltpu.VMEM((D, D), BF16),
            pltpu.VMEM((2 * PH, T1 // 2, 2 * T1), U32),
            pltpu.VMEM((7, D, HD), U32),
            pltpu.VMEM((D // 2, D), U32),
            pltpu.VMEM((2, D, NS), F32),
            pltpu.VMEM((2, D, NS), F32),
            pltpu.VMEM((D, T1), F32),
            pltpu.VMEM((8, 2, 9 * QS + 4, NS), U32),
            pltpu.VMEM((8, 9 * ZS + 4, T1), F32),
            pltpu.VMEM((PH, D, T1), BF16),
            pltpu.VMEM((NCOEF, D, 2 * T1), F32),
            pltpu.VMEM((PH, D + 8, T1), F32),
            pltpu.VMEM((PH, D, T1), BF16),
            pltpu.VMEM((2, 2 * PH, D, T1), F32),
            pltpu.VMEM((PH // 2, HD // 2, 7 * T1), U32),
            pltpu.VMEM((PH // 2, 2, D, T1), F32),
            pltpu.VMEM((WIN, D, T1), F32),
            pltpu.VMEM((WIN, HD, T1), F32),
            pltpu.VMEM((WIN, HD // 2, 7 * T1), U32),
            pltpu.SMEM((1,), I32),
            pltpu.SemaphoreType.DMA((11 + PH // 2,)),
        ],
        compiler_params=pltpu.CompilerParams(vmem_limit_bytes=100 * 1024 * 1024),
    )(A_u.reshape(T1, PH, D), A_A_re, A_A_im, A_B_re, A_B_im, A_C_re, A_C_im,
      A_log_dt, A_Dskip, B_wqkv, B_wo,
      _dft_matrices())
    return out.reshape(1, L, D)
```

```python
import numpy as np

import jax
import jax.numpy as jnp
import jax.experimental.pallas as pl
import jax.experimental.pallas.tpu as pltpu

F32, BF16, U32, I32 = jnp.float32, jnp.bfloat16, jnp.uint32, jnp.int32
L, D, NS = 2048, 512, 128
PH, T1 = 16, 128
WIN = 8
NN = (((1,), (0,)), ((), ()))
NT = (((1,), (1,)), ((), ()))
QS = 116
ZS = 28
_H = float(np.sqrt(0.5))
NCOEF = 22
HD = D // 2
RS = 64
JB = 4
EDGES = (0, 64, 192, 320, 448, D)
PROLOGUE = ((1, 0, 0, 0, 0, 0, 0, 0, 0),
            (3, 1, 0, 0, 0, 2, 0, 0, 0),
            (5, 3, 1, 0, 0, 5, 0, 0, 0),
            (7, 5, 3, 1, 0, 8, 0, 0, 0),
            (8, 7, 5, 3, 1, 8, 0, 4, 0),
            (8, 8, 7, 5, 3, 8, 2, 4, 2),
            (8, 8, 8, 7, 5, 8, 5, 4, 4),
            (8, 8, 8, 8, 8, 8, 7, 4, 8))
CB = 64


def _dft_matrices():
    t = 16 * np.arange(T1)[None, :, None] + np.arange(PH)[:, None, None]
    k = np.arange(T1)[None, None, :] + 0.5
    phi = 2.0 * np.pi * k * t / (2 * L)
    phi = np.concatenate([phi, phi.transpose(0, 2, 1)])
    f = np.concatenate([np.cos(phi), -np.sin(phi)], axis=-1).astype(np.float32)
    bits = f.astype(BF16).view(np.uint16).astype(np.uint32)
    return bits[:, 0::2] | (bits[:, 1::2] << 16)


def _cmul(a, b):
    return a[0] * b[0] - a[1] * b[1], a[0] * b[1] + a[1] * b[0]


def _csq(a):
    t = a[0] * a[1]
    return a[0] * a[0] - a[1] * a[1], t + t


def _cadd(a, b):
    return a[0] + b[0], a[1] + b[1]


def _csub(a, b):
    return a[0] - b[0], a[1] - b[1]


def _rot8(x, e):
    s, d = x[0] + x[1], x[0] - x[1]
    return {1: (d * _H, s * _H), 3: (s * -_H, d * _H), 5: (d * -_H, s * -_H), 7: (s * _H, d * -_H)}[e]


def _split(x, e):
    n = len(x) // 2
    lo, hi = x[:n], x[n:]
    if e == 4:
        return ([(a[0] - b[1], a[1] + b[0]) for a, b in zip(lo, hi)],
                [(a[0] + b[1], a[1] - b[0]) for a, b in zip(lo, hi)])
    if e:
        hi = [_rot8(b, e // 2) for b in hi]
    return [_cadd(a, b) for a, b in zip(lo, hi)], [_csub(a, b) for a, b in zip(lo, hi)]


def _merge(p, m, e):
    lo = [_cadd(a, b) for a, b in zip(p, m)]
    if e == 4:
        return lo + [(a[1] - b[1], b[0] - a[0]) for a, b in zip(p, m)]
    hi = [_csub(a, b) for a, b in zip(p, m)]
    return lo + ([_rot8(b, 8 - e // 2) for b in hi] if e else hi)


def _conv_coefs(k, e):
    if len(k) == 1:
        return [(k[0][0] * 0.5, k[0][1] * 0.5)]
    if len(k) == 2 and e % 4:
        if e % 2:
            top = _csub(_rot8(k[1], e), k[0])
        elif e == 2:
            top = (-k[1][1] - k[0][0], k[1][0] - k[0][1])
        else:
            top = (k[1][1] - k[0][0], -k[1][0] - k[0][1])
        return [k[0], top, _csub(k[1], k[0])]
    p, m = _split(k, e)
    return _conv_coefs(p, e // 2) + _conv_coefs(m, e // 2 + 4)


def _conv(x, e, coef):
    if len(x) == 1:
        return [_cmul(x[0], coef())]
    if len(x) == 2:
        yield
    if len(x) == 2 and e % 4:
        both = _cmul(_cadd(x[0], x[1]), coef())
        return [_cadd(both, _cmul(x[1], coef())), _cadd(both, _cmul(x[0], coef()))]
    p, m = _split(x, e)
    p = yield from _conv(p, e // 2, coef)
    m = yield from _conv(m, e // 2 + 4, coef)
    return _merge(p, m, e)


def _sincos(x):
    n = jnp.floor(x * float(2.0 / np.pi) + 0.5)
    r = ((x - n * 1.5703125) - n * 4.837512969970703125e-4) - n * 7.54978995489188216e-8
    z = r * r
    s = r + r * z * ((-1.9515295891e-4 * z + 8.3321608736e-3) * z - 1.6666654611e-1)
    c = 1.0 + z * (((2.443315711809948e-5 * z - 1.388731625493765e-3) * z
                    + 4.166664568298827e-2) * z - 0.5)
    q = n.astype(I32)
    odd = (q & 1) == 1
    s, c = jnp.where(odd, c, s), jnp.where(odd, s, c)
    return jnp.where((q & 2) == 2, -s, s), jnp.where(((q + 1) & 2) == 2, -c, c)


def _pk(x):
    return pltpu.bitcast(x.astype(BF16), U32)


def _zip(x):
    return jnp.concatenate(
        [pltpu.pack_elementwise([x[i:i + 8], x[i + 8:i + 16]], packed_dtype=BF16)
         for i in range(0, x.shape[0], 16)], axis=0)


def _bf(words):
    return pltpu.bitcast(words, BF16)


def _layernorm(load):
    def mean(term, every):
        acc = [term(load(i)) for i in range(4)]
        for i in range(4, D // 8):
            acc[i % 4] = acc[i % 4] + term(load(i))
            if i % every == every - 1:
                yield
        tot = jnp.sum((acc[0] + acc[1]) + (acc[2] + acc[3]), axis=0, keepdims=True)
        return jnp.broadcast_to(tot * (1.0 / D), (8, T1))

    mu = yield from mean(lambda x: x, 32)
    var = yield from mean(lambda x: (x - mu) * (x - mu), 10)
    rs = jax.lax.rsqrt(var + 1e-5)
    return lambda i: jnp.concatenate([(load(2 * i + s) - mu) * rs for s in range(2)], axis=0)


def _items(n):
    return lambda fn: lambda *args: (fn(*args), n)


def _interleave(*lists, lead=0.0, span=1.0):
    gens = [(v for g, _ in w for v in g) for w in lists]
    sizes = [sum(n for _, n in w) for w in lists]
    for _, k in sorted((i / n if k else i / n * span - lead, k)
                       for k, n in enumerate(sizes) for i in range(n)):
        next(gens[k])
    for g in gens:
        for _ in g:
            pass


def _strassen_lhs(a11, a12, a21, a22):
    return a11 + a22, a22, a21 + a22, a11 + a12, a11, a12 - a22, a21 - a11


def _strassen_rhs(b11, b12, b21, b22):
    ops = (b11 + b22, b21 - b11, b11, b22, b12 - b22, b21 + b22, b11 + b12)
    return jnp.concatenate([_zip(v) for v in ops], axis=1)


def _strassen(prod, emit):
    m4 = prod(1)
    yield
    m2 = prod(2)
    emit(1, 0, m2 + m4)
    yield
    m1 = prod(0)
    c11, c22 = m1 + m4, m1 - m2
    yield
    c11 = c11 + prod(5)
    yield
    m5 = prod(3)
    emit(0, 0, c11 - m5)
    yield
    m3 = prod(4)
    emit(0, 1, m3 + m5)
    c22 = c22 + m3
    yield
    emit(1, 1, c22 + prod(6))
    yield


def _rows(i, n):
    return slice(i * n, i * n + n)


def _kernel(u_hbm, are_hbm, aim_hbm, bre_hbm, bim_hbm, cre_hbm, cim_hbm, ldt_hbm, dsk_hbm, wqkv_hbm, wo_hbm, f_hbm, out_hbm,
            are, aim, bre, bim, cre, cim, ldt, dsk, io, wq_in, wo_in, fm, ws, wp, lam, dtc, k0s, tab, ztab, kb, kf,
            xr, xn, kv, xq, qs, oe, oo, ob, zs, sems):
    cp_u = [pltpu.make_async_copy(u_hbm.bitcast(U32).at[:, h, :], io.at[h], sems.at[3 + h])
            for h in range(PH // 2)]
    cp_o = [pltpu.make_async_copy(io.at[h], out_hbm.bitcast(U32).at[:, h, :], sems.at[3 + h])
            for h in range(PH // 2)]
    cp_f, cp_g = [pltpu.make_async_copy(f_hbm.at[_rows(i, PH)], fm.at[_rows(i, PH)], sems.at[0])
                  for i in range(2)]
    cp_wq = pltpu.make_async_copy(wqkv_hbm, wq_in, sems.at[1])
    cp_wo = pltpu.make_async_copy(wo_hbm, wo_in, sems.at[2])
    cp_p = [pltpu.make_async_copy(src, dst, sems.at[3 + PH // 2 + i]) for i, (src, dst) in enumerate(
        ((ldt_hbm, ldt), (dsk_hbm, dsk), (aim_hbm, aim), (are_hbm, are), (bre_hbm, bre), (bim_hbm, bim), (cre_hbm, cre),
         (cim_hbm, cim)))]
    for cp in cp_p:
        cp.start()

    lane = jax.lax.broadcasted_iota(I32, (8, T1), 1)
    zs[0] = 0

    def xs(p):
        return xr.at[p]

    def region(*lists, **pace):
        pl.when(zs[0] == 0)(lambda: _interleave(*lists, **pace))

    cp_p[0].wait()
    cp_p[1].wait()
    dt_row = jnp.exp(ldt[...].astype(F32).reshape(1, D)).astype(BF16).astype(F32)
    ds_row = dsk[...].astype(F32).reshape(1, D)
    for j in range(4):
        dtc[0, _rows(j, 128), :] = jnp.broadcast_to(dt_row[:, _rows(j, 128)], (128, 128)).T
        dtc[1, _rows(j, 128), :] = jnp.broadcast_to(ds_row[:, _rows(j, 128)], (128, 128)).T
    cp_p[2].wait()
    cp_p[3].wait()
    for cp in cp_u[:2]:
        cp.start()
    big = None
    for j in range(D // 16):
        r = _rows(j, 16)
        theta = dtc[0, r, :] * aim[r, :].astype(F32)
        mag = jnp.exp(dtc[0, r, :] * are[r, :].astype(F32))
        sn, cs = _sincos(theta)
        lam[0, r, :] = mag * cs
        lam[1, r, :] = mag * sn
        big = jnp.abs(theta) if big is None else jnp.maximum(big, jnp.abs(theta))

    @pl.when(jnp.logical_not(jnp.max(big) <= 8192.0))
    def _():
        def body(i, _):
            rows = pl.ds(pl.multiple_of(i * 16, 16), 16)
            th = dtc[0, rows, :] * aim[rows, :].astype(F32)
            mg = jnp.exp(dtc[0, rows, :] * are[rows, :].astype(F32))
            lam[0, rows, :] = mg * jnp.cos(th)
            lam[1, rows, :] = mg * jnp.sin(th)
        jax.lax.fori_loop(0, D // 16, body, None)

    for cp in cp_p[4:]:
        cp.wait()

    @_items(15)
    def tap_tables(blk, e):
        rows = _rows(4 * blk + e, 8)

        def part(ref):
            return ref[_rows(2 * blk + e // 2, 16), :].astype(F32)[_rows(e % 2, 8)]

        sc = dtc[0, rows, :] * (2.0 / L)
        w = _cmul((part(cre), part(cim)), (part(bre) * sc, part(bim) * sc))
        k0s[rows, :] = w[0]

        def put(row, a, b):
            for z in range(2):
                tab[blk % 8, z, pl.ds(row, 8, stride=QS), :] = pltpu.pack_elementwise(
                    [a[z], b[z]], packed_dtype=BF16)

        l1 = (lam[0, rows, :], lam[1, rows, :])
        l2 = _csq(l1)
        l16 = _csq(_csq(_csq(l2)))
        m1 = (l16[0], -l16[1])
        m2 = _csq(m1)
        a, b = _cmul(w, l1), _cmul(w, l2)
        c, d = m2, _cmul(m1, m2)
        put(16 * e, (jnp.ones_like(m1[0]), jnp.zeros_like(m1[0])), m1)
        keep = {}
        for j in range(1, 16):
            if j <= 8:
                put(64 + 12 * e + j - 1, a, b)
                keep[2 * j] = b
            if j < 8:
                a, b = _cmul(a, l2), _cmul(b, l2)
            put(16 * e + j, c, d)
            if j == 8:
                l512 = _csq((c[0], -c[1]))
                put(64 + 12 * e + 8, _cmul(keep[4], l512), _cmul(keep[12], l512))
                a, b = keep[8], keep[16]
            if j in (10, 12, 14):
                a, b = _cmul(a, l512), _cmul(b, l512)
                put(64 + 12 * e + 4 + j // 2, a, b)
            if j < 15:
                c, d = _cmul(c, m2), _cmul(d, m2)
            yield

    @_items(24)
    def tap_sums(blk):
        for i in range(8):
            re, im = [jax.lax.dot_general(_bf(tab[blk % 8, z, pl.ds(QS * i + 64, 48), :]),
                                          _bf(tab[blk % 8, z, pl.ds(QS * i, 64), :]),
                                          NT, preferred_element_type=F32) for z in range(2)]
            acc = re + im
            for r in range(3):
                pc = [acc[_rows(3 * e + r, 8)] for e in range(4)]
                ztab[blk % 8, pl.ds(ZS * i + 8 * r, 8), :] = jnp.where(
                    lane < 64, jnp.where(lane < 32, pc[0], pc[1]),
                    jnp.where(lane < 96, pc[2], pc[3]))
                yield

    def tap_rows(blk, e):
        def at(r, g):
            z = ztab[blk % 8, pl.ds(r, 8, stride=ZS), :]
            return z if g == e else pltpu.roll(z, (32 * (g - e)) % 128, 1)

        def full(r, r1):
            return jnp.where(lane < 64, jnp.where(lane < 32, at(r, 0), at(r1, 1)),
                             jnp.where(lane < 96, at(r1 + 2, 2), at(r1 + 4, 3)))

        rows = _rows(4 * blk + e, 8)
        e8, e16 = full(7, 18), full(15, 19)
        k0 = jnp.sum(k0s[rows, :], axis=1, keepdims=True) + dtc[1, rows, :] * (2.0 / L)
        e0 = jnp.where(lane == 0, k0, pltpu.roll(e16, 1, 1))
        e4 = jnp.where(lane < 32, at(3, 0), at(16, 1))
        e12 = jnp.where(lane < 32, at(11, 0), at(17, 1))
        k4, k12 = jnp.where(lane < 64, e4, e0), jnp.where(lane < 64, e12, e16)
        far = {1: e0, 2: e0, 3: k4, 5: jnp.where(lane < 64, e4, e8), 6: e8, 7: e8, 9: e8,
               10: e8, 11: jnp.where(lane < 64, e12, e8), 13: k12, 14: e16, 15: e16}
        taps = {0: e0, 4: k4, 8: e8, 12: k12}
        return lambda p: taps[p] if p in taps else jnp.where(
            lane < (16 if p % 2 else 32), at(p - 1, 0), far[p])

    @_items(2)
    def tap_blocks(blk, e2):
        a, b = tap_rows(blk, 2 * e2), tap_rows(blk, 2 * e2 + 1)
        yield
        for p in range(PH):
            kb[p, _rows(2 * blk + e2, 16), :] = jnp.concatenate([a(p), b(p)], axis=0).astype(BF16)
        yield

    def lane_dft(src, lo, hi):
        return lane_dft_items(src, lo, hi), (hi - lo) // 2

    def lane_dft_items(src, lo, hi):
        for q in range(8):
            x0, x1 = [jax.lax.dot_general(src[p, lo:hi, :], _bf(fm[p]), NN,
                                          preferred_element_type=F32) for p in (q, q + 8)]
            for i in range((hi - lo) // 8):
                r = _rows(i, 8)
                for c, v in ((q, x0[r] + x1[r]), (q + 8, x0[r] - x1[r])):
                    for z in range(2):
                        kv[0, 2 * c + z, _rows(lo // 8 + i, 8), :] = v[:, _rows(z, T1)]
                if i % 2:
                    yield

    def residues(r, odd):
        return [(kv[0, 2 * c, r, :], kv[0, 2 * c + 1, r, :]) for c in range(8 * odd, 8 * odd + 8)]

    @_items(CB // 4)
    def tap_coefs(blk):
        for i in range(CB // 8):
            r = _rows(blk * CB // 8 + i, 8)
            for odd in range(2):
                for n, v in enumerate(_conv_coefs(residues(r, odd), 4 * odd)):
                    kf[10 * odd + n, r, :T1] = v[0]
                    kf[10 * odd + n, r, T1:] = v[1]
                yield

    r0 = jax.lax.broadcasted_iota(I32, (128, 128), 0)
    ri = (r0 & ~15) + (r0 & 7) * 2 + ((r0 >> 3) & 1)
    ci = jax.lax.broadcasted_iota(I32, (128, 128), 1)
    hit = ci == (ri & 7) * 16 + (ri >> 3)

    @_items(14)
    def prep_weights(j):
        def block(c, k):
            if j < 6:
                sel = jnp.where(hit, 1.0 if j < 4 else 0.25, 0.0)
                w = wq_in[_rows(k, 128), _rows(c, 128)]
            else:
                sel = jnp.where(ri == ci, 1.0, 0.0)
                w = _bf(wp[_rows(k, 64), _rows(c, 128)])
            return jax.lax.dot_general(sel.astype(BF16), w, NT, preferred_element_type=F32)

        top, bot = (4 + j, 8 + j) if j < 4 else (j % 2, j % 2 + 2)
        for k in range(2):
            for i, a in enumerate(_strassen_lhs(block(top, k), block(top, k + 2),
                                                block(bot, k), block(bot, k + 2))):
                ws[i, _rows(j, 64), _rows(k, 128)] = _zip(a)
                yield

    @_items(8)
    def permute_wo(j):
        sel = jnp.where(ci == (r0 & 7) * 16 + (r0 >> 3), 1.0, 0.0).astype(BF16)
        wp[_rows(j, 64), :] = _zip(jnp.dot(sel, wo_in[_rows(j, 128), :],
                                           preferred_element_type=F32))
        yield from range(8)

    @_items(4)
    def load_pair(h):
        for j in range(4):
            wds = io[h, :, _rows(j, 128)].T
            xs(2 * h)[_rows(j, 128), :] = pltpu.bitcast(wds << 16, F32)
            xs(2 * h + 1)[_rows(j, 128), :] = pltpu.bitcast(wds & np.uint32(0xFFFF0000), F32)
            yield

    @_items(24)
    def norm(h):
        for p in (2 * h, 2 * h + 1):
            normed = yield from _layernorm(lambda i: xs(p)[_rows(i, 8), :])
            for i in range(D // 16):
                xn[p, _rows(i, 16), :] = normed(i).astype(BF16)
                if i % 8 == 7:
                    yield

    for i, step in enumerate(PROLOGUE):
        tables, sums, blocks, dft, coefs, loads, norms, perms, preps = [
            range(a, b) for a, b in zip(PROLOGUE[i - 1] if i else (0,) * 9, step)]
        for cp in {0: cp_u[2:5], 1: [cp_f], 2: cp_u[5:], 3: [cp_wo, cp_wq], 5: [cp_g]}.get(i, ()):
            cp.start()
        for cp, users in ((cp_f, dft), (cp_wo, perms), (cp_wq, preps)):
            if 0 in users:
                cp.wait()
        for h in loads:
            cp_u[h].wait()
        region([tap_sums(2 * b + s) for b in sums for s in range(2)]
               + [lane_dft(kb, CB * b, CB * b + CB) for b in dft]
               + [permute_wo(j) for j in perms] + [prep_weights(j) for j in preps],
               [tap_tables(2 * b + s, e) for b in tables for s in range(2) for e in range(4)]
               + [norm(h) for h in norms],
               [tap_blocks(2 * b + s, e) for b in blocks for s in range(2) for e in range(2)],
               [tap_coefs(b) for b in coefs],
               [load_pair(h) for h in loads],
               lead={3: 0.03, 5: -0.03, 7: -0.03}.get(i, 0.0),
               span={1: 0.95, 2: 1.05, 4: 1.05, 6: 0.95}.get(i, 1.0))

    cp_g.wait()

    @_items(10)
    def phase_conv(i):
        r = _rows(i, 8)
        coefs = ((kf[n, r, :T1], kf[n, r, T1:]) for n in range(NCOEF))
        for odd in range(2):
            y = yield from _conv(residues(r, odd), 4 * odd, lambda: next(coefs))
            for c, v in enumerate(y):
                for z in range(2):
                    kv[1, 16 * odd + 2 * c + z, r, :] = v[z]
            yield

    @_items(32)
    def lane_idft(lo, hi):
        for q in (0, 2, 4, 6, 1, 3, 5, 7):
            a, b = [jnp.concatenate([kv[1, 2 * c + z, lo:hi, :] for z in range(2)], axis=1)
                    for c in (q, q + 8)]
            for p, v in ((q, a + b), (q + 8, a - b)):
                inv = jnp.concatenate([fm[PH + p, :, :T1], fm[PH + p, :, T1:]], axis=0)
                d = jax.lax.dot_general(v, _bf(inv), NN, preferred_element_type=F32)
                yield
                xs(p)[lo:hi, :] += d
                yield

    @_items(32)
    def norm_pair(g):
        def unzipped(i):
            return pl.ds(16 * (i // 2) + i % 2, 8, stride=2)

        p = 4 * (g % 4) + g // 4
        a = yield from _layernorm(lambda i: xr[p, unzipped(i), :])
        b = yield from _layernorm(lambda i: xr[p + 2, unzipped(i), :])
        for r in range(HD // 16):
            xq[g, _rows(r, 8), :] = _strassen_rhs(a(r), b(r), a(HD // 16 + r), b(HD // 16 + r))
            yield

    def block_product(row0, groups, rhs, emit):
        for r in [128 // RS * hg + i for hg in groups for i in range(128 // RS)]:
            w = slice((row0 + r * RS) // 2, (row0 + r * RS + RS) // 2)
            yield from _strassen(
                lambda i: jnp.dot(_bf(ws[i, w, :]), _bf(rhs[:, _rows(i, T1)]),
                                  preferred_element_type=F32),
                lambda half, n, y: emit(half, n, r * RS, y))

    @_items(7 * HD // RS)
    def keys_values(s, g):
        def emit(half, n, row, y):
            m = 2 * (g % 4) + n
            kv[g // 4, PH * half + WIN - 1 + m, pl.ds(row, RS), :] = y
            if m:
                kv[g // 4, PH * half + m - 1, pl.ds(row, RS), :] = pltpu.roll(y, 1, 1)

        return block_product(0, (s, s + 2), xq.at[g], emit)

    @_items(7 * 128 // RS)
    def queries(s, g):
        def emit(half, n, row, y):
            qs[g, n, pl.ds(HD * half + row, RS), :] = y

        return block_product(D, (s,), xq.at[g], emit)

    @_items(34)
    def attend(par, s, m):
        for hg in (s, s + 2):
            lg = [None] * WIN
            for j0 in range(0, WIN, JB):
                for dh in range(16):
                    r = _rows(16 * hg + dh, 8)
                    q = qs[4 * par + m // 2, m % 2, r, :]
                    for j in range(j0, j0 + JB):
                        t = q * kv[par, WIN - 1 + m - j, r, :]
                        lg[j] = t if dh == 0 else lg[j] + t
                    if (dh + 1) % (16 // JB) == 0:
                        yield
            for j in range(m + 1, WIN):
                lg[j] = jnp.where(lane == 0, -1e9, lg[j])
            mx = lg[0]
            for j in range(1, WIN):
                mx = jnp.maximum(mx, lg[j])
            ex = [jnp.exp(t - mx) for t in lg]
            den = ex[0]
            for j in range(1, WIN):
                den = den + ex[j]
            inv = pltpu.reciprocal(den, full_range=False)
            pr = [t * inv for t in ex]
            yield

            def out(dh):
                r = _rows(16 * hg + dh, 8)
                acc = pr[0] * kv[par, PH + WIN - 1 + m, r, :]
                for j in range(1, WIN):
                    acc = acc + pr[j] * kv[par, PH + WIN - 1 + m - j, r, :]
                return acc

            for d2 in range(8):
                o = jnp.concatenate([out(2 * d2), out(2 * d2 + 1)], axis=0)
                r = _rows(8 * hg + d2, 16)
                if par == 0:
                    oe[m, r, :] = o
                elif hg < 2:
                    oo[m, r, :] = o
                else:
                    r1 = _rows(8 * (hg - 2) + d2, 16)
                    ob[m, _rows(8 * (hg - 2) + d2, 8), :] = _strassen_rhs(
                        oe[m, r1, :], oo[m, r1, :], oe[m, r, :], o)
                yield

    late = (1, 4)

    @_items(7 * HD // RS)
    def project(h):
        def emit(half, n, row, y):
            xs(2 * h + n)[pl.ds(HD * half + row, RS), :] += y

        for s in range(2):
            yield from block_product(D + HD, (s,), ob.at[h], emit)
            if h not in late:
                for _ in store_pair(h, (s, s + 2))[0]:
                    pass

    @_items(4)
    def store_pair(h, groups):
        for j in groups:
            io[h, :, _rows(j, 128)] = pltpu.pack_elementwise(
                [xs(2 * h + n)[_rows(j, 128), :] for n in range(2)], packed_dtype=BF16).T
            yield

    def layer(it, c):
        def send(hs):
            @pl.when(it == 1)
            def _():
                for h in hs:
                    cp_o[h].start()

        cuts = (0, 0) + EDGES + (D, D)
        for i in range(len(cuts) - 3):
            (i0, i1), (c0, c1), (f0, f1) = [cuts[i + k:i + k + 2] for k in range(3)]
            last = i0 < i1 == D
            n = CB // 2 if i < 2 or last else CB
            region([lane_dft(xn, c, c + n) for c in range(f0, f1, n)]
                   + [lane_idft(c, c + n) for c in range(i0, i1, n)],
                   [phase_conv(r) for r in range(c0 // 8, c1 // 8)]
                   + ([norm(7)] if i == 0 else []) + ([norm_pair(0)] if last else []),
                   lead=0.7 if last else 0.0, span={0: 3.0, 4: 0.95}.get(i, 1.0))
        region([keys_values(0, 0), keys_values(1, 0), queries(0, 0)],
               [norm_pair(g) for g in (1, 2, 3)])
        region([fn(0, g) for fn in (keys_values, queries) for g in (1, 2, 3)],
               [norm_pair(g) for g in (4, 5, 6, 7)])
        for par, s, kvg, qg in ((0, 0, (1, 2, 3), (0, 1, 2, 3)), (0, 1, (4, 5, 6, 7), (4, 5, 6, 7)),
                                (1, 0, (4, 5, 6, 7), (4, 5))):
            region([keys_values(1 - s, g) for g in kvg] + [queries(1 - s, g) for g in qg],
                   [attend(par, s, m) for m in range(WIN)], span=1.05)
        region([queries(1, g) for g in (6, 7)], [attend(1, 1, m) for m in (0, 1)], span=0.95)
        done = ()
        for hs, ms in (((0, 1), (2, 3, 4)), ((2, 3, 4), (5, 6, 7)), ((5, 6), ()), ((7,), ())):
            region([project(h) for h in hs],
                   [store_pair(h, range(4)) for h in done if h in late]
                   + [norm(h) for h in done] + [attend(1, 1, m) for m in ms],
                   span={0: 0.95, 5: 1.05}.get(hs[0], 1.0))
            send([h for h in done if h in late] + [h for h in hs if h not in late])
            done = hs

    jax.lax.fori_loop(0, 2, layer, None)
    for cp in cp_o:
        cp.wait()


@jax.jit
def pallas_interleave_layers__ssm_conv_s4__sliding_local_dilated__prompt_kernel(
    A_u: jax.Array,
    A_A_re: jax.Array,
    A_A_im: jax.Array,
    A_B_re: jax.Array,
    A_B_im: jax.Array,
    A_C_re: jax.Array,
    A_C_im: jax.Array,
    A_log_dt: jax.Array,
    A_Dskip: jax.Array,
    B_x: jax.Array,
    B_wqkv: jax.Array,
    B_wo: jax.Array,
):
    del B_x
    hbm = pl.BlockSpec(memory_space=pl.ANY)
    out = pl.pallas_call(
        _kernel,
        in_specs=[hbm] * 12,
        out_specs=hbm,
        out_shape=jax.ShapeDtypeStruct((T1, PH, D), BF16),
        scratch_shapes=[pltpu.VMEM((D, NS), BF16)] * 6 + [pltpu.VMEM((D,), BF16)] * 2 + [
            pltpu.VMEM((PH // 2, T1, D), U32),
            pltpu.VMEM((D, 3 * D), BF16),
            pltpu.VMEM((D, D), BF16),
            pltpu.VMEM((2 * PH, T1 // 2, 2 * T1), U32),
            pltpu.VMEM((7, D, HD), U32),
            pltpu.VMEM((D // 2, D), U32),
            pltpu.VMEM((2, D, NS), F32),
            pltpu.VMEM((2, D, NS), F32),
            pltpu.VMEM((D, T1), F32),
            pltpu.VMEM((8, 2, 9 * QS + 4, NS), U32),
            pltpu.VMEM((8, 9 * ZS + 4, T1), F32),
            pltpu.VMEM((PH, D, T1), BF16),
            pltpu.VMEM((NCOEF, D, 2 * T1), F32),
            pltpu.VMEM((PH, D + 8, T1), F32),
            pltpu.VMEM((PH, D, T1), BF16),
            pltpu.VMEM((2, 2 * PH, D, T1), F32),
            pltpu.VMEM((PH // 2, HD // 2, 7 * T1), U32),
            pltpu.VMEM((PH // 2, 2, D, T1), F32),
            pltpu.VMEM((WIN, D, T1), F32),
            pltpu.VMEM((WIN, HD, T1), F32),
            pltpu.VMEM((WIN, HD // 2, 7 * T1), U32),
            pltpu.SMEM((1,), I32),
            pltpu.SemaphoreType.DMA((11 + PH // 2,)),
        ],
        compiler_params=pltpu.CompilerParams(vmem_limit_bytes=100 * 1024 * 1024),
    )(A_u.reshape(T1, PH, D), A_A_re, A_A_im, A_B_re, A_B_im, A_C_re, A_C_im,
      A_log_dt, A_Dskip, B_wqkv, B_wo,
      _dft_matrices())
    return out.reshape(1, L, D)
```

```python
import numpy as np

import jax
import jax.numpy as jnp
import jax.experimental.pallas as pl
import jax.experimental.pallas.tpu as pltpu

F32, BF16, U32, I32 = jnp.float32, jnp.bfloat16, jnp.uint32, jnp.int32
L, D, NS = 2048, 512, 128
PH, T1 = 16, 128
WIN = 8
NN = (((1,), (0,)), ((), ()))
NT = (((1,), (1,)), ((), ()))
QS = 116
ZS = 28
_H = float(np.sqrt(0.5))
NCOEF = 22
HD = D // 2
RS = 64
JB = 4
EDGES = (0, 64, 192, 320, 448, D)
PROLOGUE = ((1, 0, 0, 0, 0, 0, 0, 0, 0),
            (3, 1, 0, 0, 0, 0, 0, 0, 0),
            (5, 3, 1, 0, 0, 2, 0, 0, 0),
            (7, 5, 3, 1, 0, 5, 0, 0, 0),
            (8, 7, 5, 3, 0, 8, 1, 0, 0),
            (8, 8, 7, 5, 3, 8, 3, 4, 1),
            (8, 8, 8, 7, 5, 8, 6, 4, 4),
            (8, 8, 8, 8, 8, 8, 7, 4, 8))
CB = 64


def _dft_matrices():
    t = 16 * np.arange(T1)[None, :, None] + np.arange(PH)[:, None, None]
    k = np.arange(T1)[None, None, :] + 0.5
    phi = 2.0 * np.pi * k * t / (2 * L)
    phi = np.concatenate([phi, phi.transpose(0, 2, 1)])
    f = np.concatenate([np.cos(phi), -np.sin(phi)], axis=-1).astype(np.float32)
    bits = f.astype(BF16).view(np.uint16).astype(np.uint32)
    return bits[:, 0::2] | (bits[:, 1::2] << 16)


def _cmul(a, b):
    return a[0] * b[0] - a[1] * b[1], a[0] * b[1] + a[1] * b[0]


def _csq(a):
    t = a[0] * a[1]
    return a[0] * a[0] - a[1] * a[1], t + t


def _cadd(a, b):
    return a[0] + b[0], a[1] + b[1]


def _csub(a, b):
    return a[0] - b[0], a[1] - b[1]


def _rot8(x, e):
    s, d = x[0] + x[1], x[0] - x[1]
    return {1: (d * _H, s * _H), 3: (s * -_H, d * _H), 5: (d * -_H, s * -_H), 7: (s * _H, d * -_H)}[e]


def _split(x, e):
    n = len(x) // 2
    lo, hi = x[:n], x[n:]
    if e == 4:
        return ([(a[0] - b[1], a[1] + b[0]) for a, b in zip(lo, hi)],
                [(a[0] + b[1], a[1] - b[0]) for a, b in zip(lo, hi)])
    if e:
        hi = [_rot8(b, e // 2) for b in hi]
    return [_cadd(a, b) for a, b in zip(lo, hi)], [_csub(a, b) for a, b in zip(lo, hi)]


def _merge(p, m, e):
    lo = [_cadd(a, b) for a, b in zip(p, m)]
    if e == 4:
        return lo + [(a[1] - b[1], b[0] - a[0]) for a, b in zip(p, m)]
    hi = [_csub(a, b) for a, b in zip(p, m)]
    return lo + ([_rot8(b, 8 - e // 2) for b in hi] if e else hi)


def _conv_coefs(k, e):
    if len(k) == 1:
        return [(k[0][0] * 0.5, k[0][1] * 0.5)]
    if len(k) == 2 and e % 4:
        if e % 2:
            top = _csub(_rot8(k[1], e), k[0])
        elif e == 2:
            top = (-k[1][1] - k[0][0], k[1][0] - k[0][1])
        else:
            top = (k[1][1] - k[0][0], -k[1][0] - k[0][1])
        return [k[0], top, _csub(k[1], k[0])]
    p, m = _split(k, e)
    return _conv_coefs(p, e // 2) + _conv_coefs(m, e // 2 + 4)


def _conv(x, e, coef):
    if len(x) == 1:
        return [_cmul(x[0], coef())]
    if len(x) == 2:
        yield
    if len(x) == 2 and e % 4:
        both = _cmul(_cadd(x[0], x[1]), coef())
        return [_cadd(both, _cmul(x[1], coef())), _cadd(both, _cmul(x[0], coef()))]
    p, m = _split(x, e)
    p = yield from _conv(p, e // 2, coef)
    m = yield from _conv(m, e // 2 + 4, coef)
    return _merge(p, m, e)


def _sincos(x):
    n = jnp.floor(x * float(2.0 / np.pi) + 0.5)
    r = ((x - n * 1.5703125) - n * 4.837512969970703125e-4) - n * 7.54978995489188216e-8
    z = r * r
    s = r + r * z * ((-1.9515295891e-4 * z + 8.3321608736e-3) * z - 1.6666654611e-1)
    c = 1.0 + z * (((2.443315711809948e-5 * z - 1.388731625493765e-3) * z
                    + 4.166664568298827e-2) * z - 0.5)
    q = n.astype(I32)
    odd = (q & 1) == 1
    s, c = jnp.where(odd, c, s), jnp.where(odd, s, c)
    return jnp.where((q & 2) == 2, -s, s), jnp.where(((q + 1) & 2) == 2, -c, c)


def _zip(x):
    return jnp.concatenate(
        [pltpu.pack_elementwise([x[i:i + 8], x[i + 8:i + 16]], packed_dtype=BF16)
         for i in range(0, x.shape[0], 16)], axis=0)


def _unzip(words, s):
    return pltpu.bitcast(words & np.uint32(0xFFFF0000) if s else words << 16, F32)


def _bf(words):
    return pltpu.bitcast(words, BF16)


def _layernorm(load):
    def mean(term, every):
        acc = [term(load(i)) for i in range(4)]
        for i in range(4, D // 8):
            acc[i % 4] = acc[i % 4] + term(load(i))
            if i % every == every - 1:
                yield
        tot = jnp.sum((acc[0] + acc[1]) + (acc[2] + acc[3]), axis=0, keepdims=True)
        return jnp.broadcast_to(tot * (1.0 / D), (8, T1))

    mu = yield from mean(lambda x: x, 32)
    var = yield from mean(lambda x: (x - mu) * (x - mu), 10)
    rs = jax.lax.rsqrt(var + 1e-5)
    return lambda i: jnp.concatenate([(load(2 * i + s) - mu) * rs for s in range(2)], axis=0)


def _items(n):
    return lambda fn: lambda *args: (fn(*args), n)


def _interleave(*lists, lead=0.0, span=1.0):
    gens = [(v for g, _ in w for v in g) for w in lists]
    sizes = [sum(n for _, n in w) for w in lists]
    for _, k in sorted((i / n if k else i / n * span - lead, k)
                       for k, n in enumerate(sizes) for i in range(n)):
        next(gens[k])
    for g in gens:
        for _ in g:
            pass


def _strassen_lhs(a11, a12, a21, a22):
    return a11 + a22, a22, a21 + a22, a11 + a12, a11, a12 - a22, a21 - a11


def _strassen_rhs(b11, b12, b21, b22):
    ops = (b11 + b22, b21 - b11, b11, b22, b12 - b22, b21 + b22, b11 + b12)
    return jnp.concatenate([_zip(v) for v in ops], axis=1)


def _strassen(prod, emit):
    m4 = prod(1)
    yield
    m2 = prod(2)
    emit(1, 0, m2 + m4)
    yield
    m1 = prod(0)
    c11, c22 = m1 + m4, m1 - m2
    yield
    c11 = c11 + prod(5)
    yield
    m5 = prod(3)
    emit(0, 0, c11 - m5)
    yield
    m3 = prod(4)
    emit(0, 1, m3 + m5)
    c22 = c22 + m3
    yield
    emit(1, 1, c22 + prod(6))
    yield


def _rows(i, n):
    return slice(i * n, i * n + n)


def _alternate(i):
    return pl.ds(16 * (i // 2) + i % 2, 8, stride=2)


def _kernel(u_hbm, are_hbm, aim_hbm, bre_hbm, bim_hbm, cre_hbm, cim_hbm, ldt_hbm, dsk_hbm, wqkv_hbm, wo_hbm, f_hbm, out_hbm,
            are, aim, bre, bim, cre, cim, ldt, dsk, io, wq_in, wo_in, fm, ws, wp, lam, dtc, k0s, tab, ztab, kb, kf,
            xr, xn, kv, xq, qs, oe, oo, ob, zs, sems):
    cp_u = [pltpu.make_async_copy(u_hbm.bitcast(U32).at[:, h, :], io.at[h], sems.at[3 + h])
            for h in range(PH // 2)]
    cp_o = [pltpu.make_async_copy(io.at[h], out_hbm.bitcast(U32).at[:, h, :], sems.at[3 + h])
            for h in range(PH // 2)]
    cp_f, cp_g = [pltpu.make_async_copy(f_hbm.at[_rows(i, PH)], fm.at[_rows(i, PH)], sems.at[0])
                  for i in range(2)]
    cp_wq = pltpu.make_async_copy(wqkv_hbm, wq_in, sems.at[1])
    cp_wo = pltpu.make_async_copy(wo_hbm, wo_in, sems.at[2])
    cp_p = [pltpu.make_async_copy(src, dst, sems.at[3 + PH // 2 + i]) for i, (src, dst) in enumerate(
        ((ldt_hbm, ldt), (dsk_hbm, dsk), (aim_hbm, aim), (are_hbm, are), (bre_hbm, bre), (bim_hbm, bim), (cre_hbm, cre),
         (cim_hbm, cim)))]
    for cp in cp_p:
        cp.start()

    lane = jax.lax.broadcasted_iota(I32, (8, T1), 1)
    zs[0] = 0

    def region(*lists, **pace):
        pl.when(zs[0] == 0)(lambda: _interleave(*lists, **pace))

    cp_p[0].wait()
    cp_p[1].wait()
    dt_row = jnp.exp(ldt[...].astype(F32).reshape(1, D)).astype(BF16).astype(F32)
    ds_row = dsk[...].astype(F32).reshape(1, D)
    for j in range(4):
        dtc[0, _rows(j, 128), :] = jnp.broadcast_to(dt_row[:, _rows(j, 128)], (128, 128)).T
        dtc[1, _rows(j, 128), :] = jnp.broadcast_to(ds_row[:, _rows(j, 128)], (128, 128)).T
    cp_p[2].wait()
    cp_p[3].wait()
    cp_u[0].start()
    cp_u[1].start()
    big = None
    for j in range(D // 16):
        r = _rows(j, 16)
        theta = dtc[0, r, :] * aim[r, :].astype(F32)
        mag = jnp.exp(dtc[0, r, :] * are[r, :].astype(F32))
        sn, cs = _sincos(theta)
        lam[0, r, :] = mag * cs
        lam[1, r, :] = mag * sn
        big = jnp.abs(theta) if big is None else jnp.maximum(big, jnp.abs(theta))

    @pl.when(jnp.logical_not(jnp.max(big) <= 8192.0))
    def _():
        def body(i, _):
            rows = pl.ds(pl.multiple_of(i * 16, 16), 16)
            th = dtc[0, rows, :] * aim[rows, :].astype(F32)
            mg = jnp.exp(dtc[0, rows, :] * are[rows, :].astype(F32))
            lam[0, rows, :] = mg * jnp.cos(th)
            lam[1, rows, :] = mg * jnp.sin(th)
        jax.lax.fori_loop(0, D // 16, body, None)

    for cp in cp_p[4:]:
        cp.wait()

    @_items(15)
    def tap_tables(blk, e, s):
        rows = pl.ds(CB * blk + 16 * e + s, 8, stride=2)

        def part(ref):
            return _unzip(pltpu.bitcast(ref[_rows(4 * blk + e, 16), :], U32), s)

        sc = dtc[0, rows, :] * (2.0 / L)
        w = _cmul((part(cre), part(cim)), (part(bre) * sc, part(bim) * sc))
        k0s[rows, :] = w[0]

        def put(row, a, b):
            for z in range(2):
                tab[blk % 4, 2 * s + z, pl.ds(row, 8, stride=QS), :] = pltpu.pack_elementwise(
                    [a[z], b[z]], packed_dtype=BF16)

        l1 = (lam[0, rows, :], lam[1, rows, :])
        l2 = _csq(l1)
        l16 = _csq(_csq(_csq(l2)))
        m1 = (l16[0], -l16[1])
        m2 = _csq(m1)
        a, b = _cmul(w, l1), _cmul(w, l2)
        c, d = m2, _cmul(m1, m2)
        put(16 * e, (jnp.ones_like(m1[0]), jnp.zeros_like(m1[0])), m1)
        keep = {}
        for j in range(1, 16):
            if j <= 8:
                put(64 + 12 * e + j - 1, a, b)
                keep[2 * j] = b
            if j < 8:
                a, b = _cmul(a, l2), _cmul(b, l2)
            put(16 * e + j, c, d)
            if j == 8:
                l512 = _csq((c[0], -c[1]))
                put(64 + 12 * e + 8, _cmul(keep[4], l512), _cmul(keep[12], l512))
                a, b = keep[8], keep[16]
            if j in (10, 12, 14):
                a, b = _cmul(a, l512), _cmul(b, l512)
                put(64 + 12 * e + 4 + j // 2, a, b)
            if j < 15:
                c, d = _cmul(c, m2), _cmul(d, m2)
            yield

    @_items(48)
    def tap_sums(blk):
        for i in range(8):
            d = [jax.lax.dot_general(_bf(tab[blk % 4, z, pl.ds(QS * i + 64, 48), :]),
                                     _bf(tab[blk % 4, z, pl.ds(QS * i, 64), :]),
                                     NT, preferred_element_type=F32) for z in range(4)]
            own = [None] * 3
            for n in range(12):
                e, r = n // 3, _rows(n, 8)
                v = pltpu.pack_elementwise([d[0][r] + d[1][r], d[2][r] + d[3][r]],
                                           packed_dtype=BF16)
                own[n % 3] = jnp.where(lane < 32 * e, own[n % 3], v) if e else v
                if n % 2:
                    yield
            for r in range(3):
                ztab[blk % 4, pl.ds(ZS * i + 8 * r, 8), :] = own[r]

    @_items(2)
    def tap_blocks(blk, e):
        def at(r, g):
            z = ztab[blk % 4, pl.ds(r, 8, stride=ZS), :]
            return z if g == e else pltpu.roll(z, (32 * (g - e)) % 128, 1)

        def full(r, r1):
            return jnp.where(lane < 64, jnp.where(lane < 32, at(r, 0), at(r1, 1)),
                             jnp.where(lane < 96, at(r1 + 2, 2), at(r1 + 4, 3)))

        halves = [pl.ds(CB * blk + 16 * e + s, 8, stride=2) for s in range(2)]
        e8, e16 = full(7, 18), full(15, 19)
        k0 = pltpu.pack_elementwise(
            [jnp.sum(k0s[r, :], axis=1, keepdims=True) + dtc[1, r, :] * (2.0 / L) for r in halves],
            packed_dtype=BF16)
        e0 = jnp.where(lane == 0, k0, pltpu.roll(e16, 1, 1))
        e4 = jnp.where(lane < 32, at(3, 0), at(16, 1))
        e12 = jnp.where(lane < 32, at(11, 0), at(17, 1))
        k4, k12 = jnp.where(lane < 64, e4, e0), jnp.where(lane < 64, e12, e16)
        far = {1: e0, 2: e0, 3: k4, 5: jnp.where(lane < 64, e4, e8), 6: e8, 7: e8, 9: e8,
               10: e8, 11: jnp.where(lane < 64, e12, e8), 13: k12, 14: e16, 15: e16}
        taps = {0: e0, 4: k4, 8: e8, 12: k12}
        yield
        for p in range(PH):
            kb[p, _rows(4 * blk + e, 8), :] = taps[p] if p in taps else jnp.where(
                lane < (16 if p % 2 else 32), at(p - 1, 0), far[p])
        yield

    @_items(CB // 2)
    def lane_dft(src, lo, hi):
        for q in range(8):
            x0, x1 = [jax.lax.dot_general(_bf(src[p, lo // 2:hi // 2, :]), _bf(fm[p]), NN,
                                          preferred_element_type=F32) for p in (q, q + 8)]
            for i in range((hi - lo) // 8):
                r = _rows(i, 8)
                for c, v in ((q, x0[r] + x1[r]), (q + 8, x0[r] - x1[r])):
                    for z in range(2):
                        kv[0, 2 * c + z, _rows(lo // 8 + i, 8), :] = v[:, _rows(z, T1)]
                if i % 2:
                    yield

    def residues(r, odd):
        return [(kv[0, 2 * c, r, :], kv[0, 2 * c + 1, r, :]) for c in range(8 * odd, 8 * odd + 8)]

    @_items(CB // 4)
    def tap_coefs(blk):
        for i in range(CB // 8):
            r = _rows(blk * CB // 8 + i, 8)
            for odd in range(2):
                for n, v in enumerate(_conv_coefs(residues(r, odd), 4 * odd)):
                    kf[10 * odd + n, r, :T1] = v[0]
                    kf[10 * odd + n, r, T1:] = v[1]
                yield

    r0 = jax.lax.broadcasted_iota(I32, (128, 128), 0)
    ri = (r0 & ~15) + (r0 & 7) * 2 + ((r0 >> 3) & 1)
    ci = jax.lax.broadcasted_iota(I32, (128, 128), 1)
    hit = ci == (ri & 7) * 16 + (ri >> 3)

    @_items(14)
    def prep_weights(j):
        def block(c, k):
            if j < 6:
                sel = jnp.where(hit, 1.0 if j < 4 else 0.25, 0.0)
                w = wq_in[_rows(k, 128), _rows(c, 128)]
            else:
                sel = jnp.where(ri == ci, 1.0, 0.0)
                w = _bf(wp[_rows(k, 64), _rows(c, 128)])
            return jax.lax.dot_general(sel.astype(BF16), w, NT, preferred_element_type=F32)

        top, bot = (4 + j, 8 + j) if j < 4 else (j % 2, j % 2 + 2)
        for k in range(2):
            for i, a in enumerate(_strassen_lhs(block(top, k), block(top, k + 2),
                                                block(bot, k), block(bot, k + 2))):
                ws[i, _rows(j, 64), _rows(k, 128)] = _zip(a)
                yield

    @_items(8)
    def permute_wo(j):
        sel = jnp.where(ci == (r0 & 7) * 16 + (r0 >> 3), 1.0, 0.0).astype(BF16)
        wp[_rows(j, 64), :] = _zip(jnp.dot(sel, wo_in[_rows(j, 128), :],
                                           preferred_element_type=F32))
        yield from range(8)

    @_items(4)
    def load_pair(h):
        for j in range(4):
            wds = io[h, :, _rows(j, 128)].T
            for s in range(2):
                xr[2 * h + s, _rows(j, 128), :] = _unzip(wds, s)
            yield

    @_items(24)
    def norm(h):
        for p in (2 * h, 2 * h + 1):
            normed = yield from _layernorm(lambda i: xr[p, _alternate(i), :])
            for i in range(D // 16):
                xn[p, _rows(i, 8), :] = _zip(normed(i))
                if i % 8 == 7:
                    yield

    for i, step in enumerate(PROLOGUE):
        tables, sums, blocks, dft, coefs, loads, norms, perms, preps = [
            range(a, b) for a, b in zip(PROLOGUE[i - 1] if i else (0,) * 9, step)]
        for cp in {0: [cp_f], 1: cp_u[2:5], 2: cp_u[5:], 3: [cp_wo, cp_wq], 5: [cp_g]}.get(i, ()):
            cp.start()
        for cp, users in ((cp_f, dft), (cp_wo, perms), (cp_wq, preps)):
            if 0 in users:
                cp.wait()
        for h in loads:
            cp_u[h].wait()
        region([tap_sums(b) for b in sums]
               + [lane_dft(kb, CB * b, CB * b + CB) for b in dft]
               + [permute_wo(j) for j in perms] + [prep_weights(j) for j in preps],
               [tap_tables(b, e, s) for b in tables for e in range(4) for s in range(2)]
               + [norm(h) for h in norms],
               [tap_blocks(b, e) for b in blocks for e in range(4)],
               [tap_coefs(b) for b in coefs],
               [load_pair(h) for h in loads],
               lead={3: 0.03, 5: -0.03, 7: -0.03}.get(i, 0.0),
               span={1: 0.95, 2: 1.05, 4: 1.05, 6: 0.95}.get(i, 1.0))

    cp_g.wait()

    @_items(10)
    def phase_conv(i):
        r = _rows(i, 8)
        coefs = ((kf[n, r, :T1], kf[n, r, T1:]) for n in range(NCOEF))
        for odd in range(2):
            y = yield from _conv(residues(r, odd), 4 * odd, lambda: next(coefs))
            for c, v in enumerate(y):
                for z in range(2):
                    kv[1, 16 * odd + 2 * c + z, r, :] = v[z]
            yield

    @_items(32)
    def lane_idft(lo, hi):
        for q in (0, 2, 4, 6, 1, 3, 5, 7):
            a, b = [jnp.concatenate([kv[1, 2 * c + z, lo:hi, :] for z in range(2)], axis=1)
                    for c in (q, q + 8)]
            for p, v in ((q, a + b), (q + 8, a - b)):
                inv = jnp.concatenate([fm[PH + p, :, :T1], fm[PH + p, :, T1:]], axis=0)
                d = jax.lax.dot_general(v, _bf(inv), NN, preferred_element_type=F32)
                yield
                xr[p, lo:hi, :] += d
                yield

    @_items(32)
    def norm_pair(g):
        p = 4 * (g % 4) + g // 4
        a = yield from _layernorm(lambda i: xr[p, _alternate(i), :])
        b = yield from _layernorm(lambda i: xr[p + 2, _alternate(i), :])
        for r in range(HD // 16):
            xq[g, _rows(r, 8), :] = _strassen_rhs(a(r), b(r), a(HD // 16 + r), b(HD // 16 + r))
            yield

    def block_product(row0, groups, rhs, emit):
        for r in [128 // RS * hg + i for hg in groups for i in range(128 // RS)]:
            w = slice((row0 + r * RS) // 2, (row0 + r * RS + RS) // 2)
            yield from _strassen(
                lambda i: jnp.dot(_bf(ws[i, w, :]), _bf(rhs[:, _rows(i, T1)]),
                                  preferred_element_type=F32),
                lambda half, n, y: emit(half, n, r * RS, y))

    @_items(7 * HD // RS)
    def keys_values(s, g):
        def emit(half, n, row, y):
            m = 2 * (g % 4) + n
            kv[g // 4, PH * half + WIN - 1 + m, pl.ds(row, RS), :] = y
            if m:
                kv[g // 4, PH * half + m - 1, pl.ds(row, RS), :] = pltpu.roll(y, 1, 1)

        return block_product(0, (s, s + 2), xq.at[g], emit)

    @_items(7 * 128 // RS)
    def queries(s, g):
        def emit(half, n, row, y):
            qs[g, n, pl.ds(HD * half + row, RS), :] = y

        return block_product(D, (s,), xq.at[g], emit)

    @_items(34)
    def attend(par, s, m):
        for hg in (s, s + 2):
            lg = [None] * WIN
            for j0 in range(0, WIN, JB):
                for dh in range(16):
                    r = _rows(16 * hg + dh, 8)
                    q = qs[4 * par + m // 2, m % 2, r, :]
                    for j in range(j0, j0 + JB):
                        t = q * kv[par, WIN - 1 + m - j, r, :]
                        lg[j] = t if dh == 0 else lg[j] + t
                    if (dh + 1) % (16 // JB) == 0:
                        yield
            for j in range(m + 1, WIN):
                lg[j] = jnp.where(lane == 0, -1e9, lg[j])
            mx = lg[0]
            for j in range(1, WIN):
                mx = jnp.maximum(mx, lg[j])
            ex = [jnp.exp(t - mx) for t in lg]
            den = ex[0]
            for j in range(1, WIN):
                den = den + ex[j]
            inv = pltpu.reciprocal(den, full_range=False)
            pr = [t * inv for t in ex]
            yield

            def out(dh):
                r = _rows(16 * hg + dh, 8)
                acc = pr[0] * kv[par, PH + WIN - 1 + m, r, :]
                for j in range(1, WIN):
                    acc = acc + pr[j] * kv[par, PH + WIN - 1 + m - j, r, :]
                return acc

            for d2 in range(8):
                o = jnp.concatenate([out(2 * d2), out(2 * d2 + 1)], axis=0)
                r = _rows(8 * hg + d2, 16)
                if par == 0:
                    oe[m, r, :] = o
                elif hg < 2:
                    oo[m, r, :] = o
                else:
                    r1 = _rows(8 * (hg - 2) + d2, 16)
                    ob[m, _rows(8 * (hg - 2) + d2, 8), :] = _strassen_rhs(
                        oe[m, r1, :], oo[m, r1, :], oe[m, r, :], o)
                yield

    late = (1, 4)

    @_items(7 * HD // RS)
    def project(h):
        def emit(half, n, row, y):
            xr[2 * h + n, pl.ds(HD * half + row, RS), :] += y

        for s in range(2):
            yield from block_product(D + HD, (s,), ob.at[h], emit)
            if h not in late:
                for _ in store_pair(h, (s, s + 2))[0]:
                    pass

    @_items(4)
    def store_pair(h, groups):
        for j in groups:
            io[h, :, _rows(j, 128)] = pltpu.pack_elementwise(
                [xr[2 * h + n, _rows(j, 128), :] for n in range(2)], packed_dtype=BF16).T
            yield

    def layer(it, c):
        def send(hs):
            @pl.when(it == 1)
            def _():
                for h in hs:
                    cp_o[h].start()

        cuts = (0, 0) + EDGES + (D, D)
        for i in range(len(cuts) - 3):
            (i0, i1), (c0, c1), (f0, f1) = [cuts[i + k:i + k + 2] for k in range(3)]
            last = i0 < i1 == D
            region([lane_dft(xn, c, c + CB) for c in range(f0, f1, CB)]
                   + [lane_idft(c, c + CB) for c in range(i0, i1, CB)],
                   [phase_conv(r) for r in range(c0 // 8, c1 // 8)]
                   + ([norm(7)] if i == 0 else []) + ([norm_pair(0)] if last else []),
                   lead=0.4 if last else 0.0, span={0: 1.5, 4: 0.95}.get(i, 1.0))
        region([keys_values(0, 0), keys_values(1, 0), queries(0, 0)],
               [norm_pair(g) for g in (1, 2, 3)])
        region([fn(0, g) for fn in (keys_values, queries) for g in (1, 2, 3)],
               [norm_pair(g) for g in (4, 5, 6, 7)])
        for par, s, kvg, qg in ((0, 0, (1, 2, 3), (0, 1, 2, 3)), (0, 1, (4, 5, 6, 7), (4, 5, 6, 7)),
                                (1, 0, (4, 5, 6, 7), (4, 5))):
            region([keys_values(1 - s, g) for g in kvg] + [queries(1 - s, g) for g in qg],
                   [attend(par, s, m) for m in range(WIN)], span=1.05)
        region([queries(1, g) for g in (6, 7)], [attend(1, 1, m) for m in (0, 1)], span=0.95)
        done = ()
        for hs, ms in (((0, 1), (2, 3, 4)), ((2, 3, 4), (5, 6, 7)), ((5, 6), ()), ((7,), ())):
            region([project(h) for h in hs],
                   [store_pair(h, range(4)) for h in done if h in late]
                   + [norm(h) for h in done] + [attend(1, 1, m) for m in ms],
                   span={0: 0.95, 5: 1.05}.get(hs[0], 1.0))
            send([h for h in done if h in late] + [h for h in hs if h not in late])
            done = hs

    jax.lax.fori_loop(0, 2, layer, None)
    for cp in cp_o:
        cp.wait()


@jax.jit
def pallas_interleave_layers__ssm_conv_s4__sliding_local_dilated__prompt_kernel(
    A_u: jax.Array,
    A_A_re: jax.Array,
    A_A_im: jax.Array,
    A_B_re: jax.Array,
    A_B_im: jax.Array,
    A_C_re: jax.Array,
    A_C_im: jax.Array,
    A_log_dt: jax.Array,
    A_Dskip: jax.Array,
    B_x: jax.Array,
    B_wqkv: jax.Array,
    B_wo: jax.Array,
):
    del B_x
    hbm = pl.BlockSpec(memory_space=pl.ANY)
    out = pl.pallas_call(
        _kernel,
        in_specs=[hbm] * 12,
        out_specs=hbm,
        out_shape=jax.ShapeDtypeStruct((T1, PH, D), BF16),
        scratch_shapes=[pltpu.VMEM((D, NS), BF16)] * 6 + [pltpu.VMEM((D,), BF16)] * 2 + [
            pltpu.VMEM((PH // 2, T1, D), U32),
            pltpu.VMEM((D, 3 * D), BF16),
            pltpu.VMEM((D, D), BF16),
            pltpu.VMEM((2 * PH, T1 // 2, 2 * T1), U32),
            pltpu.VMEM((7, D, HD), U32),
            pltpu.VMEM((D // 2, D), U32),
            pltpu.VMEM((2, D + 8, NS), F32),
            pltpu.VMEM((2, D + 8, NS), F32),
            pltpu.VMEM((D + 8, NS), F32),
            pltpu.VMEM((4, 4, 9 * QS + 4, NS), U32),
            pltpu.VMEM((4, 9 * ZS + 4, T1), U32),
            pltpu.VMEM((PH, D // 2, T1), U32),
            pltpu.VMEM((NCOEF, D, 2 * T1), F32),
            pltpu.VMEM((PH, D + 8, T1), F32),
            pltpu.VMEM((PH, D // 2, T1), U32),
            pltpu.VMEM((2, 2 * PH, D, T1), F32),
            pltpu.VMEM((PH // 2, HD // 2, 7 * T1), U32),
            pltpu.VMEM((PH // 2, 2, D, T1), F32),
            pltpu.VMEM((WIN, D, T1), F32),
            pltpu.VMEM((WIN, HD, T1), F32),
            pltpu.VMEM((WIN, HD // 2, 7 * T1), U32),
            pltpu.SMEM((1,), I32),
            pltpu.SemaphoreType.DMA((11 + PH // 2,)),
        ],
        compiler_params=pltpu.CompilerParams(vmem_limit_bytes=100 * 1024 * 1024),
    )(A_u.reshape(T1, PH, D), A_A_re, A_A_im, A_B_re, A_B_im, A_C_re, A_C_im,
      A_log_dt, A_Dskip, B_wqkv, B_wo,
      _dft_matrices())
    return out.reshape(1, L, D)
```

```python
import numpy as np

import jax
import jax.numpy as jnp
import jax.experimental.pallas as pl
import jax.experimental.pallas.tpu as pltpu

F32, BF16, U32, I32 = jnp.float32, jnp.bfloat16, jnp.uint32, jnp.int32
L, D, NS = 2048, 512, 128
PH, T1 = 16, 128
WIN = 8
NN = (((1,), (0,)), ((), ()))
NT = (((1,), (1,)), ((), ()))
QS = 116
ZS = 28
_H = float(np.sqrt(0.5))
NCOEF = 22
HD = D // 2
RS = 64
JB = 4
EDGES = (0, 64, 192, 320, 448, D)
PROLOGUE = ((1, 0, 0, 0, 0, 0, 0, 0, 0),
            (3, 1, 0, 0, 0, 0, 0, 0, 0),
            (5, 3, 1, 0, 0, 2, 0, 0, 0),
            (7, 5, 3, 1, 0, 5, 0, 0, 0),
            (8, 7, 5, 3, 0, 8, 1, 0, 0),
            (8, 8, 7, 5, 3, 8, 3, 4, 1),
            (8, 8, 8, 7, 5, 8, 6, 4, 4),
            (8, 8, 8, 8, 8, 8, 7, 4, 8))
CB = 64


def _dft_matrices():
    t = 16 * np.arange(T1)[None, :, None] + np.arange(PH)[:, None, None]
    k = np.arange(T1)[None, None, :] + 0.5
    phi = 2.0 * np.pi * k * t / (2 * L)
    phi = np.concatenate([phi, phi.transpose(0, 2, 1)])
    f = np.concatenate([np.cos(phi), -np.sin(phi)], axis=-1).astype(np.float32)
    bits = f.astype(BF16).view(np.uint16).astype(np.uint32)
    return bits[:, 0::2] | (bits[:, 1::2] << 16)


def _cmul(a, b):
    return a[0] * b[0] - a[1] * b[1], a[0] * b[1] + a[1] * b[0]


def _csq(a):
    t = a[0] * a[1]
    return a[0] * a[0] - a[1] * a[1], t + t


def _cadd(a, b):
    return a[0] + b[0], a[1] + b[1]


def _csub(a, b):
    return a[0] - b[0], a[1] - b[1]


def _rot8(x, e):
    s, d = x[0] + x[1], x[0] - x[1]
    return {1: (d * _H, s * _H), 3: (s * -_H, d * _H), 5: (d * -_H, s * -_H), 7: (s * _H, d * -_H)}[e]


def _split(x, e):
    n = len(x) // 2
    lo, hi = x[:n], x[n:]
    if e == 4:
        return ([(a[0] - b[1], a[1] + b[0]) for a, b in zip(lo, hi)],
                [(a[0] + b[1], a[1] - b[0]) for a, b in zip(lo, hi)])
    if e:
        hi = [_rot8(b, e // 2) for b in hi]
    return [_cadd(a, b) for a, b in zip(lo, hi)], [_csub(a, b) for a, b in zip(lo, hi)]


def _merge(p, m, e):
    lo = [_cadd(a, b) for a, b in zip(p, m)]
    if e == 4:
        return lo + [(a[1] - b[1], b[0] - a[0]) for a, b in zip(p, m)]
    hi = [_csub(a, b) for a, b in zip(p, m)]
    return lo + ([_rot8(b, 8 - e // 2) for b in hi] if e else hi)


def _conv_coefs(k, e):
    if len(k) == 1:
        return [(k[0][0] * 0.5, k[0][1] * 0.5)]
    if len(k) == 2 and e % 4:
        if e % 2:
            top = _csub(_rot8(k[1], e), k[0])
        elif e == 2:
            top = (-k[1][1] - k[0][0], k[1][0] - k[0][1])
        else:
            top = (k[1][1] - k[0][0], -k[1][0] - k[0][1])
        return [k[0], top, _csub(k[1], k[0])]
    p, m = _split(k, e)
    return _conv_coefs(p, e // 2) + _conv_coefs(m, e // 2 + 4)


def _conv(x, e, coef):
    if len(x) == 1:
        return [_cmul(x[0], coef())]
    if len(x) == 2:
        yield
    if len(x) == 2 and e % 4:
        both = _cmul(_cadd(x[0], x[1]), coef())
        return [_cadd(both, _cmul(x[1], coef())), _cadd(both, _cmul(x[0], coef()))]
    p, m = _split(x, e)
    p = yield from _conv(p, e // 2, coef)
    m = yield from _conv(m, e // 2 + 4, coef)
    return _merge(p, m, e)


def _sincos(x):
    n = jnp.floor(x * float(2.0 / np.pi) + 0.5)
    r = ((x - n * 1.5703125) - n * 4.837512969970703125e-4) - n * 7.54978995489188216e-8
    z = r * r
    s = r + r * z * ((-1.9515295891e-4 * z + 8.3321608736e-3) * z - 1.6666654611e-1)
    c = 1.0 + z * (((2.443315711809948e-5 * z - 1.388731625493765e-3) * z
                    + 4.166664568298827e-2) * z - 0.5)
    q = n.astype(I32)
    odd = (q & 1) == 1
    s, c = jnp.where(odd, c, s), jnp.where(odd, s, c)
    return jnp.where((q & 2) == 2, -s, s), jnp.where(((q + 1) & 2) == 2, -c, c)


def _zip(x):
    return jnp.concatenate(
        [pltpu.pack_elementwise([x[i:i + 8], x[i + 8:i + 16]], packed_dtype=BF16)
         for i in range(0, x.shape[0], 16)], axis=0)


def _unzip(words, s):
    return pltpu.bitcast(words & np.uint32(0xFFFF0000) if s else words << 16, F32)


def _bf(words):
    return pltpu.bitcast(words, BF16)


def _layernorm(load):
    def mean(term, every):
        acc = [term(load(i)) for i in range(4)]
        for i in range(4, D // 8):
            acc[i % 4] = acc[i % 4] + term(load(i))
            if i % every == every - 1:
                yield
        tot = jnp.sum((acc[0] + acc[1]) + (acc[2] + acc[3]), axis=0, keepdims=True)
        return jnp.broadcast_to(tot * (1.0 / D), (8, T1))

    mu = yield from mean(lambda x: x, 32)
    var = yield from mean(lambda x: (x - mu) * (x - mu), 10)
    rs = jax.lax.rsqrt(var + 1e-5)
    return lambda i: jnp.concatenate([(load(2 * i + s) - mu) * rs for s in range(2)], axis=0)


def _items(n):
    return lambda fn: lambda *args: (fn(*args), n)


def _interleave(*lists, lead=0.0, span=1.0):
    gens = [(v for g, _ in w for v in g) for w in lists]
    sizes = [sum(n for _, n in w) for w in lists]
    for _, k in sorted((i / n if k else i / n * span - lead, k)
                       for k, n in enumerate(sizes) for i in range(n)):
        next(gens[k])
    for g in gens:
        for _ in g:
            pass


def _strassen_lhs(a11, a12, a21, a22):
    return a11 + a22, a22, a21 + a22, a11 + a12, a11, a12 - a22, a21 - a11


def _strassen_rhs(b11, b12, b21, b22):
    return b11 + b22, b21 - b11, b11, b22, b12 - b22, b21 + b22, b11 + b12


def _strassen(prod, emit):
    m4 = prod(1)
    yield
    m2 = prod(2)
    emit(1, 0, m2 + m4)
    yield
    m1 = prod(0)
    c11, c22 = m1 + m4, m1 - m2
    yield
    c11 = c11 + prod(5)
    yield
    m5 = prod(3)
    emit(0, 0, c11 - m5)
    yield
    m3 = prod(4)
    emit(0, 1, m3 + m5)
    c22 = c22 + m3
    yield
    emit(1, 1, c22 + prod(6))
    yield


def _rows(i, n):
    return slice(i * n, i * n + n)


def _alternate(i):
    return pl.ds(16 * (i // 2) + i % 2, 8, stride=2)


def _kernel(u_hbm, are_hbm, aim_hbm, bre_hbm, bim_hbm, cre_hbm, cim_hbm, ldt_hbm, dsk_hbm, wqkv_hbm, wo_hbm, f_hbm, out_hbm,
            are, aim, bre, bim, cre, cim, ldt, dsk, io, wq_in, wo_in, fm, ws, wp, lam, dtc, k0s, tab, ztab, kb, kf,
            xr, xn, kv, xq, qs, oe, oo, ob, zs, sems):
    cp_u = [pltpu.make_async_copy(u_hbm.bitcast(U32).at[:, h, :], io.at[h], sems.at[3 + h])
            for h in range(PH // 2)]
    cp_o = [pltpu.make_async_copy(io.at[h], out_hbm.bitcast(U32).at[:, h, :], sems.at[3 + h])
            for h in range(PH // 2)]
    cp_f, cp_g = [pltpu.make_async_copy(f_hbm.at[_rows(i, PH)], fm.at[_rows(i, PH)], sems.at[0])
                  for i in range(2)]
    cp_wq = pltpu.make_async_copy(wqkv_hbm, wq_in, sems.at[1])
    cp_wo = pltpu.make_async_copy(wo_hbm, wo_in, sems.at[2])
    cp_p = [pltpu.make_async_copy(src, dst, sems.at[3 + PH // 2 + i]) for i, (src, dst) in enumerate(
        ((ldt_hbm, ldt), (dsk_hbm, dsk), (aim_hbm, aim), (are_hbm, are), (bre_hbm, bre), (bim_hbm, bim), (cre_hbm, cre),
         (cim_hbm, cim)))]
    for cp in cp_p:
        cp.start()

    lane = jax.lax.broadcasted_iota(I32, (8, T1), 1)
    zs[0] = 0

    def region(*lists, **pace):
        pl.when(zs[0] == 0)(lambda: _interleave(*lists, **pace))

    cp_p[0].wait()
    cp_p[1].wait()
    dt_row = jnp.exp(ldt[...].astype(F32).reshape(1, D)).astype(BF16).astype(F32)
    ds_row = dsk[...].astype(F32).reshape(1, D)
    for j in range(4):
        dtc[0, _rows(j, 128), :] = jnp.broadcast_to(dt_row[:, _rows(j, 128)], (128, 128)).T
        dtc[1, _rows(j, 128), :] = jnp.broadcast_to(ds_row[:, _rows(j, 128)], (128, 128)).T
    cp_p[2].wait()
    cp_p[3].wait()
    cp_u[0].start()
    cp_u[1].start()
    big = None
    for j in range(D // 16):
        r = _rows(j, 16)
        theta = dtc[0, r, :] * aim[r, :].astype(F32)
        mag = jnp.exp(dtc[0, r, :] * are[r, :].astype(F32))
        sn, cs = _sincos(theta)
        lam[0, r, :] = mag * cs
        lam[1, r, :] = mag * sn
        big = jnp.abs(theta) if big is None else jnp.maximum(big, jnp.abs(theta))

    @pl.when(jnp.logical_not(jnp.max(big) <= 8192.0))
    def _():
        def body(i, _):
            rows = pl.ds(pl.multiple_of(i * 16, 16), 16)
            th = dtc[0, rows, :] * aim[rows, :].astype(F32)
            mg = jnp.exp(dtc[0, rows, :] * are[rows, :].astype(F32))
            lam[0, rows, :] = mg * jnp.cos(th)
            lam[1, rows, :] = mg * jnp.sin(th)
        jax.lax.fori_loop(0, D // 16, body, None)

    for cp in cp_p[4:]:
        cp.wait()

    @_items(15)
    def tap_tables(blk, e, s):
        rows = pl.ds(CB * blk + 16 * e + s, 8, stride=2)

        def part(ref):
            return _unzip(pltpu.bitcast(ref[_rows(4 * blk + e, 16), :], U32), s)

        sc = dtc[0, rows, :] * (2.0 / L)
        w = _cmul((part(cre), part(cim)), (part(bre) * sc, part(bim) * sc))
        k0s[rows, :] = w[0]

        def put(row, a, b):
            for z in range(2):
                tab[blk % 4, 2 * s + z, pl.ds(row, 8, stride=QS), :] = pltpu.pack_elementwise(
                    [a[z], b[z]], packed_dtype=BF16)

        l1 = (lam[0, rows, :], lam[1, rows, :])
        l2 = _csq(l1)
        l16 = _csq(_csq(_csq(l2)))
        m1 = (l16[0], -l16[1])
        a, b = _cmul(w, l1), _cmul(w, l2)
        put(16 * e, (jnp.ones_like(m1[0]), jnp.zeros_like(m1[0])), m1)

        def columns(j, c):
            d = _cmul(c, m1)
            put(16 * e + j, c, d)
            yield c
            if j < 8:
                yield from columns(2 * j, _csq(c))
                yield from columns(2 * j + 1, _csq(d))

        keep = {}
        for j, c in enumerate(columns(1, _csq(m1)), 1):
            if j == 4:
                l512 = _csq((c[0], -c[1]))
            if j <= 8:
                put(64 + 12 * e + j - 1, a, b)
                keep[2 * j] = b
            if j < 8:
                a, b = _cmul(a, l2), _cmul(b, l2)
            if j == 8:
                put(64 + 12 * e + 8, _cmul(keep[4], l512), _cmul(keep[12], l512))
                a, b = keep[8], keep[16]
            if j in (10, 12, 14):
                a, b = _cmul(a, l512), _cmul(b, l512)
                put(64 + 12 * e + 4 + j // 2, a, b)
            yield

    @_items(48)
    def tap_sums(blk):
        for i in range(8):
            d = [jax.lax.dot_general(_bf(tab[blk % 4, z, pl.ds(QS * i + 64, 48), :]),
                                     _bf(tab[blk % 4, z, pl.ds(QS * i, 64), :]),
                                     NT, preferred_element_type=F32) for z in range(4)]
            own = [None] * 3
            for n in range(12):
                e, r = n // 3, _rows(n, 8)
                v = pltpu.pack_elementwise([d[0][r] + d[1][r], d[2][r] + d[3][r]],
                                           packed_dtype=BF16)
                own[n % 3] = jnp.where(lane < 32 * e, own[n % 3], v) if e else v
                if n % 2:
                    yield
            for r in range(3):
                ztab[blk % 4, pl.ds(ZS * i + 8 * r, 8), :] = own[r]

    @_items(2)
    def tap_blocks(blk, e):
        def at(r, g):
            z = ztab[blk % 4, pl.ds(r, 8, stride=ZS), :]
            return z if g == e else pltpu.roll(z, (32 * (g - e)) % 128, 1)

        def full(r, r1):
            return jnp.where(lane < 64, jnp.where(lane < 32, at(r, 0), at(r1, 1)),
                             jnp.where(lane < 96, at(r1 + 2, 2), at(r1 + 4, 3)))

        halves = [pl.ds(CB * blk + 16 * e + s, 8, stride=2) for s in range(2)]
        e8, e16 = full(7, 18), full(15, 19)
        k0 = pltpu.pack_elementwise(
            [jnp.sum(k0s[r, :], axis=1, keepdims=True) + dtc[1, r, :] * (2.0 / L) for r in halves],
            packed_dtype=BF16)
        e0 = jnp.where(lane == 0, k0, pltpu.roll(e16, 1, 1))
        e4 = jnp.where(lane < 32, at(3, 0), at(16, 1))
        e12 = jnp.where(lane < 32, at(11, 0), at(17, 1))
        k4, k12 = jnp.where(lane < 64, e4, e0), jnp.where(lane < 64, e12, e16)
        far = {1: e0, 2: e0, 3: k4, 5: jnp.where(lane < 64, e4, e8), 6: e8, 7: e8, 9: e8,
               10: e8, 11: jnp.where(lane < 64, e12, e8), 13: k12, 14: e16, 15: e16}
        taps = {0: e0, 4: k4, 8: e8, 12: k12}
        yield
        for p in range(PH):
            kb[p, _rows(4 * blk + e, 8), :] = taps[p] if p in taps else jnp.where(
                lane < (16 if p % 2 else 32), at(p - 1, 0), far[p])
        yield

    @_items(CB // 2)
    def lane_dft(src, lo, hi):
        for q in range(8):
            x0, x1 = [jax.lax.dot_general(_bf(src[p, lo // 2:hi // 2, :]), _bf(fm[p]), NN,
                                          preferred_element_type=F32) for p in (q, q + 8)]
            for i in range((hi - lo) // 8):
                r = _rows(i, 8)
                for c, v in ((q, x0[r] + x1[r]), (q + 8, x0[r] - x1[r])):
                    for z in range(2):
                        kv[0, 2 * c + z, _rows(lo // 8 + i, 8), :] = v[:, _rows(z, T1)]
                if i % 2:
                    yield

    def residues(r, odd):
        return [(kv[0, 2 * c, r, :], kv[0, 2 * c + 1, r, :]) for c in range(8 * odd, 8 * odd + 8)]

    @_items(CB // 4)
    def tap_coefs(blk):
        for i in range(CB // 8):
            r = _rows(blk * CB // 8 + i, 8)
            for odd in range(2):
                for n, v in enumerate(_conv_coefs(residues(r, odd), 4 * odd)):
                    kf[10 * odd + n, r, :T1] = v[0]
                    kf[10 * odd + n, r, T1:] = v[1]
                yield

    r0 = jax.lax.broadcasted_iota(I32, (128, 128), 0)
    ri = (r0 & ~15) + (r0 & 7) * 2 + ((r0 >> 3) & 1)
    ci = jax.lax.broadcasted_iota(I32, (128, 128), 1)
    hit = ci == (ri & 7) * 16 + (ri >> 3)

    @_items(14)
    def prep_weights(j):
        def block(c, k):
            if j < 6:
                sel = jnp.where(hit, 1.0 if j < 4 else 0.25, 0.0)
                w = wq_in[_rows(k, 128), _rows(c, 128)]
            else:
                sel = jnp.where(ri == ci, 1.0, 0.0)
                w = _bf(wp[_rows(k, 64), _rows(c, 128)])
            return jax.lax.dot_general(sel.astype(BF16), w, NT, preferred_element_type=F32)

        top, bot = (4 + j, 8 + j) if j < 4 else (j % 2, j % 2 + 2)
        for k in range(2):
            for i, a in enumerate(_strassen_lhs(block(top, k), block(top, k + 2),
                                                block(bot, k), block(bot, k + 2))):
                ws[i, _rows(j, 64), _rows(k, 128)] = _zip(a)
                yield

    @_items(8)
    def permute_wo(j):
        sel = jnp.where(ci == (r0 & 7) * 16 + (r0 >> 3), 1.0, 0.0).astype(BF16)
        wp[_rows(j, 64), :] = _zip(jnp.dot(sel, wo_in[_rows(j, 128), :],
                                           preferred_element_type=F32))
        yield from range(8)

    @_items(4)
    def load_pair(h):
        for j in range(4):
            wds = io[h, :, _rows(j, 128)].T
            for s in range(2):
                xr[2 * h + s, _rows(j, 128), :] = _unzip(wds, s)
            yield

    @_items(24)
    def norm(h):
        for p in (2 * h, 2 * h + 1):
            normed = yield from _layernorm(lambda i: xr[p, _alternate(i), :])
            for i in range(D // 16):
                xn[p, _rows(i, 8), :] = _zip(normed(i))
                if i % 8 == 7:
                    yield

    for i, step in enumerate(PROLOGUE):
        tables, sums, blocks, dft, coefs, loads, norms, perms, preps = [
            range(a, b) for a, b in zip(PROLOGUE[i - 1] if i else (0,) * 9, step)]
        for cp in {0: [cp_f], 1: cp_u[2:5], 2: cp_u[5:], 3: [cp_wo, cp_wq], 5: [cp_g]}.get(i, ()):
            cp.start()
        for cp, users in ((cp_f, dft), (cp_wo, perms), (cp_wq, preps)):
            if 0 in users:
                cp.wait()
        for h in loads:
            cp_u[h].wait()
        region([tap_sums(b) for b in sums]
               + [lane_dft(kb, CB * b, CB * b + CB) for b in dft]
               + [permute_wo(j) for j in perms] + [prep_weights(j) for j in preps],
               [tap_tables(b, e, s) for b in tables for e in range(4) for s in range(2)]
               + [norm(h) for h in norms],
               [tap_blocks(b, e) for b in blocks for e in range(4)],
               [tap_coefs(b) for b in coefs],
               [load_pair(h) for h in loads],
               lead={3: 0.03, 5: -0.03, 7: -0.03}.get(i, 0.0),
               span={1: 0.95, 2: 1.05, 4: 1.05, 6: 0.95}.get(i, 1.0))

    cp_g.wait()

    @_items(10)
    def phase_conv(i):
        r = _rows(i, 8)
        coefs = ((kf[n, r, :T1], kf[n, r, T1:]) for n in range(NCOEF))
        for odd in range(2):
            y = yield from _conv(residues(r, odd), 4 * odd, lambda: next(coefs))
            for c, v in enumerate(y):
                for z in range(2):
                    kv[1, 16 * odd + 2 * c + z, r, :] = v[z]
            yield

    @_items(32)
    def lane_idft(lo, hi):
        for q in (0, 2, 4, 6, 1, 3, 5, 7):
            a, b = [jnp.concatenate([kv[1, 2 * c + z, lo:hi, :] for z in range(2)], axis=1)
                    for c in (q, q + 8)]
            for p, v in ((q, a + b), (q + 8, a - b)):
                inv = jnp.concatenate([fm[PH + p, :, :T1], fm[PH + p, :, T1:]], axis=0)
                d = jax.lax.dot_general(v, _bf(inv), NN, preferred_element_type=F32)
                yield
                xr[p, lo:hi, :] += d
                yield

    @_items(32)
    def norm_pair(g):
        p = 4 * (g % 4) + g // 4
        a = yield from _layernorm(lambda i: xr[p, _alternate(i), :])
        b = yield from _layernorm(lambda i: xr[p + 2, _alternate(i), :])
        for r in range(HD // 16):
            for i, v in enumerate(_strassen_rhs(a(r), b(r), a(HD // 16 + r), b(HD // 16 + r))):
                xq[g, _rows(r, 8), _rows(i, T1)] = _zip(v)
            yield

    def block_product(row0, groups, rhs, emit):
        for r in [128 // RS * hg + i for hg in groups for i in range(128 // RS)]:
            w = slice((row0 + r * RS) // 2, (row0 + r * RS + RS) // 2)
            yield from _strassen(
                lambda i: jnp.dot(_bf(ws[i, w, :]), _bf(rhs[:, _rows(i, T1)]),
                                  preferred_element_type=F32),
                lambda half, n, y: emit(half, n, r * RS, y))

    @_items(7 * HD // RS)
    def keys_values(s, g):
        def emit(half, n, row, y):
            m = 2 * (g % 4) + n
            kv[g // 4, PH * half + WIN - 1 + m, pl.ds(row, RS), :] = y
            if m:
                kv[g // 4, PH * half + m - 1, pl.ds(row, RS), :] = pltpu.roll(y, 1, 1)

        return block_product(0, (s, s + 2), xq.at[g], emit)

    @_items(7 * 128 // RS)
    def queries(s, g):
        def emit(half, n, row, y):
            qs[g, n, pl.ds(HD * half + row, RS), :] = y

        return block_product(D, (s,), xq.at[g], emit)

    @_items(34)
    def attend(par, s, m):
        for hg in (s, s + 2):
            lg = [None] * WIN
            for j0 in range(0, WIN, JB):
                for dh in range(16):
                    r = _rows(16 * hg + dh, 8)
                    q = qs[4 * par + m // 2, m % 2, r, :]
                    for j in range(j0, j0 + JB):
                        t = q * kv[par, WIN - 1 + m - j, r, :]
                        lg[j] = t if dh == 0 else lg[j] + t
                    if (dh + 1) % (16 // JB) == 0:
                        yield
            for j in range(m + 1, WIN):
                lg[j] = jnp.where(lane == 0, -1e9, lg[j])
            mx = lg[0]
            for j in range(1, WIN):
                mx = jnp.maximum(mx, lg[j])
            ex = [jnp.exp(t - mx) for t in lg]
            den = ex[0]
            for j in range(1, WIN):
                den = den + ex[j]
            inv = pltpu.reciprocal(den, full_range=False)
            pr = [t * inv for t in ex]
            yield

            def out(dh):
                r = _rows(16 * hg + dh, 8)
                acc = pr[0] * kv[par, PH + WIN - 1 + m, r, :]
                for j in range(1, WIN):
                    acc = acc + pr[j] * kv[par, PH + WIN - 1 + m - j, r, :]
                return acc

            for d2 in range(8):
                o = jnp.concatenate([out(2 * d2), out(2 * d2 + 1)], axis=0)
                r = _rows(8 * hg + d2, 16)
                if par == 0 or hg < 2:
                    (oe, oo)[par][m, r, :] = o
                if hg >= 2:
                    r1 = _rows(8 * (hg - 2) + d2, 16)
                    ops = (_strassen_rhs(oe[m, r1, :], oo[m, r1, :], oe[m, r, :], o) if par
                           else _strassen_rhs(oe[m, r1, :], o, o, o))
                    for i in (0, 3, 4, 5, 6) if par else (1, 2):
                        ob[m, _rows(8 * (hg - 2) + d2, 8), _rows(i, T1)] = _zip(ops[i])
                yield

    late = (1, 4, 6, 7)

    @_items(7 * HD // RS)
    def project(h):
        def emit(half, n, row, y):
            xr[2 * h + n, pl.ds(HD * half + row, RS), :] += y

        for s in range(2):
            yield from block_product(D + HD, (s,), ob.at[h], emit)
            if h not in late:
                for _ in store_pair(h, (s, s + 2))[0]:
                    pass

    @_items(4)
    def store_pair(h, groups):
        for j in groups:
            io[h, :, _rows(j, 128)] = pltpu.pack_elementwise(
                [xr[2 * h + n, _rows(j, 128), :] for n in range(2)], packed_dtype=BF16).T
            yield

    def layer(it, c):
        def send(hs):
            @pl.when(it == 1)
            def _():
                for h in hs:
                    cp_o[h].start()

        cuts = (0, 0) + EDGES + (D, D)
        for i in range(len(cuts) - 3):
            (i0, i1), (c0, c1), (f0, f1) = [cuts[i + k:i + k + 2] for k in range(3)]
            last = i0 < i1 == D
            region([lane_dft(xn, c, c + CB) for c in range(f0, f1, CB)]
                   + [lane_idft(c, c + CB) for c in range(i0, i1, CB)],
                   [phase_conv(r) for r in range(c0 // 8, c1 // 8)]
                   + ([norm(7)] if i == 0 else []) + ([norm_pair(0)] if last else []),
                   lead=0.4 if last else 0.0, span={0: 1.5, 4: 0.95}.get(i, 1.0))
        region([keys_values(0, 0), keys_values(1, 0), queries(0, 0)],
               [norm_pair(g) for g in (1, 2, 3)])
        region([fn(0, g) for fn in (keys_values, queries) for g in (1, 2, 3)],
               [norm_pair(g) for g in (4, 5, 6, 7)])
        for par, s, kvg, qg in ((0, 0, (1, 2, 3), (0, 1, 2, 3)), (0, 1, (4, 5, 6, 7), (4, 5, 6, 7)),
                                (1, 0, (4, 5, 6, 7), (4, 5))):
            region([keys_values(1 - s, g) for g in kvg] + [queries(1 - s, g) for g in qg],
                   [attend(par, s, m) for m in range(WIN)], span=1.05)
        region([queries(1, g) for g in (6, 7)], [attend(1, 1, m) for m in (0, 1)], span=0.95)
        done = ()
        for hs, ms in (((0, 1), (2, 3, 4)), ((2, 3, 4), (5, 6, 7)), ((5, 6), ()), ((7,), ())):
            region([project(h) for h in hs],
                   [store_pair(h, range(4)) for h in done if h in late]
                   + [norm(h) for h in done] + [attend(1, 1, m) for m in ms],
                   span={0: 0.95, 5: 1.05}.get(hs[0], 1.0))
            send([h for h in done if h in late] + [h for h in hs if h not in late])
            done = hs

    jax.lax.fori_loop(0, 2, layer, None)
    _interleave([store_pair(7, range(4))])
    cp_o[7].start()
    for cp in cp_o:
        cp.wait()


@jax.jit
def pallas_interleave_layers__ssm_conv_s4__sliding_local_dilated__prompt_kernel(
    A_u: jax.Array,
    A_A_re: jax.Array,
    A_A_im: jax.Array,
    A_B_re: jax.Array,
    A_B_im: jax.Array,
    A_C_re: jax.Array,
    A_C_im: jax.Array,
    A_log_dt: jax.Array,
    A_Dskip: jax.Array,
    B_x: jax.Array,
    B_wqkv: jax.Array,
    B_wo: jax.Array,
):
    del B_x
    hbm = pl.BlockSpec(memory_space=pl.ANY)
    out = pl.pallas_call(
        _kernel,
        in_specs=[hbm] * 12,
        out_specs=hbm,
        out_shape=jax.ShapeDtypeStruct((T1, PH, D), BF16),
        scratch_shapes=[pltpu.VMEM((D, NS), BF16)] * 6 + [pltpu.VMEM((D,), BF16)] * 2 + [
            pltpu.VMEM((PH // 2, T1, D), U32),
            pltpu.VMEM((D, 3 * D), BF16),
            pltpu.VMEM((D, D), BF16),
            pltpu.VMEM((2 * PH, T1 // 2, 2 * T1), U32),
            pltpu.VMEM((7, D, HD), U32),
            pltpu.VMEM((D // 2, D), U32),
            pltpu.VMEM((2, D + 8, NS), F32),
            pltpu.VMEM((2, D + 8, NS), F32),
            pltpu.VMEM((D + 8, NS), F32),
            pltpu.VMEM((4, 4, 9 * QS + 4, NS), U32),
            pltpu.VMEM((4, 9 * ZS + 4, T1), U32),
            pltpu.VMEM((PH, D // 2, T1), U32),
            pltpu.VMEM((NCOEF, D, 2 * T1), F32),
            pltpu.VMEM((PH, D + 8, T1), F32),
            pltpu.VMEM((PH, D // 2, T1), U32),
            pltpu.VMEM((2, 2 * PH, D, T1), F32),
            pltpu.VMEM((PH // 2, HD // 2, 7 * T1), U32),
            pltpu.VMEM((PH // 2, 2, D, T1), F32),
            pltpu.VMEM((WIN, D, T1), F32),
            pltpu.VMEM((WIN, HD, T1), F32),
            pltpu.VMEM((WIN, HD // 2, 7 * T1), U32),
            pltpu.SMEM((1,), I32),
            pltpu.SemaphoreType.DMA((11 + PH // 2,)),
        ],
        compiler_params=pltpu.CompilerParams(vmem_limit_bytes=100 * 1024 * 1024),
    )(A_u.reshape(T1, PH, D), A_A_re, A_A_im, A_B_re, A_B_im, A_C_re, A_C_im,
      A_log_dt, A_Dskip, B_wqkv, B_wo,
      _dft_matrices())
    return out.reshape(1, L, D)
```

```python
import numpy as np

import jax
import jax.numpy as jnp
import jax.experimental.pallas as pl
import jax.experimental.pallas.tpu as pltpu

F32, BF16, U32, I32 = jnp.float32, jnp.bfloat16, jnp.uint32, jnp.int32
L, D, NS = 2048, 512, 128
PH, T1 = 16, 128
WIN = 8
NN = (((1,), (0,)), ((), ()))
NT = (((1,), (1,)), ((), ()))
QS = 116
ZS = 28
_H = float(np.sqrt(0.5))
NCOEF = 22
HD = D // 2
RS = 64
JB = 4
EDGES = (0, 64, 192, 320, 448, D)
PROLOGUE = ((1, 0, 0, 0, 0, 0, 0, 0, 0),
            (3, 1, 0, 0, 0, 1, 0, 0, 0),
            (5, 3, 1, 0, 0, 2, 0, 0, 0),
            (7, 5, 3, 1, 0, 5, 0, 0, 0),
            (8, 7, 5, 3, 1, 8, 1, 0, 0),
            (8, 8, 7, 5, 3, 8, 4, 4, 0),
            (8, 8, 8, 7, 5, 8, 6, 4, 4),
            (8, 8, 8, 8, 8, 8, 7, 4, 8))
CB = 64


def _dft_matrices():
    t = 16 * np.arange(T1)[None, :, None] + np.arange(PH)[:, None, None]
    k = np.arange(T1)[None, None, :] + 0.5
    phi = 2.0 * np.pi * k * t / (2 * L)
    phi = np.concatenate([phi, phi.transpose(0, 2, 1)])
    f = np.concatenate([np.cos(phi), -np.sin(phi)], axis=-1).astype(np.float32)
    bits = f.astype(BF16).view(np.uint16).astype(np.uint32)
    return bits[:, 0::2] | (bits[:, 1::2] << 16)


def _cmul(a, b):
    return a[0] * b[0] - a[1] * b[1], a[0] * b[1] + a[1] * b[0]


def _csq(a):
    t = a[0] * a[1]
    return a[0] * a[0] - a[1] * a[1], t + t


def _cadd(a, b):
    return a[0] + b[0], a[1] + b[1]


def _csub(a, b):
    return a[0] - b[0], a[1] - b[1]


def _rot8(x, e):
    s, d = x[0] + x[1], x[0] - x[1]
    return {1: (d * _H, s * _H), 3: (s * -_H, d * _H), 5: (d * -_H, s * -_H), 7: (s * _H, d * -_H)}[e]


def _split(x, e):
    n = len(x) // 2
    lo, hi = x[:n], x[n:]
    if e == 4:
        return ([(a[0] - b[1], a[1] + b[0]) for a, b in zip(lo, hi)],
                [(a[0] + b[1], a[1] - b[0]) for a, b in zip(lo, hi)])
    if e:
        hi = [_rot8(b, e // 2) for b in hi]
    return [_cadd(a, b) for a, b in zip(lo, hi)], [_csub(a, b) for a, b in zip(lo, hi)]


def _merge(p, m, e):
    lo = [_cadd(a, b) for a, b in zip(p, m)]
    if e == 4:
        return lo + [(a[1] - b[1], b[0] - a[0]) for a, b in zip(p, m)]
    hi = [_csub(a, b) for a, b in zip(p, m)]
    return lo + ([_rot8(b, 8 - e // 2) for b in hi] if e else hi)


def _conv_coefs(k, e):
    if len(k) == 1:
        return [(k[0][0] * 0.5, k[0][1] * 0.5)]
    if len(k) == 2 and e % 4:
        if e % 2:
            top = _csub(_rot8(k[1], e), k[0])
        elif e == 2:
            top = (-k[1][1] - k[0][0], k[1][0] - k[0][1])
        else:
            top = (k[1][1] - k[0][0], -k[1][0] - k[0][1])
        return [k[0], top, _csub(k[1], k[0])]
    p, m = _split(k, e)
    return _conv_coefs(p, e // 2) + _conv_coefs(m, e // 2 + 4)


def _conv(x, e, coef):
    if len(x) == 1:
        return [_cmul(x[0], coef())]
    if len(x) == 2:
        yield
    if len(x) == 2 and e % 4:
        both = _cmul(_cadd(x[0], x[1]), coef())
        return [_cadd(both, _cmul(x[1], coef())), _cadd(both, _cmul(x[0], coef()))]
    p, m = _split(x, e)
    p = yield from _conv(p, e // 2, coef)
    m = yield from _conv(m, e // 2 + 4, coef)
    return _merge(p, m, e)


def _sincos(x):
    n = jnp.floor(x * float(2.0 / np.pi) + 0.5)
    r = ((x - n * 1.5703125) - n * 4.837512969970703125e-4) - n * 7.54978995489188216e-8
    z = r * r
    s = r + r * z * ((-1.9515295891e-4 * z + 8.3321608736e-3) * z - 1.6666654611e-1)
    c = 1.0 + z * (((2.443315711809948e-5 * z - 1.388731625493765e-3) * z
                    + 4.166664568298827e-2) * z - 0.5)
    q = n.astype(I32)
    odd = (q & 1) == 1
    s, c = jnp.where(odd, c, s), jnp.where(odd, s, c)
    return jnp.where((q & 2) == 2, -s, s), jnp.where(((q + 1) & 2) == 2, -c, c)


def _zip(x):
    return jnp.concatenate(
        [pltpu.pack_elementwise([x[i:i + 8], x[i + 8:i + 16]], packed_dtype=BF16)
         for i in range(0, x.shape[0], 16)], axis=0)


def _unzip(words, s):
    return pltpu.bitcast(words & np.uint32(0xFFFF0000) if s else words << 16, F32)


def _bf(words):
    return pltpu.bitcast(words, BF16)


def _layernorm(load):
    def mean(term, every):
        acc = [term(load(i)) for i in range(4)]
        for i in range(4, D // 8):
            acc[i % 4] = acc[i % 4] + term(load(i))
            if i % every == every - 1:
                yield
        tot = jnp.sum((acc[0] + acc[1]) + (acc[2] + acc[3]), axis=0, keepdims=True)
        return jnp.broadcast_to(tot * (1.0 / D), (8, T1))

    mu = yield from mean(lambda x: x, 32)
    var = yield from mean(lambda x: (x - mu) * (x - mu), 10)
    rs = jax.lax.rsqrt(var + 1e-5)
    return lambda i: jnp.concatenate([(load(2 * i + s) - mu) * rs for s in range(2)], axis=0)


def _items(n):
    return lambda fn: lambda *args: (fn(*args), n)


def _interleave(*lists, lead=0.0, span=1.0):
    gens = [(v for g, _ in w for v in g) for w in lists]
    sizes = [sum(n for _, n in w) for w in lists]
    for _, k in sorted((i / n if k else i / n * span - lead, k)
                       for k, n in enumerate(sizes) for i in range(n)):
        next(gens[k])
    for g in gens:
        for _ in g:
            pass


def _strassen_lhs(a11, a12, a21, a22):
    return a11 + a22, a22, a21 + a22, a11 + a12, a11, a12 - a22, a21 - a11


def _strassen_rhs(b11, b12, b21, b22):
    return b11 + b22, b21 - b11, b11, b22, b12 - b22, b21 + b22, b11 + b12


def _strassen(prod, emit):
    m4 = prod(1)
    yield
    m2 = prod(2)
    emit(1, 0, m2 + m4)
    yield
    m1 = prod(0)
    c11, c22 = m1 + m4, m1 - m2
    yield
    c11 = c11 + prod(5)
    yield
    m5 = prod(3)
    emit(0, 0, c11 - m5)
    yield
    m3 = prod(4)
    emit(0, 1, m3 + m5)
    c22 = c22 + m3
    yield
    emit(1, 1, c22 + prod(6))
    yield


def _rows(i, n):
    return slice(i * n, i * n + n)


def _alternate(i):
    return pl.ds(16 * (i // 2) + i % 2, 8, stride=2)


def _kernel(u_hbm, are_hbm, aim_hbm, bre_hbm, bim_hbm, cre_hbm, cim_hbm, ldt_hbm, dsk_hbm, wqkv_hbm, wo_hbm, f_hbm, out_hbm,
            are, aim, bre, bim, cre, cim, ldt, dsk, io, wq_in, wo_in, fm, ws, wp, lam, dtc, k0s, tab, ztab, kb, kf,
            xr, xn, kv, xq, qs, oe, oo, ob, zs, sems):
    cp_u = [pltpu.make_async_copy(u_hbm.bitcast(U32).at[:, h, :], io.at[h], sems.at[3 + h])
            for h in range(PH // 2)]
    cp_o = [pltpu.make_async_copy(io.at[h], out_hbm.bitcast(U32).at[:, h, :], sems.at[3 + h])
            for h in range(PH // 2)]
    cp_f, cp_g = [pltpu.make_async_copy(f_hbm.at[_rows(i, PH)], fm.at[_rows(i, PH)], sems.at[0])
                  for i in range(2)]
    cp_wq = pltpu.make_async_copy(wqkv_hbm, wq_in, sems.at[1])
    cp_wo = pltpu.make_async_copy(wo_hbm, wo_in, sems.at[2])
    cp_p = [pltpu.make_async_copy(src, dst, sems.at[3 + PH // 2 + i]) for i, (src, dst) in enumerate(
        ((ldt_hbm, ldt), (dsk_hbm, dsk), (aim_hbm, aim), (are_hbm, are), (bre_hbm, bre), (bim_hbm, bim), (cre_hbm, cre),
         (cim_hbm, cim)))]
    for cp in cp_p:
        cp.start()

    lane = jax.lax.broadcasted_iota(I32, (8, T1), 1)
    zs[0] = 0

    def region(*lists, **pace):
        pl.when(zs[0] == 0)(lambda: _interleave(*lists, **pace))

    cp_p[0].wait()
    cp_p[1].wait()
    dt_row = jnp.exp(ldt[...].astype(F32).reshape(1, D)).astype(BF16).astype(F32)
    ds_row = dsk[...].astype(F32).reshape(1, D)
    for j in range(4):
        dtc[0, _rows(j, 128), :] = jnp.broadcast_to(dt_row[:, _rows(j, 128)], (128, 128)).T
        dtc[1, _rows(j, 128), :] = jnp.broadcast_to(ds_row[:, _rows(j, 128)], (128, 128)).T
    cp_p[2].wait()
    cp_p[3].wait()
    cp_u[0].start()
    cp_u[1].start()
    big = None
    for j in range(D // 16):
        r = _rows(j, 16)
        theta = dtc[0, r, :] * aim[r, :].astype(F32)
        mag = jnp.exp(dtc[0, r, :] * are[r, :].astype(F32))
        sn, cs = _sincos(theta)
        lam[0, r, :] = mag * cs
        lam[1, r, :] = mag * sn
        big = jnp.abs(theta) if big is None else jnp.maximum(big, jnp.abs(theta))

    @pl.when(jnp.logical_not(jnp.max(big) <= 8192.0))
    def _():
        def body(i, _):
            rows = pl.ds(pl.multiple_of(i * 16, 16), 16)
            th = dtc[0, rows, :] * aim[rows, :].astype(F32)
            mg = jnp.exp(dtc[0, rows, :] * are[rows, :].astype(F32))
            lam[0, rows, :] = mg * jnp.cos(th)
            lam[1, rows, :] = mg * jnp.sin(th)
        jax.lax.fori_loop(0, D // 16, body, None)

    for cp in cp_p[4:]:
        cp.wait()

    @_items(15)
    def tap_tables(blk, e, s):
        rows = pl.ds(CB * blk + 16 * e + s, 8, stride=2)

        def part(ref):
            return _unzip(pltpu.bitcast(ref[_rows(4 * blk + e, 16), :], U32), s)

        sc = dtc[0, rows, :] * (2.0 / L)
        w = _cmul((part(cre), part(cim)), (part(bre) * sc, part(bim) * sc))
        k0s[rows, :] = w[0]

        def put(row, a, b):
            for z in range(2):
                tab[blk % 4, 2 * s + z, pl.ds(row, 8, stride=QS), :] = pltpu.pack_elementwise(
                    [a[z], b[z]], packed_dtype=BF16)

        l1 = (lam[0, rows, :], lam[1, rows, :])
        l2 = _csq(l1)
        l16 = _csq(_csq(_csq(l2)))
        m1 = (l16[0], -l16[1])
        a, b = _cmul(w, l1), _cmul(w, l2)
        put(16 * e, (jnp.ones_like(m1[0]), jnp.zeros_like(m1[0])), m1)

        def columns(j, c):
            d = _cmul(c, m1)
            put(16 * e + j, c, d)
            yield c
            if j < 8:
                yield from columns(2 * j, _csq(c))
                yield from columns(2 * j + 1, _csq(d))

        keep = {}
        for j, c in enumerate(columns(1, _csq(m1)), 1):
            if j == 4:
                l512 = _csq((c[0], -c[1]))
            if j <= 8:
                put(64 + 12 * e + j - 1, a, b)
                keep[2 * j] = b
            if j < 8:
                a, b = _cmul(a, l2), _cmul(b, l2)
            if j == 8:
                put(64 + 12 * e + 8, _cmul(keep[4], l512), _cmul(keep[12], l512))
                a, b = keep[8], keep[16]
            if j in (10, 12, 14):
                a, b = _cmul(a, l512), _cmul(b, l512)
                put(64 + 12 * e + 4 + j // 2, a, b)
            yield

    @_items(48)
    def tap_sums(blk):
        for i in range(8):
            d = [jax.lax.dot_general(_bf(tab[blk % 4, z, pl.ds(QS * i + 64, 48), :]),
                                     _bf(tab[blk % 4, z, pl.ds(QS * i, 64), :]),
                                     NT, preferred_element_type=F32) for z in range(4)]
            own = [None] * 3
            for n in range(12):
                e, r = n // 3, _rows(n, 8)
                v = pltpu.pack_elementwise([d[0][r] + d[1][r], d[2][r] + d[3][r]],
                                           packed_dtype=BF16)
                own[n % 3] = jnp.where(lane < 32 * e, own[n % 3], v) if e else v
                if n % 2:
                    yield
            for r in range(3):
                ztab[blk % 4, pl.ds(ZS * i + 8 * r, 8), :] = own[r]

    @_items(2)
    def tap_blocks(blk, e):
        def at(r, g):
            z = ztab[blk % 4, pl.ds(r, 8, stride=ZS), :]
            return z if g == e else pltpu.roll(z, (32 * (g - e)) % 128, 1)

        def full(r, r1):
            return jnp.where(lane < 64, jnp.where(lane < 32, at(r, 0), at(r1, 1)),
                             jnp.where(lane < 96, at(r1 + 2, 2), at(r1 + 4, 3)))

        halves = [pl.ds(CB * blk + 16 * e + s, 8, stride=2) for s in range(2)]
        e8, e16 = full(7, 18), full(15, 19)
        k0 = pltpu.pack_elementwise(
            [jnp.sum(k0s[r, :], axis=1, keepdims=True) + dtc[1, r, :] * (2.0 / L) for r in halves],
            packed_dtype=BF16)
        e0 = jnp.where(lane == 0, k0, pltpu.roll(e16, 1, 1))
        e4 = jnp.where(lane < 32, at(3, 0), at(16, 1))
        e12 = jnp.where(lane < 32, at(11, 0), at(17, 1))
        k4, k12 = jnp.where(lane < 64, e4, e0), jnp.where(lane < 64, e12, e16)
        far = {1: e0, 2: e0, 3: k4, 5: jnp.where(lane < 64, e4, e8), 6: e8, 7: e8, 9: e8,
               10: e8, 11: jnp.where(lane < 64, e12, e8), 13: k12, 14: e16, 15: e16}
        taps = {0: e0, 4: k4, 8: e8, 12: k12}
        yield
        for p in range(PH):
            kb[p, _rows(4 * blk + e, 8), :] = taps[p] if p in taps else jnp.where(
                lane < (16 if p % 2 else 32), at(p - 1, 0), far[p])
        yield

    @_items(CB // 2)
    def lane_dft(src, lo, hi):
        for q in range(8):
            x0, x1 = [jax.lax.dot_general(_bf(src[p, lo // 2:hi // 2, :]), _bf(fm[p]), NN,
                                          preferred_element_type=F32) for p in (q, q + 8)]
            for i in range((hi - lo) // 8):
                r = _rows(i, 8)
                for c, v in ((q, x0[r] + x1[r]), (q + 8, x0[r] - x1[r])):
                    for z in range(2):
                        kv[0, 2 * c + z, _rows(lo // 8 + i, 8), :] = v[:, _rows(z, T1)]
                if i % 2:
                    yield

    def residues(r, odd):
        return [(kv[0, 2 * c, r, :], kv[0, 2 * c + 1, r, :]) for c in range(8 * odd, 8 * odd + 8)]

    @_items(CB // 4)
    def tap_coefs(blk):
        for i in range(CB // 8):
            r = _rows(blk * CB // 8 + i, 8)
            for odd in range(2):
                for n, v in enumerate(_conv_coefs(residues(r, odd), 4 * odd)):
                    kf[10 * odd + n, r, :T1] = v[0]
                    kf[10 * odd + n, r, T1:] = v[1]
                yield

    r0 = jax.lax.broadcasted_iota(I32, (128, 128), 0)
    ri = (r0 & ~15) + (r0 & 7) * 2 + ((r0 >> 3) & 1)
    ci = jax.lax.broadcasted_iota(I32, (128, 128), 1)
    hit = ci == (ri & 7) * 16 + (ri >> 3)

    @_items(14)
    def prep_weights(j):
        def block(c, k):
            if j < 6:
                sel = jnp.where(hit, 1.0 if j < 4 else 0.25, 0.0)
                w = wq_in[_rows(k, 128), _rows(c, 128)]
            else:
                sel = jnp.where(ri == ci, 1.0, 0.0)
                w = _bf(wp[_rows(k, 64), _rows(c, 128)])
            return jax.lax.dot_general(sel.astype(BF16), w, NT, preferred_element_type=F32)

        top, bot = (4 + j, 8 + j) if j < 4 else (j % 2, j % 2 + 2)
        for k in range(2):
            for i, a in enumerate(_strassen_lhs(block(top, k), block(top, k + 2),
                                                block(bot, k), block(bot, k + 2))):
                ws[i, _rows(j, 64), _rows(k, 128)] = _zip(a)
                yield

    @_items(8)
    def permute_wo(j):
        sel = jnp.where(ci == (r0 & 7) * 16 + (r0 >> 3), 1.0, 0.0).astype(BF16)
        wp[_rows(j, 64), :] = _zip(jnp.dot(sel, wo_in[_rows(j, 128), :],
                                           preferred_element_type=F32))
        yield from range(8)

    @_items(4)
    def load_pair(h):
        for j in range(4):
            wds = io[h, :, _rows(j, 128)].T
            for s in range(2):
                xr[2 * h + s, _rows(j, 128), :] = _unzip(wds, s)
            yield

    @_items(24)
    def norm(h):
        for p in (2 * h, 2 * h + 1):
            normed = yield from _layernorm(lambda i: xr[p, _alternate(i), :])
            for i in range(D // 16):
                xn[p, _rows(i, 8), :] = _zip(normed(i))
                if i % 8 == 7:
                    yield

    for i, step in enumerate(PROLOGUE):
        tables, sums, blocks, dft, coefs, loads, norms, perms, preps = [
            range(a, b) for a, b in zip(PROLOGUE[i - 1] if i else (0,) * 9, step)]
        for cp in {0: [cp_f], 1: cp_u[2:5], 2: cp_u[5:], 3: [cp_wo, cp_wq], 5: [cp_g]}.get(i, ()):
            cp.start()
        for cp, users in ((cp_f, dft), (cp_wo, perms), (cp_wq, preps)):
            if 0 in users:
                cp.wait()
        for h in loads:
            cp_u[h].wait()
        region([tap_sums(b) for b in sums]
               + [lane_dft(kb, CB * b, CB * b + CB) for b in dft]
               + [permute_wo(j) for j in perms] + [prep_weights(j) for j in preps],
               [tap_tables(b, e, s) for b in tables for e in range(4) for s in range(2)]
               + [norm(h) for h in norms],
               [tap_blocks(b, e) for b in blocks for e in range(4)],
               [tap_coefs(b) for b in coefs],
               [load_pair(h) for h in loads],
               lead={3: 0.03, 4: 0.03, 5: 0.03, 7: -0.03}.get(i, 0.0),
               span={3: 1.0, 4: 1.0, 5: 1.1}.get(i, 1.05))

    cp_g.wait()

    @_items(10)
    def phase_conv(i):
        r = _rows(i, 8)
        coefs = ((kf[n, r, :T1], kf[n, r, T1:]) for n in range(NCOEF))
        for odd in range(2):
            y = yield from _conv(residues(r, odd), 4 * odd, lambda: next(coefs))
            for c, v in enumerate(y):
                for z in range(2):
                    kv[1, 16 * odd + 2 * c + z, r, :] = v[z]
            yield

    @_items(32)
    def lane_idft(lo, hi):
        for q in (0, 2, 4, 6, 1, 3, 5, 7):
            a, b = [jnp.concatenate([kv[1, 2 * c + z, lo:hi, :] for z in range(2)], axis=1)
                    for c in (q, q + 8)]
            for p, v in ((q, a + b), (q + 8, a - b)):
                inv = jnp.concatenate([fm[PH + p, :, :T1], fm[PH + p, :, T1:]], axis=0)
                d = jax.lax.dot_general(v, _bf(inv), NN, preferred_element_type=F32)
                yield
                xr[p, lo:hi, :] += d
                yield

    @_items(32)
    def norm_pair(g):
        p = 4 * (g % 4) + g // 4
        a = yield from _layernorm(lambda i: xr[p, _alternate(i), :])
        b = yield from _layernorm(lambda i: xr[p + 2, _alternate(i), :])
        for r in range(HD // 16):
            for i, v in enumerate(_strassen_rhs(a(r), b(r), a(HD // 16 + r), b(HD // 16 + r))):
                xq[g, _rows(r, 8), _rows(i, T1)] = _zip(v)
            yield

    def block_product(row0, groups, rhs, emit):
        for r in [128 // RS * hg + i for hg in groups for i in range(128 // RS)]:
            w = slice((row0 + r * RS) // 2, (row0 + r * RS + RS) // 2)
            yield from _strassen(
                lambda i: jnp.dot(_bf(ws[i, w, :]), _bf(rhs[:, _rows(i, T1)]),
                                  preferred_element_type=F32),
                lambda half, n, y: emit(half, n, r * RS, y))

    @_items(7 * HD // RS)
    def keys_values(s, g):
        def emit(half, n, row, y):
            m = 2 * (g % 4) + n
            kv[g // 4, PH * half + WIN - 1 + m, pl.ds(row, RS), :] = y
            if m:
                kv[g // 4, PH * half + m - 1, pl.ds(row, RS), :] = pltpu.roll(y, 1, 1)

        return block_product(0, (s, s + 2), xq.at[g], emit)

    @_items(7 * 128 // RS)
    def queries(s, g):
        def emit(half, n, row, y):
            qs[g, n, pl.ds(HD * half + row, RS), :] = y

        return block_product(D, (s,), xq.at[g], emit)

    @_items(34)
    def attend(par, s, m):
        for hg in (s, s + 2):
            lg = [None] * WIN
            for j0 in range(0, WIN, JB):
                for dh in range(16):
                    r = _rows(16 * hg + dh, 8)
                    q = qs[4 * par + m // 2, m % 2, r, :]
                    for j in range(j0, j0 + JB):
                        t = q * kv[par, WIN - 1 + m - j, r, :]
                        lg[j] = t if dh == 0 else lg[j] + t
                    if (dh + 1) % (16 // JB) == 0:
                        yield
            for j in range(m + 1, WIN):
                lg[j] = jnp.where(lane == 0, -1e9, lg[j])
            mx = lg[0]
            for j in range(1, WIN):
                mx = jnp.maximum(mx, lg[j])
            ex = [jnp.exp(t - mx) for t in lg]
            den = ex[0]
            for j in range(1, WIN):
                den = den + ex[j]
            inv = pltpu.reciprocal(den, full_range=False)
            pr = [t * inv for t in ex]
            yield

            def out(dh):
                r = _rows(16 * hg + dh, 8)
                acc = pr[0] * kv[par, PH + WIN - 1 + m, r, :]
                for j in range(1, WIN):
                    acc = acc + pr[j] * kv[par, PH + WIN - 1 + m - j, r, :]
                return acc

            for d2 in range(8):
                o = jnp.concatenate([out(2 * d2), out(2 * d2 + 1)], axis=0)
                r = _rows(8 * hg + d2, 16)
                if par == 0 or hg < 2:
                    (oe, oo)[par][m, r, :] = o
                if hg >= 2:
                    r1 = _rows(8 * (hg - 2) + d2, 16)
                    ops = (_strassen_rhs(oe[m, r1, :], oo[m, r1, :], oe[m, r, :], o) if par
                           else _strassen_rhs(oe[m, r1, :], o, o, o))
                    for i in (0, 3, 4, 5, 6) if par else (1, 2):
                        ob[m, _rows(8 * (hg - 2) + d2, 8), _rows(i, T1)] = _zip(ops[i])
                yield

    late = (1, 4, 6, 7)

    @_items(7 * HD // RS)
    def project(h):
        def emit(half, n, row, y):
            xr[2 * h + n, pl.ds(HD * half + row, RS), :] += y

        for s in range(2):
            yield from block_product(D + HD, (s,), ob.at[h], emit)
            if h not in late:
                for _ in store_pair(h, (s, s + 2))[0]:
                    pass

    @_items(4)
    def store_pair(h, groups):
        for j in groups:
            io[h, :, _rows(j, 128)] = pltpu.pack_elementwise(
                [xr[2 * h + n, _rows(j, 128), :] for n in range(2)], packed_dtype=BF16).T
            yield

    def layer(it, c):
        def send(hs):
            @pl.when(it == 1)
            def _():
                for h in hs:
                    cp_o[h].start()

        cuts = (0, 0) + EDGES + (D, D)
        for i in range(len(cuts) - 3):
            (i0, i1), (c0, c1), (f0, f1) = [cuts[i + k:i + k + 2] for k in range(3)]
            last = i0 < i1 == D
            region([lane_dft(xn, c, c + CB) for c in range(f0, f1, CB)]
                   + [lane_idft(c, c + CB) for c in range(i0, i1, CB)],
                   [phase_conv(r) for r in range(c0 // 8, c1 // 8)]
                   + ([norm(7)] if i == 0 else []) + ([norm_pair(0)] if last else []),
                   lead=0.4 if last else 0.0, span={0: 1.5, 4: 0.95}.get(i, 1.0))
        region([keys_values(0, 0), keys_values(1, 0), queries(0, 0)],
               [norm_pair(g) for g in (1, 2, 3)])
        region([fn(0, g) for fn in (keys_values, queries) for g in (1, 2, 3)],
               [norm_pair(g) for g in (4, 5, 6, 7)])
        for par, s, kvg, qg in ((0, 0, (1, 2, 3), (0, 1, 2, 3)), (0, 1, (4, 5, 6, 7), (4, 5, 6, 7)),
                                (1, 0, (4, 5, 6, 7), (4, 5))):
            region([keys_values(1 - s, g) for g in kvg] + [queries(1 - s, g) for g in qg],
                   [attend(par, s, m) for m in range(WIN)], span=1.05)
        region([queries(1, g) for g in (6, 7)], [attend(1, 1, m) for m in (0, 1)], span=0.95)
        done = ()
        for hs, ms in (((0, 1), (2, 3, 4)), ((2, 3, 4), (5, 6, 7)), ((5, 6), ()), ((7,), ())):
            region([project(h) for h in hs],
                   [store_pair(h, range(4)) for h in done if h in late]
                   + [norm(h) for h in done] + [attend(1, 1, m) for m in ms],
                   span={0: 0.95, 5: 1.05}.get(hs[0], 1.0))
            send([h for h in done if h in late] + [h for h in hs if h not in late])
            done = hs

    jax.lax.fori_loop(0, 2, layer, None)
    _interleave([store_pair(7, range(4))])
    cp_o[7].start()
    for cp in cp_o:
        cp.wait()


@jax.jit
def pallas_interleave_layers__ssm_conv_s4__sliding_local_dilated__prompt_kernel(
    A_u: jax.Array,
    A_A_re: jax.Array,
    A_A_im: jax.Array,
    A_B_re: jax.Array,
    A_B_im: jax.Array,
    A_C_re: jax.Array,
    A_C_im: jax.Array,
    A_log_dt: jax.Array,
    A_Dskip: jax.Array,
    B_x: jax.Array,
    B_wqkv: jax.Array,
    B_wo: jax.Array,
):
    del B_x
    hbm = pl.BlockSpec(memory_space=pl.ANY)
    out = pl.pallas_call(
        _kernel,
        in_specs=[hbm] * 12,
        out_specs=hbm,
        out_shape=jax.ShapeDtypeStruct((T1, PH, D), BF16),
        scratch_shapes=[pltpu.VMEM((D, NS), BF16)] * 6 + [pltpu.VMEM((D,), BF16)] * 2 + [
            pltpu.VMEM((PH // 2, T1, D), U32),
            pltpu.VMEM((D, 3 * D), BF16),
            pltpu.VMEM((D, D), BF16),
            pltpu.VMEM((2 * PH, T1 // 2, 2 * T1), U32),
            pltpu.VMEM((7, D, HD), U32),
            pltpu.VMEM((D // 2, D), U32),
            pltpu.VMEM((2, D + 8, NS), F32),
            pltpu.VMEM((2, D + 8, NS), F32),
            pltpu.VMEM((D + 8, NS), F32),
            pltpu.VMEM((4, 4, 9 * QS + 4, NS), U32),
            pltpu.VMEM((4, 9 * ZS + 4, T1), U32),
            pltpu.VMEM((PH, D // 2, T1), U32),
            pltpu.VMEM((NCOEF, D, 2 * T1), F32),
            pltpu.VMEM((PH, D + 8, T1), F32),
            pltpu.VMEM((PH, D // 2, T1), U32),
            pltpu.VMEM((2, 2 * PH, D, T1), F32),
            pltpu.VMEM((PH // 2, HD // 2, 7 * T1), U32),
            pltpu.VMEM((PH // 2, 2, D, T1), F32),
            pltpu.VMEM((WIN, D, T1), F32),
            pltpu.VMEM((WIN, HD, T1), F32),
            pltpu.VMEM((WIN, HD // 2, 7 * T1), U32),
            pltpu.SMEM((1,), I32),
            pltpu.SemaphoreType.DMA((11 + PH // 2,)),
        ],
        compiler_params=pltpu.CompilerParams(vmem_limit_bytes=100 * 1024 * 1024),
    )(A_u.reshape(T1, PH, D), A_A_re, A_A_im, A_B_re, A_B_im, A_C_re, A_C_im,
      A_log_dt, A_Dskip, B_wqkv, B_wo,
      _dft_matrices())
    return out.reshape(1, L, D)
```

```python
import numpy as np

import jax
import jax.numpy as jnp
import jax.experimental.pallas as pl
import jax.experimental.pallas.tpu as pltpu

F32, BF16, U32, I32 = jnp.float32, jnp.bfloat16, jnp.uint32, jnp.int32
L, D, NS = 2048, 512, 128
PH, T1 = 16, 128
WIN = 8
NN = (((1,), (0,)), ((), ()))
NT = (((1,), (1,)), ((), ()))
QS = 116
ZS = 28
_H = float(np.sqrt(0.5))
NCOEF = 22
HD = D // 2
RS = 64
JB = 4
EDGES = (0, 64, 192, 320, 448, D)
PROLOGUE = ((1, 0, 0, 0, 0, 0, 0, 0, 0),
            (3, 1, 0, 0, 0, 1, 0, 0, 0),
            (5, 3, 1, 0, 0, 2, 0, 0, 0),
            (7, 5, 3, 1, 0, 5, 0, 0, 0),
            (8, 7, 5, 3, 1, 8, 2, 0, 0),
            (8, 8, 7, 5, 3, 8, 5, 4, 0),
            (8, 8, 8, 7, 5, 8, 8, 4, 4),
            (8, 8, 8, 8, 8, 8, 8, 4, 8))
CB = 64


def _dft_matrices():
    t = 16 * np.arange(T1)[None, :, None] + np.arange(PH)[:, None, None]
    k = np.arange(T1)[None, None, :] + 0.5
    phi = 2.0 * np.pi * k * t / (2 * L)
    phi = np.concatenate([phi, phi.transpose(0, 2, 1)])
    f = np.concatenate([np.cos(phi), -np.sin(phi)], axis=-1).astype(np.float32)
    bits = f.astype(BF16).view(np.uint16).astype(np.uint32)
    return bits[:, 0::2] | (bits[:, 1::2] << 16)


def _cmul(a, b):
    return a[0] * b[0] - a[1] * b[1], a[0] * b[1] + a[1] * b[0]


def _csq(a):
    t = a[0] * a[1]
    return a[0] * a[0] - a[1] * a[1], t + t


def _cadd(a, b):
    return a[0] + b[0], a[1] + b[1]


def _csub(a, b):
    return a[0] - b[0], a[1] - b[1]


def _rot8(x, e):
    s, d = x[0] + x[1], x[0] - x[1]
    return {1: (d * _H, s * _H), 3: (s * -_H, d * _H), 5: (d * -_H, s * -_H), 7: (s * _H, d * -_H)}[e]


def _split(x, e):
    n = len(x) // 2
    lo, hi = x[:n], x[n:]
    if e == 4:
        return ([(a[0] - b[1], a[1] + b[0]) for a, b in zip(lo, hi)],
                [(a[0] + b[1], a[1] - b[0]) for a, b in zip(lo, hi)])
    if e:
        hi = [_rot8(b, e // 2) for b in hi]
    return [_cadd(a, b) for a, b in zip(lo, hi)], [_csub(a, b) for a, b in zip(lo, hi)]


def _merge(p, m, e):
    lo = [_cadd(a, b) for a, b in zip(p, m)]
    if e == 4:
        return lo + [(a[1] - b[1], b[0] - a[0]) for a, b in zip(p, m)]
    hi = [_csub(a, b) for a, b in zip(p, m)]
    return lo + ([_rot8(b, 8 - e // 2) for b in hi] if e else hi)


def _conv_coefs(k, e):
    if len(k) == 1:
        return [(k[0][0] * 0.5, k[0][1] * 0.5)]
    if len(k) == 2 and e % 4:
        if e % 2:
            top = _csub(_rot8(k[1], e), k[0])
        elif e == 2:
            top = (-k[1][1] - k[0][0], k[1][0] - k[0][1])
        else:
            top = (k[1][1] - k[0][0], -k[1][0] - k[0][1])
        return [k[0], top, _csub(k[1], k[0])]
    p, m = _split(k, e)
    return _conv_coefs(p, e // 2) + _conv_coefs(m, e // 2 + 4)


def _conv(x, e, coef):
    if len(x) == 1:
        return [_cmul(x[0], coef())]
    if len(x) == 2:
        yield
    if len(x) == 2 and e % 4:
        both = _cmul(_cadd(x[0], x[1]), coef())
        return [_cadd(both, _cmul(x[1], coef())), _cadd(both, _cmul(x[0], coef()))]
    p, m = _split(x, e)
    p = yield from _conv(p, e // 2, coef)
    m = yield from _conv(m, e // 2 + 4, coef)
    return _merge(p, m, e)


def _sincos(x):
    n = jnp.floor(x * float(2.0 / np.pi) + 0.5)
    r = ((x - n * 1.5703125) - n * 4.837512969970703125e-4) - n * 7.54978995489188216e-8
    z = r * r
    s = r + r * z * ((-1.9515295891e-4 * z + 8.3321608736e-3) * z - 1.6666654611e-1)
    c = 1.0 + z * (((2.443315711809948e-5 * z - 1.388731625493765e-3) * z
                    + 4.166664568298827e-2) * z - 0.5)
    q = n.astype(I32)
    odd = (q & 1) == 1
    s, c = jnp.where(odd, c, s), jnp.where(odd, s, c)
    return jnp.where((q & 2) == 2, -s, s), jnp.where(((q + 1) & 2) == 2, -c, c)


def _zip(x):
    return jnp.concatenate(
        [pltpu.pack_elementwise([x[i:i + 8], x[i + 8:i + 16]], packed_dtype=BF16)
         for i in range(0, x.shape[0], 16)], axis=0)


def _unzip(words, s):
    return pltpu.bitcast(words & np.uint32(0xFFFF0000) if s else words << 16, F32)


def _bf(words):
    return pltpu.bitcast(words, BF16)


def _layernorm(load):
    def mean(term, every):
        acc = [term(load(i)) for i in range(4)]
        for i in range(4, D // 8):
            acc[i % 4] = acc[i % 4] + term(load(i))
            if i % every == every - 1:
                yield
        tot = jnp.sum((acc[0] + acc[1]) + (acc[2] + acc[3]), axis=0, keepdims=True)
        return jnp.broadcast_to(tot * (1.0 / D), (8, T1))

    mu = yield from mean(lambda x: x, 32)
    var = yield from mean(lambda x: (x - mu) * (x - mu), 10)
    rs = jax.lax.rsqrt(var + 1e-5)
    return lambda i: jnp.concatenate([(load(2 * i + s) - mu) * rs for s in range(2)], axis=0)


def _items(n):
    return lambda fn: lambda *args: (fn(*args), n)


def _interleave(*lists, lead=0.0, span=1.0):
    gens = [(v for g, _ in w for v in g) for w in lists]
    sizes = [sum(n for _, n in w) for w in lists]
    for _, k in sorted((i / n if k else i / n * span - lead, k)
                       for k, n in enumerate(sizes) for i in range(n)):
        next(gens[k])
    for g in gens:
        for _ in g:
            pass


def _strassen_lhs(a11, a12, a21, a22):
    return a11 + a22, a22, a21 + a22, a11 + a12, a11, a12 - a22, a21 - a11


def _strassen_rhs(b11, b12, b21, b22):
    return b11 + b22, b21 - b11, b11, b22, b12 - b22, b21 + b22, b11 + b12


def _strassen(prod, emit):
    m4 = prod(1)
    yield
    m2 = prod(2)
    emit(1, 0, m2 + m4)
    yield
    m1 = prod(0)
    c11, c22 = m1 + m4, m1 - m2
    yield
    c11 = c11 + prod(5)
    yield
    m5 = prod(3)
    emit(0, 0, c11 - m5)
    yield
    m3 = prod(4)
    emit(0, 1, m3 + m5)
    c22 = c22 + m3
    yield
    emit(1, 1, c22 + prod(6))
    yield


def _rows(i, n):
    return slice(i * n, i * n + n)


def _alternate(i):
    return pl.ds(16 * (i // 2) + i % 2, 8, stride=2)


def _kernel(u_hbm, are_hbm, aim_hbm, bre_hbm, bim_hbm, cre_hbm, cim_hbm, ldt_hbm, dsk_hbm,
            wqkv_hbm, wo_hbm, f_hbm, out_hbm,
            are, aim, bre, bim, cre, cim, ldt, dsk, io, wq_in, wo_in, fm, ws, wp, lam, dtc, k0s,
            tab, ztab, kb, kf, xr, xn, kv, xq, qs, oe, oo, ob, zs, sems):
    cp_u = [pltpu.make_async_copy(u_hbm.bitcast(U32).at[:, h, :], io.at[h], sems.at[3 + h])
            for h in range(PH // 2)]
    cp_o = [pltpu.make_async_copy(io.at[h], out_hbm.bitcast(U32).at[:, h, :], sems.at[3 + h])
            for h in range(PH // 2)]
    cp_f, cp_g = [pltpu.make_async_copy(f_hbm.at[_rows(i, PH)], fm.at[_rows(i, PH)], sems.at[0])
                  for i in range(2)]
    cp_wq = pltpu.make_async_copy(wqkv_hbm, wq_in, sems.at[1])
    cp_wo = pltpu.make_async_copy(wo_hbm, wo_in, sems.at[2])
    cp_p = [pltpu.make_async_copy(src, dst, sems.at[3 + PH // 2 + i])
            for i, (src, dst) in enumerate(
                ((ldt_hbm, ldt), (dsk_hbm, dsk), (aim_hbm, aim), (are_hbm, are),
                 (bre_hbm, bre), (bim_hbm, bim), (cre_hbm, cre), (cim_hbm, cim)))]
    for cp in cp_p:
        cp.start()

    lane = jax.lax.broadcasted_iota(I32, (8, T1), 1)
    zs[0] = 0

    def region(*lists, **pace):
        pl.when(zs[0] == 0)(lambda: _interleave(*lists, **pace))

    cp_p[0].wait()
    cp_p[1].wait()
    dt_row = jnp.exp(ldt[...].astype(F32).reshape(1, D)).astype(BF16).astype(F32)
    ds_row = dsk[...].astype(F32).reshape(1, D)
    for j in range(4):
        dtc[0, _rows(j, 128), :] = jnp.broadcast_to(dt_row[:, _rows(j, 128)], (128, 128)).T
        dtc[1, _rows(j, 128), :] = jnp.broadcast_to(ds_row[:, _rows(j, 128)], (128, 128)).T
    cp_p[2].wait()
    cp_p[3].wait()
    cp_u[0].start()
    cp_u[1].start()
    big = None
    for j in range(D // 16):
        r = _rows(j, 16)
        theta = dtc[0, r, :] * aim[r, :].astype(F32)
        mag = jnp.exp(dtc[0, r, :] * are[r, :].astype(F32))
        sn, cs = _sincos(theta)
        lam[0, r, :] = mag * cs
        lam[1, r, :] = mag * sn
        big = jnp.abs(theta) if big is None else jnp.maximum(big, jnp.abs(theta))

    @pl.when(jnp.logical_not(jnp.max(big) <= 8192.0))
    def _():
        def body(i, _):
            rows = pl.ds(pl.multiple_of(i * 16, 16), 16)
            th = dtc[0, rows, :] * aim[rows, :].astype(F32)
            mg = jnp.exp(dtc[0, rows, :] * are[rows, :].astype(F32))
            lam[0, rows, :] = mg * jnp.cos(th)
            lam[1, rows, :] = mg * jnp.sin(th)
        jax.lax.fori_loop(0, D // 16, body, None)

    for cp in cp_p[4:]:
        cp.wait()

    @_items(15)
    def tap_tables(blk, e, s):
        rows = pl.ds(CB * blk + 16 * e + s, 8, stride=2)

        def part(ref):
            return _unzip(pltpu.bitcast(ref[_rows(4 * blk + e, 16), :], U32), s)

        sc = dtc[0, rows, :] * (2.0 / L)
        w = _cmul((part(cre), part(cim)), (part(bre) * sc, part(bim) * sc))
        k0s[rows, :] = w[0]

        def put(row, a, b):
            for z in range(2):
                tab[blk % 4, 2 * s + z, pl.ds(row, 8, stride=QS), :] = pltpu.pack_elementwise(
                    [a[z], b[z]], packed_dtype=BF16)

        l1 = (lam[0, rows, :], lam[1, rows, :])
        l2 = _csq(l1)
        l16 = _csq(_csq(_csq(l2)))
        m1 = (l16[0], -l16[1])
        a, b = _cmul(w, l1), _cmul(w, l2)
        put(16 * e, (jnp.ones_like(m1[0]), jnp.zeros_like(m1[0])), m1)

        def columns(j, c):
            d = _cmul(c, m1)
            put(16 * e + j, c, d)
            yield c
            if j < 8:
                yield from columns(2 * j, _csq(c))
                yield from columns(2 * j + 1, _csq(d))

        keep = {}
        for j, c in enumerate(columns(1, _csq(m1)), 1):
            if j == 4:
                l512 = _csq((c[0], -c[1]))
            if j <= 8:
                put(64 + 12 * e + j - 1, a, b)
                keep[2 * j] = b
            if j < 8:
                a, b = _cmul(a, l2), _cmul(b, l2)
            if j == 8:
                put(64 + 12 * e + 8, _cmul(keep[4], l512), _cmul(keep[12], l512))
                a, b = keep[8], keep[16]
            if j in (10, 12, 14):
                a, b = _cmul(a, l512), _cmul(b, l512)
                put(64 + 12 * e + 4 + j // 2, a, b)
            yield

    @_items(48)
    def tap_sums(blk):
        for i in range(8):
            d = [jax.lax.dot_general(_bf(tab[blk % 4, z, pl.ds(QS * i + 64, 48), :]),
                                     _bf(tab[blk % 4, z, pl.ds(QS * i, 64), :]),
                                     NT, preferred_element_type=F32) for z in range(4)]
            own = [None] * 3
            for n in range(12):
                e, r = n // 3, _rows(n, 8)
                v = pltpu.pack_elementwise([d[0][r] + d[1][r], d[2][r] + d[3][r]],
                                           packed_dtype=BF16)
                own[n % 3] = jnp.where(lane < 32 * e, own[n % 3], v) if e else v
                if n % 2:
                    yield
            for r in range(3):
                ztab[blk % 4, pl.ds(ZS * i + 8 * r, 8), :] = own[r]

    @_items(2)
    def tap_blocks(blk, e):
        def at(r, g):
            z = ztab[blk % 4, pl.ds(r, 8, stride=ZS), :]
            return z if g == e else pltpu.roll(z, (32 * (g - e)) % 128, 1)

        def full(r, r1):
            return jnp.where(lane < 64, jnp.where(lane < 32, at(r, 0), at(r1, 1)),
                             jnp.where(lane < 96, at(r1 + 2, 2), at(r1 + 4, 3)))

        halves = [pl.ds(CB * blk + 16 * e + s, 8, stride=2) for s in range(2)]
        e8, e16 = full(7, 18), full(15, 19)
        k0 = pltpu.pack_elementwise(
            [jnp.sum(k0s[r, :], axis=1, keepdims=True) + dtc[1, r, :] * (2.0 / L) for r in halves],
            packed_dtype=BF16)
        e0 = jnp.where(lane == 0, k0, pltpu.roll(e16, 1, 1))
        e4 = jnp.where(lane < 32, at(3, 0), at(16, 1))
        e12 = jnp.where(lane < 32, at(11, 0), at(17, 1))
        k4, k12 = jnp.where(lane < 64, e4, e0), jnp.where(lane < 64, e12, e16)
        far = {1: e0, 2: e0, 3: k4, 5: jnp.where(lane < 64, e4, e8), 6: e8, 7: e8, 9: e8,
               10: e8, 11: jnp.where(lane < 64, e12, e8), 13: k12, 14: e16, 15: e16}
        taps = {0: e0, 4: k4, 8: e8, 12: k12}
        yield
        for p in range(PH):
            kb[p, _rows(4 * blk + e, 8), :] = taps[p] if p in taps else jnp.where(
                lane < (16 if p % 2 else 32), at(p - 1, 0), far[p])
        yield

    @_items(CB // 2)
    def lane_dft(src, lo, hi):
        for q in range(8):
            x0, x1 = [jax.lax.dot_general(_bf(src[p, lo // 2:hi // 2, :]), _bf(fm[p]), NN,
                                          preferred_element_type=F32) for p in (q, q + 8)]
            for i in range((hi - lo) // 8):
                r = _rows(i, 8)
                for c, v in ((q, x0[r] + x1[r]), (q + 8, x0[r] - x1[r])):
                    for z in range(2):
                        kv[0, 2 * c + z, _rows(lo // 8 + i, 8), :] = v[:, _rows(z, T1)]
                if i % 2:
                    yield

    def residues(r, odd):
        return [(kv[0, 2 * c, r, :], kv[0, 2 * c + 1, r, :]) for c in range(8 * odd, 8 * odd + 8)]

    @_items(CB // 4)
    def tap_coefs(blk):
        for i in range(CB // 8):
            r = _rows(blk * CB // 8 + i, 8)
            for odd in range(2):
                for n, v in enumerate(_conv_coefs(residues(r, odd), 4 * odd)):
                    kf[10 * odd + n, r, :T1] = v[0]
                    kf[10 * odd + n, r, T1:] = v[1]
                yield

    r0 = jax.lax.broadcasted_iota(I32, (128, 128), 0)
    ri = (r0 & ~15) + (r0 & 7) * 2 + ((r0 >> 3) & 1)
    ci = jax.lax.broadcasted_iota(I32, (128, 128), 1)
    hit = ci == (ri & 7) * 16 + (ri >> 3)

    @_items(14)
    def prep_weights(j):
        def block(c, k):
            if j < 6:
                sel = jnp.where(hit, 1.0 if j < 4 else 0.25, 0.0)
                w = wq_in[_rows(k, 128), _rows(c, 128)]
            else:
                sel = jnp.where(ri == ci, 1.0, 0.0)
                w = _bf(wp[_rows(k, 64), _rows(c, 128)])
            return jax.lax.dot_general(sel.astype(BF16), w, NT, preferred_element_type=F32)

        top, bot = (4 + j, 8 + j) if j < 4 else (j % 2, j % 2 + 2)
        for k in range(2):
            for i, a in enumerate(_strassen_lhs(block(top, k), block(top, k + 2),
                                                block(bot, k), block(bot, k + 2))):
                ws[i, _rows(j, 64), _rows(k, 128)] = _zip(a)
                yield

    @_items(8)
    def permute_wo(j):
        sel = jnp.where(ci == (r0 & 7) * 16 + (r0 >> 3), 1.0, 0.0).astype(BF16)
        wp[_rows(j, 64), :] = _zip(jnp.dot(sel, wo_in[_rows(j, 128), :],
                                           preferred_element_type=F32))
        yield from range(8)

    @_items(4)
    def load_pair(h):
        for j in range(4):
            wds = io[h, :, _rows(j, 128)].T
            for s in range(2):
                xr[2 * h + s, _rows(j, 128), :] = _unzip(wds, s)
            yield

    @_items(24)
    def norm(h):
        for p in (2 * h, 2 * h + 1):
            normed = yield from _layernorm(lambda i: xr[p, _alternate(i), :])
            for i in range(D // 16):
                xn[p, _rows(i, 8), :] = _zip(normed(i))
                if i % 8 == 7:
                    yield

    for i, step in enumerate(PROLOGUE):
        tables, sums, blocks, dft, coefs, loads, norms, perms, preps = [
            range(a, b) for a, b in zip(PROLOGUE[i - 1] if i else (0,) * 9, step)]
        for cp in {0: [cp_f], 1: cp_u[2:5], 2: cp_u[5:], 3: [cp_wo, cp_wq], 5: [cp_g]}.get(i, ()):
            cp.start()
        for cp, users in ((cp_f, dft), (cp_wo, perms), (cp_wq, preps)):
            if 0 in users:
                cp.wait()
        for h in loads:
            cp_u[h].wait()
        region([tap_sums(b) for b in sums]
               + [lane_dft(kb, CB * b, CB * b + CB) for b in dft]
               + [permute_wo(j) for j in perms] + [prep_weights(j) for j in preps]
               + ([lane_dft(xn, 0, CB)] if step is PROLOGUE[-1] else []),
               [tap_tables(b, e, s) for b in tables for e in range(4) for s in range(2)]
               + [norm(h) for h in norms],
               [tap_blocks(b, e) for b in blocks for e in range(4)],
               [tap_coefs(b) for b in coefs],
               [load_pair(h) for h in loads],
               lead={3: 0.03, 4: 0.03, 5: 0.03, 7: -0.03}.get(i, 0.0),
               span={3: 1.0, 4: 1.0, 5: 1.1}.get(i, 1.05))

    cp_g.wait()

    @_items(10)
    def phase_conv(i):
        r = _rows(i, 8)
        coefs = ((kf[n, r, :T1], kf[n, r, T1:]) for n in range(NCOEF))
        for odd in range(2):
            y = yield from _conv(residues(r, odd), 4 * odd, lambda: next(coefs))
            for c, v in enumerate(y):
                for z in range(2):
                    kv[1, 16 * odd + 2 * c + z, r, :] = v[z]
            yield

    @_items(32)
    def lane_idft(lo, hi):
        for q in (0, 2, 4, 6, 1, 3, 5, 7):
            a, b = [jnp.concatenate([kv[1, 2 * c + z, lo:hi, :] for z in range(2)], axis=1)
                    for c in (q, q + 8)]
            for p, v in ((q, a + b), (q + 8, a - b)):
                inv = jnp.concatenate([fm[PH + p, :, :T1], fm[PH + p, :, T1:]], axis=0)
                d = jax.lax.dot_general(v, _bf(inv), NN, preferred_element_type=F32)
                yield
                xr[p, lo:hi, :] += d
                yield

    @_items(32)
    def norm_pair(g):
        p = 4 * (g % 4) + g // 4
        a = yield from _layernorm(lambda i: xr[p, _alternate(i), :])
        b = yield from _layernorm(lambda i: xr[p + 2, _alternate(i), :])
        for r in range(HD // 16):
            for i, v in enumerate(_strassen_rhs(a(r), b(r), a(HD // 16 + r), b(HD // 16 + r))):
                xq[g, _rows(r, 8), _rows(i, T1)] = _zip(v)
            yield

    def block_product(row0, groups, rhs, emit):
        for r in [128 // RS * hg + i for hg in groups for i in range(128 // RS)]:
            w = slice((row0 + r * RS) // 2, (row0 + r * RS + RS) // 2)
            yield from _strassen(
                lambda i: jnp.dot(_bf(ws[i, w, :]), _bf(rhs[:, _rows(i, T1)]),
                                  preferred_element_type=F32),
                lambda half, n, y: emit(half, n, r * RS, y))

    @_items(7 * HD // RS)
    def keys_values(s, g):
        def emit(half, n, row, y):
            m = 2 * (g % 4) + n
            kv[g // 4, PH * half + WIN - 1 + m, pl.ds(row, RS), :] = y
            if m:
                kv[g // 4, PH * half + m - 1, pl.ds(row, RS), :] = pltpu.roll(y, 1, 1)

        return block_product(0, (s, s + 2), xq.at[g], emit)

    @_items(7 * 128 // RS)
    def queries(s, g):
        def emit(half, n, row, y):
            qs[g, n, pl.ds(HD * half + row, RS), :] = y

        return block_product(D, (s,), xq.at[g], emit)

    @_items(34)
    def attend(par, s, m):
        for hg in (s, s + 2):
            lg = [None] * WIN
            for j0 in range(0, WIN, JB):
                for dh in range(16):
                    r = _rows(16 * hg + dh, 8)
                    q = qs[4 * par + m // 2, m % 2, r, :]
                    for j in range(j0, j0 + JB):
                        t = q * kv[par, WIN - 1 + m - j, r, :]
                        lg[j] = t if dh == 0 else lg[j] + t
                    if (dh + 1) % (16 // JB) == 0:
                        yield
            for j in range(m + 1, WIN):
                lg[j] = jnp.where(lane == 0, -1e9, lg[j])
            mx = lg[0]
            for j in range(1, WIN):
                mx = jnp.maximum(mx, lg[j])
            ex = [jnp.exp(t - mx) for t in lg]
            den = ex[0]
            for j in range(1, WIN):
                den = den + ex[j]
            inv = pltpu.reciprocal(den, full_range=False)
            pr = [t * inv for t in ex]
            yield

            def out(dh):
                r = _rows(16 * hg + dh, 8)
                acc = pr[0] * kv[par, PH + WIN - 1 + m, r, :]
                for j in range(1, WIN):
                    acc = acc + pr[j] * kv[par, PH + WIN - 1 + m - j, r, :]
                return acc

            for d2 in range(8):
                o = jnp.concatenate([out(2 * d2), out(2 * d2 + 1)], axis=0)
                r = _rows(8 * hg + d2, 16)
                if par == 0 or hg < 2:
                    (oe, oo)[par][m, r, :] = o
                if hg >= 2:
                    r1 = _rows(8 * (hg - 2) + d2, 16)
                    ops = (_strassen_rhs(oe[m, r1, :], oo[m, r1, :], oe[m, r, :], o) if par
                           else _strassen_rhs(oe[m, r1, :], o, o, o))
                    for i in (0, 3, 4, 5, 6) if par else (1, 2):
                        ob[m, _rows(8 * (hg - 2) + d2, 8), _rows(i, T1)] = _zip(ops[i])
                yield

    late = (1, 4, 6)

    @_items(7 * HD // RS)
    def project(h, store):
        def emit(half, n, row, y):
            xr[2 * h + n, pl.ds(HD * half + row, RS), :] += y

        for s in range(2):
            yield from block_product(D + HD, (s,), ob.at[h], emit)
            if store:
                for _ in store_pair(h, (s, s + 2))[0]:
                    pass

    @_items(4)
    def store_pair(h, groups):
        for j in groups:
            io[h, :, _rows(j, 128)] = pltpu.pack_elementwise(
                [xr[2 * h + n, _rows(j, 128), :] for n in range(2)], packed_dtype=BF16).T
            yield

    def layer(it, c):
        def send(hs):
            @pl.when(it == 1)
            def _():
                for h in hs:
                    cp_o[h].start()

        cuts = (0, 0) + EDGES + (D, D)
        for i in range(1, len(cuts) - 3):
            (i0, i1), (c0, c1), (f0, f1) = [cuts[i + k:i + k + 2] for k in range(3)]
            last = i0 < i1 == D
            region([lane_dft(xn, c, c + CB) for c in range(f0, f1, CB)]
                   + [lane_idft(c, c + CB) for c in range(i0, i1, CB)],
                   [phase_conv(r) for r in range(c0 // 8, c1 // 8)]
                   + ([norm_pair(0)] if last else []),
                   lead=0.4 if last else 0.0, span=0.95 if i == 4 else 1.0)
        region([keys_values(0, 0), keys_values(1, 0), queries(0, 0)],
               [norm_pair(g) for g in (1, 2, 3)])
        region([fn(0, g) for fn in (keys_values, queries) for g in (1, 2, 3)],
               [norm_pair(g) for g in (4, 5, 6, 7)])
        for par, s, kvg, qg in ((0, 0, (1, 2, 3), (0, 1, 2, 3)), (0, 1, (4, 5, 6, 7), (4, 5, 6, 7)),
                                (1, 0, (4, 5, 6, 7), (4, 5))):
            region([keys_values(1 - s, g) for g in kvg] + [queries(1 - s, g) for g in qg],
                   [attend(par, s, m) for m in range(WIN)], span=1.05)
        region([queries(1, g) for g in (6, 7)], [attend(1, 1, m) for m in (0, 1)], span=0.95)
        done = ()
        for hs, ms in (((0, 1), (2, 3, 4)), ((2, 3, 4), (5, 6, 7)), ((5, 6), ())):
            region([project(h, h not in late) for h in hs],
                   [store_pair(h, range(4)) for h in done if h in late]
                   + [norm(h) for h in done] + [attend(1, 1, m) for m in ms],
                   span={0: 0.95, 5: 1.05}.get(hs[0], 1.0))
            send([h for h in done if h in late] + [h for h in hs if h not in late])
            done = hs

        @pl.when(it == 0)
        def _():
            _interleave([project(7, False)], [norm(5), norm(6)])
            _interleave([lane_dft(xn, 0, CB)], [norm(7)], span=1.5)

    @_items(1)
    def send_now(h):
        cp_o[h].start()
        yield

    jax.lax.fori_loop(0, 2, layer, None)
    _interleave([project(7, True)], [store_pair(6, range(4)), send_now(6)], span=4.0)
    cp_o[7].start()
    for cp in cp_o:
        cp.wait()


@jax.jit
def pallas_interleave_layers__ssm_conv_s4__sliding_local_dilated__prompt_kernel(
    A_u: jax.Array,
    A_A_re: jax.Array,
    A_A_im: jax.Array,
    A_B_re: jax.Array,
    A_B_im: jax.Array,
    A_C_re: jax.Array,
    A_C_im: jax.Array,
    A_log_dt: jax.Array,
    A_Dskip: jax.Array,
    B_x: jax.Array,
    B_wqkv: jax.Array,
    B_wo: jax.Array,
):
    del B_x
    hbm = pl.BlockSpec(memory_space=pl.ANY)
    out = pl.pallas_call(
        _kernel,
        in_specs=[hbm] * 12,
        out_specs=hbm,
        out_shape=jax.ShapeDtypeStruct((T1, PH, D), BF16),
        scratch_shapes=[pltpu.VMEM((D, NS), BF16)] * 6 + [pltpu.VMEM((D,), BF16)] * 2 + [
            pltpu.VMEM((PH // 2, T1, D), U32),
            pltpu.VMEM((D, 3 * D), BF16),
            pltpu.VMEM((D, D), BF16),
            pltpu.VMEM((2 * PH, T1 // 2, 2 * T1), U32),
            pltpu.VMEM((7, D, HD), U32),
            pltpu.VMEM((D // 2, D), U32),
            pltpu.VMEM((2, D + 8, NS), F32),
            pltpu.VMEM((2, D + 8, NS), F32),
            pltpu.VMEM((D + 8, NS), F32),
            pltpu.VMEM((4, 4, 9 * QS + 4, NS), U32),
            pltpu.VMEM((4, 9 * ZS + 4, T1), U32),
            pltpu.VMEM((PH, D // 2, T1), U32),
            pltpu.VMEM((NCOEF, D, 2 * T1), F32),
            pltpu.VMEM((PH, D + 8, T1), F32),
            pltpu.VMEM((PH, D // 2, T1), U32),
            pltpu.VMEM((2, 2 * PH, D, T1), F32),
            pltpu.VMEM((PH // 2, HD // 2, 7 * T1), U32),
            pltpu.VMEM((PH // 2, 2, D, T1), F32),
            pltpu.VMEM((WIN, D, T1), F32),
            pltpu.VMEM((WIN, HD, T1), F32),
            pltpu.VMEM((WIN, HD // 2, 7 * T1), U32),
            pltpu.SMEM((1,), I32),
            pltpu.SemaphoreType.DMA((11 + PH // 2,)),
        ],
        compiler_params=pltpu.CompilerParams(vmem_limit_bytes=100 * 1024 * 1024),
    )(A_u.reshape(T1, PH, D), A_A_re, A_A_im, A_B_re, A_B_im, A_C_re, A_C_im,
      A_log_dt, A_Dskip, B_wqkv, B_wo,
      _dft_matrices())
    return out.reshape(1, L, D)
```

```python
import numpy as np

import jax
import jax.numpy as jnp
import jax.experimental.pallas as pl
import jax.experimental.pallas.tpu as pltpu

F32, BF16, U32, I32 = jnp.float32, jnp.bfloat16, jnp.uint32, jnp.int32
L, D, NS = 2048, 512, 128
PH, T1 = 16, 128
WIN = 8
NN = (((1,), (0,)), ((), ()))
NT = (((1,), (1,)), ((), ()))
QS = 116
ZS = 28
_H = float(np.sqrt(0.5))
NCOEF = 22
HD = D // 2
RS = 64
JB = 4
EDGES = (0, 64, 192, 320, 448, D)
PROLOGUE = ((2, 0, 0, 0, 0, 0, 0, 0, 0),
            (4, 2, 0, 0, 0, 1, 0, 0, 0),
            (6, 4, 2, 0, 0, 2, 0, 0, 0),
            (8, 6, 4, 2, 0, 5, 0, 0, 0),
            (8, 8, 6, 4, 2, 8, 3, 0, 0),
            (8, 8, 8, 6, 4, 8, 5, 4, 2),
            (8, 8, 8, 8, 6, 8, 8, 4, 6),
            (8, 8, 8, 8, 8, 8, 8, 4, 8))
CB = 64


def _dft_matrices():
    t = 16 * np.arange(T1)[None, :, None] + np.arange(PH)[:, None, None]
    k = np.arange(T1)[None, None, :] + 0.5
    phi = 2.0 * np.pi * k * t / (2 * L)
    phi = np.concatenate([phi, phi.transpose(0, 2, 1)])
    f = np.concatenate([np.cos(phi), -np.sin(phi)], axis=-1).astype(np.float32)
    bits = f.astype(BF16).view(np.uint16).astype(np.uint32)
    return bits[:, 0::2] | (bits[:, 1::2] << 16)


def _cmul(a, b):
    return a[0] * b[0] - a[1] * b[1], a[0] * b[1] + a[1] * b[0]


def _csq(a):
    t = a[0] * a[1]
    return a[0] * a[0] - a[1] * a[1], t + t


def _cadd(a, b):
    return a[0] + b[0], a[1] + b[1]


def _csub(a, b):
    return a[0] - b[0], a[1] - b[1]


def _rot8(x, e):
    s, d = x[0] + x[1], x[0] - x[1]
    return {1: (d * _H, s * _H), 3: (s * -_H, d * _H), 5: (d * -_H, s * -_H), 7: (s * _H, d * -_H)}[e]


def _split(x, e):
    n = len(x) // 2
    lo, hi = x[:n], x[n:]
    if e == 4:
        return ([(a[0] - b[1], a[1] + b[0]) for a, b in zip(lo, hi)],
                [(a[0] + b[1], a[1] - b[0]) for a, b in zip(lo, hi)])
    if e:
        hi = [_rot8(b, e // 2) for b in hi]
    return [_cadd(a, b) for a, b in zip(lo, hi)], [_csub(a, b) for a, b in zip(lo, hi)]


def _merge(p, m, e):
    lo = [_cadd(a, b) for a, b in zip(p, m)]
    if e == 4:
        return lo + [(a[1] - b[1], b[0] - a[0]) for a, b in zip(p, m)]
    hi = [_csub(a, b) for a, b in zip(p, m)]
    return lo + ([_rot8(b, 8 - e // 2) for b in hi] if e else hi)


def _conv_coefs(k, e):
    if len(k) == 1:
        return [(k[0][0] * 0.5, k[0][1] * 0.5)]
    if len(k) == 2 and e % 4:
        if e % 2:
            top = _csub(_rot8(k[1], e), k[0])
        elif e == 2:
            top = (-k[1][1] - k[0][0], k[1][0] - k[0][1])
        else:
            top = (k[1][1] - k[0][0], -k[1][0] - k[0][1])
        return [k[0], top, _csub(k[1], k[0])]
    p, m = _split(k, e)
    return _conv_coefs(p, e // 2) + _conv_coefs(m, e // 2 + 4)


def _conv(x, e, coef):
    if len(x) == 1:
        return [_cmul(x[0], coef())]
    if len(x) == 2:
        yield
    if len(x) == 2 and e % 4:
        both = _cmul(_cadd(x[0], x[1]), coef())
        return [_cadd(both, _cmul(x[1], coef())), _cadd(both, _cmul(x[0], coef()))]
    p, m = _split(x, e)
    p = yield from _conv(p, e // 2, coef)
    m = yield from _conv(m, e // 2 + 4, coef)
    return _merge(p, m, e)


def _sincos(x):
    n = jnp.floor(x * float(2.0 / np.pi) + 0.5)
    r = ((x - n * 1.5703125) - n * 4.837512969970703125e-4) - n * 7.54978995489188216e-8
    z = r * r
    s = r + r * z * ((-1.9515295891e-4 * z + 8.3321608736e-3) * z - 1.6666654611e-1)
    c = 1.0 + z * (((2.443315711809948e-5 * z - 1.388731625493765e-3) * z
                    + 4.166664568298827e-2) * z - 0.5)
    q = n.astype(I32)
    odd = (q & 1) == 1
    s, c = jnp.where(odd, c, s), jnp.where(odd, s, c)
    return jnp.where((q & 2) == 2, -s, s), jnp.where(((q + 1) & 2) == 2, -c, c)


def _zip(x):
    return jnp.concatenate(
        [pltpu.pack_elementwise([x[i:i + 8], x[i + 8:i + 16]], packed_dtype=BF16)
         for i in range(0, x.shape[0], 16)], axis=0)


def _unzip(words, s):
    return pltpu.bitcast(words & np.uint32(0xFFFF0000) if s else words << 16, F32)


def _bf(words):
    return pltpu.bitcast(words, BF16)


def _layernorm(load):
    def mean(term, every):
        acc = [term(load(i)) for i in range(4)]
        for i in range(4, D // 8):
            acc[i % 4] = acc[i % 4] + term(load(i))
            if i % every == every - 1:
                yield
        tot = jnp.sum((acc[0] + acc[1]) + (acc[2] + acc[3]), axis=0, keepdims=True)
        return jnp.broadcast_to(tot * (1.0 / D), (8, T1))

    mu = yield from mean(lambda x: x, 32)
    var = yield from mean(lambda x: (x - mu) * (x - mu), 10)
    rs = jax.lax.rsqrt(var + 1e-5)
    return lambda i: jnp.concatenate([(load(2 * i + s) - mu) * rs for s in range(2)], axis=0)


def _items(n):
    return lambda fn: lambda *args: (fn(*args), n)


def _interleave(*lists, lead=0.0, span=1.0):
    gens = [(v for g, _ in w for v in g) for w in lists]
    sizes = [sum(n for _, n in w) for w in lists]
    for _, k in sorted((i / n if k else i / n * span - lead, k)
                       for k, n in enumerate(sizes) for i in range(n)):
        next(gens[k])
    for g in gens:
        for _ in g:
            pass


def _strassen_lhs(a11, a12, a21, a22):
    return a11 + a22, a22, a21 + a22, a11 + a12, a11, a12 - a22, a21 - a11


def _strassen_rhs(b11, b12, b21, b22):
    return b11 + b22, b21 - b11, b11, b22, b12 - b22, b21 + b22, b11 + b12


def _strassen(prod, emit):
    m4 = prod(1)
    yield
    m2 = prod(2)
    emit(1, 0, m2 + m4)
    yield
    m1 = prod(0)
    c11, c22 = m1 + m4, m1 - m2
    yield
    c11 = c11 + prod(5)
    yield
    m5 = prod(3)
    emit(0, 0, c11 - m5)
    yield
    m3 = prod(4)
    emit(0, 1, m3 + m5)
    c22 = c22 + m3
    yield
    emit(1, 1, c22 + prod(6))
    yield


def _rows(i, n):
    return slice(i * n, i * n + n)


def _alternate(i):
    return pl.ds(16 * (i // 2) + i % 2, 8, stride=2)


def _kernel(u_hbm, are_hbm, aim_hbm, bre_hbm, bim_hbm, cre_hbm, cim_hbm, ldt_hbm, dsk_hbm,
            wqkv_hbm, wo_hbm, f_hbm, out_hbm,
            are, aim, bre, bim, cre, cim, ldt, dsk, io, wq_in, wo_in, fm, ws, wp, lam, dtc, k0s,
            tab, ztab, kb, kf, xr, xn, kv, xq, qs, oe, oo, ob, zs, sems):
    cp_u = [pltpu.make_async_copy(u_hbm.bitcast(U32).at[:, h, :], io.at[h], sems.at[3 + h])
            for h in range(PH // 2)]
    cp_o = [pltpu.make_async_copy(io.at[h], out_hbm.bitcast(U32).at[:, h, :], sems.at[3 + h])
            for h in range(PH // 2)]
    cp_f, cp_g = [pltpu.make_async_copy(f_hbm.at[_rows(i, PH)], fm.at[_rows(i, PH)], sems.at[0])
                  for i in range(2)]
    cp_wq = pltpu.make_async_copy(wqkv_hbm, wq_in, sems.at[1])
    cp_wo = pltpu.make_async_copy(wo_hbm, wo_in, sems.at[2])
    cp_p = [pltpu.make_async_copy(src, dst, sems.at[3 + PH // 2 + i])
            for i, (src, dst) in enumerate(
                ((ldt_hbm, ldt), (dsk_hbm, dsk), (aim_hbm, aim), (are_hbm, are),
                 (bre_hbm, bre), (bim_hbm, bim), (cre_hbm, cre), (cim_hbm, cim)))]
    for cp in cp_p:
        cp.start()

    lane = jax.lax.broadcasted_iota(I32, (8, T1), 1)
    zs[0] = 0

    def region(*lists, **pace):
        pl.when(zs[0] == 0)(lambda: _interleave(*lists, **pace))

    cp_p[0].wait()
    cp_p[1].wait()
    dt_row = jnp.exp(ldt[...].astype(F32).reshape(1, D)).astype(BF16).astype(F32)
    ds_row = dsk[...].astype(F32).reshape(1, D)
    for j in range(4):
        dtc[0, _rows(j, 128), :] = jnp.broadcast_to(dt_row[:, _rows(j, 128)], (128, 128)).T
        dtc[1, _rows(j, 128), :] = jnp.broadcast_to(ds_row[:, _rows(j, 128)], (128, 128)).T
    cp_p[2].wait()
    cp_p[3].wait()
    cp_u[0].start()
    cp_u[1].start()
    big = None
    for j in range(D // 16):
        r = _rows(j, 16)
        theta = dtc[0, r, :] * aim[r, :].astype(F32)
        mag = jnp.exp(dtc[0, r, :] * are[r, :].astype(F32))
        sn, cs = _sincos(theta)
        lam[0, r, :] = mag * cs
        lam[1, r, :] = mag * sn
        big = jnp.abs(theta) if big is None else jnp.maximum(big, jnp.abs(theta))

    @pl.when(jnp.logical_not(jnp.max(big) <= 8192.0))
    def _():
        def body(i, _):
            rows = pl.ds(pl.multiple_of(i * 16, 16), 16)
            th = dtc[0, rows, :] * aim[rows, :].astype(F32)
            mg = jnp.exp(dtc[0, rows, :] * are[rows, :].astype(F32))
            lam[0, rows, :] = mg * jnp.cos(th)
            lam[1, rows, :] = mg * jnp.sin(th)
        jax.lax.fori_loop(0, D // 16, body, None)

    for cp in cp_p[4:]:
        cp.wait()

    @_items(15)
    def tap_tables(blk, e, s):
        rows = pl.ds(CB * blk + 16 * e + s, 8, stride=2)

        def part(ref):
            return _unzip(pltpu.bitcast(ref[_rows(4 * blk + e, 16), :], U32), s)

        sc = dtc[0, rows, :] * (2.0 / L)
        w = _cmul((part(cre), part(cim)), (part(bre) * sc, part(bim) * sc))
        k0s[rows, :] = w[0]

        def put(row, a, b):
            for z in range(2):
                tab[blk % 4, 2 * s + z, pl.ds(row, 8, stride=QS), :] = pltpu.pack_elementwise(
                    [a[z], b[z]], packed_dtype=BF16)

        l1 = (lam[0, rows, :], lam[1, rows, :])
        l2 = _csq(l1)
        l16 = _csq(_csq(_csq(l2)))
        m1 = (l16[0], -l16[1])
        a, b = _cmul(w, l1), _cmul(w, l2)
        put(16 * e, (jnp.ones_like(m1[0]), jnp.zeros_like(m1[0])), m1)

        def columns(j, c):
            d = _cmul(c, m1)
            put(16 * e + j, c, d)
            yield c
            if j < 8:
                yield from columns(2 * j, _csq(c))
                yield from columns(2 * j + 1, _csq(d))

        keep = {}
        for j, c in enumerate(columns(1, _csq(m1)), 1):
            if j == 4:
                l512 = _csq((c[0], -c[1]))
            if j <= 8:
                put(64 + 12 * e + j - 1, a, b)
                keep[2 * j] = b
            if j < 8:
                a, b = _cmul(a, l2), _cmul(b, l2)
            if j == 8:
                put(64 + 12 * e + 8, _cmul(keep[4], l512), _cmul(keep[12], l512))
                a, b = keep[8], keep[16]
            if j in (10, 12, 14):
                a, b = _cmul(a, l512), _cmul(b, l512)
                put(64 + 12 * e + 4 + j // 2, a, b)
            yield

    @_items(48)
    def tap_sums(blk):
        for i in range(8):
            d = [jax.lax.dot_general(_bf(tab[blk % 4, z, pl.ds(QS * i + 64, 48), :]),
                                     _bf(tab[blk % 4, z, pl.ds(QS * i, 64), :]),
                                     NT, preferred_element_type=F32) for z in range(4)]
            own = [None] * 3
            for n in range(12):
                e, r = n // 3, _rows(n, 8)
                v = pltpu.pack_elementwise([d[0][r] + d[1][r], d[2][r] + d[3][r]],
                                           packed_dtype=BF16)
                own[n % 3] = jnp.where(lane < 32 * e, own[n % 3], v) if e else v
                if n % 2:
                    yield
            for r in range(3):
                ztab[blk % 4, pl.ds(ZS * i + 8 * r, 8), :] = own[r]

    @_items(2)
    def tap_blocks(blk, e):
        def at(r, g):
            z = ztab[blk % 4, pl.ds(r, 8, stride=ZS), :]
            return z if g == e else pltpu.roll(z, (32 * (g - e)) % 128, 1)

        def full(r, r1):
            return jnp.where(lane < 64, jnp.where(lane < 32, at(r, 0), at(r1, 1)),
                             jnp.where(lane < 96, at(r1 + 2, 2), at(r1 + 4, 3)))

        halves = [pl.ds(CB * blk + 16 * e + s, 8, stride=2) for s in range(2)]
        e8, e16 = full(7, 18), full(15, 19)
        k0 = pltpu.pack_elementwise(
            [jnp.sum(k0s[r, :], axis=1, keepdims=True) + dtc[1, r, :] * (2.0 / L) for r in halves],
            packed_dtype=BF16)
        e0 = jnp.where(lane == 0, k0, pltpu.roll(e16, 1, 1))
        e4 = jnp.where(lane < 32, at(3, 0), at(16, 1))
        e12 = jnp.where(lane < 32, at(11, 0), at(17, 1))
        k4, k12 = jnp.where(lane < 64, e4, e0), jnp.where(lane < 64, e12, e16)
        far = {1: e0, 2: e0, 3: k4, 5: jnp.where(lane < 64, e4, e8), 6: e8, 7: e8, 9: e8,
               10: e8, 11: jnp.where(lane < 64, e12, e8), 13: k12, 14: e16, 15: e16}
        taps = {0: e0, 4: k4, 8: e8, 12: k12}
        yield
        for p in range(PH):
            kb[p, _rows(4 * blk + e, 8), :] = taps[p] if p in taps else jnp.where(
                lane < (16 if p % 2 else 32), at(p - 1, 0), far[p])
        yield

    @_items(CB // 2)
    def lane_dft(src, lo, hi):
        for q in range(8):
            x0, x1 = [jax.lax.dot_general(_bf(src[p, lo // 2:hi // 2, :]), _bf(fm[p]), NN,
                                          preferred_element_type=F32) for p in (q, q + 8)]
            for i in range((hi - lo) // 8):
                r = _rows(i, 8)
                for c, v in ((q, x0[r] + x1[r]), (q + 8, x0[r] - x1[r])):
                    for z in range(2):
                        kv[0, 2 * c + z, _rows(lo // 8 + i, 8), :] = v[:, _rows(z, T1)]
                if i % 2:
                    yield

    def residues(r, odd):
        return [(kv[0, 2 * c, r, :], kv[0, 2 * c + 1, r, :]) for c in range(8 * odd, 8 * odd + 8)]

    @_items(CB // 4)
    def tap_coefs(blk):
        for i in range(CB // 8):
            r = _rows(blk * CB // 8 + i, 8)
            for odd in range(2):
                for n, v in enumerate(_conv_coefs(residues(r, odd), 4 * odd)):
                    kf[10 * odd + n, r, :T1] = v[0]
                    kf[10 * odd + n, r, T1:] = v[1]
                yield

    r0 = jax.lax.broadcasted_iota(I32, (128, 128), 0)
    ri = (r0 & ~15) + (r0 & 7) * 2 + ((r0 >> 3) & 1)
    ci = jax.lax.broadcasted_iota(I32, (128, 128), 1)
    hit = ci == (ri & 7) * 16 + (ri >> 3)

    @_items(14)
    def prep_weights(j):
        def block(c, k):
            if j < 6:
                sel = jnp.where(hit, 1.0 if j < 4 else 0.25, 0.0)
                w = wq_in[_rows(k, 128), _rows(c, 128)]
            else:
                sel = jnp.where(ri == ci, 1.0, 0.0)
                w = _bf(wp[_rows(k, 64), _rows(c, 128)])
            return jax.lax.dot_general(sel.astype(BF16), w, NT, preferred_element_type=F32)

        top, bot = (4 + j, 8 + j) if j < 4 else (j % 2, j % 2 + 2)
        for k in range(2):
            for i, a in enumerate(_strassen_lhs(block(top, k), block(top, k + 2),
                                                block(bot, k), block(bot, k + 2))):
                ws[i, _rows(j, 64), _rows(k, 128)] = _zip(a)
                yield

    @_items(8)
    def permute_wo(j):
        sel = jnp.where(ci == (r0 & 7) * 16 + (r0 >> 3), 1.0, 0.0).astype(BF16)
        wp[_rows(j, 64), :] = _zip(jnp.dot(sel, wo_in[_rows(j, 128), :],
                                           preferred_element_type=F32))
        yield from range(8)

    @_items(4)
    def load_pair(h):
        for j in range(4):
            wds = io[h, :, _rows(j, 128)].T
            for s in range(2):
                xr[2 * h + s, _rows(j, 128), :] = _unzip(wds, s)
            yield

    @_items(24)
    def norm(h):
        for p in (2 * h, 2 * h + 1):
            normed = yield from _layernorm(lambda i: xr[p, _alternate(i), :])
            for i in range(D // 16):
                xn[p, _rows(i, 8), :] = _zip(normed(i))
                if i % 8 == 7:
                    yield

    for i, step in enumerate(PROLOGUE):
        tables, sums, blocks, dft, coefs, loads, norms, perms, preps = [
            range(a, b) for a, b in zip(PROLOGUE[i - 1] if i else (0,) * 9, step)]
        for cp in {0: [cp_f], 1: cp_u[2:5], 2: cp_u[5:], 3: [cp_wo, cp_wq], 5: [cp_g]}.get(i, ()):
            cp.start()
        for cp, users in ((cp_f, dft), (cp_wo, perms), (cp_wq, preps)):
            if 0 in users:
                cp.wait()
        for h in loads:
            cp_u[h].wait()
        region([tap_sums(b) for b in sums]
               + [lane_dft(kb, CB * b, CB * b + CB) for b in dft]
               + [permute_wo(j) for j in perms] + [prep_weights(j) for j in preps]
               + ([lane_dft(xn, 0, CB)] if step is PROLOGUE[-1] else []),
               [tap_tables(b, e, s) for b in tables for e in range(4) for s in range(2)]
               + [norm(h) for h in norms],
               [tap_blocks(b, e) for b in blocks for e in range(4)],
               [tap_coefs(b) for b in coefs],
               [load_pair(h) for h in loads],
               lead={1: 0.06, 3: 0.06, 4: 0.06, 5: 0.03}.get(i, 0.0),
               span={1: 1.0, 3: 1.0, 5: 1.1}.get(i, 1.05))

    cp_g.wait()

    @_items(10)
    def phase_conv(i):
        r = _rows(i, 8)
        coefs = ((kf[n, r, :T1], kf[n, r, T1:]) for n in range(NCOEF))
        for odd in range(2):
            y = yield from _conv(residues(r, odd), 4 * odd, lambda: next(coefs))
            for c, v in enumerate(y):
                for z in range(2):
                    kv[1, 16 * odd + 2 * c + z, r, :] = v[z]
            yield

    @_items(32)
    def lane_idft(lo, hi):
        for q in (0, 2, 4, 6, 1, 3, 5, 7):
            a, b = [jnp.concatenate([kv[1, 2 * c + z, lo:hi, :] for z in range(2)], axis=1)
                    for c in (q, q + 8)]
            for p, v in ((q, a + b), (q + 8, a - b)):
                inv = jnp.concatenate([fm[PH + p, :, :T1], fm[PH + p, :, T1:]], axis=0)
                d = jax.lax.dot_general(v, _bf(inv), NN, preferred_element_type=F32)
                yield
                xr[p, lo:hi, :] += d
                yield

    @_items(32)
    def norm_pair(g):
        p = 4 * (g % 4) + g // 4
        a = yield from _layernorm(lambda i: xr[p, _alternate(i), :])
        b = yield from _layernorm(lambda i: xr[p + 2, _alternate(i), :])
        for r in range(HD // 16):
            for i, v in enumerate(_strassen_rhs(a(r), b(r), a(HD // 16 + r), b(HD // 16 + r))):
                xq[g, _rows(r, 8), _rows(i, T1)] = _zip(v)
            yield

    def block_product(row0, groups, rhs, emit):
        for r in [128 // RS * hg + i for hg in groups for i in range(128 // RS)]:
            w = slice((row0 + r * RS) // 2, (row0 + r * RS + RS) // 2)
            yield from _strassen(
                lambda i: jnp.dot(_bf(ws[i, w, :]), _bf(rhs[:, _rows(i, T1)]),
                                  preferred_element_type=F32),
                lambda half, n, y: emit(half, n, r * RS, y))

    @_items(7 * HD // RS)
    def keys_values(s, g):
        def emit(half, n, row, y):
            m = 2 * (g % 4) + n
            kv[g // 4, PH * half + WIN - 1 + m, pl.ds(row, RS), :] = y
            if m:
                kv[g // 4, PH * half + m - 1, pl.ds(row, RS), :] = pltpu.roll(y, 1, 1)

        return block_product(0, (s, s + 2), xq.at[g], emit)

    @_items(7 * 128 // RS)
    def queries(s, g):
        def emit(half, n, row, y):
            qs[g, n, pl.ds(HD * half + row, RS), :] = y

        return block_product(D, (s,), xq.at[g], emit)

    @_items(34)
    def attend(par, s, m):
        for hg in (s, s + 2):
            lg = [None] * WIN
            for j0 in range(0, WIN, JB):
                for dh in range(16):
                    r = _rows(16 * hg + dh, 8)
                    q = qs[4 * par + m // 2, m % 2, r, :]
                    for j in range(j0, j0 + JB):
                        t = q * kv[par, WIN - 1 + m - j, r, :]
                        lg[j] = t if dh == 0 else lg[j] + t
                    if (dh + 1) % (16 // JB) == 0:
                        yield
            for j in range(m + 1, WIN):
                lg[j] = jnp.where(lane == 0, -1e9, lg[j])
            mx = lg[0]
            for j in range(1, WIN):
                mx = jnp.maximum(mx, lg[j])
            ex = [jnp.exp(t - mx) for t in lg]
            den = ex[0]
            for j in range(1, WIN):
                den = den + ex[j]
            inv = pltpu.reciprocal(den, full_range=False)
            pr = [t * inv for t in ex]
            yield

            def out(dh):
                r = _rows(16 * hg + dh, 8)
                acc = pr[0] * kv[par, PH + WIN - 1 + m, r, :]
                for j in range(1, WIN):
                    acc = acc + pr[j] * kv[par, PH + WIN - 1 + m - j, r, :]
                return acc

            for d2 in range(8):
                o = jnp.concatenate([out(2 * d2), out(2 * d2 + 1)], axis=0)
                r = _rows(8 * hg + d2, 16)
                if par == 0 or hg < 2:
                    (oe, oo)[par][m, r, :] = o
                if hg >= 2:
                    r1 = _rows(8 * (hg - 2) + d2, 16)
                    ops = (_strassen_rhs(oe[m, r1, :], oo[m, r1, :], oe[m, r, :], o) if par
                           else _strassen_rhs(oe[m, r1, :], o, o, o))
                    for i in (0, 3, 4, 5, 6) if par else (1, 2):
                        ob[m, _rows(8 * (hg - 2) + d2, 8), _rows(i, T1)] = _zip(ops[i])
                yield

    late = (1, 4, 6)

    @_items(7 * HD // RS)
    def project(h, store):
        def emit(half, n, row, y):
            xr[2 * h + n, pl.ds(HD * half + row, RS), :] += y

        for s in range(2):
            yield from block_product(D + HD, (s,), ob.at[h], emit)
            if store:
                for _ in store_pair(h, (s, s + 2))[0]:
                    pass

    @_items(4)
    def store_pair(h, groups):
        for j in groups:
            io[h, :, _rows(j, 128)] = pltpu.pack_elementwise(
                [xr[2 * h + n, _rows(j, 128), :] for n in range(2)], packed_dtype=BF16).T
            yield

    def layer(it, c):
        def send(hs):
            @pl.when(it == 1)
            def _():
                for h in hs:
                    cp_o[h].start()

        cuts = (0, 0) + EDGES + (D, D)
        for i in range(1, len(cuts) - 3):
            (i0, i1), (c0, c1), (f0, f1) = [cuts[i + k:i + k + 2] for k in range(3)]
            last = i0 < i1 == D
            region([lane_dft(xn, c, c + CB) for c in range(f0, f1, CB)]
                   + [lane_idft(c, c + CB) for c in range(i0, i1, CB)],
                   [phase_conv(r) for r in range(c0 // 8, c1 // 8)]
                   + ([norm_pair(0)] if last else []),
                   lead=0.4 if last else 0.0, span=0.95 if i == 4 else 1.0)
        region([keys_values(0, 0), keys_values(1, 0), queries(0, 0)],
               [norm_pair(g) for g in (1, 2, 3)])
        region([fn(0, g) for fn in (keys_values, queries) for g in (1, 2, 3)],
               [norm_pair(g) for g in (4, 5, 6, 7)])
        for par, s, kvg, qg in ((0, 0, (1, 2, 3), (0, 1, 2, 3)), (0, 1, (4, 5, 6, 7), (4, 5, 6, 7)),
                                (1, 0, (4, 5, 6, 7), (4, 5))):
            region([keys_values(1 - s, g) for g in kvg] + [queries(1 - s, g) for g in qg],
                   [attend(par, s, m) for m in range(WIN)], span=1.05)
        region([queries(1, g) for g in (6, 7)], [attend(1, 1, m) for m in (0, 1)], span=0.95)
        done = ()
        for hs, ms in (((0, 1), (2, 3, 4)), ((2, 3, 4), (5, 6, 7)), ((5, 6), ())):
            region([project(h, h not in late) for h in hs],
                   [store_pair(h, range(4)) for h in done if h in late]
                   + [norm(h) for h in done] + [attend(1, 1, m) for m in ms],
                   span={0: 0.95, 5: 1.05}.get(hs[0], 1.0))
            send([h for h in done if h in late] + [h for h in hs if h not in late])
            done = hs

        @pl.when(it == 0)
        def _():
            _interleave([project(7, False)], [norm(5), norm(6)])
            _interleave([lane_dft(xn, 0, CB)], [norm(7)], span=1.5)

    @_items(1)
    def send_now(h):
        cp_o[h].start()
        yield

    jax.lax.fori_loop(0, 2, layer, None)
    _interleave([project(7, True)], [store_pair(6, range(4)), send_now(6)], span=4.0)
    cp_o[7].start()
    for cp in cp_o:
        cp.wait()


@jax.jit
def pallas_interleave_layers__ssm_conv_s4__sliding_local_dilated__prompt_kernel(
    A_u: jax.Array,
    A_A_re: jax.Array,
    A_A_im: jax.Array,
    A_B_re: jax.Array,
    A_B_im: jax.Array,
    A_C_re: jax.Array,
    A_C_im: jax.Array,
    A_log_dt: jax.Array,
    A_Dskip: jax.Array,
    B_x: jax.Array,
    B_wqkv: jax.Array,
    B_wo: jax.Array,
):
    del B_x
    hbm = pl.BlockSpec(memory_space=pl.ANY)
    out = pl.pallas_call(
        _kernel,
        in_specs=[hbm] * 12,
        out_specs=hbm,
        out_shape=jax.ShapeDtypeStruct((T1, PH, D), BF16),
        scratch_shapes=[pltpu.VMEM((D, NS), BF16)] * 6 + [pltpu.VMEM((D,), BF16)] * 2 + [
            pltpu.VMEM((PH // 2, T1, D), U32),
            pltpu.VMEM((D, 3 * D), BF16),
            pltpu.VMEM((D, D), BF16),
            pltpu.VMEM((2 * PH, T1 // 2, 2 * T1), U32),
            pltpu.VMEM((7, D, HD), U32),
            pltpu.VMEM((D // 2, D), U32),
            pltpu.VMEM((2, D + 8, NS), F32),
            pltpu.VMEM((2, D + 8, NS), F32),
            pltpu.VMEM((D + 8, NS), F32),
            pltpu.VMEM((4, 4, 9 * QS + 4, NS), U32),
            pltpu.VMEM((4, 9 * ZS + 4, T1), U32),
            pltpu.VMEM((PH, D // 2, T1), U32),
            pltpu.VMEM((NCOEF, D, 2 * T1), F32),
            pltpu.VMEM((PH, D + 8, T1), F32),
            pltpu.VMEM((PH, D // 2, T1), U32),
            pltpu.VMEM((2, 2 * PH, D, T1), F32),
            pltpu.VMEM((PH // 2, HD // 2, 7 * T1), U32),
            pltpu.VMEM((PH // 2, 2, D, T1), F32),
            pltpu.VMEM((WIN, D, T1), F32),
            pltpu.VMEM((WIN, HD, T1), F32),
            pltpu.VMEM((WIN, HD // 2, 7 * T1), U32),
            pltpu.SMEM((1,), I32),
            pltpu.SemaphoreType.DMA((11 + PH // 2,)),
        ],
        compiler_params=pltpu.CompilerParams(vmem_limit_bytes=100 * 1024 * 1024),
    )(A_u.reshape(T1, PH, D), A_A_re, A_A_im, A_B_re, A_B_im, A_C_re, A_C_im,
      A_log_dt, A_Dskip, B_wqkv, B_wo,
      _dft_matrices())
    return out.reshape(1, L, D)
```

```python
import numpy as np

import jax
import jax.numpy as jnp
import jax.experimental.pallas as pl
import jax.experimental.pallas.tpu as pltpu

F32, BF16, U32, I32 = jnp.float32, jnp.bfloat16, jnp.uint32, jnp.int32
L, D, NS = 2048, 512, 128
PH, T1 = 16, 128
WIN = 8
NN = (((1,), (0,)), ((), ()))
NT = (((1,), (1,)), ((), ()))
QS = 116
ZS = 28
_H = float(np.sqrt(0.5))
NCOEF = 22
HD = D // 2
RS = 64
JB = 4
EDGES = (0, 64, 192, 320, 448, D)
PROLOGUE = ((2, 0, 0, 0, 0, 0, 0, 0, 0),
            (4, 2, 0, 0, 0, 1, 0, 0, 0),
            (6, 4, 2, 0, 0, 2, 0, 0, 0),
            (8, 6, 4, 2, 0, 5, 0, 0, 0),
            (8, 8, 6, 4, 2, 8, 3, 0, 0),
            (8, 8, 8, 6, 4, 8, 5, 4, 2),
            (8, 8, 8, 8, 6, 8, 8, 4, 6),
            (8, 8, 8, 8, 8, 8, 8, 4, 8))
CB = 64


def _dft_matrices():
    t = 16 * np.arange(T1)[None, :, None] + np.arange(PH)[:, None, None]
    k = np.arange(T1)[None, None, :] + 0.5
    phi = 2.0 * np.pi * k * t / (2 * L)
    phi = np.concatenate([phi, phi.transpose(0, 2, 1)])
    f = np.concatenate([np.cos(phi), -np.sin(phi)], axis=-1).astype(np.float32)
    bits = f.astype(BF16).view(np.uint16).astype(np.uint32)
    return bits[:, 0::2] | (bits[:, 1::2] << 16)


def _cmul(a, b):
    return a[0] * b[0] - a[1] * b[1], a[0] * b[1] + a[1] * b[0]


def _csq(a):
    t = a[0] * a[1]
    return a[0] * a[0] - a[1] * a[1], t + t


def _cadd(a, b):
    return a[0] + b[0], a[1] + b[1]


def _csub(a, b):
    return a[0] - b[0], a[1] - b[1]


def _rot8(x, e):
    s, d = x[0] + x[1], x[0] - x[1]
    return {1: (d * _H, s * _H), 3: (s * -_H, d * _H), 5: (d * -_H, s * -_H), 7: (s * _H, d * -_H)}[e]


def _split(x, e):
    n = len(x) // 2
    lo, hi = x[:n], x[n:]
    if e == 4:
        return ([(a[0] - b[1], a[1] + b[0]) for a, b in zip(lo, hi)],
                [(a[0] + b[1], a[1] - b[0]) for a, b in zip(lo, hi)])
    if e:
        hi = [_rot8(b, e // 2) for b in hi]
    return [_cadd(a, b) for a, b in zip(lo, hi)], [_csub(a, b) for a, b in zip(lo, hi)]


def _merge(p, m, e):
    lo = [_cadd(a, b) for a, b in zip(p, m)]
    if e == 4:
        return lo + [(a[1] - b[1], b[0] - a[0]) for a, b in zip(p, m)]
    hi = [_csub(a, b) for a, b in zip(p, m)]
    return lo + ([_rot8(b, 8 - e // 2) for b in hi] if e else hi)


def _conv_coefs(k, e):
    if len(k) == 1:
        return [(k[0][0] * 0.5, k[0][1] * 0.5)]
    if len(k) == 2 and e % 4:
        if e % 2:
            top = _csub(_rot8(k[1], e), k[0])
        elif e == 2:
            top = (-k[1][1] - k[0][0], k[1][0] - k[0][1])
        else:
            top = (k[1][1] - k[0][0], -k[1][0] - k[0][1])
        return [k[0], top, _csub(k[1], k[0])]
    p, m = _split(k, e)
    return _conv_coefs(p, e // 2) + _conv_coefs(m, e // 2 + 4)


def _conv(x, e, coef):
    if len(x) == 1:
        return [_cmul(x[0], coef())]
    if len(x) == 2:
        yield
    if len(x) == 2 and e % 4:
        both = _cmul(_cadd(x[0], x[1]), coef())
        return [_cadd(both, _cmul(x[1], coef())), _cadd(both, _cmul(x[0], coef()))]
    p, m = _split(x, e)
    p = yield from _conv(p, e // 2, coef)
    m = yield from _conv(m, e // 2 + 4, coef)
    return _merge(p, m, e)


def _sincos(x):
    n = jnp.floor(x * float(2.0 / np.pi) + 0.5)
    r = ((x - n * 1.5703125) - n * 4.837512969970703125e-4) - n * 7.54978995489188216e-8
    z = r * r
    s = r + r * z * ((-1.9515295891e-4 * z + 8.3321608736e-3) * z - 1.6666654611e-1)
    c = 1.0 + z * (((2.443315711809948e-5 * z - 1.388731625493765e-3) * z
                    + 4.166664568298827e-2) * z - 0.5)
    q = n.astype(I32)
    odd = (q & 1) == 1
    s, c = jnp.where(odd, c, s), jnp.where(odd, s, c)
    return jnp.where((q & 2) == 2, -s, s), jnp.where(((q + 1) & 2) == 2, -c, c)


def _zip(x):
    return jnp.concatenate(
        [pltpu.pack_elementwise([x[i:i + 8], x[i + 8:i + 16]], packed_dtype=BF16)
         for i in range(0, x.shape[0], 16)], axis=0)


def _unzip(words, s):
    return pltpu.bitcast(words & np.uint32(0xFFFF0000) if s else words << 16, F32)


def _bf(words):
    return pltpu.bitcast(words, BF16)


def _layernorms(loads):
    def mean(load, term, every):
        acc = [term(load(i)) for i in range(4)]
        for i in range(4, D // 8):
            acc[i % 4] = acc[i % 4] + term(load(i))
            if i % every == every - 1:
                yield
        tot = jnp.sum(_tree(jnp.add, acc), axis=0, keepdims=True)
        return jnp.broadcast_to(tot * (1.0 / D), (8, T1))

    def normed(load, mu, rs):
        return lambda i: jnp.concatenate([(load(2 * i + s) - mu) * rs for s in range(2)], axis=0)

    mus, out = [], []
    for load in loads:
        mus.append((yield from mean(load, lambda x: x, 32)))
    for load, mu in zip(loads, mus):
        var = yield from mean(load, lambda x: (x - mu) * (x - mu), 10)
        out.append(normed(load, mu, jax.lax.rsqrt(var + 1e-5)))
    return out


def _items(n):
    return lambda fn: lambda *args: (fn(*args), n)


def _interleave(*lists, lead=0.0, span=1.0):
    gens = [(v for g, _ in w for v in g) for w in lists]
    sizes = [sum(n for _, n in w) for w in lists]
    for _, k in sorted((i / n if k else i / n * span - lead, k)
                       for k, n in enumerate(sizes) for i in range(n)):
        next(gens[k])
    for g in gens:
        for _ in g:
            pass


def _strassen_lhs(a11, a12, a21, a22):
    return a11 + a22, a22, a21 + a22, a11 + a12, a11, a12 - a22, a21 - a11


def _strassen_rhs(b11, b12, b21, b22):
    return b11 + b22, b21 - b11, b11, b22, b12 - b22, b21 + b22, b11 + b12


def _strassen(prod, emit):
    m4 = prod(1)
    yield
    m2 = prod(2)
    emit(1, 0, m2 + m4)
    yield
    m1 = prod(0)
    c11, c22 = m1 + m4, m1 - m2
    yield
    c11 = c11 + prod(5)
    yield
    m5 = prod(3)
    emit(0, 0, c11 - m5)
    yield
    m3 = prod(4)
    emit(0, 1, m3 + m5)
    c22 = c22 + m3
    yield
    emit(1, 1, c22 + prod(6))
    yield


def _tree(op, xs):
    return xs[0] if len(xs) == 1 else op(_tree(op, xs[:len(xs) // 2]), _tree(op, xs[len(xs) // 2:]))


def _rows(i, n):
    return slice(i * n, i * n + n)


def _alternate(i):
    return pl.ds(16 * (i // 2) + i % 2, 8, stride=2)


def _kernel(u_hbm, are_hbm, aim_hbm, bre_hbm, bim_hbm, cre_hbm, cim_hbm, ldt_hbm, dsk_hbm,
            wqkv_hbm, wo_hbm, f_hbm, out_hbm,
            are, aim, bre, bim, cre, cim, ldt, dsk, io, wq_in, wo_in, fm, ws, wp, lam, dtc, k0s,
            tab, ztab, kb, kf, xr, xn, kv, xq, qs, oe, oo, ob, zs, sems):
    cp_u = [pltpu.make_async_copy(u_hbm.bitcast(U32).at[:, h, :], io.at[h], sems.at[3 + h])
            for h in range(PH // 2)]
    cp_o = [pltpu.make_async_copy(io.at[h], out_hbm.bitcast(U32).at[:, h, :], sems.at[3 + h])
            for h in range(PH // 2)]
    cp_f, cp_g = [pltpu.make_async_copy(f_hbm.at[_rows(i, PH)], fm.at[_rows(i, PH)], sems.at[0])
                  for i in range(2)]
    cp_wq = pltpu.make_async_copy(wqkv_hbm, wq_in, sems.at[1])
    cp_wo = pltpu.make_async_copy(wo_hbm, wo_in, sems.at[2])
    cp_p = [pltpu.make_async_copy(src, dst, sems.at[3 + PH // 2 + i])
            for i, (src, dst) in enumerate(
                ((ldt_hbm, ldt), (dsk_hbm, dsk), (aim_hbm, aim), (are_hbm, are),
                 (bre_hbm, bre), (bim_hbm, bim), (cre_hbm, cre), (cim_hbm, cim)))]
    for cp in cp_p:
        cp.start()

    lane = jax.lax.broadcasted_iota(I32, (8, T1), 1)
    zs[0] = 0

    def region(*lists, **pace):
        pl.when(zs[0] == 0)(lambda: _interleave(*lists, **pace))

    cp_p[0].wait()
    cp_p[1].wait()
    dt_row = jnp.exp(ldt[...].astype(F32).reshape(1, D)).astype(BF16).astype(F32)
    ds_row = dsk[...].astype(F32).reshape(1, D)
    for j in range(4):
        dtc[0, _rows(j, 128), :] = jnp.broadcast_to(dt_row[:, _rows(j, 128)], (128, 128)).T
        dtc[1, _rows(j, 128), :] = jnp.broadcast_to(ds_row[:, _rows(j, 128)], (128, 128)).T
    cp_p[2].wait()
    cp_p[3].wait()
    cp_u[0].start()
    cp_u[1].start()
    big = None
    for j in range(D // 16):
        r = _rows(j, 16)
        theta = dtc[0, r, :] * aim[r, :].astype(F32)
        mag = jnp.exp(dtc[0, r, :] * are[r, :].astype(F32))
        sn, cs = _sincos(theta)
        lam[0, r, :] = mag * cs
        lam[1, r, :] = mag * sn
        big = jnp.abs(theta) if big is None else jnp.maximum(big, jnp.abs(theta))

    @pl.when(jnp.logical_not(jnp.max(big) <= 8192.0))
    def _():
        def body(i, _):
            rows = pl.ds(pl.multiple_of(i * 16, 16), 16)
            th = dtc[0, rows, :] * aim[rows, :].astype(F32)
            mg = jnp.exp(dtc[0, rows, :] * are[rows, :].astype(F32))
            lam[0, rows, :] = mg * jnp.cos(th)
            lam[1, rows, :] = mg * jnp.sin(th)
        jax.lax.fori_loop(0, D // 16, body, None)

    for cp in cp_p[4:]:
        cp.wait()

    @_items(15)
    def tap_tables(blk, e, s):
        rows = pl.ds(CB * blk + 16 * e + s, 8, stride=2)

        def part(ref):
            return _unzip(pltpu.bitcast(ref[_rows(4 * blk + e, 16), :], U32), s)

        sc = dtc[0, rows, :] * (2.0 / L)
        w = _cmul((part(cre), part(cim)), (part(bre) * sc, part(bim) * sc))
        k0s[rows, :] = w[0]

        def put(row, a, b):
            for z in range(2):
                tab[blk % 4, 2 * s + z, pl.ds(row, 8, stride=QS), :] = pltpu.pack_elementwise(
                    [a[z], b[z]], packed_dtype=BF16)

        l1 = (lam[0, rows, :], lam[1, rows, :])
        l2 = _csq(l1)
        l16 = _csq(_csq(_csq(l2)))
        m1 = (l16[0], -l16[1])
        a, b = _cmul(w, l1), _cmul(w, l2)
        put(16 * e, (jnp.ones_like(m1[0]), jnp.zeros_like(m1[0])), m1)

        def columns(j, c):
            d = _cmul(c, m1)
            put(16 * e + j, c, d)
            yield c
            if j < 8:
                yield from columns(2 * j, _csq(c))
                yield from columns(2 * j + 1, _csq(d))

        keep = {}
        for j, c in enumerate(columns(1, _csq(m1)), 1):
            if j == 4:
                l512 = _csq((c[0], -c[1]))
            if j <= 8:
                put(64 + 12 * e + j - 1, a, b)
                keep[2 * j] = b
            if j < 8:
                a, b = _cmul(a, l2), _cmul(b, l2)
            if j == 8:
                put(64 + 12 * e + 8, _cmul(keep[4], l512), _cmul(keep[12], l512))
                a, b = keep[8], keep[16]
            if j in (10, 12, 14):
                a, b = _cmul(a, l512), _cmul(b, l512)
                put(64 + 12 * e + 4 + j // 2, a, b)
            yield

    @_items(48)
    def tap_sums(blk):
        for i in range(8):
            d = [jax.lax.dot_general(_bf(tab[blk % 4, z, pl.ds(QS * i + 64, 48), :]),
                                     _bf(tab[blk % 4, z, pl.ds(QS * i, 64), :]),
                                     NT, preferred_element_type=F32) for z in range(4)]
            own = [None] * 3
            for n in range(12):
                e, r = n // 3, _rows(n, 8)
                v = pltpu.pack_elementwise([d[0][r] + d[1][r], d[2][r] + d[3][r]],
                                           packed_dtype=BF16)
                own[n % 3] = jnp.where(lane < 32 * e, own[n % 3], v) if e else v
                if n % 2:
                    yield
            for r in range(3):
                ztab[blk % 4, pl.ds(ZS * i + 8 * r, 8), :] = own[r]

    @_items(2)
    def tap_blocks(blk, e):
        def at(r, g):
            z = ztab[blk % 4, pl.ds(r, 8, stride=ZS), :]
            return z if g == e else pltpu.roll(z, (32 * (g - e)) % 128, 1)

        def full(r, r1):
            return jnp.where(lane < 64, jnp.where(lane < 32, at(r, 0), at(r1, 1)),
                             jnp.where(lane < 96, at(r1 + 2, 2), at(r1 + 4, 3)))

        halves = [pl.ds(CB * blk + 16 * e + s, 8, stride=2) for s in range(2)]
        e8, e16 = full(7, 18), full(15, 19)
        k0 = pltpu.pack_elementwise(
            [jnp.sum(k0s[r, :], axis=1, keepdims=True) + dtc[1, r, :] * (2.0 / L) for r in halves],
            packed_dtype=BF16)
        e0 = jnp.where(lane == 0, k0, pltpu.roll(e16, 1, 1))
        e4 = jnp.where(lane < 32, at(3, 0), at(16, 1))
        e12 = jnp.where(lane < 32, at(11, 0), at(17, 1))
        k4, k12 = jnp.where(lane < 64, e4, e0), jnp.where(lane < 64, e12, e16)
        far = {1: e0, 2: e0, 3: k4, 5: jnp.where(lane < 64, e4, e8), 6: e8, 7: e8, 9: e8,
               10: e8, 11: jnp.where(lane < 64, e12, e8), 13: k12, 14: e16, 15: e16}
        taps = {0: e0, 4: k4, 8: e8, 12: k12}
        yield
        for p in range(PH):
            kb[p, _rows(4 * blk + e, 8), :] = taps[p] if p in taps else jnp.where(
                lane < (16 if p % 2 else 32), at(p - 1, 0), far[p])
        yield

    @_items(CB // 2)
    def lane_dft(src, lo, hi):
        for q in range(8):
            x0, x1 = [jax.lax.dot_general(_bf(src[p, lo // 2:hi // 2, :]), _bf(fm[p]), NN,
                                          preferred_element_type=F32) for p in (q, q + 8)]
            for i in range((hi - lo) // 8):
                r = _rows(i, 8)
                for c, v in ((q, x0[r] + x1[r]), (q + 8, x0[r] - x1[r])):
                    for z in range(2):
                        kv[0, 2 * c + z, _rows(lo // 8 + i, 8), :] = v[:, _rows(z, T1)]
                if i % 2:
                    yield

    def residues(r, odd):
        return [(kv[0, 2 * c, r, :], kv[0, 2 * c + 1, r, :]) for c in range(8 * odd, 8 * odd + 8)]

    @_items(CB // 4)
    def tap_coefs(blk):
        for i in range(CB // 8):
            r = _rows(blk * CB // 8 + i, 8)
            for odd in range(2):
                for n, v in enumerate(_conv_coefs(residues(r, odd), 4 * odd)):
                    kf[10 * odd + n, r, :T1] = v[0]
                    kf[10 * odd + n, r, T1:] = v[1]
                yield

    r0 = jax.lax.broadcasted_iota(I32, (128, 128), 0)
    ri = (r0 & ~15) + (r0 & 7) * 2 + ((r0 >> 3) & 1)
    ci = jax.lax.broadcasted_iota(I32, (128, 128), 1)
    hit = ci == (ri & 7) * 16 + (ri >> 3)

    @_items(14)
    def prep_weights(j):
        def block(c, k):
            if j < 6:
                sel = jnp.where(hit, 1.0 if j < 4 else 0.25, 0.0)
                w = wq_in[_rows(k, 128), _rows(c, 128)]
            else:
                sel = jnp.where(ri == ci, 1.0, 0.0)
                w = _bf(wp[_rows(k, 64), _rows(c, 128)])
            return jax.lax.dot_general(sel.astype(BF16), w, NT, preferred_element_type=F32)

        top, bot = (4 + j, 8 + j) if j < 4 else (j % 2, j % 2 + 2)
        for k in range(2):
            for i, a in enumerate(_strassen_lhs(block(top, k), block(top, k + 2),
                                                block(bot, k), block(bot, k + 2))):
                ws[i, _rows(j, 64), _rows(k, 128)] = _zip(a)
                yield

    @_items(8)
    def permute_wo(j):
        sel = jnp.where(ci == (r0 & 7) * 16 + (r0 >> 3), 1.0, 0.0).astype(BF16)
        wp[_rows(j, 64), :] = _zip(jnp.dot(sel, wo_in[_rows(j, 128), :],
                                           preferred_element_type=F32))
        yield from range(8)

    @_items(4)
    def load_pair(h):
        for j in range(4):
            wds = io[h, :, _rows(j, 128)].T
            for s in range(2):
                xr[2 * h + s, _rows(j, 128), :] = _unzip(wds, s)
            yield

    def phase(p):
        return lambda i: xr[p, _alternate(i), :]

    @_items(24)
    def norm(h):
        both = yield from _layernorms([phase(2 * h), phase(2 * h + 1)])
        for p, normed in enumerate(both, 2 * h):
            for i in range(D // 16):
                xn[p, _rows(i, 8), :] = _zip(normed(i))
                if i % 8 == 7:
                    yield

    for i, step in enumerate(PROLOGUE):
        tables, sums, blocks, dft, coefs, loads, norms, perms, preps = [
            range(a, b) for a, b in zip(PROLOGUE[i - 1] if i else (0,) * 9, step)]
        for cp in {0: [cp_f], 1: cp_u[2:5], 2: cp_u[5:], 3: [cp_wo, cp_wq], 5: [cp_g]}.get(i, ()):
            cp.start()
        for cp, users in ((cp_f, dft), (cp_wo, perms), (cp_wq, preps)):
            if 0 in users:
                cp.wait()
        for h in loads:
            cp_u[h].wait()
        region([tap_sums(b) for b in sums]
               + [lane_dft(kb, CB * b, CB * b + CB) for b in dft]
               + [permute_wo(j) for j in perms] + [prep_weights(j) for j in preps]
               + ([lane_dft(xn, 0, CB)] if step is PROLOGUE[-1] else []),
               [tap_tables(b, e, s) for b in tables for e in range(4) for s in range(2)]
               + [norm(h) for h in norms],
               [tap_blocks(b, e) for b in blocks for e in range(4)],
               [tap_coefs(b) for b in coefs],
               [load_pair(h) for h in loads],
               lead={1: 0.06, 3: 0.06, 4: 0.06, 5: 0.03}.get(i, 0.0),
               span={1: 1.0, 3: 1.0, 5: 1.1}.get(i, 1.05))

    cp_g.wait()

    @_items(10)
    def phase_conv(i):
        r = _rows(i, 8)
        coefs = ((kf[n, r, :T1], kf[n, r, T1:]) for n in range(NCOEF))
        for odd in range(2):
            y = yield from _conv(residues(r, odd), 4 * odd, lambda: next(coefs))
            for c, v in enumerate(y):
                for z in range(2):
                    kv[1, 16 * odd + 2 * c + z, r, :] = v[z]
            yield

    @_items(32)
    def lane_idft(lo, hi):
        for q in (0, 2, 4, 6, 1, 3, 5, 7):
            a, b = [jnp.concatenate([kv[1, 2 * c + z, lo:hi, :] for z in range(2)], axis=1)
                    for c in (q, q + 8)]
            for p, v in ((q, a + b), (q + 8, a - b)):
                inv = jnp.concatenate([fm[PH + p, :, :T1], fm[PH + p, :, T1:]], axis=0)
                d = jax.lax.dot_general(v, _bf(inv), NN, preferred_element_type=F32)
                yield
                xr[p, lo:hi, :] += d
                yield

    @_items(32)
    def norm_pair(g):
        p = 4 * (g % 4) + g // 4
        a, b = yield from _layernorms([phase(p), phase(p + 2)])
        for r in range(HD // 16):
            for i, v in enumerate(_strassen_rhs(a(r), b(r), a(HD // 16 + r), b(HD // 16 + r))):
                xq[g, _rows(r, 8), _rows(i, T1)] = _zip(v)
            yield

    def block_product(row0, groups, rhs, emit):
        for r in [128 // RS * hg + i for hg in groups for i in range(128 // RS)]:
            w = slice((row0 + r * RS) // 2, (row0 + r * RS + RS) // 2)
            yield from _strassen(
                lambda i: jnp.dot(_bf(ws[i, w, :]), _bf(rhs[:, _rows(i, T1)]),
                                  preferred_element_type=F32),
                lambda half, n, y: emit(half, n, r * RS, y))

    @_items(7 * HD // RS)
    def keys_values(s, g):
        def emit(half, n, row, y):
            m = 2 * (g % 4) + n
            kv[g // 4, PH * half + WIN - 1 + m, pl.ds(row, RS), :] = y
            if m:
                kv[g // 4, PH * half + m - 1, pl.ds(row, RS), :] = pltpu.roll(y, 1, 1)

        return block_product(0, (s, s + 2), xq.at[g], emit)

    @_items(7 * 128 // RS)
    def queries(s, g):
        def emit(half, n, row, y):
            qs[g, n, pl.ds(HD * half + row, RS), :] = y

        return block_product(D, (s,), xq.at[g], emit)

    @_items(34)
    def attend(par, s, m):
        def group(hg):
            lg = [None] * WIN
            for j0 in range(0, WIN, JB):
                for dh in range(16):
                    r = _rows(16 * hg + dh, 8)
                    q = qs[4 * par + m // 2, m % 2, r, :]
                    for j in range(j0, j0 + JB):
                        t = q * kv[par, WIN - 1 + m - j, r, :]
                        lg[j] = t if dh == 0 else lg[j] + t
                    if (dh + 1) % (16 // JB) == 0:
                        yield
            for j in range(m + 1, WIN):
                lg[j] = jnp.where(lane == 0, -1e9, lg[j])
            mx = _tree(jnp.maximum, lg)
            ex = [jnp.exp(t - mx) for t in lg]
            den = _tree(jnp.add, ex)
            inv = pltpu.reciprocal(den, full_range=False)
            pr = [t * inv for t in ex]
            yield

            def out(dh):
                r = _rows(16 * hg + dh, 8)
                acc = pr[0] * kv[par, PH + WIN - 1 + m, r, :]
                for j in range(1, WIN):
                    acc = acc + pr[j] * kv[par, PH + WIN - 1 + m - j, r, :]
                return acc

            for d2 in range(8):
                o = jnp.concatenate([out(2 * d2), out(2 * d2 + 1)], axis=0)
                r = _rows(8 * hg + d2, 16)
                if par == 0 or hg < 2:
                    (oe, oo)[par][m, r, :] = o
                if hg >= 2:
                    r1 = _rows(8 * (hg - 2) + d2, 16)
                    ops = (_strassen_rhs(oe[m, r1, :], oo[m, r1, :], oe[m, r, :], o) if par
                           else _strassen_rhs(oe[m, r1, :], o, o, o))
                    for i in (0, 3, 4, 5, 6) if par else (1, 2):
                        ob[m, _rows(8 * (hg - 2) + d2, 8), _rows(i, T1)] = _zip(ops[i])
                yield

        a, b = group(s), group(s + 2)
        for g, n in ((a, 9), (b, 9), (a, 8), (b, 8)):
            for _ in range(n):
                yield next(g)

    late = (1, 4, 6)

    @_items(7 * HD // RS)
    def project(h, store):
        def emit(half, n, row, y):
            xr[2 * h + n, pl.ds(HD * half + row, RS), :] += y

        for s in range(2):
            yield from block_product(D + HD, (s,), ob.at[h], emit)
            if store:
                for _ in store_pair(h, (s, s + 2))[0]:
                    pass

    @_items(4)
    def store_pair(h, groups):
        for j in groups:
            io[h, :, _rows(j, 128)] = pltpu.pack_elementwise(
                [xr[2 * h + n, _rows(j, 128), :] for n in range(2)], packed_dtype=BF16).T
            yield

    def layer(it, c):
        def send(hs):
            @pl.when(it == 1)
            def _():
                for h in hs:
                    cp_o[h].start()

        cuts = (0, 0) + EDGES + (D, D)
        for i in range(1, len(cuts) - 3):
            (i0, i1), (c0, c1), (f0, f1) = [cuts[i + k:i + k + 2] for k in range(3)]
            last = i0 < i1 == D
            region([lane_dft(xn, c, c + CB) for c in range(f0, f1, CB)]
                   + [lane_idft(c, c + CB) for c in range(i0, i1, CB)],
                   [phase_conv(r) for r in range(c0 // 8, c1 // 8)]
                   + ([norm_pair(0)] if last else []),
                   lead=0.4 if last else 0.0, span=0.95 if i == 4 else 1.0)
        region([keys_values(0, 0), keys_values(1, 0), queries(0, 0)],
               [norm_pair(g) for g in (1, 2, 3)])
        region([fn(0, g) for fn in (keys_values, queries) for g in (1, 2, 3)],
               [norm_pair(g) for g in (4, 5, 6, 7)])
        for par, s, kvg, qg in ((0, 0, (1, 2, 3), (0, 1, 2, 3)), (0, 1, (4, 5, 6, 7), (4, 5, 6, 7)),
                                (1, 0, (4, 5, 6, 7), (4, 5))):
            region([keys_values(1 - s, g) for g in kvg] + [queries(1 - s, g) for g in qg],
                   [attend(par, s, m) for m in range(WIN)], span=1.05)
        region([queries(1, g) for g in (6, 7)], [attend(1, 1, m) for m in (0, 1)], span=0.95)
        done = ()
        for hs, ms in (((0, 1), (2, 3, 4)), ((2, 3, 4), (5, 6, 7)), ((5, 6), ())):
            region([project(h, h not in late) for h in hs],
                   [store_pair(h, range(4)) for h in done if h in late]
                   + [norm(h) for h in done] + [attend(1, 1, m) for m in ms],
                   span={0: 0.95, 5: 1.05}.get(hs[0], 1.0))
            send([h for h in done if h in late] + [h for h in hs if h not in late])
            done = hs

        @pl.when(it == 0)
        def _():
            _interleave([project(7, False)], [norm(5), norm(6)])
            _interleave([lane_dft(xn, 0, CB)], [norm(7)], span=1.5)

    @_items(1)
    def send_now(h):
        cp_o[h].start()
        yield

    jax.lax.fori_loop(0, 2, layer, None)
    _interleave([project(7, True)], [store_pair(6, range(4)), send_now(6)], span=4.0)
    cp_o[7].start()
    for cp in cp_o:
        cp.wait()


@jax.jit
def pallas_interleave_layers__ssm_conv_s4__sliding_local_dilated__prompt_kernel(
    A_u: jax.Array,
    A_A_re: jax.Array,
    A_A_im: jax.Array,
    A_B_re: jax.Array,
    A_B_im: jax.Array,
    A_C_re: jax.Array,
    A_C_im: jax.Array,
    A_log_dt: jax.Array,
    A_Dskip: jax.Array,
    B_x: jax.Array,
    B_wqkv: jax.Array,
    B_wo: jax.Array,
):
    del B_x
    hbm = pl.BlockSpec(memory_space=pl.ANY)
    out = pl.pallas_call(
        _kernel,
        in_specs=[hbm] * 12,
        out_specs=hbm,
        out_shape=jax.ShapeDtypeStruct((T1, PH, D), BF16),
        scratch_shapes=[pltpu.VMEM((D, NS), BF16)] * 6 + [pltpu.VMEM((D,), BF16)] * 2 + [
            pltpu.VMEM((PH // 2, T1, D), U32),
            pltpu.VMEM((D, 3 * D), BF16),
            pltpu.VMEM((D, D), BF16),
            pltpu.VMEM((2 * PH, T1 // 2, 2 * T1), U32),
            pltpu.VMEM((7, D, HD), U32),
            pltpu.VMEM((D // 2, D), U32),
            pltpu.VMEM((2, D + 8, NS), F32),
            pltpu.VMEM((2, D + 8, NS), F32),
            pltpu.VMEM((D + 8, NS), F32),
            pltpu.VMEM((4, 4, 9 * QS + 4, NS), U32),
            pltpu.VMEM((4, 9 * ZS + 4, T1), U32),
            pltpu.VMEM((PH, D // 2, T1), U32),
            pltpu.VMEM((NCOEF, D, 2 * T1), F32),
            pltpu.VMEM((PH, D + 8, T1), F32),
            pltpu.VMEM((PH, D // 2, T1), U32),
            pltpu.VMEM((2, 2 * PH, D, T1), F32),
            pltpu.VMEM((PH // 2, HD // 2, 7 * T1), U32),
            pltpu.VMEM((PH // 2, 2, D, T1), F32),
            pltpu.VMEM((WIN, D, T1), F32),
            pltpu.VMEM((WIN, HD, T1), F32),
            pltpu.VMEM((WIN, HD // 2, 7 * T1), U32),
            pltpu.SMEM((1,), I32),
            pltpu.SemaphoreType.DMA((11 + PH // 2,)),
        ],
        compiler_params=pltpu.CompilerParams(vmem_limit_bytes=100 * 1024 * 1024),
    )(A_u.reshape(T1, PH, D), A_A_re, A_A_im, A_B_re, A_B_im, A_C_re, A_C_im,
      A_log_dt, A_Dskip, B_wqkv, B_wo,
      _dft_matrices())
    return out.reshape(1, L, D)
```

```python
import numpy as np

import jax
import jax.numpy as jnp
import jax.experimental.pallas as pl
import jax.experimental.pallas.tpu as pltpu

F32, BF16, U32, I32 = jnp.float32, jnp.bfloat16, jnp.uint32, jnp.int32
L, D, NS = 2048, 512, 128
PH, T1 = 16, 128
WIN = 8
NN = (((1,), (0,)), ((), ()))
NT = (((1,), (1,)), ((), ()))
QS = 116
ZS = 28
_H = float(np.sqrt(0.5))
NCOEF = 22
HD = D // 2
RS = 64
DFT = (2, 6, 10, 14, 16, 16, 16)
CONV = (0, 8, 24, 40, 56, 64, 64)
IDFT = (0, 0, 2, 6, 10, 14, 16)
PROLOGUE = ((2, 0, 0, 0, 0, 0, 0, 0, 0),
            (4, 2, 0, 0, 0, 1, 0, 0, 0),
            (6, 4, 2, 0, 0, 2, 0, 0, 0),
            (8, 6, 4, 2, 0, 5, 0, 0, 0),
            (8, 8, 6, 4, 2, 8, 3, 0, 0),
            (8, 8, 8, 6, 4, 8, 5, 4, 2),
            (8, 8, 8, 8, 6, 8, 8, 4, 6),
            (8, 8, 8, 8, 8, 8, 8, 4, 8))
CB = 64


def _dft_matrices():
    t = 16 * np.arange(T1)[None, :, None] + np.arange(PH)[:, None, None]
    k = np.arange(T1)[None, None, :] + 0.5
    phi = 2.0 * np.pi * k * t / (2 * L)
    phi = np.concatenate([phi, phi.transpose(0, 2, 1)])
    f = np.concatenate([np.cos(phi), -np.sin(phi)], axis=-1).astype(np.float32)
    bits = f.astype(BF16).view(np.uint16).astype(np.uint32)
    return bits[:, 0::2] | (bits[:, 1::2] << 16)


def _cmul(a, b):
    return a[0] * b[0] - a[1] * b[1], a[0] * b[1] + a[1] * b[0]


def _csq(a):
    t = a[0] * a[1]
    return a[0] * a[0] - a[1] * a[1], t + t


def _cadd(a, b):
    return a[0] + b[0], a[1] + b[1]


def _csub(a, b):
    return a[0] - b[0], a[1] - b[1]


def _rot8(x, e):
    s, d = x[0] + x[1], x[0] - x[1]
    return {1: (d * _H, s * _H), 3: (s * -_H, d * _H), 5: (d * -_H, s * -_H), 7: (s * _H, d * -_H)}[e]


def _split(x, e):
    n = len(x) // 2
    lo, hi = x[:n], x[n:]
    if e == 4:
        return ([(a[0] - b[1], a[1] + b[0]) for a, b in zip(lo, hi)],
                [(a[0] + b[1], a[1] - b[0]) for a, b in zip(lo, hi)])
    if e:
        hi = [_rot8(b, e // 2) for b in hi]
    return [_cadd(a, b) for a, b in zip(lo, hi)], [_csub(a, b) for a, b in zip(lo, hi)]


def _merge(p, m, e):
    lo = [_cadd(a, b) for a, b in zip(p, m)]
    if e == 4:
        return lo + [(a[1] - b[1], b[0] - a[0]) for a, b in zip(p, m)]
    hi = [_csub(a, b) for a, b in zip(p, m)]
    return lo + ([_rot8(b, 8 - e // 2) for b in hi] if e else hi)


def _conv_coefs(k, e):
    if len(k) == 1:
        return [(k[0][0] * 0.5, k[0][1] * 0.5)]
    if len(k) == 2 and e % 4:
        if e % 2:
            top = _csub(_rot8(k[1], e), k[0])
        elif e == 2:
            top = (-k[1][1] - k[0][0], k[1][0] - k[0][1])
        else:
            top = (k[1][1] - k[0][0], -k[1][0] - k[0][1])
        return [k[0], top, _csub(k[1], k[0])]
    p, m = _split(k, e)
    return _conv_coefs(p, e // 2) + _conv_coefs(m, e // 2 + 4)


def _conv(x, e, coef):
    if len(x) == 1:
        return [_cmul(x[0], coef())]
    if len(x) == 2:
        yield
    if len(x) == 2 and e % 4:
        both = _cmul(_cadd(x[0], x[1]), coef())
        return [_cadd(both, _cmul(x[1], coef())), _cadd(both, _cmul(x[0], coef()))]
    p, m = _split(x, e)
    p = yield from _conv(p, e // 2, coef)
    m = yield from _conv(m, e // 2 + 4, coef)
    return _merge(p, m, e)


def _sincos(x):
    n = jnp.floor(x * float(2.0 / np.pi) + 0.5)
    r = ((x - n * 1.5703125) - n * 4.837512969970703125e-4) - n * 7.54978995489188216e-8
    z = r * r
    s = r + r * z * ((-1.9515295891e-4 * z + 8.3321608736e-3) * z - 1.6666654611e-1)
    c = 1.0 + z * (((2.443315711809948e-5 * z - 1.388731625493765e-3) * z
                    + 4.166664568298827e-2) * z - 0.5)
    q = n.astype(I32)
    odd = (q & 1) == 1
    s, c = jnp.where(odd, c, s), jnp.where(odd, s, c)
    return jnp.where((q & 2) == 2, -s, s), jnp.where(((q + 1) & 2) == 2, -c, c)


def _zip(x):
    return jnp.concatenate(
        [pltpu.pack_elementwise([x[i:i + 8], x[i + 8:i + 16]], packed_dtype=BF16)
         for i in range(0, x.shape[0], 16)], axis=0)


def _unzip(words, s):
    return pltpu.bitcast(words & np.uint32(0xFFFF0000) if s else words << 16, F32)


def _bf(words):
    return pltpu.bitcast(words, BF16)


def _layernorms(loads):
    def mean(load, term, every):
        acc = [term(load(i)) for i in range(4)]
        for i in range(4, D // 8):
            acc[i % 4] = acc[i % 4] + term(load(i))
            if i % every == every - 1:
                yield
        tot = jnp.sum(_tree(jnp.add, acc), axis=0, keepdims=True)
        return jnp.broadcast_to(tot * (1.0 / D), (8, T1))

    def normed(load, mu, rs):
        return lambda i: jnp.concatenate([(load(2 * i + s) - mu) * rs for s in range(2)], axis=0)

    mus, out = [], []
    for load in loads:
        mus.append((yield from mean(load, lambda x: x, 32)))
    for load, mu in zip(loads, mus):
        var = yield from mean(load, lambda x: (x - mu) * (x - mu), 10)
        out.append(normed(load, mu, jax.lax.rsqrt(var + 1e-5)))
    return out


def _items(n):
    return lambda fn: lambda *args: (fn(*args), n)


def _interleave(*lists, lead=0.0, span=1.0):
    gens = [(v for g, _ in w for v in g) for w in lists]
    sizes = [sum(n for _, n in w) for w in lists]
    for _, k in sorted((i / n if k else i / n * span - lead, k)
                       for k, n in enumerate(sizes) for i in range(n)):
        next(gens[k])
    for g in gens:
        for _ in g:
            pass


def _strassen_lhs(a11, a12, a21, a22):
    return a11 + a22, a22, a21 + a22, a11 + a12, a11, a12 - a22, a21 - a11


def _strassen_rhs(b11, b12, b21, b22):
    return b11 + b22, b21 - b11, b11, b22, b12 - b22, b21 + b22, b11 + b12


def _strassen(prod, emit):
    m4 = prod(1)
    yield
    m2 = prod(2)
    emit(1, 0, m2 + m4)
    yield
    m1 = prod(0)
    c11, c22 = m1 + m4, m1 - m2
    yield
    c11 = c11 + prod(5)
    yield
    m5 = prod(3)
    emit(0, 0, c11 - m5)
    yield
    m3 = prod(4)
    emit(0, 1, m3 + m5)
    c22 = c22 + m3
    yield
    emit(1, 1, c22 + prod(6))
    yield


def _tree(op, xs):
    return xs[0] if len(xs) == 1 else op(_tree(op, xs[:len(xs) // 2]), _tree(op, xs[len(xs) // 2:]))


def _rows(i, n):
    return slice(i * n, i * n + n)


def _alternate(i):
    return pl.ds(16 * (i // 2) + i % 2, 8, stride=2)


def _kernel(u_hbm, are_hbm, aim_hbm, bre_hbm, bim_hbm, cre_hbm, cim_hbm, ldt_hbm, dsk_hbm,
            wqkv_hbm, wo_hbm, f_hbm, out_hbm,
            are, aim, bre, bim, cre, cim, ldt, dsk, io, wq_in, wo_in, fm, ws, wp, lam, dtc, k0s,
            tab, ztab, kb, kf, xr, xn, kv, xq, qs, oe, oo, ob, zs, sems):
    cp_u = [pltpu.make_async_copy(u_hbm.bitcast(U32).at[:, h, :], io.at[h], sems.at[3 + h])
            for h in range(PH // 2)]
    cp_o = [pltpu.make_async_copy(io.at[h], out_hbm.bitcast(U32).at[:, h, :], sems.at[3 + h])
            for h in range(PH // 2)]
    cp_f, cp_g = [pltpu.make_async_copy(f_hbm.at[_rows(i, PH)], fm.at[_rows(i, PH)], sems.at[0])
                  for i in range(2)]
    cp_wq = pltpu.make_async_copy(wqkv_hbm, wq_in, sems.at[1])
    cp_wo = pltpu.make_async_copy(wo_hbm, wo_in, sems.at[2])
    cp_p = [pltpu.make_async_copy(src, dst, sems.at[3 + PH // 2 + i])
            for i, (src, dst) in enumerate(
                ((ldt_hbm, ldt), (dsk_hbm, dsk), (aim_hbm, aim), (are_hbm, are),
                 (bre_hbm, bre), (bim_hbm, bim), (cre_hbm, cre), (cim_hbm, cim)))]
    for cp in cp_p:
        cp.start()

    lane = jax.lax.broadcasted_iota(I32, (8, T1), 1)
    zs[0] = 0

    def region(*lists, **pace):
        pl.when(zs[0] == 0)(lambda: _interleave(*lists, **pace))

    cp_p[0].wait()
    cp_p[1].wait()
    dt_row = jnp.exp(ldt[...].astype(F32).reshape(1, D)).astype(BF16).astype(F32)
    ds_row = dsk[...].astype(F32).reshape(1, D)
    for j in range(4):
        dtc[0, _rows(j, 128), :] = jnp.broadcast_to(dt_row[:, _rows(j, 128)], (128, 128)).T
        dtc[1, _rows(j, 128), :] = jnp.broadcast_to(ds_row[:, _rows(j, 128)], (128, 128)).T
    cp_p[2].wait()
    cp_p[3].wait()
    cp_u[0].start()
    cp_u[1].start()
    big = None
    for j in range(D // 16):
        r = _rows(j, 16)
        theta = dtc[0, r, :] * aim[r, :].astype(F32)
        mag = jnp.exp(dtc[0, r, :] * are[r, :].astype(F32))
        sn, cs = _sincos(theta)
        lam[0, r, :] = mag * cs
        lam[1, r, :] = mag * sn
        big = jnp.abs(theta) if big is None else jnp.maximum(big, jnp.abs(theta))

    @pl.when(jnp.logical_not(jnp.max(big) <= 8192.0))
    def _():
        def body(i, _):
            rows = pl.ds(pl.multiple_of(i * 16, 16), 16)
            th = dtc[0, rows, :] * aim[rows, :].astype(F32)
            mg = jnp.exp(dtc[0, rows, :] * are[rows, :].astype(F32))
            lam[0, rows, :] = mg * jnp.cos(th)
            lam[1, rows, :] = mg * jnp.sin(th)
        jax.lax.fori_loop(0, D // 16, body, None)

    for cp in cp_p[4:]:
        cp.wait()

    @_items(15)
    def tap_tables(blk, e, s):
        rows = pl.ds(CB * blk + 16 * e + s, 8, stride=2)

        def part(ref):
            return _unzip(pltpu.bitcast(ref[_rows(4 * blk + e, 16), :], U32), s)

        sc = dtc[0, rows, :] * (2.0 / L)
        w = _cmul((part(cre), part(cim)), (part(bre) * sc, part(bim) * sc))
        k0s[rows, :] = w[0]

        def put(row, a, b):
            for z in range(2):
                tab[blk % 4, 2 * s + z, pl.ds(row, 8, stride=QS), :] = pltpu.pack_elementwise(
                    [a[z], b[z]], packed_dtype=BF16)

        l1 = (lam[0, rows, :], lam[1, rows, :])
        l2 = _csq(l1)
        l16 = _csq(_csq(_csq(l2)))
        m1 = (l16[0], -l16[1])
        a, b = _cmul(w, l1), _cmul(w, l2)
        put(16 * e, (jnp.ones_like(m1[0]), jnp.zeros_like(m1[0])), m1)

        def columns(j, c):
            d = _cmul(c, m1)
            put(16 * e + j, c, d)
            yield c
            if j < 8:
                yield from columns(2 * j, _csq(c))
                yield from columns(2 * j + 1, _csq(d))

        keep = {}
        for j, c in enumerate(columns(1, _csq(m1)), 1):
            if j == 4:
                l512 = _csq((c[0], -c[1]))
            if j <= 8:
                put(64 + 12 * e + j - 1, a, b)
                keep[2 * j] = b
            if j < 8:
                a, b = _cmul(a, l2), _cmul(b, l2)
            if j == 8:
                put(64 + 12 * e + 8, _cmul(keep[4], l512), _cmul(keep[12], l512))
                a, b = keep[8], keep[16]
            if j in (10, 12, 14):
                a, b = _cmul(a, l512), _cmul(b, l512)
                put(64 + 12 * e + 4 + j // 2, a, b)
            yield

    @_items(48)
    def tap_sums(blk):
        for i in range(8):
            d = [jax.lax.dot_general(_bf(tab[blk % 4, z, pl.ds(QS * i + 64, 48), :]),
                                     _bf(tab[blk % 4, z, pl.ds(QS * i, 64), :]),
                                     NT, preferred_element_type=F32) for z in range(4)]
            own = [None] * 3
            for n in range(12):
                e, r = n // 3, _rows(n, 8)
                v = pltpu.pack_elementwise([d[0][r] + d[1][r], d[2][r] + d[3][r]],
                                           packed_dtype=BF16)
                own[n % 3] = jnp.where(lane < 32 * e, own[n % 3], v) if e else v
                if n % 2:
                    yield
            for r in range(3):
                ztab[blk % 4, pl.ds(ZS * i + 8 * r, 8), :] = own[r]

    @_items(2)
    def tap_blocks(blk, e):
        def at(r, g):
            z = ztab[blk % 4, pl.ds(r, 8, stride=ZS), :]
            return z if g == e else pltpu.roll(z, (32 * (g - e)) % 128, 1)

        def full(r, r1):
            return jnp.where(lane < 64, jnp.where(lane < 32, at(r, 0), at(r1, 1)),
                             jnp.where(lane < 96, at(r1 + 2, 2), at(r1 + 4, 3)))

        halves = [pl.ds(CB * blk + 16 * e + s, 8, stride=2) for s in range(2)]
        e8, e16 = full(7, 18), full(15, 19)
        k0 = pltpu.pack_elementwise(
            [jnp.sum(k0s[r, :], axis=1, keepdims=True) + dtc[1, r, :] * (2.0 / L) for r in halves],
            packed_dtype=BF16)
        e0 = jnp.where(lane == 0, k0, pltpu.roll(e16, 1, 1))
        e4 = jnp.where(lane < 32, at(3, 0), at(16, 1))
        e12 = jnp.where(lane < 32, at(11, 0), at(17, 1))
        k4, k12 = jnp.where(lane < 64, e4, e0), jnp.where(lane < 64, e12, e16)
        far = {1: e0, 2: e0, 3: k4, 5: jnp.where(lane < 64, e4, e8), 6: e8, 7: e8, 9: e8,
               10: e8, 11: jnp.where(lane < 64, e12, e8), 13: k12, 14: e16, 15: e16}
        taps = {0: e0, 4: k4, 8: e8, 12: k12}
        yield
        for p in range(PH):
            kb[p, _rows(4 * blk + e, 8), :] = taps[p] if p in taps else jnp.where(
                lane < (16 if p % 2 else 32), at(p - 1, 0), far[p])
        yield

    @_items(CB // 4)
    def lane_dft(src, blk, half):
        lo, hi = CB * blk, CB * blk + CB
        for q in range(4 * half, 4 * half + 4):
            x0, x1 = [jax.lax.dot_general(_bf(src[p, lo // 2:hi // 2, :]), _bf(fm[p]), NN,
                                          preferred_element_type=F32) for p in (q, q + 8)]
            for i in range((hi - lo) // 8):
                r = _rows(i, 8)
                for c, v in ((q, x0[r] + x1[r]), (q + 8, x0[r] - x1[r])):
                    for z in range(2):
                        kv[0, 2 * c + z, _rows(lo // 8 + i, 8), :] = v[:, _rows(z, T1)]
                if i % 2:
                    yield

    def residues(r, odd):
        return [(kv[0, 2 * c, r, :], kv[0, 2 * c + 1, r, :]) for c in range(8 * odd, 8 * odd + 8)]

    @_items(CB // 4)
    def tap_coefs(blk):
        for i in range(CB // 8):
            r = _rows(blk * CB // 8 + i, 8)
            for odd in range(2):
                for n, v in enumerate(_conv_coefs(residues(r, odd), 4 * odd)):
                    kf[10 * odd + n, r, :T1] = v[0]
                    kf[10 * odd + n, r, T1:] = v[1]
                yield

    r0 = jax.lax.broadcasted_iota(I32, (128, 128), 0)
    ri = (r0 & ~15) + (r0 & 7) * 2 + ((r0 >> 3) & 1)
    ci = jax.lax.broadcasted_iota(I32, (128, 128), 1)
    hit = ci == (ri & 7) * 16 + (ri >> 3)

    @_items(14)
    def prep_weights(j):
        def block(c, k):
            if j < 6:
                sel = jnp.where(hit, 1.0 if j < 4 else 0.25, 0.0)
                w = wq_in[_rows(k, 128), _rows(c, 128)]
            else:
                sel = jnp.where(ri == ci, 1.0, 0.0)
                w = _bf(wp[_rows(k, 64), _rows(c, 128)])
            return jax.lax.dot_general(sel.astype(BF16), w, NT, preferred_element_type=F32)

        top, bot = (4 + j, 8 + j) if j < 4 else (j % 2, j % 2 + 2)
        for k in range(2):
            for i, a in enumerate(_strassen_lhs(block(top, k), block(top, k + 2),
                                                block(bot, k), block(bot, k + 2))):
                ws[i, _rows(j, 64), _rows(k, 128)] = _zip(a)
                yield

    @_items(8)
    def permute_wo(j):
        sel = jnp.where(ci == (r0 & 7) * 16 + (r0 >> 3), 1.0, 0.0).astype(BF16)
        wp[_rows(j, 64), :] = _zip(jnp.dot(sel, wo_in[_rows(j, 128), :],
                                           preferred_element_type=F32))
        yield from range(8)

    @_items(4)
    def load_pair(h):
        for j in range(4):
            wds = io[h, :, _rows(j, 128)].T
            for s in range(2):
                xr[2 * h + s, _rows(j, 128), :] = _unzip(wds, s)
            yield

    def phase(p):
        return lambda i: xr[p, _alternate(i), :]

    @_items(24)
    def norm(h):
        both = yield from _layernorms([phase(2 * h), phase(2 * h + 1)])
        for p, normed in enumerate(both, 2 * h):
            for i in range(D // 16):
                xn[p, _rows(i, 8), :] = _zip(normed(i))
                if i % 8 == 7:
                    yield

    for i, step in enumerate(PROLOGUE):
        tables, sums, blocks, dft, coefs, loads, norms, perms, preps = [
            range(a, b) for a, b in zip(PROLOGUE[i - 1] if i else (0,) * 9, step)]
        for cp in {0: [cp_f], 1: cp_u[2:5], 2: cp_u[5:], 3: [cp_wo, cp_wq], 5: [cp_g]}.get(i, ()):
            cp.start()
        for cp, users in ((cp_f, dft), (cp_wo, perms), (cp_wq, preps)):
            if 0 in users:
                cp.wait()
        for h in loads:
            cp_u[h].wait()
        region([tap_sums(b) for b in sums]
               + [lane_dft(kb, b, s) for b in dft for s in range(2)]
               + [permute_wo(j) for j in perms] + [prep_weights(j) for j in preps]
               + ([lane_dft(xn, 0, 0), lane_dft(xn, 0, 1)] if step is PROLOGUE[-1] else []),
               [tap_tables(b, e, s) for b in tables for e in range(4) for s in range(2)]
               + [norm(h) for h in norms],
               [tap_blocks(b, e) for b in blocks for e in range(4)],
               [tap_coefs(b) for b in coefs],
               [load_pair(h) for h in loads],
               lead={1: 0.06, 3: 0.06, 4: 0.06, 5: 0.03}.get(i, 0.0),
               span={1: 1.0, 3: 1.0, 5: 1.1}.get(i, 1.05))

    cp_g.wait()

    @_items(10)
    def phase_conv(i):
        r = _rows(i, 8)
        coefs = ((kf[n, r, :T1], kf[n, r, T1:]) for n in range(NCOEF))
        for odd in range(2):
            y = yield from _conv(residues(r, odd), 4 * odd, lambda: next(coefs))
            for c, v in enumerate(y):
                for z in range(2):
                    kv[1, 16 * odd + 2 * c + z, r, :] = v[z]
            yield

    @_items(16)
    def lane_idft(blk, half):
        lo, hi = CB * blk, CB * blk + CB
        for q in range(half, 8, 2):
            a, b = [jnp.concatenate([kv[1, 2 * c + z, lo:hi, :] for z in range(2)], axis=1)
                    for c in (q, q + 8)]
            for p, v in ((q, a + b), (q + 8, a - b)):
                inv = jnp.concatenate([fm[PH + p, :, :T1], fm[PH + p, :, T1:]], axis=0)
                d = jax.lax.dot_general(v, _bf(inv), NN, preferred_element_type=F32)
                yield
                xr[p, lo:hi, :] += d
                yield

    @_items(32)
    def norm_pair(g):
        p = 4 * (g % 4) + g // 4
        a, b = yield from _layernorms([phase(p), phase(p + 2)])
        for r in range(HD // 16):
            for i, v in enumerate(_strassen_rhs(a(r), b(r), a(HD // 16 + r), b(HD // 16 + r))):
                xq[g, _rows(r, 8), _rows(i, T1)] = _zip(v)
            yield

    def block_product(row0, groups, rhs, emit):
        for r in [128 // RS * hg + i for hg in groups for i in range(128 // RS)]:
            w = slice((row0 + r * RS) // 2, (row0 + r * RS + RS) // 2)
            yield from _strassen(
                lambda i: jnp.dot(_bf(ws[i, w, :]), _bf(rhs[:, _rows(i, T1)]),
                                  preferred_element_type=F32),
                lambda half, n, y: emit(half, n, r * RS, y))

    @_items(7 * HD // RS)
    def keys_values(s, g):
        def emit(half, n, row, y):
            m = 2 * (g % 4) + n
            kv[g // 4, PH * half + WIN - 1 + m, pl.ds(row, RS), :] = y
            if m:
                kv[g // 4, PH * half + m - 1, pl.ds(row, RS), :] = pltpu.roll(y, 1, 1)

        return block_product(0, (s, s + 2), xq.at[g], emit)

    @_items(7 * 128 // RS)
    def queries(s, g):
        def emit(half, n, row, y):
            qs[g, n, pl.ds(HD * half + row, RS), :] = y

        return block_product(D, (s,), xq.at[g], emit)

    @_items(34)
    def attend(par, s, m):
        def group(hg):
            lg = [None] * WIN
            for dh in range(16):
                r = _rows(16 * hg + dh, 8)
                q = qs[4 * par + m // 2, m % 2, r, :]
                for j in range(WIN):
                    t = q * kv[par, WIN - 1 + m - j, r, :]
                    lg[j] = t if dh == 0 else lg[j] + t
                if dh % 2:
                    yield
            for j in range(m + 1, WIN):
                lg[j] = jnp.where(lane == 0, -1e9, lg[j])
            mx = _tree(jnp.maximum, lg)
            ex = [jnp.exp(t - mx) for t in lg]
            den = _tree(jnp.add, ex)
            inv = pltpu.reciprocal(den, full_range=False)
            pr = [t * inv for t in ex]
            yield

            def out(dh):
                r = _rows(16 * hg + dh, 8)
                acc = pr[0] * kv[par, PH + WIN - 1 + m, r, :]
                for j in range(1, WIN):
                    acc = acc + pr[j] * kv[par, PH + WIN - 1 + m - j, r, :]
                return acc

            for d2 in range(8):
                o = jnp.concatenate([out(2 * d2), out(2 * d2 + 1)], axis=0)
                r = _rows(8 * hg + d2, 16)
                if par == 0 or hg < 2:
                    (oe, oo)[par][m, r, :] = o
                if hg >= 2:
                    r1 = _rows(8 * (hg - 2) + d2, 16)
                    ops = (_strassen_rhs(oe[m, r1, :], oo[m, r1, :], oe[m, r, :], o) if par
                           else _strassen_rhs(oe[m, r1, :], o, o, o))
                    for i in (0, 3, 4, 5, 6) if par else (1, 2):
                        ob[m, _rows(8 * (hg - 2) + d2, 8), _rows(i, T1)] = _zip(ops[i])
                yield

        a, b = group(s), group(s + 2)
        for g, n in ((a, 9), (b, 9), (a, 8), (b, 8)):
            for _ in range(n):
                yield next(g)

    late = (1, 4, 6)

    @_items(7 * HD // RS)
    def project(h, store):
        def emit(half, n, row, y):
            xr[2 * h + n, pl.ds(HD * half + row, RS), :] += y

        for s in range(2):
            yield from block_product(D + HD, (s,), ob.at[h], emit)
            if store:
                for _ in store_pair(h, (s, s + 2))[0]:
                    pass

    @_items(4)
    def store_pair(h, groups):
        for j in groups:
            io[h, :, _rows(j, 128)] = pltpu.pack_elementwise(
                [xr[2 * h + n, _rows(j, 128), :] for n in range(2)], packed_dtype=BF16).T
            yield

    def layer(it, c):
        def send(hs):
            @pl.when(it == 1)
            def _():
                for h in hs:
                    cp_o[h].start()

        for i in range(len(DFT) - 1):
            last = i == len(DFT) - 2
            region([lane_dft(xn, c // 2, c % 2) for c in range(*DFT[i:i + 2])]
                   + [lane_idft(c // 2, c % 2) for c in range(*IDFT[i:i + 2])],
                   [phase_conv(r) for r in range(*CONV[i:i + 2])]
                   + ([norm_pair(0)] if last else []),
                   lead=0.4 if last else 0.0, span=0.95 if i == 3 else 1.0)
        region([keys_values(0, 0), keys_values(1, 0), queries(0, 0)],
               [norm_pair(g) for g in (1, 2, 3)])
        region([fn(0, g) for fn in (keys_values, queries) for g in (1, 2, 3)],
               [norm_pair(g) for g in (4, 5, 6, 7)])
        for par, s, kvg, qg in ((0, 0, (1, 2, 3), (0, 1, 2, 3)), (0, 1, (4, 5, 6, 7), (4, 5, 6, 7)),
                                (1, 0, (4, 5, 6, 7), (4, 5))):
            region([keys_values(1 - s, g) for g in kvg] + [queries(1 - s, g) for g in qg],
                   [attend(par, s, m) for m in range(WIN)], span=1.05)
        region([queries(1, g) for g in (6, 7)], [attend(1, 1, m) for m in (0, 1)], span=0.95)
        done = ()
        for hs, ms in (((0, 1), (2, 3, 4)), ((2, 3, 4), (5, 6, 7)), ((5, 6), ())):
            region([project(h, h not in late) for h in hs],
                   [store_pair(h, range(4)) for h in done if h in late]
                   + [norm(h) for h in done] + [attend(1, 1, m) for m in ms],
                   span=1.0 if ms else 1.05)
            send([h for h in done if h in late] + [h for h in hs if h not in late])
            done = hs

        @pl.when(it == 0)
        def _():
            _interleave([project(7, False)], [norm(5), norm(6)])
            _interleave([lane_dft(xn, 0, 0), lane_dft(xn, 0, 1)], [norm(7)], span=1.5)

    @_items(1)
    def send_now(h):
        cp_o[h].start()
        yield

    jax.lax.fori_loop(0, 2, layer, None)
    _interleave([project(7, True)], [store_pair(6, range(4)), send_now(6)], span=4.0)
    cp_o[7].start()
    for cp in cp_o:
        cp.wait()


@jax.jit
def pallas_interleave_layers__ssm_conv_s4__sliding_local_dilated__prompt_kernel(
    A_u: jax.Array,
    A_A_re: jax.Array,
    A_A_im: jax.Array,
    A_B_re: jax.Array,
    A_B_im: jax.Array,
    A_C_re: jax.Array,
    A_C_im: jax.Array,
    A_log_dt: jax.Array,
    A_Dskip: jax.Array,
    B_x: jax.Array,
    B_wqkv: jax.Array,
    B_wo: jax.Array,
):
    del B_x
    hbm = pl.BlockSpec(memory_space=pl.ANY)
    out = pl.pallas_call(
        _kernel,
        in_specs=[hbm] * 12,
        out_specs=hbm,
        out_shape=jax.ShapeDtypeStruct((T1, PH, D), BF16),
        scratch_shapes=[pltpu.VMEM((D, NS), BF16)] * 6 + [pltpu.VMEM((D,), BF16)] * 2 + [
            pltpu.VMEM((PH // 2, T1, D), U32),
            pltpu.VMEM((D, 3 * D), BF16),
            pltpu.VMEM((D, D), BF16),
            pltpu.VMEM((2 * PH, T1 // 2, 2 * T1), U32),
            pltpu.VMEM((7, D, HD), U32),
            pltpu.VMEM((D // 2, D), U32),
            pltpu.VMEM((2, D + 8, NS), F32),
            pltpu.VMEM((2, D + 8, NS), F32),
            pltpu.VMEM((D + 8, NS), F32),
            pltpu.VMEM((4, 4, 9 * QS + 4, NS), U32),
            pltpu.VMEM((4, 9 * ZS + 4, T1), U32),
            pltpu.VMEM((PH, D // 2, T1), U32),
            pltpu.VMEM((NCOEF, D, 2 * T1), F32),
            pltpu.VMEM((PH, D + 8, T1), F32),
            pltpu.VMEM((PH, D // 2, T1), U32),
            pltpu.VMEM((2, 2 * PH, D, T1), F32),
            pltpu.VMEM((PH // 2, HD // 2, 7 * T1), U32),
            pltpu.VMEM((PH // 2, 2, D, T1), F32),
            pltpu.VMEM((WIN, D, T1), F32),
            pltpu.VMEM((WIN, HD, T1), F32),
            pltpu.VMEM((WIN, HD // 2, 7 * T1), U32),
            pltpu.SMEM((1,), I32),
            pltpu.SemaphoreType.DMA((11 + PH // 2,)),
        ],
        compiler_params=pltpu.CompilerParams(vmem_limit_bytes=100 * 1024 * 1024),
    )(A_u.reshape(T1, PH, D), A_A_re, A_A_im, A_B_re, A_B_im, A_C_re, A_C_im,
      A_log_dt, A_Dskip, B_wqkv, B_wo,
      _dft_matrices())
    return out.reshape(1, L, D)
```

```python
import numpy as np

import jax
import jax.numpy as jnp
import jax.experimental.pallas as pl
import jax.experimental.pallas.tpu as pltpu

F32, BF16, U32, I32 = jnp.float32, jnp.bfloat16, jnp.uint32, jnp.int32
L, D, NS = 2048, 512, 128
PH, T1 = 16, 128
WIN = 8
NN = (((1,), (0,)), ((), ()))
NT = (((1,), (1,)), ((), ()))
QS = 116
ZS = 28
_H = float(np.sqrt(0.5))
NCOEF = 22
HD = D // 2
RS = 64
DFT = (2, 6, 10, 14, 16, 16, 16)
CONV = (0, 8, 24, 40, 56, 64, 64)
IDFT = (0, 0, 2, 6, 10, 14, 16)
PROLOGUE = ((2, 0, 0, 0, 0, 0, 0, 0, 0),
            (4, 2, 0, 0, 0, 1, 0, 0, 0),
            (6, 4, 2, 0, 0, 2, 0, 0, 0),
            (8, 6, 4, 2, 0, 5, 0, 0, 0),
            (8, 8, 6, 4, 2, 8, 3, 0, 0),
            (8, 8, 8, 6, 4, 8, 5, 4, 2),
            (8, 8, 8, 8, 6, 8, 8, 4, 6),
            (8, 8, 8, 8, 8, 8, 8, 4, 8))
CB = 64


def _dft_matrices():
    t = 16 * np.arange(T1)[None, :, None] + np.arange(PH)[:, None, None]
    k = np.arange(T1)[None, None, :] + 0.5
    phi = 2.0 * np.pi * k * t / (2 * L)
    phi = np.concatenate([phi, phi.transpose(0, 2, 1)])
    f = np.concatenate([np.cos(phi), -np.sin(phi)], axis=-1).astype(np.float32)
    bits = f.astype(BF16).view(np.uint16).astype(np.uint32)
    return bits[:, 0::2] | (bits[:, 1::2] << 16)


def _cmul(a, b):
    return a[0] * b[0] - a[1] * b[1], a[0] * b[1] + a[1] * b[0]


def _csq(a):
    t = a[0] * a[1]
    return a[0] * a[0] - a[1] * a[1], t + t


def _cadd(a, b):
    return a[0] + b[0], a[1] + b[1]


def _csub(a, b):
    return a[0] - b[0], a[1] - b[1]


def _rot8(x, e):
    s, d = x[0] + x[1], x[0] - x[1]
    return {1: (d * _H, s * _H), 3: (s * -_H, d * _H), 5: (d * -_H, s * -_H), 7: (s * _H, d * -_H)}[e]


def _split(x, e):
    n = len(x) // 2
    lo, hi = x[:n], x[n:]
    if e == 4:
        return ([(a[0] - b[1], a[1] + b[0]) for a, b in zip(lo, hi)],
                [(a[0] + b[1], a[1] - b[0]) for a, b in zip(lo, hi)])
    if e:
        hi = [_rot8(b, e // 2) for b in hi]
    return [_cadd(a, b) for a, b in zip(lo, hi)], [_csub(a, b) for a, b in zip(lo, hi)]


def _merge(p, m, e):
    lo = [_cadd(a, b) for a, b in zip(p, m)]
    if e == 4:
        return lo + [(a[1] - b[1], b[0] - a[0]) for a, b in zip(p, m)]
    hi = [_csub(a, b) for a, b in zip(p, m)]
    return lo + ([_rot8(b, 8 - e // 2) for b in hi] if e else hi)


def _conv_coefs(k, e):
    if len(k) == 1:
        return [(k[0][0] * 0.5, k[0][1] * 0.5)]
    if len(k) == 2 and e % 4:
        if e % 2:
            top = _csub(_rot8(k[1], e), k[0])
        elif e == 2:
            top = (-k[1][1] - k[0][0], k[1][0] - k[0][1])
        else:
            top = (k[1][1] - k[0][0], -k[1][0] - k[0][1])
        return [k[0], top, _csub(k[1], k[0])]
    p, m = _split(k, e)
    return _conv_coefs(p, e // 2) + _conv_coefs(m, e // 2 + 4)


def _conv(x, e, coef):
    if len(x) == 1:
        return [_cmul(x[0], coef())]
    if len(x) == 2:
        yield
    if len(x) == 2 and e % 4:
        both = _cmul(_cadd(x[0], x[1]), coef())
        return [_cadd(both, _cmul(x[1], coef())), _cadd(both, _cmul(x[0], coef()))]
    p, m = _split(x, e)
    p = yield from _conv(p, e // 2, coef)
    m = yield from _conv(m, e // 2 + 4, coef)
    return _merge(p, m, e)


def _sincos(x):
    n = jnp.floor(x * float(2.0 / np.pi) + 0.5)
    r = ((x - n * 1.5703125) - n * 4.837512969970703125e-4) - n * 7.54978995489188216e-8
    z = r * r
    s = r + r * z * ((-1.9515295891e-4 * z + 8.3321608736e-3) * z - 1.6666654611e-1)
    c = 1.0 + z * (((2.443315711809948e-5 * z - 1.388731625493765e-3) * z
                    + 4.166664568298827e-2) * z - 0.5)
    q = n.astype(I32)
    odd = (q & 1) == 1
    s, c = jnp.where(odd, c, s), jnp.where(odd, s, c)
    return jnp.where((q & 2) == 2, -s, s), jnp.where(((q + 1) & 2) == 2, -c, c)


def _zip(x):
    return jnp.concatenate(
        [pltpu.pack_elementwise([x[i:i + 8], x[i + 8:i + 16]], packed_dtype=BF16)
         for i in range(0, x.shape[0], 16)], axis=0)


def _unzip(words, s):
    return pltpu.bitcast(words & np.uint32(0xFFFF0000) if s else words << 16, F32)


def _bf(words):
    return pltpu.bitcast(words, BF16)


def _layernorms(loads):
    def mean(load, term, every):
        acc = [term(load(i)) for i in range(4)]
        for i in range(4, D // 8):
            acc[i % 4] = acc[i % 4] + term(load(i))
            if i % every == every - 1:
                yield
        tot = jnp.sum(_tree(jnp.add, acc), axis=0, keepdims=True)
        return jnp.broadcast_to(tot * (1.0 / D), (8, T1))

    def normed(load, mu, rs):
        return lambda i: jnp.concatenate([(load(2 * i + s) - mu) * rs for s in range(2)], axis=0)

    mus, out = [], []
    for load in loads:
        mus.append((yield from mean(load, lambda x: x, 32)))
    for load, mu in zip(loads, mus):
        var = yield from mean(load, lambda x: (x - mu) * (x - mu), 10)
        out.append(normed(load, mu, jax.lax.rsqrt(var + 1e-5)))
    return out


def _items(n):
    return lambda fn: lambda *args: (fn(*args), n)


def _interleave(*lists, lead=0.0, span=1.0):
    gens = [(v for g, _ in w for v in g) for w in lists]
    sizes = [sum(n for _, n in w) for w in lists]
    for _, k in sorted((i / n if k else i / n * span - lead, k)
                       for k, n in enumerate(sizes) for i in range(n)):
        next(gens[k])
    for g in gens:
        for _ in g:
            pass


def _strassen_lhs(a11, a12, a21, a22):
    return a11 + a22, a22, a21 + a22, a11 + a12, a11, a12 - a22, a21 - a11


def _strassen_rhs(b11, b12, b21, b22):
    return b11 + b22, b21 - b11, b11, b22, b12 - b22, b21 + b22, b11 + b12


def _strassen(prod, emit):
    m4 = prod(1)
    yield
    m2 = prod(2)
    emit(1, 0, m2 + m4)
    yield
    m1 = prod(0)
    c11, c22 = m1 + m4, m1 - m2
    yield
    c11 = c11 + prod(5)
    yield
    m5 = prod(3)
    emit(0, 0, c11 - m5)
    yield
    m3 = prod(4)
    emit(0, 1, m3 + m5)
    c22 = c22 + m3
    yield
    emit(1, 1, c22 + prod(6))
    yield


def _tree(op, xs):
    return xs[0] if len(xs) == 1 else op(_tree(op, xs[:len(xs) // 2]), _tree(op, xs[len(xs) // 2:]))


def _rows(i, n):
    return slice(i * n, i * n + n)


def _alternate(i):
    return pl.ds(16 * (i // 2) + i % 2, 8, stride=2)


def _kernel(u_hbm, are_hbm, aim_hbm, bre_hbm, bim_hbm, cre_hbm, cim_hbm, ldt_hbm, dsk_hbm,
            wqkv_hbm, wo_hbm, f_hbm, out_hbm,
            are, aim, bre, bim, cre, cim, ldt, dsk, io, wq_in, wo_in, fm, ws, wp, lam, dtc, k0s,
            tab, ztab, kb, kf, xr, xn, kv, xq, qs, oe, oo, ob, zs, sems):
    cp_u = [pltpu.make_async_copy(u_hbm.bitcast(U32).at[:, h, :], io.at[h], sems.at[3 + h])
            for h in range(PH // 2)]
    cp_o = [pltpu.make_async_copy(io.at[h], out_hbm.bitcast(U32).at[:, h, :], sems.at[3 + h])
            for h in range(PH // 2)]
    cp_f, cp_g = [pltpu.make_async_copy(f_hbm.at[_rows(i, PH)], fm.at[_rows(i, PH)], sems.at[0])
                  for i in range(2)]
    cp_wq = pltpu.make_async_copy(wqkv_hbm, wq_in, sems.at[1])
    cp_wo = pltpu.make_async_copy(wo_hbm, wo_in, sems.at[2])
    cp_p = [pltpu.make_async_copy(src, dst, sems.at[3 + PH // 2 + i])
            for i, (src, dst) in enumerate(
                ((ldt_hbm, ldt), (dsk_hbm, dsk), (aim_hbm, aim), (are_hbm, are),
                 (bre_hbm, bre), (bim_hbm, bim), (cre_hbm, cre), (cim_hbm, cim)))]
    for cp in cp_p[:4]:
        cp.start()

    lane = jax.lax.broadcasted_iota(I32, (8, T1), 1)
    zs[0] = 0

    def region(*lists, **pace):
        pl.when(zs[0] == 0)(lambda: _interleave(*lists, **pace))

    cp_p[0].wait()
    cp_p[1].wait()
    for cp in cp_p[4:]:
        cp.start()
    dt_row = jnp.exp(ldt[...].astype(F32).reshape(1, D)).astype(BF16).astype(F32)
    ds_row = dsk[...].astype(F32).reshape(1, D)
    for j in range(4):
        dtc[0, _rows(j, 128), :] = jnp.broadcast_to(dt_row[:, _rows(j, 128)], (128, 128)).T
        dtc[1, _rows(j, 128), :] = jnp.broadcast_to(ds_row[:, _rows(j, 128)], (128, 128)).T
    cp_p[2].wait()
    cp_p[3].wait()
    big = None
    for j in range(D // 16):
        r = _rows(j, 16)
        theta = dtc[0, r, :] * aim[r, :].astype(F32)
        mag = jnp.exp(dtc[0, r, :] * are[r, :].astype(F32))
        sn, cs = _sincos(theta)
        lam[0, r, :] = mag * cs
        lam[1, r, :] = mag * sn
        big = jnp.abs(theta) if big is None else jnp.maximum(big, jnp.abs(theta))

    @pl.when(jnp.logical_not(jnp.max(big) <= 8192.0))
    def _():
        def body(i, _):
            rows = pl.ds(pl.multiple_of(i * 16, 16), 16)
            th = dtc[0, rows, :] * aim[rows, :].astype(F32)
            mg = jnp.exp(dtc[0, rows, :] * are[rows, :].astype(F32))
            lam[0, rows, :] = mg * jnp.cos(th)
            lam[1, rows, :] = mg * jnp.sin(th)
        jax.lax.fori_loop(0, D // 16, body, None)

    for cp in cp_p[4:]:
        cp.wait()

    @_items(15)
    def tap_tables(blk, e, s):
        rows = pl.ds(CB * blk + 16 * e + s, 8, stride=2)

        def part(ref):
            return _unzip(pltpu.bitcast(ref[_rows(4 * blk + e, 16), :], U32), s)

        sc = dtc[0, rows, :] * (2.0 / L)
        w = _cmul((part(cre), part(cim)), (part(bre) * sc, part(bim) * sc))
        k0s[rows, :] = w[0]

        def put(row, a, b):
            for z in range(2):
                tab[blk % 4, 2 * s + z, pl.ds(row, 8, stride=QS), :] = pltpu.pack_elementwise(
                    [a[z], b[z]], packed_dtype=BF16)

        l1 = (lam[0, rows, :], lam[1, rows, :])
        l2 = _csq(l1)
        l16 = _csq(_csq(_csq(l2)))
        m1 = (l16[0], -l16[1])
        a, b = _cmul(w, l1), _cmul(w, l2)
        put(16 * e, (jnp.ones_like(m1[0]), jnp.zeros_like(m1[0])), m1)

        def columns(j, c):
            d = _cmul(c, m1)
            put(16 * e + j, c, d)
            yield c
            if j < 8:
                yield from columns(2 * j, _csq(c))
                yield from columns(2 * j + 1, _csq(d))

        keep = {}
        for j, c in enumerate(columns(1, _csq(m1)), 1):
            if j == 4:
                l512 = _csq((c[0], -c[1]))
            if j <= 8:
                put(64 + 12 * e + j - 1, a, b)
                keep[2 * j] = b
            if j < 8:
                a, b = _cmul(a, l2), _cmul(b, l2)
            if j == 8:
                put(64 + 12 * e + 8, _cmul(keep[4], l512), _cmul(keep[12], l512))
                a, b = keep[8], keep[16]
            if j in (10, 12, 14):
                a, b = _cmul(a, l512), _cmul(b, l512)
                put(64 + 12 * e + 4 + j // 2, a, b)
            yield

    @_items(48)
    def tap_sums(blk):
        for i in range(8):
            d = [jax.lax.dot_general(_bf(tab[blk % 4, z, pl.ds(QS * i + 64, 48), :]),
                                     _bf(tab[blk % 4, z, pl.ds(QS * i, 64), :]),
                                     NT, preferred_element_type=F32) for z in range(4)]
            own = [None] * 3
            for n in range(12):
                e, r = n // 3, _rows(n, 8)
                v = pltpu.pack_elementwise([d[0][r] + d[1][r], d[2][r] + d[3][r]],
                                           packed_dtype=BF16)
                own[n % 3] = jnp.where(lane < 32 * e, own[n % 3], v) if e else v
                if n % 2:
                    yield
            for r in range(3):
                ztab[blk % 4, pl.ds(ZS * i + 8 * r, 8), :] = own[r]

    @_items(2)
    def tap_blocks(blk, e):
        def at(r, g):
            z = ztab[blk % 4, pl.ds(r, 8, stride=ZS), :]
            return z if g == e else pltpu.roll(z, (32 * (g - e)) % 128, 1)

        def full(r, r1):
            return jnp.where(lane < 64, jnp.where(lane < 32, at(r, 0), at(r1, 1)),
                             jnp.where(lane < 96, at(r1 + 2, 2), at(r1 + 4, 3)))

        halves = [pl.ds(CB * blk + 16 * e + s, 8, stride=2) for s in range(2)]
        e8, e16 = full(7, 18), full(15, 19)
        k0 = pltpu.pack_elementwise(
            [jnp.sum(k0s[r, :], axis=1, keepdims=True) + dtc[1, r, :] * (2.0 / L) for r in halves],
            packed_dtype=BF16)
        e0 = jnp.where(lane == 0, k0, pltpu.roll(e16, 1, 1))
        e4 = jnp.where(lane < 32, at(3, 0), at(16, 1))
        e12 = jnp.where(lane < 32, at(11, 0), at(17, 1))
        k4, k12 = jnp.where(lane < 64, e4, e0), jnp.where(lane < 64, e12, e16)
        far = {1: e0, 2: e0, 3: k4, 5: jnp.where(lane < 64, e4, e8), 6: e8, 7: e8, 9: e8,
               10: e8, 11: jnp.where(lane < 64, e12, e8), 13: k12, 14: e16, 15: e16}
        taps = {0: e0, 4: k4, 8: e8, 12: k12}
        yield
        for p in range(PH):
            kb[p, _rows(4 * blk + e, 8), :] = taps[p] if p in taps else jnp.where(
                lane < (16 if p % 2 else 32), at(p - 1, 0), far[p])
        yield

    @_items(CB // 4)
    def lane_dft(src, blk, half):
        lo, hi = CB * blk, CB * blk + CB
        for q in range(4 * half, 4 * half + 4):
            x0, x1 = [jax.lax.dot_general(_bf(src[p, lo // 2:hi // 2, :]), _bf(fm[p]), NN,
                                          preferred_element_type=F32) for p in (q, q + 8)]
            for i in range((hi - lo) // 8):
                r = _rows(i, 8)
                for c, v in ((q, x0[r] + x1[r]), (q + 8, x0[r] - x1[r])):
                    for z in range(2):
                        kv[0, 2 * c + z, _rows(lo // 8 + i, 8), :] = v[:, _rows(z, T1)]
                if i % 2:
                    yield

    def residues(r, odd):
        return [(kv[0, 2 * c, r, :], kv[0, 2 * c + 1, r, :]) for c in range(8 * odd, 8 * odd + 8)]

    @_items(CB // 4)
    def tap_coefs(blk):
        for i in range(CB // 8):
            r = _rows(blk * CB // 8 + i, 8)
            for odd in range(2):
                for n, v in enumerate(_conv_coefs(residues(r, odd), 4 * odd)):
                    kf[10 * odd + n, r, :T1] = v[0]
                    kf[10 * odd + n, r, T1:] = v[1]
                yield

    r0 = jax.lax.broadcasted_iota(I32, (128, 128), 0)
    ri = (r0 & ~15) + (r0 & 7) * 2 + ((r0 >> 3) & 1)
    ci = jax.lax.broadcasted_iota(I32, (128, 128), 1)
    hit = ci == (ri & 7) * 16 + (ri >> 3)

    @_items(14)
    def prep_weights(j):
        def block(c, k):
            if j < 6:
                sel = jnp.where(hit, 1.0 if j < 4 else 0.25, 0.0)
                w = wq_in[_rows(k, 128), _rows(c, 128)]
            else:
                sel = jnp.where(ri == ci, 1.0, 0.0)
                w = _bf(wp[_rows(k, 64), _rows(c, 128)])
            return jax.lax.dot_general(sel.astype(BF16), w, NT, preferred_element_type=F32)

        top, bot = (4 + j, 8 + j) if j < 4 else (j % 2, j % 2 + 2)
        for k in range(2):
            for i, a in enumerate(_strassen_lhs(block(top, k), block(top, k + 2),
                                                block(bot, k), block(bot, k + 2))):
                ws[i, _rows(j, 64), _rows(k, 128)] = _zip(a)
                yield

    @_items(8)
    def permute_wo(j):
        sel = jnp.where(ci == (r0 & 7) * 16 + (r0 >> 3), 1.0, 0.0).astype(BF16)
        wp[_rows(j, 64), :] = _zip(jnp.dot(sel, wo_in[_rows(j, 128), :],
                                           preferred_element_type=F32))
        yield from range(8)

    @_items(4)
    def load_pair(h):
        for j in range(4):
            wds = io[h, :, _rows(j, 128)].T
            for s in range(2):
                xr[2 * h + s, _rows(j, 128), :] = _unzip(wds, s)
            yield

    def phase(p):
        return lambda i: xr[p, _alternate(i), :]

    @_items(24)
    def norm(h):
        both = yield from _layernorms([phase(2 * h), phase(2 * h + 1)])
        for p, normed in enumerate(both, 2 * h):
            for i in range(D // 16):
                xn[p, _rows(i, 8), :] = _zip(normed(i))
                if i % 8 == 7:
                    yield

    for i, step in enumerate(PROLOGUE):
        tables, sums, blocks, dft, coefs, loads, norms, perms, preps = [
            range(a, b) for a, b in zip(PROLOGUE[i - 1] if i else (0,) * 9, step)]
        for cp in {0: cp_u[:2], 1: [cp_f] + cp_u[2:5], 2: cp_u[5:], 3: [cp_wo, cp_wq], 5: [cp_g]}.get(i, ()):
            cp.start()
        for cp, users in ((cp_f, dft), (cp_wo, perms), (cp_wq, preps)):
            if 0 in users:
                cp.wait()
        for h in loads:
            cp_u[h].wait()
        region([tap_sums(b) for b in sums]
               + [lane_dft(kb, b, s) for b in dft for s in range(2)]
               + [permute_wo(j) for j in perms] + [prep_weights(j) for j in preps]
               + ([lane_dft(xn, 0, 0), lane_dft(xn, 0, 1)] if step is PROLOGUE[-1] else []),
               [tap_tables(b, e, s) for b in tables for e in range(4) for s in range(2)]
               + [norm(h) for h in norms],
               [tap_blocks(b, e) for b in blocks for e in range(4)],
               [tap_coefs(b) for b in coefs],
               [load_pair(h) for h in loads],
               lead={1: 0.06, 3: 0.06, 4: 0.06, 5: 0.03}.get(i, 0.0),
               span={1: 1.0, 3: 1.0, 5: 1.1}.get(i, 1.05))

    cp_g.wait()

    @_items(10)
    def phase_conv(i):
        r = _rows(i, 8)
        coefs = ((kf[n, r, :T1], kf[n, r, T1:]) for n in range(NCOEF))
        for odd in range(2):
            y = yield from _conv(residues(r, odd), 4 * odd, lambda: next(coefs))
            for c, v in enumerate(y):
                for z in range(2):
                    kv[1, 16 * odd + 2 * c + z, r, :] = v[z]
            yield

    @_items(16)
    def lane_idft(blk, half):
        lo, hi = CB * blk, CB * blk + CB
        for q in range(half, 8, 2):
            a, b = [jnp.concatenate([kv[1, 2 * c + z, lo:hi, :] for z in range(2)], axis=1)
                    for c in (q, q + 8)]
            for p, v in ((q, a + b), (q + 8, a - b)):
                inv = jnp.concatenate([fm[PH + p, :, :T1], fm[PH + p, :, T1:]], axis=0)
                d = jax.lax.dot_general(v, _bf(inv), NN, preferred_element_type=F32)
                yield
                xr[p, lo:hi, :] += d
                yield

    @_items(32)
    def norm_pair(g):
        p = 4 * (g % 4) + g // 4
        a, b = yield from _layernorms([phase(p), phase(p + 2)])
        for r in range(HD // 16):
            for i, v in enumerate(_strassen_rhs(a(r), b(r), a(HD // 16 + r), b(HD // 16 + r))):
                xq[g, _rows(r, 8), _rows(i, T1)] = _zip(v)
            yield

    def block_product(row0, groups, rhs, emit):
        for r in [128 // RS * hg + i for hg in groups for i in range(128 // RS)]:
            w = slice((row0 + r * RS) // 2, (row0 + r * RS + RS) // 2)
            yield from _strassen(
                lambda i: jnp.dot(_bf(ws[i, w, :]), _bf(rhs[:, _rows(i, T1)]),
                                  preferred_element_type=F32),
                lambda half, n, y: emit(half, n, r * RS, y))

    @_items(7 * HD // RS)
    def keys_values(s, g):
        def emit(half, n, row, y):
            m = 2 * (g % 4) + n
            kv[g // 4, PH * half + WIN - 1 + m, pl.ds(row, RS), :] = y
            if m:
                kv[g // 4, PH * half + m - 1, pl.ds(row, RS), :] = pltpu.roll(y, 1, 1)

        return block_product(0, (s, s + 2), xq.at[g], emit)

    @_items(7 * 128 // RS)
    def queries(s, g):
        def emit(half, n, row, y):
            qs[g, n, pl.ds(HD * half + row, RS), :] = y

        return block_product(D, (s,), xq.at[g], emit)

    @_items(34)
    def attend(par, s, m):
        def group(hg):
            lg = [None] * WIN
            for dh in range(16):
                r = _rows(16 * hg + dh, 8)
                q = qs[4 * par + m // 2, m % 2, r, :]
                for j in range(WIN):
                    t = q * kv[par, WIN - 1 + m - j, r, :]
                    lg[j] = t if dh == 0 else lg[j] + t
                if dh % 2:
                    yield
            for j in range(m + 1, WIN):
                lg[j] = jnp.where(lane == 0, -1e9, lg[j])
            mx = _tree(jnp.maximum, lg)
            ex = [jnp.exp(t - mx) for t in lg]
            den = _tree(jnp.add, ex)
            inv = pltpu.reciprocal(den, full_range=False)
            pr = [t * inv for t in ex]
            yield

            def out(dh):
                r = _rows(16 * hg + dh, 8)
                acc = pr[0] * kv[par, PH + WIN - 1 + m, r, :]
                for j in range(1, WIN):
                    acc = acc + pr[j] * kv[par, PH + WIN - 1 + m - j, r, :]
                return acc

            for d2 in range(8):
                o = jnp.concatenate([out(2 * d2), out(2 * d2 + 1)], axis=0)
                r = _rows(8 * hg + d2, 16)
                if par == 0 or hg < 2:
                    (oe, oo)[par][m, r, :] = o
                if hg >= 2:
                    r1 = _rows(8 * (hg - 2) + d2, 16)
                    ops = (_strassen_rhs(oe[m, r1, :], oo[m, r1, :], oe[m, r, :], o) if par
                           else _strassen_rhs(oe[m, r1, :], o, o, o))
                    for i in (0, 3, 4, 5, 6) if par else (1, 2):
                        ob[m, _rows(8 * (hg - 2) + d2, 8), _rows(i, T1)] = _zip(ops[i])
                yield

        a, b = group(s), group(s + 2)
        for g, n in ((a, 9), (b, 9), (a, 8), (b, 8)):
            for _ in range(n):
                yield next(g)

    late = (1, 4, 6)

    @_items(7 * HD // RS)
    def project(h, store):
        def emit(half, n, row, y):
            xr[2 * h + n, pl.ds(HD * half + row, RS), :] += y

        for s in range(2):
            yield from block_product(D + HD, (s,), ob.at[h], emit)
            if store:
                for _ in store_pair(h, (s, s + 2))[0]:
                    pass

    @_items(4)
    def store_pair(h, groups):
        for j in groups:
            io[h, :, _rows(j, 128)] = pltpu.pack_elementwise(
                [xr[2 * h + n, _rows(j, 128), :] for n in range(2)], packed_dtype=BF16).T
            yield

    def layer(it, c):
        def send(hs):
            @pl.when(it == 1)
            def _():
                for h in hs:
                    cp_o[h].start()

        for i in range(len(DFT) - 1):
            last = i == len(DFT) - 2
            region([lane_dft(xn, c // 2, c % 2) for c in range(*DFT[i:i + 2])]
                   + [lane_idft(c // 2, c % 2) for c in range(*IDFT[i:i + 2])],
                   [phase_conv(r) for r in range(*CONV[i:i + 2])]
                   + ([norm_pair(0)] if last else []),
                   lead=0.4 if last else 0.0, span=0.95 if i == 3 else 1.0)
        region([keys_values(0, 0), keys_values(1, 0), queries(0, 0)],
               [norm_pair(g) for g in (1, 2, 3)])
        region([fn(0, g) for fn in (keys_values, queries) for g in (1, 2, 3)],
               [norm_pair(g) for g in (4, 5, 6, 7)])
        for par, s, kvg, qg in ((0, 0, (1, 2, 3), (0, 1, 2, 3)), (0, 1, (4, 5, 6, 7), (4, 5, 6, 7)),
                                (1, 0, (4, 5, 6, 7), (4, 5))):
            region([keys_values(1 - s, g) for g in kvg] + [queries(1 - s, g) for g in qg],
                   [attend(par, s, m) for m in range(WIN)], span=1.05)
        region([queries(1, g) for g in (6, 7)], [attend(1, 1, m) for m in (0, 1)], span=0.95)
        done = ()
        for hs, ms in (((0, 1), (2, 3, 4)), ((2, 3, 4), (5, 6, 7)), ((5, 6), ())):
            region([project(h, h not in late) for h in hs],
                   [store_pair(h, range(4)) for h in done if h in late]
                   + [norm(h) for h in done] + [attend(1, 1, m) for m in ms],
                   span=1.0 if ms else 1.05)
            send([h for h in done if h in late] + [h for h in hs if h not in late])
            done = hs

        @pl.when(it == 0)
        def _():
            _interleave([project(7, False)], [norm(5), norm(6)])
            _interleave([lane_dft(xn, 0, 0), lane_dft(xn, 0, 1)], [norm(7)], span=1.5)

    @_items(1)
    def send_now(h):
        cp_o[h].start()
        yield

    jax.lax.fori_loop(0, 2, layer, None)
    _interleave([project(7, True)], [store_pair(6, range(4)), send_now(6)], span=4.0)
    cp_o[7].start()
    for cp in cp_o:
        cp.wait()


@jax.jit
def pallas_interleave_layers__ssm_conv_s4__sliding_local_dilated__prompt_kernel(
    A_u: jax.Array,
    A_A_re: jax.Array,
    A_A_im: jax.Array,
    A_B_re: jax.Array,
    A_B_im: jax.Array,
    A_C_re: jax.Array,
    A_C_im: jax.Array,
    A_log_dt: jax.Array,
    A_Dskip: jax.Array,
    B_x: jax.Array,
    B_wqkv: jax.Array,
    B_wo: jax.Array,
):
    del B_x
    hbm = pl.BlockSpec(memory_space=pl.ANY)
    out = pl.pallas_call(
        _kernel,
        in_specs=[hbm] * 12,
        out_specs=hbm,
        out_shape=jax.ShapeDtypeStruct((T1, PH, D), BF16),
        scratch_shapes=[pltpu.VMEM((D, NS), BF16)] * 6 + [pltpu.VMEM((D,), BF16)] * 2 + [
            pltpu.VMEM((PH // 2, T1, D), U32),
            pltpu.VMEM((D, 3 * D), BF16),
            pltpu.VMEM((D, D), BF16),
            pltpu.VMEM((2 * PH, T1 // 2, 2 * T1), U32),
            pltpu.VMEM((7, D, HD), U32),
            pltpu.VMEM((D // 2, D), U32),
            pltpu.VMEM((2, D + 8, NS), F32),
            pltpu.VMEM((2, D + 8, NS), F32),
            pltpu.VMEM((D + 8, NS), F32),
            pltpu.VMEM((4, 4, 9 * QS + 4, NS), U32),
            pltpu.VMEM((4, 9 * ZS + 4, T1), U32),
            pltpu.VMEM((PH, D // 2, T1), U32),
            pltpu.VMEM((NCOEF, D, 2 * T1), F32),
            pltpu.VMEM((PH, D + 8, T1), F32),
            pltpu.VMEM((PH, D // 2, T1), U32),
            pltpu.VMEM((2, 2 * PH, D, T1), F32),
            pltpu.VMEM((PH // 2, HD // 2, 7 * T1), U32),
            pltpu.VMEM((PH // 2, 2, D, T1), F32),
            pltpu.VMEM((WIN, D, T1), F32),
            pltpu.VMEM((WIN, HD, T1), F32),
            pltpu.VMEM((WIN, HD // 2, 7 * T1), U32),
            pltpu.SMEM((1,), I32),
            pltpu.SemaphoreType.DMA((11 + PH // 2,)),
        ],
        compiler_params=pltpu.CompilerParams(vmem_limit_bytes=100 * 1024 * 1024),
    )(A_u.reshape(T1, PH, D), A_A_re, A_A_im, A_B_re, A_B_im, A_C_re, A_C_im,
      A_log_dt, A_Dskip, B_wqkv, B_wo,
      _dft_matrices())
    return out.reshape(1, L, D)
```
